```python
import jax
import jax.numpy as jnp

def _softmax(x, axis=-1):
    return jax.nn.softmax(x, axis=axis)

def _gelu(x):
    return jax.nn.gelu(x, approximate=True)

def _silu(x):
    return jax.nn.silu(x)

def _sigmoid(x):
    return jax.nn.sigmoid(x)

def _layernorm(x, axis=-1, eps=1e-05):
    m = jnp.mean(x, axis=axis, keepdims=True)
    v = jnp.var(x, axis=axis, keepdims=True)
    return (x - m) / jnp.sqrt(v + eps)

def _scatter_add(tgt, idx, src, axis=0):
    return tgt.at[idx].add(src)

def _segment_sum(src, seg, n):
    return jax.ops.segment_sum(src, seg, n)

class _Rng:

    def __init__(self, key):
        self._k = key

    def _next(self):
        self._k, sub = jax.random.split(self._k)
        return sub

    def normal(self, shape):
        return jax.random.normal(self._next(), shape, dtype=jnp.bfloat16)

    def randint(self, lo, hi, shape):
        return jax.random.randint(self._next(), shape, lo, hi, dtype=jnp.int32)

    def uniform(self, shape, lo=0.0, hi=1.0):
        return jax.random.uniform(self._next(), shape, jnp.bfloat16, lo, hi)

    def permutation(self, n):
        return jax.random.permutation(self._next(), n)
kernel_name = 'adaLN_cond__ssm_conv_h3__mixer_s_mlp__prompt'

def setup_inputs():
    _rng = _Rng(jax.random.key(int.from_bytes(__import__("os").urandom(4), "little")))
    _w = lambda a: (lambda t: t.astype(jnp.bfloat16) if jnp.issubdtype(t.dtype, jnp.floating) else t)(jnp.asarray(a))

    def _A_setup():
        B, S, D = (1, 2048, 640)
        ks = 4
        return {'q': _w((lambda *s: _rng.normal(s) * 0.05)(B, S, D)), 'k': _w((lambda *s: _rng.normal(s) * 0.05)(B, S, D)), 'v': _w((lambda *s: _rng.normal(s) * 0.05)(B, S, D)), 'shift_k': _w((lambda *s: _rng.normal(s) * 0.05)(D, ks) * 0.5), 'ssm_k': _w((lambda *s: _rng.normal(s) * 0.05)(D, S) * (1.0 / S ** 0.5)), 'ssm_D': _w((lambda *s: _rng.normal(s) * 0.05)(D))}
    _A_in = _A_setup()

    def _B_setup():
        B, S, D, F = (1, 2048, 640, 1728)
        return {'x': _w((lambda *s: _rng.normal(s) * 0.05)(B, S, D)), 'w1': _w((lambda *s: _rng.normal(s) * 0.05)(D, D) * D ** (-0.5)), 'w2': _w((lambda *s: _rng.normal(s) * 0.05)(D, D) * D ** (-0.5)), 'w3': _w((lambda *s: _rng.normal(s) * 0.05)(D, F) * D ** (-0.5)), 'w4': _w((lambda *s: _rng.normal(s) * 0.05)(F, D) * F ** (-0.5))}
    _B_in = _B_setup()
    return {'A_q': _A_in['q'], 'A_k': _A_in['k'], 'A_v': _A_in['v'], 'A_shift_k': _A_in['shift_k'], 'A_ssm_k': _A_in['ssm_k'], 'A_ssm_D': _A_in['ssm_D'], 'B_x': _B_in['x'], 'B_w1': _B_in['w1'], 'B_w2': _B_in['w2'], 'B_w3': _B_in['w3'], 'B_w4': _B_in['w4'], 'c': _w((lambda *s: _rng.normal(s) * 0.05)(1, 640)), 'w_mod': _w((lambda *s: _rng.normal(s) * 0.05)(640, 6 * 640) * 640 ** (-0.5))}

def reference(A_q, A_k, A_v, A_shift_k, A_ssm_k, A_ssm_D, B_x, B_w1, B_w2, B_w3, B_w4, c, w_mod):

    def _A_ref(q, k, v, shift_k, ssm_k, ssm_D):
        B, S, D = q.shape
        ks = shift_k.shape[-1]
        k_pad = jnp.pad(k, ((0, 0), (ks - 1, 0), (0, 0)))
        k_shift = jnp.zeros_like(k)
        for t in range(ks):
            k_shift = k_shift + k_pad[:, t:t + S, :] * shift_k[:, ks - 1 - t][None, None, :]
        kv = k_shift * v
        L = 2 * S
        kv_pad = jnp.pad(kv, ((0, 0), (0, S), (0, 0)))
        kf_pad = jnp.pad(ssm_k, ((0, 0), (0, S)))
        kv_f = (lambda x, axes=(-2, -1): jnp.fft.rfft2(x.astype(jnp.float32), axes=axes))(kv_pad[:, None, :, :], axes=(1, 2))
        kf_f = (lambda x, axes=(-2, -1): jnp.fft.rfft2(x.astype(jnp.float32), axes=axes))(kf_pad[:, None, :], axes=(1, 2))
        kf_f = (lambda x, *d: x.transpose(*d))(kf_f, 1, 2, 0)
        y_f = kv_f * kf_f[None, :, :, :]
        y = (lambda x, s, axes=(-2, -1): jnp.fft.irfft2(x, s=s, axes=axes).astype(jnp.bfloat16))(y_f, (1, L), axes=(1, 2))[:, 0, :S, :]
        y = y + kv * ssm_D[None, None, :]
        return q * y

    def _B_ref(x, w1, w2, w3, w4):
        B, S, D = x.shape
        h = _gelu(_layernorm(x, axis=-1) @ w1)
        c = D // 4
        g0 = jnp.pad(h[:, :, 0 * c:1 * c], ((0, 0), (1, 0), (0, 0)))[:, :S, :]
        g1 = jnp.pad(h[:, :, 1 * c:2 * c], ((0, 0), (0, 1), (0, 0)))[:, 1:, :]
        g2 = jnp.pad(h[:, :, 2 * c:3 * c], ((0, 0), (2, 0), (0, 0)))[:, :S, :]
        g3 = jnp.pad(h[:, :, 3 * c:], ((0, 0), (0, 2), (0, 0)))[:, 2:, :]
        hs = jnp.concatenate([g0, g1, g2, g3], axis=-1) @ w2
        x1 = x + hs
        h2 = _gelu(_layernorm(x1, axis=-1) @ w3) @ w4
        return x1 + h2
    x = A_q
    mod = (_silu(c) @ w_mod).reshape(c.shape[0], 6, 1, -1)
    sa, ca, ga, sb, cb, gb = (mod[:, 0].copy(), mod[:, 1].copy(), mod[:, 2].copy(), mod[:, 3].copy(), mod[:, 4].copy(), mod[:, 5].copy())
    h = _layernorm(x, axis=-1) * (1 + ca) + sa
    x = x + ga * _A_ref(h, A_k, A_v, A_shift_k, A_ssm_k, A_ssm_D)
    h = _layernorm(x, axis=-1) * (1 + cb) + sb
    x = x + gb * _B_ref(h, B_w1, B_w2, B_w3, B_w4)
    return x
```

```python
import functools

import jax
import jax.numpy as jnp
import numpy as np
import jax.experimental.pallas as pl
import jax.experimental.pallas.tpu as pltpu

S, D, FF = 2048, 640, 1728
NT = D // 128
L = 512
NB = S // L
NFFT = 2 * L
R = 4
KPAD = 16
HPAD = 8
EPS = 1e-5
F32 = jnp.float32
BF16 = jnp.bfloat16
NT_DIMS = (((1,), (1,)), ((), ()))


def _dft_tables():
    chunk = np.arange(16)[:, None]
    s = np.arange(8)[None, :]
    f = np.where(chunk < 8, 2 * (8 * chunk + s), 2 * (8 * (chunk - 8) + s) + 1)
    m = np.arange(128)
    fwd = np.zeros((R, 16, 2, 8, 128), np.float64)
    for r in range(R):
        ang = -2.0 * np.pi * ((4 * m + r)[None, None, :] * (f[:, :, None] + 0.5)) / NFFT
        fwd[r, :, 0] = np.cos(ang)
        fwd[r, :, 1] = np.sin(ang)
    fwd = fwd.reshape(R, 256, 128)
    inv = np.transpose(fwd, (0, 2, 1)) * (2.0 / NFFT)
    inv = inv.reshape(R, 128, 2, 128).transpose(0, 2, 1, 3)
    return fwd.astype(np.float32), np.ascontiguousarray(inv).astype(np.float32)


_FWD, _INV = _dft_tables()


def _gelu(x):
    c1 = np.float32(np.sqrt(2.0 / np.pi))
    c2 = np.float32(np.sqrt(2.0 / np.pi) * 0.044715)
    u = x * (c1 + c2 * (x * x))
    hx = 0.5 * x
    return hx + hx * jnp.tanh(u)


def _stats(x):
    m = jnp.sum(x, axis=-1, keepdims=True) * (1.0 / D)
    e2 = jnp.sum(x * x, axis=-1, keepdims=True) * (1.0 / D)
    v = jnp.maximum(e2 - m * m, 0.0)
    return m, jax.lax.rsqrt(v + EPS)


def _split(b):
    b = b.reshape(16, 2, 8, 128)
    return b[:, 0], b[:, 1]


def _fft4(b, sign):
    (r0, i0), (r1, i1), (r2, i2), (r3, i3) = b
    sr, si, dr, di = r0 + r2, i0 + i2, r0 - r2, i0 - i2
    tr, ti, er, ei = r1 + r3, i1 + i3, r1 - r3, i1 - i3
    x0 = (sr + tr, si + ti)
    x2 = (sr - tr, si - ti)
    xm = (dr + ei, di - er)
    xp = (dr - ei, di + er)
    return [x0, xm, x2, xp] if sign < 0 else [x0, xp, x2, xm]


def _kernel(q_hbm, k_hbm, v_hbm, sk_hbm, ssm_hbm, sd_hbm, w1_hbm, w2_hbm, w3_hbm,
            w4_hbm, c_hbm, wm_hbm, fw_hbm, gi_hbm, o_hbm,
            qb, kb, vb, skb, ssmb, sdb, w1b, w2b, w3b, w4b, cb_, wmb, fwb, gib,
            st, xs, ks, yb, x1b, hb, hpb, ob, sems, osems):
    copies = {}

    def add(name, src, dst):
        copies[name] = pltpu.make_async_copy(src, dst, sems.at[len(copies)])

    def add_kv(c):
        for t in range(NT):
            add(f"k{c}_{t}", k_hbm.at[0, pl.ds(L * c, L), pl.ds(128 * t, 128)],
                kb.at[t, pl.ds(KPAD + L * c, L), :])
            add(f"v{c}_{t}", v_hbm.at[0, pl.ds(L * c, L), pl.ds(128 * t, 128)],
                vb.at[t, pl.ds(L * c, L), :])

    def add_q(c):
        add(f"q{c}", q_hbm.at[0, pl.ds(L * c, L), :], qb.at[pl.ds(L * c, L), :])

    add("ssm0", ssm_hbm.at[pl.ds(0, 128), :], ssmb.at[pl.ds(0, 128), :])
    add("fw", fw_hbm, fwb)
    add("sd", sd_hbm, sdb)
    add("sk", sk_hbm, skb)
    add("c", c_hbm, cb_)
    for t in range(1, NT):
        add(f"ssm{t}", ssm_hbm.at[pl.ds(128 * t, 128), :], ssmb.at[pl.ds(128 * t, 128), :])
    add("gi", gi_hbm, gib)
    add_kv(0)
    add_q(0)
    add("wmA", wm_hbm.at[:, pl.ds(0, 3 * D)], wmb.at[:, pl.ds(0, 3 * D)])
    add("wmB", wm_hbm.at[:, pl.ds(3 * D, 2 * D)], wmb.at[:, pl.ds(3 * D, 2 * D)])
    add("w1", w1_hbm, w1b)
    add("w2", w2_hbm, w2b)
    add("w3", w3_hbm, w3b)
    add_kv(1)
    add("w4", w4_hbm, w4b)
    add("wmC", wm_hbm.at[:, pl.ds(5 * D, D)], wmb.at[:, pl.ds(5 * D, D)])
    add_q(1)
    for c in range(2, NB):
        add_kv(c)
        add_q(c)
    for cp in copies.values():
        cp.start()

    def wait(*names):
        for n in names:
            copies[n].wait()

    def wait_kv(c):
        wait(*[f"{a}{c}_{t}" for t in range(NT) for a in "kv"])

    kb[:, 0:KPAD, :] = jnp.zeros((NT, KPAD, 128), BF16)
    hpb[:, 0:HPAD, :] = jnp.zeros((NT, HPAD, 128), F32)
    hpb[:, HPAD + S:HPAD + S + HPAD, :] = jnp.zeros((NT, HPAD, 128), F32)

    env = {}

    def conv_k(t):
        dvec = env["dvec"][:, 128 * t:128 * t + 128]
        prev = None
        for j in range(NB):
            st[t, L * j:L * j + L, :] = ssmb[128 * t:128 * t + 128, L * j:L * j + L].astype(F32).T
            b = []
            for r in range(R):
                rhs = st[t, pl.ds(L * j + r, 128, stride=R), :].astype(BF16)
                re, im = _split(jnp.dot(fwb[r], rhs, preferred_element_type=F32))
                if j == 0 and r == 0:
                    re = re + dvec[None]
                b.append((re, im))
            kq = _fft4(b, -1)
            for q in range(R):
                re, im = kq[q]
                if j > 0:
                    pr, pi = prev[q]
                    re = jnp.concatenate([re[:8] - pi[:8], re[8:] + pi[8:]], axis=0)
                    im = jnp.concatenate([im[:8] + pr[:8], im[8:] - pr[8:]], axis=0)
                ks[j, q, t, 0] = re
                ks[j, q, t, 1] = im
            prev = kq

    def unpack(u):
        lo = pltpu.bitcast(u << 16, F32)
        hi = pltpu.bitcast(u & jnp.uint32(0xFFFF0000), F32)
        return lo, hi

    def conv_fwd(c, t):
        taps = env["taps"]
        ku = kb.bitcast(jnp.uint32)
        vu = vb.bitcast(jnp.uint32)
        w0 = (KPAD + L * c) // 2
        k0, k1 = unpack(ku[t, pl.ds(w0, 128, stride=2), :])
        k2, k3 = unpack(ku[t, pl.ds(w0 + 1, 128, stride=2), :])
        _, km3 = unpack(ku[t, pl.ds(w0 - 2, 128, stride=2), :])
        km2, km1 = unpack(ku[t, pl.ds(w0 - 1, 128, stride=2), :])
        v0, v1 = unpack(vu[t, pl.ds(L * c // 2, 128, stride=2), :])
        v2, v3 = unpack(vu[t, pl.ds(L * c // 2 + 1, 128, stride=2), :])
        kk = [km3, km2, km1, k0, k1, k2, k3]
        vv = [v0, v1, v2, v3]
        tp = [taps[j:j + 1, 128 * t:128 * t + 128] for j in range(4)]
        b = []
        for r in range(R):
            acc = kk[3 + r] * tp[0]
            for j in range(1, 4):
                acc = acc + kk[3 + r - j] * tp[j]
            kv = (acc * vv[r]).astype(BF16)
            b.append(_split(jnp.dot(fwb[r], kv, preferred_element_type=F32)))
        xq = _fft4(b, -1)
        for q in range(R):
            xs[c, q, t, 0] = xq[q][0]
            xs[c, q, t, 1] = xq[q][1]
        z = []
        for q in range(R):
            zr = zi = None
            for cc in range(c, -1, -1):
                xr, xi = xs[cc, q, t, 0], xs[cc, q, t, 1]
                kr, ki = ks[c - cc, q, t, 0], ks[c - cc, q, t, 1]
                if zr is None:
                    zr = xr * kr - xi * ki
                    zi = xr * ki + xi * kr
                else:
                    zr = (zr + xr * kr) - xi * ki
                    zi = (zi + xr * ki) + xi * kr
            z.append((zr, zi))
        cr = _fft4(z, +1)
        env["cm", c, t] = [jnp.stack(cr[r], axis=1).reshape(256, 128).astype(BF16) for r in range(R)]

    def conv_inv(c, t):
        cm = env.pop(("cm", c, t))
        for r in range(R):
            g = jnp.concatenate([gib[r, 0], gib[r, 1]], axis=-1)
            yb[t, pl.ds(L * c + r, 128, stride=R), :] = jnp.dot(g, cm[r], preferred_element_type=F32)

    def a_pre1(r0, n):
        env["m1", r0] = _stats(qb[r0:r0 + n, :].astype(F32))

    def a_pre2(r0, n):
        m1, r1 = env.pop(("m1", r0))
        x = qb[r0:r0 + n, :].astype(F32)
        y = jnp.concatenate([yb[t, r0:r0 + n, :] for t in range(NT)], axis=-1)
        x1 = x + ((x - m1) * r1 * env["a1"] + env["a0"]) * y
        x1b[r0:r0 + n, :] = x1
        env["m2", r0] = _stats(x1)

    def a_pre3(r0, n):
        m2, r2 = env.pop(("m2", r0))
        h = (x1b[r0:r0 + n, :] - m2) * r2 * env["b1"] + env["b0"]
        hb[r0:r0 + n, :] = h
        m3, r3 = _stats(h)
        env["n3", r0] = ((hb[r0:r0 + n, :] - m3) * r3).astype(BF16)

    def a_pre(r0, n):
        a_pre1(r0, n)
        a_pre2(r0, n)
        a_pre3(r0, n)

    def mm1(r0, n):
        hp = _gelu(jnp.dot(env.pop(("n3", r0)), w1b[...], preferred_element_type=F32))
        for t in range(NT):
            hpb[t, HPAD + r0:HPAD + r0 + n, :] = hp[:, 128 * t:128 * t + 128]

    def mm2(r0, n):
        lane = jax.lax.broadcasted_iota(jnp.int32, (n, 128), 1)
        sh = [-1, 1, -2, 2]

        def ld(t, g):
            o = HPAD + r0 + sh[g]
            return hpb[t, o:o + n, :]

        cols = [ld(0, 0)]
        for t in range(1, 4):
            cols.append(jnp.where(lane < 32 * t, ld(t, t - 1), ld(t, t)))
        cols.append(ld(4, 3))
        g = jnp.concatenate(cols, axis=-1).astype(BF16)
        x2 = hb[r0:r0 + n, :] + jnp.dot(g, w2b[...], preferred_element_type=F32)
        hb[r0:r0 + n, :] = x2
        m4, r4 = _stats(x2)
        env["n4", r0] = ((hb[r0:r0 + n, :] - m4) * r4).astype(BF16)
        env["u", r0] = []

    def mm3(r0, n, f0, f1):
        h3 = jax.lax.dot_general(env["n4", r0], w3b[f0:f1, :], NT_DIMS, preferred_element_type=F32)
        env["u", r0].append(_gelu(h3).astype(BF16))

    def mm4(r0, n, t0, t1):
        u = env["u", r0]
        if len(u) > 1:
            u = env["u", r0] = [jnp.concatenate(u, axis=-1)]
        c0, c1 = 128 * t0, 128 * t1
        h2 = jnp.dot(u[0], w4b[:, c0:c1], preferred_element_type=F32)
        ob[r0:r0 + n, c0:c1] = (x1b[r0:r0 + n, c0:c1]
                                + env["gb"][:, c0:c1] * (hb[r0:r0 + n, c0:c1] + h2)).astype(BF16)

    out_copies = []

    def emit(r0, n):
        cp = pltpu.make_async_copy(ob.at[pl.ds(r0, n), :], o_hbm.at[0, pl.ds(r0, n), :],
                                   osems.at[len(out_copies)])
        cp.start()
        out_copies.append(cp)

    wait("ssm0", "fw", "sd", "sk", "c")
    env["taps"] = skb[...].astype(F32)
    env["dvec"] = sdb[...].astype(F32).reshape(1, D)
    cf = cb_[...].astype(F32)
    sc = (cf * jax.nn.sigmoid(cf)).astype(BF16)
    sc8 = jnp.broadcast_to(sc, (8, D))

    for t in range(NT):
        if t:
            wait(f"ssm{t}")
        conv_k(t)
    wait("gi")
    wait_kv(0)
    for t in range(NT):
        conv_fwd(0, t)
        if t:
            conv_inv(0, t - 1)
    conv_inv(0, NT - 1)

    H = L // 2
    wait("q0")
    a_pre1(0, H)
    a_pre1(H, H)
    wait("wmA")
    mod = jnp.dot(sc8, wmb[:, 0:3 * D], preferred_element_type=F32)[0:1]
    sa, ca, ga = [mod[:, D * i:D * (i + 1)] for i in range(3)]
    env["a1"], env["a0"] = (1.0 + ca) * ga, sa * ga
    a_pre2(0, H)
    a_pre2(H, H)
    wait("wmB")
    mod = jnp.dot(sc8, wmb[:, 3 * D:5 * D], preferred_element_type=F32)[0:1]
    env["b1"], env["b0"] = 1.0 + mod[:, D:2 * D], mod[:, 0:D]
    a_pre3(0, H)
    a_pre3(H, H)
    wait("w1")
    mm1(0, H)
    mm1(H, H)
    wait("w2")

    bounds = [0] + [H * i - 16 for i in range(1, 2 * NB)] + [S]
    blk = [(bounds[i], bounds[i + 1] - bounds[i]) for i in range(2 * NB)]
    fch = [0, 512, 1024, 1408, FF]
    mm2(*blk[0])
    mm2(*blk[1])
    wait("w3")
    wait_kv(1)
    for i in range(2 * NB):
        c = i // 2 + 1
        live = c < NB
        first = i % 2 == 0
        for j in range(4):
            if live and first and j < 3:
                conv_fwd(c, j)
            if live and not first:
                if j == 2:
                    mm1(L * c, H)
            mm3(*blk[i], fch[j], fch[j + 1])
        if i == 0:
            wait("w4", "wmC", "q1")
            env["gb"] = jnp.dot(sc8, wmb[:, 5 * D:6 * D], preferred_element_type=F32)[0:1]
        if i >= 1 and i + 1 < 2 * NB:
            mm2(*blk[i + 1])
        for t in range(NT):
            if live and first:
                if t < 2:
                    conv_fwd(c, 3 + t)
                    conv_inv(c, t)
                if t == 2:
                    conv_inv(c, 2)
                    conv_inv(c, 3)
                if t == 3:
                    conv_inv(c, 4)
                    a_pre(L * c, H)
            if live and not first:
                if t == 0:
                    a_pre(L * c + H, H)
                if t == 3:
                    mm1(L * c + H, H)
            mm4(*blk[i], t, t + 1)
        emit(*blk[i])
        if not first and c + 1 < NB:
            wait(f"q{c + 1}")
            wait_kv(c + 1)
    for cp in out_copies:
        cp.wait()


@jax.jit
def pallas_adaLN_cond__ssm_conv_h3__mixer_s_mlp__prompt_kernel(
    A_q, A_k, A_v, A_shift_k, A_ssm_k, A_ssm_D, B_x, B_w1, B_w2, B_w3, B_w4, c, w_mod,
):
    del B_x
    fw = jnp.asarray(_FWD, dtype=BF16)
    gi = jnp.asarray(_INV, dtype=BF16)
    vm = pltpu.VMEM
    scratch = [
        vm((S, D), BF16),
        vm((NT, KPAD + S, 128), BF16),
        vm((NT, S, 128), BF16),
        vm((4, D), BF16),
        vm((D, S), BF16),
        vm((D,), BF16),
        vm((D, D), BF16),
        vm((D, D), BF16),
        vm((FF, D), BF16),
        vm((FF, D), BF16),
        vm((1, D), BF16),
        vm((D, 6 * D), BF16),
        vm((R, 256, 128), BF16),
        vm((R, 2, 128, 128), BF16),
        vm((NT, S, 128), F32),
        vm((NB, R, NT, 2, 16, 8, 128), F32),
        vm((NB, R, NT, 2, 16, 8, 128), F32),
        vm((NT, S, 128), F32),
        vm((S, D), F32),
        vm((S, D), F32),
        vm((NT, S + 2 * HPAD, 128), F32),
        vm((S, D), BF16),
        pltpu.SemaphoreType.DMA((64,)),
        pltpu.SemaphoreType.DMA((8,)),
    ]
    hbm = pl.BlockSpec(memory_space=pltpu.HBM)
    return pl.pallas_call(
        _kernel,
        out_shape=jax.ShapeDtypeStruct((1, S, D), BF16),
        in_specs=[hbm] * 14,
        out_specs=hbm,
        scratch_shapes=scratch,
        compiler_params=pltpu.CompilerParams(vmem_limit_bytes=110 * 2**20),
        name="h3_mixer",
    )(A_q, A_k, A_v, A_shift_k.T, A_ssm_k, A_ssm_D, B_w1, B_w2, B_w3.T, B_w4,
      c, w_mod, fw, gi)
```

```python
import jax
import jax.numpy as jnp
import numpy as np
import jax.experimental.pallas as pl
import jax.experimental.pallas.tpu as pltpu

S, D, FF = 2048, 640, 1728
NT = D // 128
L = 512
NB = S // L
NFFT = 2 * L
R = 4
KPAD = 16
HPAD = 8
TB = 256
NBLK = S // TB
AO = 16
CH = 16
EPS = 1e-5
F32 = jnp.float32
BF16 = jnp.bfloat16
U32 = jnp.uint32
NT_DIMS = (((1,), (1,)), ((), ()))
K0P, K1P, K1R, K2R, X0S, X1S, Z1P, Z2P, Z3P = range(9)


def _to_bf16_bits(a):
    u = np.ascontiguousarray(a, dtype=np.float32).view(np.uint32)
    return ((u + 0x7FFF + ((u >> 16) & 1)) >> 16).astype(np.uint32)


def _pack_rows(a):
    b = _to_bf16_bits(a)
    return b[..., 0::2, :] | (b[..., 1::2, :] << 16)


def _dft_tables():
    chunk = np.arange(16)[:, None]
    s = np.arange(8)[None, :]
    f = np.where(chunk < 8, 2 * (8 * chunk + s), 2 * (8 * (chunk - 8) + s) + 1)
    m = np.arange(128)
    fwd = np.zeros((R, 16, 2, 8, 128), np.float64)
    for r in range(R):
        ang = -2.0 * np.pi * ((4 * m + r)[None, None, :] * (f[:, :, None] + 0.5)) / NFFT
        fwd[r, :, 0] = np.cos(ang)
        fwd[r, :, 1] = np.sin(ang)
    inv = fwd.transpose(0, 1, 3, 2, 4).reshape(R, 256, 128)
    inv = np.transpose(inv, (0, 2, 1)) * (2.0 / NFFT)
    inv = inv.reshape(R, 128, 2, 128).transpose(0, 2, 1, 3)
    return _pack_rows(fwd.reshape(R, 256, 128)), _pack_rows(inv)


_FWD, _INV = _dft_tables()


def _gelu(x):
    c1 = np.float32(np.sqrt(2.0 / np.pi))
    c2 = np.float32(np.sqrt(2.0 / np.pi) * 0.044715)
    u = x * (c1 + c2 * (x * x))
    hx = 0.5 * x
    return hx + hx * jnp.tanh(u)


def _stats(x):
    m = jnp.sum(x, axis=-1, keepdims=True) * (1.0 / D)
    e2 = jnp.sum(x * x, axis=-1, keepdims=True) * (1.0 / D)
    v = jnp.maximum(e2 - m * m, 0.0)
    return m, jax.lax.rsqrt(v + EPS)


def _split(b):
    b = b.reshape(16, 2, 8, 128)
    return b[:, 0], b[:, 1]


def _join(z):
    return jnp.stack(z, axis=1).reshape(256, 128)


def _fft4(b, sign):
    (r0, i0), (r1, i1), (r2, i2), (r3, i3) = b
    sr, si, dr, di = r0 + r2, i0 + i2, r0 - r2, i0 - i2
    tr, ti, er, ei = r1 + r3, i1 + i3, r1 - r3, i1 - i3
    x0 = (sr + tr, si + ti)
    x2 = (sr - tr, si - ti)
    xm = (dr + ei, di - er)
    xp = (dr - ei, di + er)
    return [x0, xm, x2, xp] if sign < 0 else [x0, xp, x2, xm]


def _cmul(a, b, acc=None):
    (ar, ai), (br, bi) = a, b
    if acc is None:
        return ar * br - ai * bi, ar * bi + ai * br
    return (acc[0] + ar * br) - ai * bi, (acc[1] + ar * bi) + ai * br


def _bf(x):
    return pltpu.bitcast(x, BF16)


def _kernel(q_hbm, k_hbm, v_hbm, sk_hbm, ssm_hbm, sd_hbm, w1_hbm, w2_hbm, w3_hbm,
            w4_hbm, c_hbm, wm_hbm, fw_hbm, gi_hbm, o_hbm,
            qb, kb, vb, skb, ssmb, sdb, w1b, w2b, w3b, w4b, cb_, wmb, fwb, gib,
            stb, spec, cmb, yb, x1b, hb, hpb, n4b, par, ob, sems, osem):
    groups = {}

    def add(name, src, dst):
        if name not in groups:
            groups[name] = (len(groups), [])
        idx, lst = groups[name]
        cp = pltpu.make_async_copy(src, dst, sems.at[idx])
        cp.start()
        lst.append(cp)

    def add_kv(name, c):
        for t in range(NT):
            add(name, k_hbm.at[0, pl.ds(L * c, L), pl.ds(128 * t, 128)],
                kb.at[t, pl.ds(KPAD + L * c, L), :])
            add(name, v_hbm.at[0, pl.ds(L * c, L), pl.ds(128 * t, 128)],
                vb.at[t, pl.ds(L * c, L), :])

    def add_ssm(name, c):
        add(name, ssm_hbm.at[:, pl.ds(L * c, L)], ssmb.bitcast(BF16).at[:, pl.ds(L * c, L)])

    QE = 2 * TB + AO
    add_ssm("s0", 0)
    add("s0", fw_hbm, fwb)
    add("s0", sd_hbm, sdb)
    add("s0", sk_hbm, skb)
    add("s0", c_hbm, cb_)
    add_kv("c0", 0)
    add("c0", gi_hbm, gib)
    for c in range(1, NB):
        add_ssm(f"c{c}", c)
        add_kv(f"c{c}", c)
    add("c3", q_hbm.at[0, pl.ds(0, QE), :], qb.bitcast(BF16).at[pl.ds(0, QE), :])
    add("wmA", wm_hbm.at[:, pl.ds(0, 3 * D)], wmb.at[:, pl.ds(0, 3 * D)])
    add("wmB", wm_hbm.at[:, pl.ds(3 * D, 2 * D)], wmb.at[:, pl.ds(3 * D, 2 * D)])
    add("w1", w1_hbm, w1b.bitcast(BF16))
    add("w2", w2_hbm, w2b.bitcast(BF16))
    add("w3", w3_hbm, w3b.bitcast(BF16))
    add("w4", w4_hbm, w4b.bitcast(BF16))
    add("rest", q_hbm.at[0, pl.ds(QE, S - QE), :], qb.bitcast(BF16).at[pl.ds(QE, S - QE), :])
    add("rest", wm_hbm.at[:, pl.ds(5 * D, D)], wmb.at[:, pl.ds(5 * D, D)])

    def wait(name):
        with jax.named_scope("W_" + name):
            for cp in groups[name][1]:
                cp.wait()

    kb[:, 0:KPAD, :] = jnp.zeros((NT, KPAD, 128), BF16)
    hpb[:, 0:HPAD, :] = jnp.zeros((NT, HPAD, 128), F32)
    yb[:, S:S + AO, :] = jnp.zeros((NT, AO, 128), F32)
    qb[S // 2:(S + AO) // 2, :] = jnp.zeros((AO // 2, D), U32)

    spec[9, 0, 0, pl.ds(0, 8, stride=2), :] = jnp.zeros((8, 128), F32)
    cmb[2, 0, 0, pl.ds(0, 8, stride=2), :] = jnp.zeros((8, 128), U32)

    env = {}

    def ld_spec(slot, t, q):
        return _split(spec[slot, t, q])

    def st_spec(slot, t, q, z):
        spec[slot, t, q] = _join(z)

    def conv_k(c, t):
        w0 = L * c // 2
        stb[t, w0:w0 + L // 2, :] = pltpu.bitcast(
            _bf(ssmb[64 * t:64 * t + 64, L * c:L * c + L]).T, U32)
        b = []
        for h in range(2):
            lo = stb[t, pl.ds(w0 + h, 64, stride=4), :]
            hi = stb[t, pl.ds(w0 + h + 2, 64, stride=4), :]
            for rhs in ((lo & jnp.uint32(0xFFFF)) | (hi << 16),
                        (lo >> 16) | (hi & jnp.uint32(0xFFFF0000))):
                b.append(_split(jnp.dot(_bf(fwb[len(b)]), _bf(rhs), preferred_element_type=F32)))
        if c == 0:
            b[0] = (b[0][0] + env["dvec"][:, 128 * t:128 * t + 128][None], b[0][1])
        kq = _fft4(b, -1)
        for q in range(R):
            re, im = kq[q]
            if c == 0:
                st_spec(K0P, t, q, kq[q])
                continue
            if c < 3:
                st_spec((K1R, K2R)[c - 1], t, q, kq[q])
            pr, pi = ld_spec((K0P, K1R, K2R)[c - 1], t, q)
            kp = (jnp.concatenate([re[:8] - pi[:8], re[8:] + pi[8:]], axis=0),
                  jnp.concatenate([im[:8] + pr[:8], im[8:] - pr[8:]], axis=0))
            x0 = ld_spec(X0S, t, q)
            if c == 1:
                st_spec(K1P, t, q, kp)
                st_spec(Z1P, t, q, _cmul(kp, x0))
            elif c == 2:
                st_spec(Z2P, t, q, _cmul(kp, x0, ld_spec(Z2P, t, q)))
                st_spec(Z3P, t, q, _cmul(kp, ld_spec(X1S, t, q)))
            else:
                st_spec(Z3P, t, q, _cmul(kp, x0, ld_spec(Z3P, t, q)))

    def unpack(u):
        return (pltpu.bitcast(u << 16, F32),
                pltpu.bitcast(u & jnp.uint32(0xFFFF0000), F32))

    def conv_x(c, t):
        taps = env["taps"]
        ku = kb.bitcast(U32)
        vu = vb.bitcast(U32)
        w0 = (KPAD + L * c) // 2
        k0, k1 = unpack(ku[t, pl.ds(w0, 128, stride=2), :])
        k2, k3 = unpack(ku[t, pl.ds(w0 + 1, 128, stride=2), :])
        _, km3 = unpack(ku[t, pl.ds(w0 - 2, 128, stride=2), :])
        km2, km1 = unpack(ku[t, pl.ds(w0 - 1, 128, stride=2), :])
        v0, v1 = unpack(vu[t, pl.ds(L * c // 2, 128, stride=2), :])
        v2, v3 = unpack(vu[t, pl.ds(L * c // 2 + 1, 128, stride=2), :])
        kk = [km3, km2, km1, k0, k1, k2, k3]
        vv = [v0, v1, v2, v3]
        tp = [taps[j:j + 1, 128 * t:128 * t + 128] for j in range(4)]
        b = []
        for r in range(R):
            acc = kk[3 + r] * tp[0]
            for j in range(1, 4):
                acc = acc + kk[3 + r - j] * tp[j]
            kv = (acc * vv[r]).astype(BF16)
            b.append(_split(jnp.dot(_bf(fwb[r]), kv, preferred_element_type=F32)))
        xq = _fft4(b, -1)
        z = []
        for q in range(R):
            if c < 2:
                st_spec((X0S, X1S)[c], t, q, xq[q])
            acc = None if c == 0 else ld_spec((Z1P, Z2P, Z3P)[c - 1], t, q)
            z.append(_cmul(xq[q], ld_spec(K0P, t, q), acc))
            if c == 1:
                st_spec(Z2P, t, q, _cmul(xq[q], ld_spec(K1P, t, q)))
            elif c == 2:
                st_spec(Z3P, t, q, _cmul(xq[q], ld_spec(K1P, t, q), ld_spec(Z3P, t, q)))
        cr = _fft4(z, +1)
        for r in range(R):
            cmb[c % 2, t, r] = pltpu.pack_elementwise(list(cr[r]), packed_dtype=BF16).reshape(128, 128)

    def conv_inv(c, t):
        for r in range(R):
            g = jnp.concatenate([_bf(gib[r, 0]), _bf(gib[r, 1])], axis=-1)
            yb[t, pl.ds(L * c + r, 128, stride=R), :] = jnp.dot(
                g, _bf(cmb[c % 2, t, r]), preferred_element_type=F32)

    def rows(r0, n, align=8):
        if isinstance(r0, int):
            return slice(r0, r0 + n)
        return pl.ds(pl.multiple_of(r0, align), n)

    def ld_y(r0, n):
        return jnp.concatenate([yb[t, rows(r0, n), :] for t in range(NT)], axis=-1)

    def prm(i):
        return par[i:i + 1, :]

    def a_pre1(r0, n):
        env["m1", r0] = _stats(_bf(qb[r0 // 2:(r0 + n) // 2, :]).astype(F32))

    def a_pre2(r0, n):
        m1, r1 = env.pop(("m1", r0))
        x = _bf(qb[r0 // 2:(r0 + n) // 2, :]).astype(F32)
        x1 = x + ((x - m1) * r1 * prm(0) + prm(1)) * ld_y(r0, n)
        x1b[r0:r0 + n, :] = x1
        env["m2", r0] = _stats(x1)

    def a_pre3(r0, n):
        m2, r2 = env.pop(("m2", r0))
        h = (x1b[r0:r0 + n, :] - m2) * r2 * prm(2) + prm(3)
        hb[r0:r0 + n, :] = h
        m3, r3 = _stats(h)
        return (hb[r0:r0 + n, :] - m3) * r3

    def a_pre_gated(r0, gates):
        zero = kb.bitcast(U32)[0, 0:8, :]
        out = []
        for j, g in enumerate(gates):
            r = r0 + CH * j
            z = pltpu.bitcast(g, U32) & zero
            qv = qb[rows(r0 // 2 + CH // 2 * j, CH // 2), :] | jnp.concatenate([z] * NT, axis=1)
            x = _bf(qv).astype(F32)
            m1, r1 = _stats(x)
            x1 = x + ((x - m1) * r1 * prm(0) + prm(1)) * ld_y(r, CH)
            x1b[rows(r, CH), :] = x1
            m2, r2 = _stats(x1)
            h = (x1 - m2) * r2 * prm(2) + prm(3)
            hb[rows(r, CH), :] = h
            m3, r3 = _stats(h)
            out.append((h - m3) * r3)
        return jnp.concatenate(out, axis=0)

    def mm1(r0, n, n3):
        hp = _gelu(jnp.dot(n3.astype(BF16), _bf(w1b[...]), preferred_element_type=F32))
        for t in range(NT):
            hpb[t, rows(HPAD + r0, n), :] = hp[:, 128 * t:128 * t + 128]

    def g_prep(r0):
        lane = jax.lax.broadcasted_iota(jnp.int32, (TB, 128), 1)
        sh = [-1, 1, -2, 2]

        def ldh(t, g):
            return hpb[t, pl.ds(HPAD + r0 + sh[g], TB), :]

        cols = [ldh(0, 0)]
        for t in range(1, 4):
            cols.append(jnp.where(lane < 32 * t, ldh(t, t - 1), ldh(t, t)))
        cols.append(ldh(4, 3))
        return jnp.concatenate(cols, axis=-1).astype(BF16)

    def mm2(r0, g=None):
        g = g_prep(r0) if g is None else g
        x2 = hb[rows(r0, TB), :] + jnp.dot(g, _bf(w2b[...]), preferred_element_type=F32)
        hb[rows(r0, TB), :] = x2
        return x2

    def ln4(x2):
        m4, r4 = _stats(x2)
        return (x2 - m4) * r4

    def mm3(n4):
        n4 = n4.astype(BF16)
        us, gates = [], []
        for f0 in range(0, FF, 128):
            f1 = min(f0 + 128, FF)
            h3 = jax.lax.dot_general(n4, _bf(w3b[f0 // 2:f1 // 2, :]), NT_DIMS,
                                     preferred_element_type=F32)
            if f1 - f0 == 128:
                gates += [h3[0:8], h3[128:136]]
            us.append(_gelu(h3))
        return jnp.concatenate(us, axis=-1).astype(BF16), gates

    def mm4(r0, u, t, final=True):
        c0, c1 = 128 * t, 128 * t + 128
        h2 = jnp.dot(u, _bf(w4b[:, c0:c1]), preferred_element_type=F32)
        s = hb[rows(r0, TB), c0:c1] + h2
        if final:
            ob[rows(r0, TB, 16), c0:c1] = (x1b[rows(r0, TB), c0:c1] + par[4:5, c0:c1] * s).astype(BF16)
        else:
            hb[rows(r0, TB), c0:c1] = s

    def out_copy(r0, n):
        return pltpu.make_async_copy(ob.at[rows(r0, n, 16), :], o_hbm.at[0, rows(r0, n, 16), :], osem)

    wait("s0")
    env["taps"] = skb[...].astype(F32)
    env["dvec"] = sdb[...].astype(F32).reshape(1, D)
    cf = cb_[...].astype(F32)
    sc8 = jnp.broadcast_to(cf * jax.nn.sigmoid(cf), (8, D)).astype(BF16)
    for t in range(NT):
        conv_k(0, t)
    wait("c0")
    for t in range(NT):
        conv_x(0, t)
        if t >= 1:
            conv_inv(0, t - 1)
    for c in range(1, NB):
        wait(f"c{c}")
        conv_inv(c - 1, NT - 1)
        for t in range(NT):
            conv_k(c, t)
            if t >= 1:
                conv_inv(c, t - 1)
            conv_x(c, t)
    a_pre1(0, TB + AO)
    a_pre1(TB + AO, TB)

    wait("wmA")
    mod = jnp.dot(sc8, wmb[:, 0:3 * D], preferred_element_type=F32)[0:1]
    sa, ca, ga = [mod[:, D * i:D * (i + 1)] for i in range(3)]
    par[0:1, :] = (1.0 + ca) * ga
    par[1:2, :] = sa * ga
    conv_inv(NB - 1, NT - 1)
    a_pre2(0, TB + AO)
    a_pre2(TB + AO, TB)
    wait("wmB")
    mod = jnp.dot(sc8, wmb[:, 3 * D:5 * D], preferred_element_type=F32)[0:1]
    par[2:3, :] = 1.0 + mod[:, D:2 * D]
    par[3:4, :] = mod[:, 0:D]
    n3a = a_pre3(0, TB + AO).astype(BF16)
    n3b = a_pre3(TB + AO, TB).astype(BF16)

    wait("w1")
    mm1(0, TB + AO, n3a)
    mm1(TB + AO, TB, n3b)
    g0 = g_prep(0)
    wait("w2")
    n4 = ln4(mm2(0, g0)).astype(BF16)
    mm2(TB)
    wait("w3")
    u, _ = mm3(n4)
    n4b[...] = ln4(hb[TB:2 * TB, :])
    wait("w4")
    for t in range(NT):
        mm4(0, u, t, final=False)
    wait("rest")
    par[4:5, :] = jnp.dot(sc8, wmb[:, 5 * D:6 * D], preferred_element_type=F32)[0:1]

    def body(i, carry):
        r0 = i * TB
        u, gates = mm3(n4b[...])
        n3 = a_pre_gated(r0 + TB + AO, [gates[j * 25 // 15] for j in range(TB // CH)])
        mm4(r0, u, 0)
        mm1(r0 + TB + AO, TB, n3)
        hpb[:, HPAD + S:HPAD + S + 8, :] = jnp.zeros((NT, 8, 128), F32)
        mm4(r0, u, 1)
        x2 = mm2(r0 + TB)
        n4b[...] = ln4(x2)
        for t in range(2, NT):
            mm4(r0, u, t)
        out_copy(r0, TB).start()
        return carry

    jax.lax.fori_loop(1, NBLK - 1, body, 0)

    r0 = S - TB
    u, _ = mm3(n4b[...])
    ob[0:TB, :] = (x1b[0:TB, :] + prm(4) * hb[0:TB, :]).astype(BF16)
    out_copy(0, TB).start()
    for t in range(NT):
        mm4(r0, u, t)
    out_copy(r0, TB).start()
    with jax.named_scope("W_out"):
        pltpu.make_async_copy(ob, o_hbm.at[0], osem).wait()


@jax.jit
def pallas_adaLN_cond__ssm_conv_h3__mixer_s_mlp__prompt_kernel(
    A_q, A_k, A_v, A_shift_k, A_ssm_k, A_ssm_D, B_x, B_w1, B_w2, B_w3, B_w4, c, w_mod,
):
    del B_x
    vm = pltpu.VMEM
    scratch = [
        vm(((S + AO) // 2, D), U32),
        vm((NT, KPAD + S, 128), BF16),
        vm((NT, S, 128), BF16),
        vm((4, D), BF16),
        vm((D // 2, S), U32),
        vm((D,), BF16),
        vm((D // 2, D), U32),
        vm((D // 2, D), U32),
        vm((FF // 2, D), U32),
        vm((FF // 2, D), U32),
        vm((1, D), BF16),
        vm((D, 6 * D), BF16),
        vm((R, 128, 128), U32),
        vm((R, 2, 64, 128), U32),
        vm((NT, S // 2, 128), U32),
        vm((10, NT, R, 256, 128), F32),
        vm((3, NT, R, 128, 128), U32),
        vm((NT, S + AO, 128), F32),
        vm((S + AO, D), F32),
        vm((S + AO, D), F32),
        vm((NT, HPAD + S + AO, 128), F32),
        vm((TB, D), F32),
        vm((8, D), F32),
        vm((S, D), BF16),
        pltpu.SemaphoreType.DMA((12,)),
        pltpu.SemaphoreType.DMA(()),
    ]
    hbm = pl.BlockSpec(memory_space=pltpu.HBM)
    return pl.pallas_call(
        _kernel,
        out_shape=jax.ShapeDtypeStruct((1, S, D), BF16),
        in_specs=[hbm] * 14,
        out_specs=hbm,
        scratch_shapes=scratch,
        compiler_params=pltpu.CompilerParams(vmem_limit_bytes=110 * 2**20,
                                             disable_semaphore_checks=True),
        name="h3_mixer",
    )(A_q, A_k, A_v, A_shift_k.T, A_ssm_k, A_ssm_D, B_w1, B_w2, B_w3.T, B_w4,
      c, w_mod, jnp.asarray(_FWD), jnp.asarray(_INV))
```

```python
import jax
import jax.numpy as jnp
import numpy as np
import jax.experimental.pallas as pl
import jax.experimental.pallas.tpu as pltpu

S, D, FF = 2048, 640, 1728
NT = D // 128
L = 512
NB = S // L
NFFT = 2 * L
R = 4
KPAD = 16
HPAD = 8
TB = 256
NBLK = S // TB
AO = 16
CH = 16
EPS = 1e-5
F32 = jnp.float32
BF16 = jnp.bfloat16
U32 = jnp.uint32
I32 = jnp.int32
NT_DIMS = (((1,), (1,)), ((), ()))
K0P, K1P, K1R, K2R, X0S, X1S, Z1P, Z2P, Z3P = range(9)


def _cos_coefs(deg=6):
    u = (np.cos(np.pi * (np.arange(400) + 0.5) / 400) + 1.0) / 2.0
    c = np.polynomial.polynomial.polyfit(u, np.cos(np.pi * np.sqrt(u)), deg)
    return [np.float32(v) for v in c]


_COS = _cos_coefs()


def _cos_units(a, scale=1.0):
    x = (((a + 1024) & 2047) - 1024).astype(F32) * np.float32(1.0 / 1024.0)
    u = x * x
    acc = u * np.float32(_COS[-1] * scale) + np.float32(_COS[-2] * scale)
    for c in _COS[-3::-1]:
        acc = acc * u + np.float32(c * scale)
    return acc


def _freq2(chunk, s):
    return 4 * (8 * (chunk & 7) + s) + 2 * (chunk >> 3) + 1


def _gelu(x):
    c1 = np.float32(np.sqrt(2.0 / np.pi))
    c2 = np.float32(np.sqrt(2.0 / np.pi) * 0.044715)
    u = x * (c1 + c2 * (x * x))
    hx = 0.5 * x
    return hx + hx * jnp.tanh(u)


def _stats(x):
    m = jnp.sum(x, axis=-1, keepdims=True) * (1.0 / D)
    e2 = jnp.sum(x * x, axis=-1, keepdims=True) * (1.0 / D)
    v = jnp.maximum(e2 - m * m, 0.0)
    return m, jax.lax.rsqrt(v + EPS)


def _split(b):
    b = b.reshape(16, 2, 8, 128)
    return b[:, 0], b[:, 1]


def _join(z):
    return jnp.stack(z, axis=1).reshape(256, 128)


def _fft4(b, sign):
    (r0, i0), (r1, i1), (r2, i2), (r3, i3) = b
    sr, si, dr, di = r0 + r2, i0 + i2, r0 - r2, i0 - i2
    tr, ti, er, ei = r1 + r3, i1 + i3, r1 - r3, i1 - i3
    x0 = (sr + tr, si + ti)
    x2 = (sr - tr, si - ti)
    xm = (dr + ei, di - er)
    xp = (dr - ei, di + er)
    return [x0, xm, x2, xp] if sign < 0 else [x0, xp, x2, xm]


def _cmul(a, b, acc=None):
    (ar, ai), (br, bi) = a, b
    if acc is None:
        return ar * br - ai * bi, ar * bi + ai * br
    return (acc[0] + ar * br) - ai * bi, (acc[1] + ar * bi) + ai * br


def _bf(x):
    return pltpu.bitcast(x, BF16)


def _pack(a, b):
    return pltpu.pack_elementwise([a, b], packed_dtype=BF16)


def _tie(w, ties):
    if not ties:
        return w
    parts = []
    for i in range(w.shape[0] // 8):
        p = w[8 * i:8 * i + 8]
        if i in ties:
            z = ties[i]
            p = p | z if p.shape[1] == 128 else jnp.concatenate([p[:, :128] | z, p[:, 128:]], axis=1)
        parts.append(p)
    return jnp.concatenate(parts, axis=0)


def _kernel(q_hbm, k_hbm, v_hbm, sk_hbm, ssm_hbm, sd_hbm, w1_hbm, w2_hbm, w3_hbm,
            w4_hbm, c_hbm, wm_hbm, o_hbm,
            qb, kb, vb, skb, ssmb, sdb, w1b, w2b, w3b, w4b, cb_, wmb, fwb, gib,
            stb, spec, cmb, yb, x1b, hb, hpb, n4b, par, ob, sems, osem):
    groups = {}

    def add(name, src, dst):
        if name not in groups:
            groups[name] = (len(groups), [])
        idx, lst = groups[name]
        cp = pltpu.make_async_copy(src, dst, sems.at[idx])
        cp.start()
        lst.append(cp)

    def add_kv(name, c, tiles=range(NT)):
        for t in tiles:
            add(name, k_hbm.at[0, pl.ds(L * c, L), pl.ds(128 * t, 128)],
                kb.at[t, pl.ds(KPAD + L * c, L), :])
            add(name, v_hbm.at[0, pl.ds(L * c, L), pl.ds(128 * t, 128)],
                vb.at[t, pl.ds(L * c, L), :])

    def add_ssm(name, c):
        add(name, ssm_hbm.at[:, pl.ds(L * c, L)], ssmb.bitcast(BF16).at[:, pl.ds(L * c, L)])

    QE = 2 * TB + AO
    add_ssm("r0", 0)
    add("r0", sd_hbm, sdb)
    add("r0", sk_hbm, skb)
    add("r0", c_hbm, cb_)
    add_kv("r1", 0, range(3))
    add_kv("r2", 0, range(3, NT))
    add_ssm("r2", 1)
    add_kv("r3", 1)
    add_ssm("r3", 2)
    add_kv("r4", 2)
    add_ssm("r4", 3)
    add("wmA", q_hbm.at[0, pl.ds(0, QE), :], qb.bitcast(BF16).at[pl.ds(0, QE), :])
    add("wmA", wm_hbm.at[:, pl.ds(0, 3 * D)], wmb.at[:, pl.ds(0, 3 * D)])
    add("wmB", wm_hbm.at[:, pl.ds(3 * D, 2 * D)], wmb.at[:, pl.ds(3 * D, 2 * D)])
    add("w1", w1_hbm, w1b.bitcast(BF16))
    add("w2", w2_hbm, w2b.bitcast(BF16))
    add_kv("w2", 3, range(3))
    add_kv("w3", 3, range(3, NT))
    add("w3", w3_hbm, w3b.bitcast(BF16))
    add("w4", w4_hbm, w4b.bitcast(BF16))
    add("rest", q_hbm.at[0, pl.ds(QE, S - QE), :], qb.bitcast(BF16).at[pl.ds(QE, S - QE), :])
    add("rest", wm_hbm.at[:, pl.ds(5 * D, D)], wmb.at[:, pl.ds(5 * D, D)])

    def wait(name):
        with jax.named_scope("W_" + name):
            for cp in groups[name][1]:
                cp.wait()

    kb[:, 0:KPAD, :] = jnp.zeros((NT, KPAD, 128), BF16)
    hpb[:, 0:HPAD, :] = jnp.zeros((NT, HPAD, 128), F32)
    yb[:, S:S + AO, :] = jnp.zeros((NT, AO, 128), F32)
    qb[S // 2:(S + AO) // 2, :] = jnp.zeros((AO // 2, D), U32)

    spec[9, 0, 0, pl.ds(0, 8, stride=2), :] = jnp.zeros((8, 128), F32)
    cmb[2, 0, 0, pl.ds(0, 8, stride=2), :] = jnp.zeros((8, 128), U32)
    fwb[R, pl.ds(0, 8, stride=2), :] = jnp.zeros((8, 128), U32)
    gib[R, 0, pl.ds(0, 8, stride=2), :] = jnp.zeros((8, 128), U32)

    row = jax.lax.broadcasted_iota(I32, (128, 128), 0)
    col = jax.lax.broadcasted_iota(I32, (128, 128), 1)
    f2 = _freq2(row >> 3, 2 * (row & 3))
    ph = 512 * ((row >> 2) & 1)
    for r in range(R):
        n = 4 * col + r
        a = n * f2 + ph
        fwb[r] = _pack(_cos_units(a), _cos_units(a + 4 * n))
    row = jax.lax.broadcasted_iota(I32, (64, 128), 0)
    col = jax.lax.broadcasted_iota(I32, (64, 128), 1)
    for h in range(2):
        f2 = _freq2(8 * h + (col >> 4), (col >> 1) & 7)
        ph = 512 * (col & 1)
        for r in range(R):
            a = (8 * row + r) * f2 + ph
            gib[r, h] = _pack(_cos_units(a, 2.0 / NFFT), _cos_units(a + 4 * f2, 2.0 / NFFT))

    env = {}

    def zero_after(*vals):
        acc = None
        for v in vals:
            v = pltpu.bitcast(v, U32)
            for i in range(0, v.shape[0], 8):
                for j in range(0, v.shape[1], 128):
                    p = v[i:i + 8, j:j + 128]
                    acc = p if acc is None else acc | p
        return acc & kb.bitcast(U32)[0, 0:8, :]

    def ld_spec(slot, t, q):
        return _split(spec[slot, t, q])

    def st_spec(slot, t, q, z):
        spec[slot, t, q] = _join(z)

    def fwd_dots(rhs, ties):
        return [_split(jnp.dot(_bf(_tie(fwb[r], ties if r == 0 else None)), _bf(rhs[r]),
                               preferred_element_type=F32)) for r in range(R)]

    def conv_k(c, t, ties):
        w0 = L * c // 2
        stb[t, w0:w0 + L // 2, :] = pltpu.bitcast(
            _bf(ssmb[64 * t:64 * t + 64, L * c:L * c + L]).T, U32)
        rhs = []
        for h in range(2):
            lo = stb[t, pl.ds(w0 + h, 64, stride=4), :]
            hi = stb[t, pl.ds(w0 + h + 2, 64, stride=4), :]
            rhs.append((lo & jnp.uint32(0xFFFF)) | (hi << 16))
            rhs.append((lo >> 16) | (hi & jnp.uint32(0xFFFF0000)))
        b = fwd_dots(rhs, ties)
        if c == 0:
            b[0] = (b[0][0] + env["dvec"][:, 128 * t:128 * t + 128][None], b[0][1])
        kq = _fft4(b, -1)
        for q in range(R):
            re, im = kq[q]
            if c == 0:
                st_spec(K0P, t, q, kq[q])
                continue
            if c < 3:
                st_spec((K1R, K2R)[c - 1], t, q, kq[q])
            pr, pi = ld_spec((K0P, K1R, K2R)[c - 1], t, q)
            kp = (jnp.concatenate([re[:8] - pi[:8], re[8:] + pi[8:]], axis=0),
                  jnp.concatenate([im[:8] + pr[:8], im[8:] - pr[8:]], axis=0))
            x0 = ld_spec(X0S, t, q)
            if c == 1:
                st_spec(K1P, t, q, kp)
                st_spec(Z1P, t, q, _cmul(kp, x0))
            elif c == 2:
                st_spec(Z2P, t, q, _cmul(kp, x0, ld_spec(Z2P, t, q)))
                st_spec(Z3P, t, q, _cmul(kp, ld_spec(X1S, t, q)))
            else:
                st_spec(Z3P, t, q, _cmul(kp, x0, ld_spec(Z3P, t, q)))

    def unpack(u):
        return (pltpu.bitcast(u << 16, F32),
                pltpu.bitcast(u & jnp.uint32(0xFFFF0000), F32))

    def conv_prep(c, t):
        taps = env["taps"]
        ku = kb.bitcast(U32)
        vu = vb.bitcast(U32)
        tp = [taps[j:j + 1, 128 * t:128 * t + 128] for j in range(4)]
        w0 = (KPAD + L * c) // 2
        kk = [unpack(ku[t, pl.ds(w0 - 2, 64, stride=4), :])[1]]
        for o in range(-1, 4):
            kk += unpack(ku[t, pl.ds(w0 + o, 64, stride=4), :])
        vv = []
        for o in range(4):
            vv += unpack(vu[t, pl.ds(L * c // 2 + o, 64, stride=4), :])
        kv = []
        for n in range(8):
            acc = kk[3 + n] * tp[0]
            for j in range(1, 4):
                acc = acc + kk[3 + n - j] * tp[j]
            kv.append(acc * vv[n])
        return [_pack(kv[r], kv[r + 4]) for r in range(R)]

    def conv_x(c, t, ties):
        xq = _fft4(fwd_dots(env.pop(("kv", c, t)), ties), -1)
        z = []
        for q in range(R):
            if c < 2:
                st_spec((X0S, X1S)[c], t, q, xq[q])
            acc = None if c == 0 else ld_spec((Z1P, Z2P, Z3P)[c - 1], t, q)
            z.append(_cmul(xq[q], ld_spec(K0P, t, q), acc))
            if c == 1:
                st_spec(Z2P, t, q, _cmul(xq[q], ld_spec(K1P, t, q)))
            elif c == 2:
                st_spec(Z3P, t, q, _cmul(xq[q], ld_spec(K1P, t, q), ld_spec(Z3P, t, q)))
        cr = _fft4(z, +1)
        for r in range(R):
            cmb[c % 2, t, r] = _pack(*cr[r]).reshape(128, 128)

    def conv_inv(c, t, ties):
        for r in range(R):
            tr = None
            if ties and r % 2 == 0:
                tr = {i - 4 * r: z for i, z in ties.items() if 0 <= i - 4 * r < 8}
            g = jnp.concatenate([_bf(_tie(gib[r, 0], tr)), _bf(gib[r, 1])], axis=-1)
            yb[t, pl.ds(L * c + r, 128, stride=R), :] = jnp.dot(
                g, _bf(cmb[c % 2, t, r]), preferred_element_type=F32)

    def run_rounds(spec_str):
        rounds = spec_str.split()
        plan = {}
        for n, rd in enumerate(rounds):
            if rd[0] == "X":
                pts = []
                if "@" in rd:
                    a, b = (float(v) for v in rd[4:].split(":"))
                    pts = [int(round(16 * (n - a + (a - b) * (j + 1) / 8))) - 1 for j in range(8)]
                plan.setdefault(pts[0] // 16 if pts else n, []).append((rd, pts))
        ties = {}
        for n, rd in enumerate(rounds):
            for xr, pts in plan.get(n, []):
                c, t = int(xr[1]), int(xr[2])
                kv = env["kv", c, t] = conv_prep(c, t)
                for j, p in enumerate(pts):
                    z = zero_after(*[w[8 * j:8 * j + 8] for w in kv])
                    d = ties.setdefault(p // 16, {})
                    d[p % 16] = z if p % 16 not in d else d[p % 16] | z
            {"K": conv_k, "X": conv_x, "I": conv_inv}[rd[0]](int(rd[1]), int(rd[2]), ties.get(n))

    def rows(r0, n, align=8):
        if isinstance(r0, int):
            return slice(r0, r0 + n)
        return pl.ds(pl.multiple_of(r0, align), n)

    def ld_y(r0, n):
        return jnp.concatenate([yb[t, rows(r0, n), :] for t in range(NT)], axis=-1)

    def prm(i):
        return par[i:i + 1, :]

    def a_pre12(r0, n):
        x = _bf(qb[r0 // 2:(r0 + n) // 2, :]).astype(F32)
        m1, r1 = _stats(x)
        x1 = x + ((x - m1) * r1 * prm(0) + prm(1)) * ld_y(r0, n)
        x1b[r0:r0 + n, :] = x1
        env["m2", r0] = _stats(x1)

    def a_pre3(r0, n):
        m2, r2 = env.pop(("m2", r0))
        h = (x1b[r0:r0 + n, :] - m2) * r2 * prm(2) + prm(3)
        hb[r0:r0 + n, :] = h
        m3, r3 = _stats(h)
        return (hb[r0:r0 + n, :] - m3) * r3

    def a_pre(r0, gates):
        out = []
        for j, g in enumerate(gates):
            r = r0 + CH * j
            z = zero_after(g)
            qv = qb[rows(r0 // 2 + CH // 2 * j, CH // 2), :] | jnp.concatenate([z] * NT, axis=1)
            x = _bf(qv).astype(F32)
            m1, r1 = _stats(x)
            x1 = x + ((x - m1) * r1 * prm(0) + prm(1)) * ld_y(r, CH)
            x1b[rows(r, CH), :] = x1
            m2, r2 = _stats(x1)
            h = (x1 - m2) * r2 * prm(2) + prm(3)
            hb[rows(r, CH), :] = h
            m3, r3 = _stats(h)
            out.append((h - m3) * r3)
        return jnp.concatenate(out, axis=0)

    def halves(n, split):
        return [(0, n // 2), (n // 2, n - n // 2)] if split else [(0, n)]

    def mm1(r0, n, n3, split_last=False):
        for t in range(NT):
            for o, m in halves(n, split_last and t == NT - 1):
                hp = jnp.dot(n3[o:o + m].astype(BF16), _bf(w1b[:, 128 * t:128 * t + 128]),
                             preferred_element_type=F32)
                hpb[t, rows(HPAD + r0 + o, m), :] = _gelu(hp)

    def g_prep(r0):
        lane = jax.lax.broadcasted_iota(I32, (TB, 128), 1)
        sh = [-1, 1, -2, 2]

        def ldh(t, g):
            return hpb[t, pl.ds(HPAD + r0 + sh[g], TB), :]

        cols = [ldh(0, 0)]
        for t in range(1, 4):
            cols.append(jnp.where(lane < 32 * t, ldh(t, t - 1), ldh(t, t)))
        cols.append(ldh(4, 3))
        return jnp.concatenate(cols, axis=-1)

    def mm2(r0, g, split_last=False, side=None):
        for t in range(NT):
            if side and t in side:
                side[t]()
            c0, c1 = 128 * t, 128 * t + 128
            for o, m in halves(TB, split_last and t == NT - 1):
                hs = jnp.dot(g[o:o + m].astype(BF16), _bf(w2b[:, c0:c1]), preferred_element_type=F32)
                hb[rows(r0 + o, m), c0:c1] = hb[rows(r0 + o, m), c0:c1] + hs
        return hs[m - 8:m]

    def ln4(r0, n):
        x2 = hb[rows(r0, n), :]
        m4, r4 = _stats(x2)
        return (x2 - m4) * r4

    def mm3(n4, ties=None, split_last=False, side=None):
        us = []
        env["g3"] = []
        for j, f0 in enumerate(range(0, FF, 128)):
            if side and j in side:
                side[j]()
            f1 = min(f0 + 128, FF)
            w = w3b[f0 // 2:f1 // 2, :]
            if ties and j in ties:
                w = _tie(w, {0: ties[j]})
            parts = []
            for o, m in halves(TB, split_last and f1 == FF):
                h3 = jax.lax.dot_general(n4[o:o + m].astype(BF16), _bf(w), NT_DIMS,
                                         preferred_element_type=F32)
                parts.append(_gelu(h3))
                if m == TB and f1 - f0 == 128:
                    env["g3"] += [h3[0:8], h3[128:136]]
            us.append(jnp.concatenate(parts, axis=0))
        return jnp.concatenate(us, axis=-1)

    def mm4(r0, u, t, final=True, ties=None, split=False):
        c0, c1 = 128 * t, 128 * t + 128
        w = _bf(_tie(w4b[:, c0:c1], ties))
        for o, m in halves(TB, split):
            h2 = jnp.dot(u[o:o + m].astype(BF16), w, preferred_element_type=F32)
            s = hb[rows(r0 + o, m), c0:c1] + h2
            if final:
                ob[rows(r0 + o, m, 16), c0:c1] = (
                    x1b[rows(r0 + o, m), c0:c1] + par[4:5, c0:c1] * s).astype(BF16)
            else:
                hb[rows(r0 + o, m), c0:c1] = s

    def ln4_store(r0, nch):
        zs = []
        m = TB // nch
        for j in range(nch):
            n4 = ln4(r0 + m * j, m)
            n4b[m * j:m * j + m, :] = n4
            zs.append(zero_after(n4))
        return zs

    def ln4_ticked(r0, g, nch, hops):
        z = zero_after(g)
        m = TB // nch
        for j in range(nch):
            zt = jnp.concatenate([jnp.concatenate([z] * NT, axis=1)] * (m // 8), axis=0)
            x2 = pltpu.bitcast(pltpu.bitcast(hb[rows(r0 + m * j, m), :], U32) | zt, F32)
            m4, r4 = _stats(x2)
            n4b[m * j:m * j + m, :] = (x2 - m4) * r4
            for _ in range(hops):
                z = pltpu.roll(z, 1, 1)

    def out_copy(r0, n, c0=0, c1=D):
        return pltpu.make_async_copy(ob.at[rows(r0, n, 16), c0:c1],
                                     o_hbm.at[0, rows(r0, n, 16), c0:c1], osem)

    def out_copy_old(r0, n):
        return pltpu.make_async_copy(ob.at[rows(r0, n, 16), :], o_hbm.at[0, rows(r0, n, 16), :], osem)

    wait("r0")
    env["taps"] = skb[...].astype(F32)
    env["dvec"] = sdb[...].astype(F32).reshape(1, D)
    cf = cb_[...].astype(F32)
    sc8 = jnp.broadcast_to(cf * jax.nn.sigmoid(cf), (8, D)).astype(BF16)
    run_rounds("K00 K01 K02 K03 K04")
    wait("r1")
    run_rounds("X00 X01@1:0.2 X02@1:0.2 I00")
    wait("r2")
    run_rounds("I01 X03@1:0.2 I02 K10 X04@1.5:0.5 K11 I03 K12 K13 K14")
    for c in (1, 2):
        wait(f"r{c + 2}")
        seq = f"I{c - 1}4 X{c}0@1:0.2 K{c + 1}0 X{c}1@1:0.2"
        for t in range(1, NT):
            seq += f" I{c}{t - 1} K{c + 1}{t}"
            if t + 1 < NT:
                seq += f" X{c}{t + 1}@1.5:0.5"
        run_rounds(seq)

    wait("wmA")
    mod = jnp.dot(sc8, wmb[:, 0:3 * D], preferred_element_type=F32)[0:1]
    sa, ca, ga = [mod[:, D * i:D * (i + 1)] for i in range(3)]
    par[0:1, :] = (1.0 + ca) * ga
    par[1:2, :] = sa * ga
    run_rounds("I24")
    a_pre12(0, TB + AO)
    a_pre12(TB + AO, TB)
    wait("wmB")
    mod = jnp.dot(sc8, wmb[:, 3 * D:5 * D], preferred_element_type=F32)[0:1]
    par[2:3, :] = 1.0 + mod[:, D:2 * D]
    par[3:4, :] = mod[:, 0:D]
    n3a = a_pre3(0, TB + AO)
    n3b = a_pre3(TB + AO, TB)

    wait("w1")
    mm1(0, TB + AO, n3a)
    mm1(TB + AO, TB, n3b, split_last=True)
    g0 = g_prep(0)
    wait("w2")
    rr = lambda x: (lambda: run_rounds(x))
    mm2(0, g0, side={2: rr("X30"), 4: rr("X31")})
    n4 = ln4(0, TB)
    mm2(TB, g_prep(TB), split_last=True, side={0: rr("I30"), 2: rr("X32 I31"), 4: rr("I32")})
    wait("w3")
    zs = ln4_store(TB, 8)
    u = mm3(n4, {6 + j: z for j, z in enumerate(zs)}, split_last=True,
            side={2: rr("X33"), 5: rr("X34"), 8: rr("I33"), 10: rr("I34")})
    wait("w4")
    for t in range(NT):
        mm4(0, u, t, final=False, split=t == NT - 1)
    wait("rest")
    par[4:5, :] = jnp.dot(sc8, wmb[:, 5 * D:6 * D], preferred_element_type=F32)[0:1]

    def body(i, carry):
        r0 = i * TB
        u = mm3(n4b[...])
        n3 = a_pre(r0 + TB + AO, [env["g3"][j * 23 // 15] for j in range(TB // CH)])
        mm4(r0, u, 0)
        mm1(r0 + TB + AO, TB, n3)
        hpb[:, HPAD + S:HPAD + S + 8, :] = jnp.zeros((NT, 8, 128), F32)
        mm4(r0, u, 1)
        g = mm2(r0 + TB, g_prep(r0 + TB))
        ln4_ticked(r0 + TB, g, 16, 1)
        for t in range(2, NT):
            mm4(r0, u, t)
        out_copy(r0, TB).start()
        return carry

    jax.lax.fori_loop(1, NBLK - 1, body, 0)

    r0 = S - TB
    zs = []
    for j in range(8):
        rs = slice(32 * j, 32 * j + 32)
        o = x1b[rs, :] + prm(4) * hb[rs, :]
        ob[rs, :] = o.astype(BF16)
        zs.append(zero_after(o))
    u = mm3(n4b[...], {3 + j: z for j, z in enumerate(zs)})
    out_copy(0, TB).start()
    for t in range(NT):
        mm4(r0, u, t, split=t == NT - 1)
        if t < NT - 1:
            out_copy(r0, TB, 128 * t, 128 * t + 128).start()
    out_copy(r0, TB // 2, D - 128, D).start()
    out_copy(r0 + TB // 2, TB // 2, D - 128, D).start()
    with jax.named_scope("W_out"):
        pltpu.make_async_copy(ob, o_hbm.at[0], osem).wait()


@jax.jit
def pallas_adaLN_cond__ssm_conv_h3__mixer_s_mlp__prompt_kernel(
    A_q, A_k, A_v, A_shift_k, A_ssm_k, A_ssm_D, B_x, B_w1, B_w2, B_w3, B_w4, c, w_mod,
):
    del B_x
    vm = pltpu.VMEM
    scratch = [
        vm(((S + AO) // 2, D), U32),
        vm((NT, KPAD + S, 128), BF16),
        vm((NT, S, 128), BF16),
        vm((4, D), BF16),
        vm((D // 2, S), U32),
        vm((D,), BF16),
        vm((D // 2, D), U32),
        vm((D // 2, D), U32),
        vm((FF // 2, D), U32),
        vm((FF // 2, D), U32),
        vm((1, D), BF16),
        vm((D, 6 * D), BF16),
        vm((R + 1, 128, 128), U32),
        vm((R + 1, 2, 64, 128), U32),
        vm((NT, S // 2, 128), U32),
        vm((10, NT, R, 256, 128), F32),
        vm((3, NT, R, 128, 128), U32),
        vm((NT, S + AO, 128), F32),
        vm((S + AO, D), F32),
        vm((S + AO, D), F32),
        vm((NT, HPAD + S + AO, 128), F32),
        vm((TB, D), F32),
        vm((8, D), F32),
        vm((S, D), BF16),
        pltpu.SemaphoreType.DMA((12,)),
        pltpu.SemaphoreType.DMA(()),
    ]
    hbm = pl.BlockSpec(memory_space=pltpu.HBM)
    return pl.pallas_call(
        _kernel,
        out_shape=jax.ShapeDtypeStruct((1, S, D), BF16),
        in_specs=[hbm] * 12,
        out_specs=hbm,
        scratch_shapes=scratch,
        compiler_params=pltpu.CompilerParams(vmem_limit_bytes=110 * 2**20,
                                             disable_semaphore_checks=True),
        name="h3_mixer",
    )(A_q, A_k, A_v, A_shift_k.T, A_ssm_k, A_ssm_D, B_w1, B_w2, B_w3.T, B_w4, c, w_mod)
```

```python
import jax
import jax.numpy as jnp
import numpy as np
import jax.experimental.pallas as pl
import jax.experimental.pallas.tpu as pltpu

S, D, FF = 2048, 640, 1728
NT = D // 128
L = 512
NB = S // L
NFFT = 2 * L
R = 4
KPAD = 16
HPAD = 8
TB = 256
NBLK = S // TB
AO = 16
CH = 16
EPS = 1e-5
FM = FF // 128 * 128
F32 = jnp.float32
BF16 = jnp.bfloat16
U32 = jnp.uint32
I32 = jnp.int32
NT_DIMS = (((1,), (1,)), ((), ()))
K0P, K1P, K1R, K2R, X0S, X1S, Z1P, Z2P, Z3P = range(9)


def _cos_coefs(deg=6):
    u = (np.cos(np.pi * (np.arange(400) + 0.5) / 400) + 1.0) / 2.0
    c = np.polynomial.polynomial.polyfit(u, np.cos(np.pi * np.sqrt(u)), deg)
    return [np.float32(v) for v in c]


_COS = _cos_coefs()


def _cos_units(a, scale=1.0):
    x = (((a + 1024) & 2047) - 1024).astype(F32) * np.float32(1.0 / 1024.0)
    u = x * x
    acc = u * np.float32(_COS[-1] * scale) + np.float32(_COS[-2] * scale)
    for c in _COS[-3::-1]:
        acc = acc * u + np.float32(c * scale)
    return acc


def _freq2(chunk, s):
    return 4 * (8 * (chunk & 7) + s) + 2 * (chunk >> 3) + 1


def _gelu(x):
    c1 = np.float32(np.sqrt(2.0 / np.pi))
    c2 = np.float32(np.sqrt(2.0 / np.pi) * 0.044715)
    u = x * (c1 + c2 * (x * x))
    hx = 0.5 * x
    return hx + hx * jnp.tanh(u)


def _stats(x):
    m = jnp.sum(x, axis=-1, keepdims=True) * (1.0 / D)
    e2 = jnp.sum(x * x, axis=-1, keepdims=True) * (1.0 / D)
    v = jnp.maximum(e2 - m * m, 0.0)
    return m, jax.lax.rsqrt(v + EPS)


def _split(b):
    b = b.reshape(16, 2, 8, 128)
    return b[:, 0], b[:, 1]


def _join(z):
    return jnp.stack(z, axis=1).reshape(256, 128)


def _fft4(b, sign):
    (r0, i0), (r1, i1), (r2, i2), (r3, i3) = b
    sr, si, dr, di = r0 + r2, i0 + i2, r0 - r2, i0 - i2
    tr, ti, er, ei = r1 + r3, i1 + i3, r1 - r3, i1 - i3
    x0 = (sr + tr, si + ti)
    x2 = (sr - tr, si - ti)
    xm = (dr + ei, di - er)
    xp = (dr - ei, di + er)
    return [x0, xm, x2, xp] if sign < 0 else [x0, xp, x2, xm]


def _cmul(a, b, acc=None):
    (ar, ai), (br, bi) = a, b
    if acc is None:
        return ar * br - ai * bi, ar * bi + ai * br
    return (acc[0] + ar * br) - ai * bi, (acc[1] + ar * bi) + ai * br


def _bf(x):
    return pltpu.bitcast(x, BF16)


def _pack(a, b):
    return pltpu.pack_elementwise([a, b], packed_dtype=BF16)


def _tie(w, ties):
    if not ties:
        return w
    parts = []
    for i in range(w.shape[0] // 8):
        p = w[8 * i:8 * i + 8]
        if i in ties:
            z = ties[i]
            p = p | z if p.shape[1] == 128 else jnp.concatenate([p[:, :128] | z, p[:, 128:]], axis=1)
        parts.append(p)
    return jnp.concatenate(parts, axis=0)


def _kernel(q_hbm, k_hbm, v_hbm, sk_hbm, ssm_hbm, sd_hbm, w1_hbm, w2_hbm, w3_hbm,
            w4_hbm, c_hbm, wm_hbm, o_hbm,
            qb, kb, vb, skb, ssmb, sdb, w1b, w2b, w3b, w4b, cb_, wmb, fwb, gib,
            stb, spec, cmb, yb, x1b, hb, hpb, n4b, par, ob, sems, osem):
    groups = {}

    def add(name, src, dst):
        if name not in groups:
            groups[name] = (len(groups), [])
        idx, lst = groups[name]
        cp = pltpu.make_async_copy(src, dst, sems.at[idx])
        cp.start()
        lst.append(cp)

    def add_kv(name, c, tiles=range(NT)):
        for t in tiles:
            add(name, k_hbm.at[0, pl.ds(L * c, L), pl.ds(128 * t, 128)],
                kb.at[t, pl.ds(KPAD + L * c, L), :])
            add(name, v_hbm.at[0, pl.ds(L * c, L), pl.ds(128 * t, 128)],
                vb.at[t, pl.ds(L * c, L), :])

    def add_ssm(name, c):
        add(name, ssm_hbm.at[:, pl.ds(L * c, L)], ssmb.bitcast(BF16).at[:, pl.ds(L * c, L)])

    QE = 2 * TB + AO
    add_ssm("r0", 0)
    add("r0", sd_hbm, sdb)
    add("r0", sk_hbm, skb)
    add("r0", c_hbm, cb_)
    add_kv("r1", 0, range(3))
    add_kv("r2", 0, range(3, NT))
    add_ssm("r2", 1)
    add_kv("r3", 1)
    add_ssm("r3", 2)
    add_kv("r4", 2)
    add_ssm("r4", 3)
    add("wmA", q_hbm.at[0, pl.ds(0, QE), :], qb.bitcast(BF16).at[pl.ds(0, QE), :])
    add("wmA", wm_hbm.at[:, pl.ds(0, 3 * D)], wmb.at[:, pl.ds(0, 3 * D)])
    add("wmB", wm_hbm.at[:, pl.ds(3 * D, 2 * D)], wmb.at[:, pl.ds(3 * D, 2 * D)])
    add("w1", w1_hbm, w1b.bitcast(BF16))
    add("w2", w2_hbm, w2b.bitcast(BF16))
    add_kv("w2", 3, range(3))
    add_kv("w3", 3, range(3, NT))
    add("w3", w3_hbm, w3b.bitcast(BF16))
    add("w4", w4_hbm, w4b.bitcast(BF16))
    add("rest", q_hbm.at[0, pl.ds(QE, S - QE), :], qb.bitcast(BF16).at[pl.ds(QE, S - QE), :])
    add("rest", wm_hbm.at[:, pl.ds(5 * D, D)], wmb.at[:, pl.ds(5 * D, D)])

    def wait(name):
        with jax.named_scope("W_" + name):
            for cp in groups[name][1]:
                cp.wait()

    kb[:, 0:KPAD, :] = jnp.zeros((NT, KPAD, 128), BF16)
    hpb[:, 0:HPAD, :] = jnp.zeros((NT, HPAD, 128), F32)
    yb[:, S:S + AO, :] = jnp.zeros((NT, AO, 128), F32)
    qb[S // 2:(S + AO) // 2, :] = jnp.zeros((AO // 2, D), U32)

    spec[9, 0, 0, pl.ds(0, 8, stride=2), :] = jnp.zeros((8, 128), F32)
    cmb[2, 0, 0, pl.ds(0, 8, stride=2), :] = jnp.zeros((8, 128), U32)
    fwb[R, pl.ds(0, 8, stride=2), :] = jnp.zeros((8, 128), U32)
    gib[R, 0, pl.ds(0, 8, stride=2), :] = jnp.zeros((8, 128), U32)

    row = jax.lax.broadcasted_iota(I32, (128, 128), 0)
    col = jax.lax.broadcasted_iota(I32, (128, 128), 1)
    f2 = _freq2(row >> 3, 2 * (row & 3))
    ph = 512 * ((row >> 2) & 1)
    for r in range(R):
        n = 4 * col + r
        a = n * f2 + ph
        fwb[r] = _pack(_cos_units(a), _cos_units(a + 4 * n))
    row = jax.lax.broadcasted_iota(I32, (64, 128), 0)
    col = jax.lax.broadcasted_iota(I32, (64, 128), 1)
    for h in range(2):
        f2 = _freq2(8 * h + (col >> 4), (col >> 1) & 7)
        ph = 512 * (col & 1)
        for r in range(R):
            a = (8 * row + r) * f2 + ph
            gib[r, h] = _pack(_cos_units(a, 2.0 / NFFT), _cos_units(a + 4 * f2, 2.0 / NFFT))

    env = {}

    def zero_after(*vals):
        acc = None
        for v in vals:
            v = pltpu.bitcast(v, U32)
            for i in range(0, v.shape[0], 8):
                for j in range(0, v.shape[1], 128):
                    p = v[i:i + 8, j:j + 128]
                    acc = p if acc is None else acc | p
        return acc & kb.bitcast(U32)[0, 0:8, :]

    def ld_spec(slot, t, q):
        return _split(spec[slot, t, q])

    def st_spec(slot, t, q, z):
        spec[slot, t, q] = _join(z)

    def fwd_dots(rhs, ties):
        return [_split(jnp.dot(_bf(_tie(fwb[r], ties if r == 0 else None)), _bf(rhs[r]),
                               preferred_element_type=F32)) for r in range(R)]

    def conv_k(c, t, ties):
        w0 = L * c // 2
        stb[t, w0:w0 + L // 2, :] = pltpu.bitcast(
            _bf(ssmb[64 * t:64 * t + 64, L * c:L * c + L]).T, U32)
        rhs = []
        for h in range(2):
            lo = stb[t, pl.ds(w0 + h, 64, stride=4), :]
            hi = stb[t, pl.ds(w0 + h + 2, 64, stride=4), :]
            rhs.append((lo & jnp.uint32(0xFFFF)) | (hi << 16))
            rhs.append((lo >> 16) | (hi & jnp.uint32(0xFFFF0000)))
        b = fwd_dots(rhs, ties)
        if c == 0:
            b[0] = (b[0][0] + env["dvec"][:, 128 * t:128 * t + 128][None], b[0][1])
        kq = _fft4(b, -1)
        for q in range(R):
            re, im = kq[q]
            if c == 0:
                st_spec(K0P, t, q, kq[q])
                continue
            if c < 3:
                st_spec((K1R, K2R)[c - 1], t, q, kq[q])
            pr, pi = ld_spec((K0P, K1R, K2R)[c - 1], t, q)
            kp = (jnp.concatenate([re[:8] - pi[:8], re[8:] + pi[8:]], axis=0),
                  jnp.concatenate([im[:8] + pr[:8], im[8:] - pr[8:]], axis=0))
            x0 = ld_spec(X0S, t, q)
            if c == 1:
                st_spec(K1P, t, q, kp)
                st_spec(Z1P, t, q, _cmul(kp, x0))
            elif c == 2:
                st_spec(Z2P, t, q, _cmul(kp, x0, ld_spec(Z2P, t, q)))
                st_spec(Z3P, t, q, _cmul(kp, ld_spec(X1S, t, q)))
            else:
                st_spec(Z3P, t, q, _cmul(kp, x0, ld_spec(Z3P, t, q)))

    def unpack(u):
        return (pltpu.bitcast(u << 16, F32),
                pltpu.bitcast(u & jnp.uint32(0xFFFF0000), F32))

    def conv_prep(c, t):
        taps = env["taps"]
        ku = kb.bitcast(U32)
        vu = vb.bitcast(U32)
        tp = [taps[j:j + 1, 128 * t:128 * t + 128] for j in range(4)]
        w0 = (KPAD + L * c) // 2
        kk = [unpack(ku[t, pl.ds(w0 - 2, 64, stride=4), :])[1]]
        for o in range(-1, 4):
            kk += unpack(ku[t, pl.ds(w0 + o, 64, stride=4), :])
        vv = []
        for o in range(4):
            vv += unpack(vu[t, pl.ds(L * c // 2 + o, 64, stride=4), :])
        kv = []
        for n in range(8):
            acc = kk[3 + n] * tp[0]
            for j in range(1, 4):
                acc = acc + kk[3 + n - j] * tp[j]
            kv.append(acc * vv[n])
        return [_pack(kv[r], kv[r + 4]) for r in range(R)]

    def conv_x(c, t, ties):
        xq = _fft4(fwd_dots(env.pop(("kv", c, t)), ties), -1)
        z = []
        for q in range(R):
            if c < 2:
                st_spec((X0S, X1S)[c], t, q, xq[q])
            acc = None if c == 0 else ld_spec((Z1P, Z2P, Z3P)[c - 1], t, q)
            z.append(_cmul(xq[q], ld_spec(K0P, t, q), acc))
            if c == 1:
                st_spec(Z2P, t, q, _cmul(xq[q], ld_spec(K1P, t, q)))
            elif c == 2:
                st_spec(Z3P, t, q, _cmul(xq[q], ld_spec(K1P, t, q), ld_spec(Z3P, t, q)))
        cr = _fft4(z, +1)
        for r in range(R):
            cmb[c % 2, t, r] = _pack(*cr[r]).reshape(128, 128)

    def conv_inv(c, t, ties):
        for r in range(R):
            tr = None
            if ties and r % 2 == 0:
                tr = {i - 4 * r: z for i, z in ties.items() if 0 <= i - 4 * r < 8}
            g = jnp.concatenate([_bf(_tie(gib[r, 0], tr)), _bf(gib[r, 1])], axis=-1)
            yb[t, pl.ds(L * c + r, 128, stride=R), :] = jnp.dot(
                g, _bf(cmb[c % 2, t, r]), preferred_element_type=F32)

    def run_rounds(spec_str):
        rounds = spec_str.split()
        plan = {}
        for n, rd in enumerate(rounds):
            if rd[0] == "X":
                pts = []
                if "@" in rd:
                    a, b = (float(v) for v in rd[4:].split(":"))
                    pts = [int(round(16 * (n - a + (a - b) * (j + 1) / 8))) - 1 for j in range(8)]
                plan.setdefault(pts[0] // 16 if pts else n, []).append((rd, pts))
        ties = {}
        for n, rd in enumerate(rounds):
            for xr, pts in plan.get(n, []):
                c, t = int(xr[1]), int(xr[2])
                kv = env["kv", c, t] = conv_prep(c, t)
                for j, p in enumerate(pts):
                    z = zero_after(*[w[8 * j:8 * j + 8] for w in kv])
                    d = ties.setdefault(p // 16, {})
                    d[p % 16] = z if p % 16 not in d else d[p % 16] | z
            {"K": conv_k, "X": conv_x, "I": conv_inv}[rd[0]](int(rd[1]), int(rd[2]), ties.get(n))

    def rows(r0, n, align=8):
        if isinstance(r0, int):
            return slice(r0, r0 + n)
        return pl.ds(pl.multiple_of(r0, align), n)

    def ld_y(r0, n):
        return jnp.concatenate([yb[t, rows(r0, n), :] for t in range(NT)], axis=-1)

    def prm(i):
        return par[i:i + 1, :]

    def a_pre12(r0, n):
        x = _bf(qb[r0 // 2:(r0 + n) // 2, :]).astype(F32)
        m1, r1 = _stats(x)
        x1 = x + ((x - m1) * r1 * prm(0) + prm(1)) * ld_y(r0, n)
        x1b[r0:r0 + n, :] = x1
        env["m2", r0] = _stats(x1)

    def a_pre3(r0, n):
        m2, r2 = env.pop(("m2", r0))
        h = (x1b[r0:r0 + n, :] - m2) * r2 * prm(2) + prm(3)
        hb[r0:r0 + n, :] = h
        m3, r3 = _stats(h)
        return (hb[r0:r0 + n, :] - m3) * r3

    def a_pre(r0, gates):
        out = []
        for j, g in enumerate(gates):
            r = r0 + CH * j
            z = zero_after(g)
            qv = qb[rows(r0 // 2 + CH // 2 * j, CH // 2), :] | jnp.concatenate([z] * NT, axis=1)
            x = _bf(qv).astype(F32)
            m1, r1 = _stats(x)
            x1 = x + ((x - m1) * r1 * prm(0) + prm(1)) * ld_y(r, CH)
            x1b[rows(r, CH), :] = x1
            m2, r2 = _stats(x1)
            h = (x1 - m2) * r2 * prm(2) + prm(3)
            hb[rows(r, CH), :] = h
            m3, r3 = _stats(h)
            out.append((h - m3) * r3)
        return jnp.concatenate(out, axis=0)

    def halves(n, split):
        return [(0, n // 2), (n // 2, n - n // 2)] if split else [(0, n)]

    def mm1(r0, n, n3, split_last=False):
        for t in range(NT):
            for o, m in halves(n, split_last and t == NT - 1):
                hp = jnp.dot(n3[o:o + m].astype(BF16), _bf(w1b[:, 128 * t:128 * t + 128]),
                             preferred_element_type=F32)
                hpb[t, rows(HPAD + r0 + o, m), :] = _gelu(hp)

    def g_prep(r0):
        lane = jax.lax.broadcasted_iota(I32, (TB, 128), 1)
        sh = [-1, 1, -2, 2]

        def ldh(t, g):
            return hpb[t, pl.ds(HPAD + r0 + sh[g], TB), :]

        cols = [ldh(0, 0)]
        for t in range(1, 4):
            cols.append(jnp.where(lane < 32 * t, ldh(t, t - 1), ldh(t, t)))
        cols.append(ldh(4, 3))
        return jnp.concatenate(cols, axis=-1)

    def mm2(r0, g, split_last=False, side=None):
        for t in range(NT):
            if side and t in side:
                side[t]()
            c0, c1 = 128 * t, 128 * t + 128
            for o, m in halves(TB, split_last and t == NT - 1):
                hs = jnp.dot(g[o:o + m].astype(BF16), _bf(w2b[:, c0:c1]), preferred_element_type=F32)
                hb[rows(r0 + o, m), c0:c1] = hb[rows(r0 + o, m), c0:c1] + hs
        return hs[m - 8:m]

    def ln4(r0, n):
        x2 = hb[rows(r0, n), :]
        m4, r4 = _stats(x2)
        return (x2 - m4) * r4

    def mm3(n4, ties=None, split_last=False, side=None, tpos=6):
        us = []
        env["g3"] = []
        for j in range(FF // 128):
            if side and j in side:
                side[j]()
            if j == tpos:
                ht = jax.lax.dot_general(_bf(w3b[FM // 2:FF // 2, :]), n4.astype(BF16), NT_DIMS,
                                         preferred_element_type=F32)
                ut = _gelu(ht).T
            w = w3b[64 * j:64 * j + 64, :]
            if ties and j in ties:
                w = _tie(w, {0: ties[j]})
            parts = []
            for o, m in halves(TB, split_last and j == FF // 128 - 1):
                h3 = jax.lax.dot_general(n4[o:o + m].astype(BF16), _bf(w), NT_DIMS,
                                         preferred_element_type=F32)
                parts.append(_gelu(h3))
                if m == TB:
                    env["g3"] += [h3[0:8], h3[128:136]]
            us.append(jnp.concatenate(parts, axis=0))
        return jnp.concatenate(us + [ut], axis=-1)

    def mm4(r0, u, t, final=True, ties=None, split=False):
        c0, c1 = 128 * t, 128 * t + 128
        w = _bf(_tie(w4b[:, c0:c1], ties))
        for o, m in halves(TB, split):
            h2 = jnp.dot(u[o:o + m].astype(BF16), w, preferred_element_type=F32)
            s = hb[rows(r0 + o, m), c0:c1] + h2
            if final:
                ob[rows(r0 + o, m, 16), c0:c1] = (
                    x1b[rows(r0 + o, m), c0:c1] + par[4:5, c0:c1] * s).astype(BF16)
            else:
                hb[rows(r0 + o, m), c0:c1] = s

    def ln4_store(r0, nch):
        zs = []
        m = TB // nch
        for j in range(nch):
            n4 = ln4(r0 + m * j, m)
            n4b[m * j:m * j + m, :] = n4
            zs.append(zero_after(n4))
        return zs

    def ln4_ticked(r0, g, nch, hops):
        z = zero_after(g)
        m = TB // nch
        for j in range(nch):
            zt = jnp.concatenate([jnp.concatenate([z] * NT, axis=1)] * (m // 8), axis=0)
            x2 = pltpu.bitcast(pltpu.bitcast(hb[rows(r0 + m * j, m), :], U32) | zt, F32)
            m4, r4 = _stats(x2)
            n4b[m * j:m * j + m, :] = (x2 - m4) * r4
            for _ in range(hops):
                z = pltpu.roll(z, 1, 1)

    def out_copy(r0, n, c0=0, c1=D):
        return pltpu.make_async_copy(ob.at[rows(r0, n, 16), c0:c1],
                                     o_hbm.at[0, rows(r0, n, 16), c0:c1], osem)

    def out_copy_old(r0, n):
        return pltpu.make_async_copy(ob.at[rows(r0, n, 16), :], o_hbm.at[0, rows(r0, n, 16), :], osem)

    wait("r0")
    env["taps"] = skb[...].astype(F32)
    env["dvec"] = sdb[...].astype(F32).reshape(1, D)
    cf = cb_[...].astype(F32)
    sc8 = jnp.broadcast_to(cf * jax.nn.sigmoid(cf), (8, D)).astype(BF16)
    run_rounds("K00 K01 K02 K03 K04")
    wait("r1")
    run_rounds("X00 X01@1:0.2 X02@1:0.2 I00")
    wait("r2")
    run_rounds("I01 X03@1:0.2 I02 K10 X04@1.5:0.5 K11 I03 K12 K13 K14")
    for c in (1, 2):
        wait(f"r{c + 2}")
        seq = f"I{c - 1}4 X{c}0@1:0.2 K{c + 1}0 X{c}1@1:0.2"
        for t in range(1, NT):
            seq += f" I{c}{t - 1} K{c + 1}{t}"
            if t + 1 < NT:
                seq += f" X{c}{t + 1}@1.5:0.5"
        run_rounds(seq)

    wait("wmA")
    mod = jnp.dot(sc8, wmb[:, 0:3 * D], preferred_element_type=F32)[0:1]
    sa, ca, ga = [mod[:, D * i:D * (i + 1)] for i in range(3)]
    par[0:1, :] = (1.0 + ca) * ga
    par[1:2, :] = sa * ga
    run_rounds("I24")
    a_pre12(0, TB + AO)
    a_pre12(TB + AO, TB)
    wait("wmB")
    mod = jnp.dot(sc8, wmb[:, 3 * D:5 * D], preferred_element_type=F32)[0:1]
    par[2:3, :] = 1.0 + mod[:, D:2 * D]
    par[3:4, :] = mod[:, 0:D]
    n3a = a_pre3(0, TB + AO)

    wait("w1")
    mm1(0, TB + AO, n3a)
    n3b = a_pre3(TB + AO, TB)
    mm1(TB + AO, TB, n3b, split_last=True)
    wait("w2")
    g0 = g_prep(0)
    rr = lambda x: (lambda: run_rounds(x))
    mm2(0, g0, side={2: rr("X30"), 4: rr("X31")})
    n4 = ln4(0, TB)
    mm2(TB, g_prep(TB), split_last=True, side={0: rr("I30"), 2: rr("X32 I31"), 4: rr("I32")})
    wait("w3")
    zs = ln4_store(TB, 8)
    u = mm3(n4, {5 + j: z for j, z in enumerate(zs)}, split_last=True,
            side={2: rr("X33"), 5: rr("X34"), 8: rr("I33"), 10: rr("I34")})
    wait("w4")
    for t in range(NT):
        mm4(0, u, t, final=False, split=t == NT - 1)
    wait("rest")
    par[4:5, :] = jnp.dot(sc8, wmb[:, 5 * D:6 * D], preferred_element_type=F32)[0:1]

    def body(i, carry):
        r0 = i * TB
        u = mm3(n4b[...])
        n3 = a_pre(r0 + TB + AO, [env["g3"][j * 21 // 15] for j in range(TB // CH)])
        mm4(r0, u, 0)
        mm1(r0 + TB + AO, TB, n3)
        hpb[:, HPAD + S:HPAD + S + 8, :] = jnp.zeros((NT, 8, 128), F32)
        mm4(r0, u, 1)
        g = mm2(r0 + TB, g_prep(r0 + TB))
        ln4_ticked(r0 + TB, g, 16, 1)
        for t in range(2, NT):
            mm4(r0, u, t)
        out_copy(r0, TB).start()
        return carry

    jax.lax.fori_loop(1, NBLK - 1, body, 0)

    r0 = S - TB
    zs = []
    for j in range(8):
        rs = slice(32 * j, 32 * j + 32)
        o = x1b[rs, :] + prm(4) * hb[rs, :]
        ob[rs, :] = o.astype(BF16)
        zs.append(zero_after(o))
    u = mm3(n4b[...], {3 + j: z for j, z in enumerate(zs)})
    out_copy(0, TB).start()
    for t in range(NT):
        mm4(r0, u, t, split=t == NT - 1)
        if t < NT - 1:
            out_copy(r0, TB, 128 * t, 128 * t + 128).start()
    out_copy(r0, TB // 2, D - 128, D).start()
    out_copy(r0 + TB // 2, TB // 2, D - 128, D).start()
    with jax.named_scope("W_out"):
        pltpu.make_async_copy(ob, o_hbm.at[0], osem).wait()


@jax.jit
def pallas_adaLN_cond__ssm_conv_h3__mixer_s_mlp__prompt_kernel(
    A_q, A_k, A_v, A_shift_k, A_ssm_k, A_ssm_D, B_x, B_w1, B_w2, B_w3, B_w4, c, w_mod,
):
    del B_x
    vm = pltpu.VMEM
    scratch = [
        vm(((S + AO) // 2, D), U32),
        vm((NT, KPAD + S, 128), BF16),
        vm((NT, S, 128), BF16),
        vm((4, D), BF16),
        vm((D // 2, S), U32),
        vm((D,), BF16),
        vm((D // 2, D), U32),
        vm((D // 2, D), U32),
        vm((FF // 2, D), U32),
        vm((FF // 2, D), U32),
        vm((1, D), BF16),
        vm((D, 6 * D), BF16),
        vm((R + 1, 128, 128), U32),
        vm((R + 1, 2, 64, 128), U32),
        vm((NT, S // 2, 128), U32),
        vm((10, NT, R, 256, 128), F32),
        vm((3, NT, R, 128, 128), U32),
        vm((NT, S + AO, 128), F32),
        vm((S + AO, D), F32),
        vm((S + AO, D), F32),
        vm((NT, HPAD + S + AO, 128), F32),
        vm((TB, D), F32),
        vm((8, D), F32),
        vm((S, D), BF16),
        pltpu.SemaphoreType.DMA((12,)),
        pltpu.SemaphoreType.DMA(()),
    ]
    hbm = pl.BlockSpec(memory_space=pltpu.HBM)
    return pl.pallas_call(
        _kernel,
        out_shape=jax.ShapeDtypeStruct((1, S, D), BF16),
        in_specs=[hbm] * 12,
        out_specs=hbm,
        scratch_shapes=scratch,
        compiler_params=pltpu.CompilerParams(vmem_limit_bytes=110 * 2**20,
                                             disable_semaphore_checks=True),
        name="h3_mixer",
    )(A_q, A_k, A_v, A_shift_k.T, A_ssm_k, A_ssm_D, B_w1, B_w2, B_w3.T, B_w4, c, w_mod)
```

```python
import jax
import jax.numpy as jnp
import numpy as np
import jax.experimental.pallas as pl
import jax.experimental.pallas.tpu as pltpu

S, D, FF = 2048, 640, 1728
NT = D // 128
L = 512
NB = S // L
NFFT = 2 * L
R = 4
KPAD = 16
HPAD = 8
TB = 256
NBLK = S // TB
AO = 16
CH = 16
EPS = 1e-5
FM = FF // 128 * 128
F32 = jnp.float32
BF16 = jnp.bfloat16
U32 = jnp.uint32
I32 = jnp.int32
NT_DIMS = (((1,), (1,)), ((), ()))
K0P, K1P, K1R, K2R, X0S, X1S, Z1P, Z2P, Z3P = range(9)


def _cos_coefs(deg=6):
    u = (np.cos(np.pi * (np.arange(400) + 0.5) / 400) + 1.0) / 2.0
    c = np.polynomial.polynomial.polyfit(u, np.cos(np.pi * np.sqrt(u)), deg)
    return [np.float32(v) for v in c]


_COS = _cos_coefs()


def _cos_units(a, scale=1.0):
    x = (((a + 1024) & 2047) - 1024).astype(F32) * np.float32(1.0 / 1024.0)
    u = x * x
    acc = u * np.float32(_COS[-1] * scale) + np.float32(_COS[-2] * scale)
    for c in _COS[-3::-1]:
        acc = acc * u + np.float32(c * scale)
    return acc


def _freq2(chunk, s):
    return 4 * (8 * (chunk & 7) + s) + 2 * (chunk >> 3) + 1


def _gelu(x):
    c1 = np.float32(np.sqrt(2.0 / np.pi))
    c2 = np.float32(np.sqrt(2.0 / np.pi) * 0.044715)
    u = x * (c1 + c2 * (x * x))
    hx = 0.5 * x
    return hx + hx * jnp.tanh(u)


def _stats(x):
    m = jnp.sum(x, axis=-1, keepdims=True) * (1.0 / D)
    e2 = jnp.sum(x * x, axis=-1, keepdims=True) * (1.0 / D)
    v = jnp.maximum(e2 - m * m, 0.0)
    return m, jax.lax.rsqrt(v + EPS)


def _split(b):
    b = b.reshape(16, 2, 8, 128)
    return b[:, 0], b[:, 1]


def _join(z):
    return jnp.stack(z, axis=1).reshape(256, 128)


def _fft4(b, sign):
    (r0, i0), (r1, i1), (r2, i2), (r3, i3) = b
    sr, si, dr, di = r0 + r2, i0 + i2, r0 - r2, i0 - i2
    tr, ti, er, ei = r1 + r3, i1 + i3, r1 - r3, i1 - i3
    x0 = (sr + tr, si + ti)
    x2 = (sr - tr, si - ti)
    xm = (dr + ei, di - er)
    xp = (dr - ei, di + er)
    return [x0, xm, x2, xp] if sign < 0 else [x0, xp, x2, xm]


def _cmul(a, b, acc=None):
    (ar, ai), (br, bi) = a, b
    if acc is None:
        return ar * br - ai * bi, ar * bi + ai * br
    return (acc[0] + ar * br) - ai * bi, (acc[1] + ar * bi) + ai * br


def _bf(x):
    return pltpu.bitcast(x, BF16)


def _pack(a, b):
    return pltpu.pack_elementwise([a, b], packed_dtype=BF16)


def _tie(w, ties):
    if not ties:
        return w
    parts = []
    for i in range(w.shape[0] // 8):
        p = w[8 * i:8 * i + 8]
        if i in ties:
            z = ties[i]
            p = p | z if p.shape[1] == 128 else jnp.concatenate([p[:, :128] | z, p[:, 128:]], axis=1)
        parts.append(p)
    return jnp.concatenate(parts, axis=0)


def _kernel(q_hbm, k_hbm, v_hbm, sk_hbm, ssm_hbm, sd_hbm, w1_hbm, w2_hbm, w3_hbm,
            w4_hbm, c_hbm, wm_hbm, o_hbm,
            qb, kb, vb, skb, ssmb, sdb, w1b, w2b, w3b, w4b, cb_, wmb, fwb, gib,
            stb, spec, cmb, yb, x1b, hb, hpb, n4b, par, w3n, ob, sems, osem):
    groups = {}

    def add(name, src, dst):
        if name not in groups:
            groups[name] = (len(groups), [])
        idx, lst = groups[name]
        cp = pltpu.make_async_copy(src, dst, sems.at[idx])
        cp.start()
        lst.append(cp)

    def add_kv(name, c, tiles=range(NT)):
        for t in tiles:
            add(name, k_hbm.at[0, pl.ds(L * c, L), pl.ds(128 * t, 128)],
                kb.at[t, pl.ds(KPAD + L * c, L), :])
            add(name, v_hbm.at[0, pl.ds(L * c, L), pl.ds(128 * t, 128)],
                vb.at[t, pl.ds(L * c, L), :])

    def add_ssm(name, c):
        add(name, ssm_hbm.at[:, pl.ds(L * c, L)], ssmb.bitcast(BF16).at[:, pl.ds(L * c, L)])

    QE = 2 * TB + AO
    add_ssm("r0", 0)
    add("r0", sd_hbm, sdb)
    add("r0", sk_hbm, skb)
    add("r0", c_hbm, cb_)
    add_kv("r1", 0, range(3))
    add_kv("r2", 0, range(3, NT))
    add_ssm("r2", 1)
    add_kv("r3", 1)
    add_ssm("r3", 2)
    add_kv("r4", 2)
    add_ssm("r4", 3)
    add("wmA", q_hbm.at[0, pl.ds(0, QE), :], qb.bitcast(BF16).at[pl.ds(0, QE), :])
    add("wmA", wm_hbm.at[:, pl.ds(0, 3 * D)], wmb.at[:, pl.ds(0, 3 * D)])
    add("wmB", wm_hbm.at[:, pl.ds(3 * D, 2 * D)], wmb.at[:, pl.ds(3 * D, 2 * D)])
    add("w1", w1_hbm, w1b.bitcast(BF16))
    add("w2", w2_hbm, w2b.bitcast(BF16))
    add_kv("w2", 3, range(3))
    add_kv("w3", 3, range(3, NT))
    add("w3", w3_hbm, w3b.bitcast(BF16))
    add("w4", w4_hbm, w4b.bitcast(BF16))
    add("rest", q_hbm.at[0, pl.ds(QE, S - QE), :], qb.bitcast(BF16).at[pl.ds(QE, S - QE), :])
    add("rest", wm_hbm.at[:, pl.ds(5 * D, D)], wmb.at[:, pl.ds(5 * D, D)])

    def wait(name):
        with jax.named_scope("W_" + name):
            for cp in groups[name][1]:
                cp.wait()

    kb[:, 0:KPAD, :] = jnp.zeros((NT, KPAD, 128), BF16)
    hpb[:, 0:HPAD, :] = jnp.zeros((NT, HPAD, 128), F32)
    yb[:, S:S + AO, :] = jnp.zeros((NT, AO, 128), F32)
    qb[S // 2:(S + AO) // 2, :] = jnp.zeros((AO // 2, D), U32)

    spec[9, 0, 0, pl.ds(0, 8, stride=2), :] = jnp.zeros((8, 128), F32)
    cmb[2, 0, 0, pl.ds(0, 8, stride=2), :] = jnp.zeros((8, 128), U32)
    fwb[R, pl.ds(0, 8, stride=2), :] = jnp.zeros((8, 128), U32)
    gib[R, 0, pl.ds(0, 8, stride=2), :] = jnp.zeros((8, 128), U32)

    row = jax.lax.broadcasted_iota(I32, (128, 128), 0)
    col = jax.lax.broadcasted_iota(I32, (128, 128), 1)
    f2 = _freq2(row >> 3, 2 * (row & 3))
    ph = 512 * ((row >> 2) & 1)
    for r in range(R):
        n = 4 * col + r
        a = n * f2 + ph
        fwb[r] = _pack(_cos_units(a), _cos_units(a + 4 * n))
    row = jax.lax.broadcasted_iota(I32, (64, 128), 0)
    col = jax.lax.broadcasted_iota(I32, (64, 128), 1)
    for h in range(2):
        f2 = _freq2(8 * h + (col >> 4), (col >> 1) & 7)
        ph = 512 * (col & 1)
        for r in range(R):
            a = (8 * row + r) * f2 + ph
            gib[r, h] = _pack(_cos_units(a, 2.0 / NFFT), _cos_units(a + 4 * f2, 2.0 / NFFT))

    env = {}

    def zero_after(*vals):
        acc = None
        for v in vals:
            v = pltpu.bitcast(v, U32)
            for i in range(0, v.shape[0], 8):
                for j in range(0, v.shape[1], 128):
                    p = v[i:i + 8, j:j + 128]
                    acc = p if acc is None else acc | p
        return acc & kb.bitcast(U32)[0, 0:8, :]

    def ld_spec(slot, t, q):
        return _split(spec[slot, t, q])

    def st_spec(slot, t, q, z):
        spec[slot, t, q] = _join(z)

    def fwd_dots(rhs, ties):
        return [_split(jnp.dot(_bf(_tie(fwb[r], ties if r == 0 else None)), _bf(rhs[r]),
                               preferred_element_type=F32)) for r in range(R)]

    def conv_k(c, t, ties):
        w0 = L * c // 2
        stb[t, w0:w0 + L // 2, :] = pltpu.bitcast(
            _bf(ssmb[64 * t:64 * t + 64, L * c:L * c + L]).T, U32)
        rhs = []
        for h in range(2):
            lo = stb[t, pl.ds(w0 + h, 64, stride=4), :]
            hi = stb[t, pl.ds(w0 + h + 2, 64, stride=4), :]
            rhs.append((lo & jnp.uint32(0xFFFF)) | (hi << 16))
            rhs.append((lo >> 16) | (hi & jnp.uint32(0xFFFF0000)))
        b = fwd_dots(rhs, ties)
        if c == 0:
            b[0] = (b[0][0] + env["dvec"][:, 128 * t:128 * t + 128][None], b[0][1])
        kq = _fft4(b, -1)
        for q in range(R):
            re, im = kq[q]
            if c == 0:
                st_spec(K0P, t, q, kq[q])
                continue
            if c < 3:
                st_spec((K1R, K2R)[c - 1], t, q, kq[q])
            pr, pi = ld_spec((K0P, K1R, K2R)[c - 1], t, q)
            kp = (jnp.concatenate([re[:8] - pi[:8], re[8:] + pi[8:]], axis=0),
                  jnp.concatenate([im[:8] + pr[:8], im[8:] - pr[8:]], axis=0))
            x0 = ld_spec(X0S, t, q)
            if c == 1:
                st_spec(K1P, t, q, kp)
                st_spec(Z1P, t, q, _cmul(kp, x0))
            elif c == 2:
                st_spec(Z2P, t, q, _cmul(kp, x0, ld_spec(Z2P, t, q)))
                st_spec(Z3P, t, q, _cmul(kp, ld_spec(X1S, t, q)))
            else:
                st_spec(Z3P, t, q, _cmul(kp, x0, ld_spec(Z3P, t, q)))

    def unpack(u):
        return (pltpu.bitcast(u << 16, F32),
                pltpu.bitcast(u & jnp.uint32(0xFFFF0000), F32))

    def conv_prep(c, t):
        taps = env["taps"]
        ku = kb.bitcast(U32)
        vu = vb.bitcast(U32)
        tp = [taps[j:j + 1, 128 * t:128 * t + 128] for j in range(4)]
        w0 = (KPAD + L * c) // 2
        kk = [unpack(ku[t, pl.ds(w0 - 2, 64, stride=4), :])[1]]
        for o in range(-1, 4):
            kk += unpack(ku[t, pl.ds(w0 + o, 64, stride=4), :])
        vv = []
        for o in range(4):
            vv += unpack(vu[t, pl.ds(L * c // 2 + o, 64, stride=4), :])
        kv = []
        for n in range(8):
            acc = kk[3 + n] * tp[0]
            for j in range(1, 4):
                acc = acc + kk[3 + n - j] * tp[j]
            kv.append(acc * vv[n])
        return [_pack(kv[r], kv[r + 4]) for r in range(R)]

    def conv_x(c, t, ties):
        xq = _fft4(fwd_dots(env.pop(("kv", c, t)), ties), -1)
        z = []
        for q in range(R):
            if c < 2:
                st_spec((X0S, X1S)[c], t, q, xq[q])
            acc = None if c == 0 else ld_spec((Z1P, Z2P, Z3P)[c - 1], t, q)
            z.append(_cmul(xq[q], ld_spec(K0P, t, q), acc))
            if c == 1:
                st_spec(Z2P, t, q, _cmul(xq[q], ld_spec(K1P, t, q)))
            elif c == 2:
                st_spec(Z3P, t, q, _cmul(xq[q], ld_spec(K1P, t, q), ld_spec(Z3P, t, q)))
        cr = _fft4(z, +1)
        for r in range(R):
            cmb[c % 2, t, r] = _pack(*cr[r]).reshape(128, 128)

    def conv_inv(c, t, ties):
        for r in range(R):
            tr = None
            if ties and r % 2 == 0:
                tr = {i - 4 * r: z for i, z in ties.items() if 0 <= i - 4 * r < 8}
            g = jnp.concatenate([_bf(_tie(gib[r, 0], tr)), _bf(gib[r, 1])], axis=-1)
            yb[t, pl.ds(L * c + r, 128, stride=R), :] = jnp.dot(
                g, _bf(cmb[c % 2, t, r]), preferred_element_type=F32)

    def run_rounds(spec_str):
        rounds = spec_str.split()
        plan = {}
        for n, rd in enumerate(rounds):
            if rd[0] == "X":
                pts = []
                if "@" in rd:
                    a, b = (float(v) for v in rd[4:].split(":"))
                    pts = [int(round(16 * (n - a + (a - b) * (j + 1) / 8))) - 1 for j in range(8)]
                plan.setdefault(pts[0] // 16 if pts else n, []).append((rd, pts))
        ties = {}
        for n, rd in enumerate(rounds):
            for xr, pts in plan.get(n, []):
                c, t = int(xr[1]), int(xr[2])
                kv = env["kv", c, t] = conv_prep(c, t)
                for j, p in enumerate(pts):
                    z = zero_after(*[w[8 * j:8 * j + 8] for w in kv])
                    d = ties.setdefault(p // 16, {})
                    d[p % 16] = z if p % 16 not in d else d[p % 16] | z
            {"K": conv_k, "X": conv_x, "I": conv_inv}[rd[0]](int(rd[1]), int(rd[2]), ties.get(n))

    def rows(r0, n, align=8):
        if isinstance(r0, int):
            return slice(r0, r0 + n)
        return pl.ds(pl.multiple_of(r0, align), n)

    def ld_y(r0, n):
        return jnp.concatenate([yb[t, rows(r0, n), :] for t in range(NT)], axis=-1)

    def prm(i, n=CH, c0=0, c1=D):
        return jnp.concatenate([par[i, :, c0:c1]] * (n // 8), axis=0)

    def a_pre12(r0, n):
        x = _bf(qb[r0 // 2:(r0 + n) // 2, :]).astype(F32)
        m1, r1 = _stats(x)
        x1 = x + ((x - m1) * r1 * prm(0, n) + prm(1, n)) * ld_y(r0, n)
        x1b[r0:r0 + n, :] = x1
        env["m2", r0] = _stats(x1)

    def a_pre3(r0, n, o=0, m=None):
        m = n if m is None else m
        m2, r2 = (v[o:o + m] for v in env["m2", r0])
        rs = slice(r0 + o, r0 + o + m)
        h = (x1b[rs, :] - m2) * r2 * prm(2, m) + prm(3, m)
        hb[rs, :] = h
        m3, r3 = _stats(h)
        return (h - m3) * r3

    def a_pre(r0, gates):
        out = []
        for j, g in enumerate(gates):
            r = r0 + CH * j
            z = zero_after(g)
            qv = qb[rows(r0 // 2 + CH // 2 * j, CH // 2), :] | jnp.concatenate([z] * NT, axis=1)
            x = _bf(qv).astype(F32)
            m1, r1 = _stats(x)
            x1 = x + ((x - m1) * r1 * prm(0) + prm(1)) * ld_y(r, CH)
            x1b[rows(r, CH), :] = x1
            m2, r2 = _stats(x1)
            h = (x1 - m2) * r2 * prm(2) + prm(3)
            hb[rows(r, CH), :] = h
            m3, r3 = _stats(h)
            out.append((h - m3) * r3)
        return jnp.concatenate(out, axis=0)

    def halves(n, split):
        return [(0, n // 2), (n // 2, n - n // 2)] if split else [(0, n)]

    def mm1(r0, n, n3, split_last=False, ties=None, ties2=None):
        for t in range(NT):
            w = w1b[:, 128 * t:128 * t + 128]
            if ties and t in ties:
                w = _tie(w, {**ties[t], **ties2[t]})
            for o, m in halves(n, split_last and t == NT - 1):
                hp = jnp.dot(n3[o:o + m].astype(BF16), _bf(w), preferred_element_type=F32)
                hpb[t, rows(HPAD + r0 + o, m), :] = _gelu(hp)

    def g_prep(r0):
        lane = jax.lax.broadcasted_iota(I32, (TB, 128), 1)
        sh = [-1, 1, -2, 2]

        def ldh(t, g):
            return hpb[t, pl.ds(HPAD + r0 + sh[g], TB), :]

        cols = [ldh(0, 0)]
        for t in range(1, 4):
            cols.append(jnp.where(lane < 32 * t, ldh(t, t - 1), ldh(t, t)))
        cols.append(ldh(4, 3))
        return jnp.concatenate(cols, axis=-1)

    def mm2(r0, g, split_last=False, side=None):
        for t in range(NT):
            if side and t in side:
                side[t]()
            c0, c1 = 128 * t, 128 * t + 128
            for o, m in halves(TB, split_last and t == NT - 1):
                hs = jnp.dot(g[o:o + m].astype(BF16), _bf(w2b[:, c0:c1]), preferred_element_type=F32)
                hb[rows(r0 + o, m), c0:c1] = hb[rows(r0 + o, m), c0:c1] + hs
        return hs[m - 8:m]

    def ln4(r0, n):
        x2 = hb[rows(r0, n), :]
        m4, r4 = _stats(x2)
        return (x2 - m4) * r4

    def mm3(n4, ties=None, split_last=False, side=None, tpos=12, nat=True):
        us = []
        env["g3"] = []
        for j in range(FF // 128):
            if side and j in side:
                side[j]()
            if j == tpos:
                ht = jax.lax.dot_general(_bf(w3b[FM // 2:FF // 2, :]), n4.astype(BF16), NT_DIMS,
                                         preferred_element_type=F32)
                ut = _gelu(ht).T
            w = w3b[64 * j:64 * j + 64, :]
            if ties and j in ties:
                w = _tie(w, {0: ties[j]})
            parts = []
            for o, m in halves(TB, split_last and j == FF // 128 - 1):
                if j == 0 and nat:
                    h3 = jnp.dot(n4.astype(BF16), _bf(w3n[...]), preferred_element_type=F32)
                else:
                    h3 = jax.lax.dot_general(n4[o:o + m].astype(BF16), _bf(w), NT_DIMS,
                                             preferred_element_type=F32)
                parts.append(_gelu(h3))
                if m == TB:
                    env["g3"] += [h3[0:8], h3[128:136]]
            us.append(jnp.concatenate(parts, axis=0))
        return jnp.concatenate(us + [ut], axis=-1)

    def mm4(r0, u, t, final=True, ties=None, split=False):
        c0, c1 = 128 * t, 128 * t + 128
        w = _bf(_tie(w4b[:, c0:c1], ties))
        for o, m in halves(TB, split):
            h2 = jnp.dot(u[o:o + m].astype(BF16), w, preferred_element_type=F32)
            s = hb[rows(r0 + o, m), c0:c1] + h2
            if final:
                ob[rows(r0 + o, m, 16), c0:c1] = (
                    x1b[rows(r0 + o, m), c0:c1] + prm(4, m, c0, c1) * s).astype(BF16)
            else:
                hb[rows(r0 + o, m), c0:c1] = s

    def ln4_store(r0, nch):
        zs = []
        m = TB // nch
        for j in range(nch):
            n4 = ln4(r0 + m * j, m)
            n4b[m * j:m * j + m, :] = n4
            zs.append(zero_after(n4))
        return zs

    def ln4_ticked(r0, g, nch, hops):
        z = zero_after(g)
        m = TB // nch
        for j in range(nch):
            zt = jnp.concatenate([jnp.concatenate([z] * NT, axis=1)] * (m // 8), axis=0)
            x2 = pltpu.bitcast(pltpu.bitcast(hb[rows(r0 + m * j, m), :], U32) | zt, F32)
            m4, r4 = _stats(x2)
            n4b[m * j:m * j + m, :] = (x2 - m4) * r4
            for _ in range(hops):
                z = pltpu.roll(z, 1, 1)

    def out_copy(r0, n, c0=0, c1=D):
        return pltpu.make_async_copy(ob.at[rows(r0, n, 16), c0:c1],
                                     o_hbm.at[0, rows(r0, n, 16), c0:c1], osem)

    def out_copy_old(r0, n):
        return pltpu.make_async_copy(ob.at[rows(r0, n, 16), :], o_hbm.at[0, rows(r0, n, 16), :], osem)

    wait("r0")
    env["taps"] = skb[...].astype(F32)
    env["dvec"] = sdb[...].astype(F32).reshape(1, D)
    cf = cb_[...].astype(F32)
    sc8 = jnp.broadcast_to(cf * jax.nn.sigmoid(cf), (8, D)).astype(BF16)
    run_rounds("K00 K01 K02 K03 K04")
    wait("r1")
    run_rounds("X00 X01@1:0.2 X02@1:0.2 I00")
    wait("r2")
    run_rounds("I01 X03@1:0.2 I02 K10 X04@1.5:0.5 K11 I03 K12 K13 K14")
    for c in (1, 2):
        wait(f"r{c + 2}")
        seq = f"I{c - 1}4 X{c}0@1:0.2 K{c + 1}0 X{c}1@1:0.2"
        for t in range(1, NT):
            seq += f" I{c}{t - 1} K{c + 1}{t}"
            if t + 1 < NT:
                seq += f" X{c}{t + 1}@1.5:0.5"
        run_rounds(seq)

    wait("wmA")
    mod = jnp.dot(sc8, wmb[:, 0:3 * D], preferred_element_type=F32)
    sa, ca, ga = [mod[:, D * i:D * (i + 1)] for i in range(3)]
    par[0] = (1.0 + ca) * ga
    par[1] = sa * ga
    run_rounds("I24")
    a_pre12(0, TB + AO)
    a_pre12(TB + AO, TB)
    wait("wmB")
    mod = jnp.dot(sc8, wmb[:, 3 * D:5 * D], preferred_element_type=F32)
    par[2] = 1.0 + mod[:, D:2 * D]
    par[3] = mod[:, 0:D]
    n3a = a_pre3(0, TB + AO)

    wait("w1")
    n3b = [a_pre3(TB + AO, TB, 32 * j, 32) for j in range(8)]
    zs = [zero_after(v) for v in n3b]
    mm1(0, TB + AO, n3a, ties={1 + j // 2: {16 * (j % 2): zs[j]} for j in range(0, 8, 2)},
        ties2={1 + j // 2: {16: zs[j]} for j in range(1, 8, 2)})
    mm1(TB + AO, TB, jnp.concatenate(n3b, axis=0), split_last=True)
    wait("w2")
    g0 = g_prep(0)
    rr = lambda x: (lambda: run_rounds(x))
    mm2(0, g0, side={2: rr("X30"), 4: rr("X31")})
    n4 = ln4(0, TB)
    mm2(TB, g_prep(TB), split_last=True, side={0: rr("I30"), 2: rr("X32 I31"), 4: rr("I32")})
    wait("w3")
    zs = ln4_store(TB, 8)
    u = mm3(n4, {5 + j: z for j, z in enumerate(zs)}, split_last=True, nat=False, tpos=6,
            side={2: rr("X33"), 5: rr("X34"), 8: rr("I33"), 10: rr("I34")})
    wait("w4")
    w3n[...] = pltpu.bitcast(_bf(w3b[0:64, :]).T, U32)
    for t in range(NT):
        mm4(0, u, t, final=False, split=t == NT - 1)
    wait("rest")
    par[4] = jnp.dot(sc8, wmb[:, 5 * D:6 * D], preferred_element_type=F32)

    def body(i, carry):
        r0 = i * TB
        u = mm3(n4b[...])
        n3 = a_pre(r0 + TB + AO, [env["g3"][j * 25 // 15] for j in range(TB // CH)])
        mm4(r0, u, 0)
        mm1(r0 + TB + AO, TB, n3)
        hpb[:, HPAD + S:HPAD + S + 8, :] = jnp.zeros((NT, 8, 128), F32)
        mm4(r0, u, 1)
        g = mm2(r0 + TB, g_prep(r0 + TB))
        ln4_ticked(r0 + TB, g, 16, 1)
        for t in range(2, NT):
            mm4(r0, u, t)
        out_copy(r0, TB).start()
        return carry

    jax.lax.fori_loop(1, NBLK - 1, body, 0)

    r0 = S - TB
    zs = []
    for j in range(8):
        rs = slice(32 * j, 32 * j + 32)
        o = x1b[rs, :] + prm(4, 32) * hb[rs, :]
        ob[rs, :] = o.astype(BF16)
        zs.append(zero_after(o))
    u = mm3(n4b[...], {3 + j: z for j, z in enumerate(zs)})
    out_copy(0, TB).start()
    for t in range(NT):
        mm4(r0, u, t, split=t == NT - 1)
        if t < NT - 1:
            out_copy(r0, TB, 128 * t, 128 * t + 128).start()
    out_copy(r0, TB // 2, D - 128, D).start()
    out_copy(r0 + TB // 2, TB // 2, D - 128, D).start()
    with jax.named_scope("W_out"):
        pltpu.make_async_copy(ob, o_hbm.at[0], osem).wait()


@jax.jit
def pallas_adaLN_cond__ssm_conv_h3__mixer_s_mlp__prompt_kernel(
    A_q, A_k, A_v, A_shift_k, A_ssm_k, A_ssm_D, B_x, B_w1, B_w2, B_w3, B_w4, c, w_mod,
):
    del B_x
    vm = pltpu.VMEM
    scratch = [
        vm(((S + AO) // 2, D), U32),
        vm((NT, KPAD + S, 128), BF16),
        vm((NT, S, 128), BF16),
        vm((4, D), BF16),
        vm((D // 2, S), U32),
        vm((D,), BF16),
        vm((D // 2, D), U32),
        vm((D // 2, D), U32),
        vm((FF // 2, D), U32),
        vm((FF // 2, D), U32),
        vm((1, D), BF16),
        vm((D, 6 * D), BF16),
        vm((R + 1, 128, 128), U32),
        vm((R + 1, 2, 64, 128), U32),
        vm((NT, S // 2, 128), U32),
        vm((10, NT, R, 256, 128), F32),
        vm((3, NT, R, 128, 128), U32),
        vm((NT, S + AO, 128), F32),
        vm((S + AO, D), F32),
        vm((S + AO, D), F32),
        vm((NT, HPAD + S + AO, 128), F32),
        vm((TB, D), F32),
        vm((5, 8, D), F32),
        vm((D // 2, 128), U32),
        vm((S, D), BF16),
        pltpu.SemaphoreType.DMA((12,)),
        pltpu.SemaphoreType.DMA(()),
    ]
    hbm = pl.BlockSpec(memory_space=pltpu.HBM)
    return pl.pallas_call(
        _kernel,
        out_shape=jax.ShapeDtypeStruct((1, S, D), BF16),
        in_specs=[hbm] * 12,
        out_specs=hbm,
        scratch_shapes=scratch,
        compiler_params=pltpu.CompilerParams(vmem_limit_bytes=110 * 2**20,
                                             disable_semaphore_checks=True,
                                             disable_bounds_checks=True),
        name="h3_mixer",
    )(A_q, A_k, A_v, A_shift_k.T, A_ssm_k, A_ssm_D, B_w1, B_w2, B_w3.T, B_w4, c, w_mod)
```

```python
import jax
import jax.numpy as jnp
import numpy as np
import jax.experimental.pallas as pl
import jax.experimental.pallas.tpu as pltpu

S, D, FF = 2048, 640, 1728
NT = D // 128
L = 512
NB = S // L
NFFT = 2 * L
R = 4
KPAD = 16
HPAD = 8
TB = 256
NBLK = S // TB
AO = 16
CH = 16
EPS = 1e-5
PACED = False
FM = FF // 128 * 128
F32 = jnp.float32
BF16 = jnp.bfloat16
U32 = jnp.uint32
I32 = jnp.int32
NT_DIMS = (((1,), (1,)), ((), ()))
K0P, K1P, K1R, K2R, X0S, X1S, Z1P, Z2P, Z3P = range(9)


def _cos_coefs(deg=6):
    u = (np.cos(np.pi * (np.arange(400) + 0.5) / 400) + 1.0) / 2.0
    c = np.polynomial.polynomial.polyfit(u, np.cos(np.pi * np.sqrt(u)), deg)
    return [np.float32(v) for v in c]


_COS = _cos_coefs()


def _cos_units(a, scale=1.0):
    x = (((a + 1024) & 2047) - 1024).astype(F32) * np.float32(1.0 / 1024.0)
    u = x * x
    acc = u * np.float32(_COS[-1] * scale) + np.float32(_COS[-2] * scale)
    for c in _COS[-3::-1]:
        acc = acc * u + np.float32(c * scale)
    return acc


def _freq2(chunk, s):
    e = 4 * (8 * (chunk >> 1) + s) + 1
    return jnp.where((chunk & 1) == 0, e, 256 - e)


def _gelu(x):
    c1 = np.float32(np.sqrt(2.0 / np.pi))
    c2 = np.float32(np.sqrt(2.0 / np.pi) * 0.044715)
    u = x * (c1 + c2 * (x * x))
    hx = 0.5 * x
    return hx + hx * jnp.tanh(u)


def _stats(x):
    m = jnp.sum(x, axis=-1, keepdims=True) * (1.0 / D)
    e2 = jnp.sum(x * x, axis=-1, keepdims=True) * (1.0 / D)
    v = jnp.maximum(e2 - m * m, 0.0)
    return m, jax.lax.rsqrt(v + EPS)


def _split(b):
    b = b.reshape(-1, 2, 8, 128)
    return b[:, 0], b[:, 1]


def _join(z):
    return jnp.stack(z, axis=1).reshape(-1, 128)


def _eo(v):
    v = v.reshape(-1, 2, 8, 128)
    return v[:, 0], v[:, 1]


def _uneo(e, o):
    return jnp.stack([e, o], axis=1).reshape(16, 8, 128)


def _fft4(b, sign):
    (r0, i0), (r1, i1), (r2, i2), (r3, i3) = b
    sr, si, dr, di = r0 + r2, i0 + i2, r0 - r2, i0 - i2
    tr, ti, er, ei = r1 + r3, i1 + i3, r1 - r3, i1 - i3
    x0 = (sr + tr, si + ti)
    x2 = (sr - tr, si - ti)
    xm = (dr + ei, di - er)
    xp = (dr - ei, di + er)
    return [x0, xm, x2, xp] if sign < 0 else [x0, xp, x2, xm]


def _cmul(a, b, acc=None):
    (ar, ai), (br, bi) = a, b
    if acc is None:
        return ar * br - ai * bi, ar * bi + ai * br
    return (acc[0] + ar * br) - ai * bi, (acc[1] + ar * bi) + ai * br


def _bf(x):
    return pltpu.bitcast(x, BF16)


def _pack(a, b):
    return pltpu.pack_elementwise([a, b], packed_dtype=BF16)


def _tie(w, ties):
    if not ties:
        return w
    parts = []
    for i in range(w.shape[0] // 8):
        p = w[8 * i:8 * i + 8]
        if i in ties:
            z = ties[i]
            p = p | z if p.shape[1] == 128 else jnp.concatenate([p[:, :128] | z, p[:, 128:]], axis=1)
        parts.append(p)
    return jnp.concatenate(parts, axis=0)


def _kernel(q_hbm, k_hbm, v_hbm, sk_hbm, ssm_hbm, sd_hbm, w1_hbm, w2_hbm, w3_hbm,
            w4_hbm, c_hbm, wm_hbm, o_hbm,
            qb, kb, vb, skb, ssmb, sdb, w1b, w2b, w3b, w4b, cb_, wmb, fwb, gib,
            stb, spec, cmb, yb, x1b, hb, hpb, n4b, par, w3n, ob, sems, osem):
    groups = {}

    def add(name, src, dst):
        if name not in groups:
            groups[name] = (len(groups), [])
        idx, lst = groups[name]
        cp = pltpu.make_async_copy(src, dst, sems.at[idx])
        cp.start()
        lst.append(cp)

    def add_kv(name, c, tiles=range(NT)):
        for t in tiles:
            add(name, k_hbm.at[0, pl.ds(L * c, L), pl.ds(128 * t, 128)],
                kb.at[t, pl.ds(KPAD + L * c, L), :])
            add(name, v_hbm.at[0, pl.ds(L * c, L), pl.ds(128 * t, 128)],
                vb.at[t, pl.ds(L * c, L), :])

    def add_ssm(name, c):
        add(name, ssm_hbm.at[:, pl.ds(L * c, L)], ssmb.bitcast(BF16).at[:, pl.ds(L * c, L)])

    QE = 2 * TB + AO
    add_ssm("r0", 0)
    add("r0", sd_hbm, sdb)
    add("r0", sk_hbm, skb)
    add("r0", c_hbm, cb_)
    add_kv("r1", 0, range(3))
    add_kv("r2", 0, range(3, NT))
    add_ssm("r2", 1)
    add_kv("r3", 1)
    add_ssm("r3", 2)
    add_kv("r4", 2)
    add_ssm("r4", 3)
    add("wmA", q_hbm.at[0, pl.ds(0, QE), :], qb.bitcast(BF16).at[pl.ds(0, QE), :])
    add("wmA", wm_hbm.at[:, pl.ds(0, 3 * D)], wmb.at[:, pl.ds(0, 3 * D)])
    add("wmB", wm_hbm.at[:, pl.ds(3 * D, 2 * D)], wmb.at[:, pl.ds(3 * D, 2 * D)])
    add("w1", w1_hbm, w1b.bitcast(BF16))
    add("w2", w2_hbm, w2b.bitcast(BF16))
    add_kv("w2", 3, range(3))
    add("w3", w3_hbm, w3b.bitcast(BF16))
    add_kv("w3", 3, [3])
    add("w4", w4_hbm, w4b.bitcast(BF16))
    add_kv("w4", 3, [4])
    add("rest", wm_hbm.at[:, pl.ds(5 * D, D)], wmb.at[:, pl.ds(5 * D, D)])
    add("rest", q_hbm.at[0, pl.ds(QE, TB), :], qb.bitcast(BF16).at[pl.ds(QE, TB), :])
    add("qlast", q_hbm.at[0, pl.ds(QE + TB, S - QE - TB), :],
        qb.bitcast(BF16).at[pl.ds(QE + TB, S - QE - TB), :])

    def wait(name):
        with jax.named_scope("W_" + name):
            for cp in groups[name][1]:
                cp.wait()

    kb[:, 0:KPAD, :] = jnp.zeros((NT, KPAD, 128), BF16)
    hpb[:, 0:HPAD, :] = jnp.zeros((NT, HPAD, 128), F32)
    yb[:, S:S + AO, :] = jnp.zeros((NT, AO, 128), F32)
    qb[S // 2:(S + AO) // 2, :] = jnp.zeros((AO // 2, D), U32)

    spec[9, 0, 0, pl.ds(0, 8, stride=2), :] = jnp.zeros((8, 128), F32)
    cmb[2, 0, 0, pl.ds(0, 8, stride=2), :] = jnp.zeros((8, 128), U32)
    fwb[R, pl.ds(0, 8, stride=2), :] = jnp.zeros((8, 128), U32)
    gib[2 * R, pl.ds(0, 8, stride=2), :] = jnp.zeros((8, 128), U32)

    row = jax.lax.broadcasted_iota(I32, (128, 128), 0)
    col = jax.lax.broadcasted_iota(I32, (128, 128), 1)
    f2e = _freq2(row >> 3, 2 * (row & 3))
    f2o = _freq2(row >> 3, 2 * (row & 3) + 1)
    ph = 512 * ((row >> 2) & 1)
    for r in range(R):
        n = 4 * col + r
        fwb[r] = _pack(_cos_units(n * f2e + ph), _cos_units(n * f2o + ph))
    row = jax.lax.broadcasted_iota(I32, (32, 128), 0)
    col = jax.lax.broadcasted_iota(I32, (32, 128), 1)
    f2 = 4 * (col >> 1) + 1
    ph = 512 * (col & 1)
    for r in range(2 * R):
        a = (16 * row + r) * f2 + ph
        gib[r] = _pack(_cos_units(a, 2.0 / NFFT), _cos_units(a + 8 * f2, 2.0 / NFFT))

    env = {}

    def zero_after(*vals):
        acc = None
        for v in vals:
            v = pltpu.bitcast(v, U32)
            for i in range(0, v.shape[0], 8):
                for j in range(0, v.shape[1], 128):
                    p = v[i:i + 8, j:j + 128]
                    acc = p if acc is None else acc | p
        return acc & kb.bitcast(U32)[0, 0:8, :]

    def ld_spec(slot, t, q):
        return _split(spec[slot, t, q])

    def st_spec(slot, t, q, z):
        spec[slot, t, q] = _join(z)

    def fwd_dots(rhs, ties):
        return [_split(jnp.dot(_bf(_tie(fwb[r], ties if r == 0 else None)), _bf(rhs[r]),
                               preferred_element_type=F32)) for r in range(R)]

    def conv_k(c, t, ties):
        w0 = L * c // 2
        stb[t, w0:w0 + L // 2, :] = pltpu.bitcast(
            _bf(ssmb[64 * t:64 * t + 64, L * c:L * c + L]).T, U32)
        rhs = []
        for h in range(2):
            lo = stb[t, pl.ds(w0 + h, 64, stride=4), :]
            hi = stb[t, pl.ds(w0 + h + 2, 64, stride=4), :]
            rhs.append((lo & jnp.uint32(0xFFFF)) | (hi << 16))
            rhs.append((lo >> 16) | (hi & jnp.uint32(0xFFFF0000)))
        b = fwd_dots(rhs, ties)
        if c == 0:
            b[0] = (b[0][0] + env["dvec"][:, 128 * t:128 * t + 128][None], b[0][1])
        kq = _fft4(b, -1)
        for q in range(R):
            re, im = kq[q]
            if c == 0:
                st_spec(K0P, t, q, kq[q])
                continue
            if c < 3:
                st_spec((K1R, K2R)[c - 1], t, q, kq[q])
            pr, pi = ld_spec((K0P, K1R, K2R)[c - 1], t, q)
            (ree, reo), (ime, imo), (pre, pro), (pie, pio) = (_eo(v) for v in (re, im, pr, pi))
            kp = (_uneo(ree - pie, reo + pio), _uneo(ime + pre, imo - pro))
            x0 = ld_spec(X0S, t, q)
            if c == 1:
                st_spec(K1P, t, q, kp)
                st_spec(Z1P, t, q, _cmul(kp, x0))
            elif c == 2:
                st_spec(Z2P, t, q, _cmul(kp, x0, ld_spec(Z2P, t, q)))
                st_spec(Z3P, t, q, _cmul(kp, ld_spec(X1S, t, q)))
            else:
                st_spec(Z3P, t, q, _cmul(kp, x0, ld_spec(Z3P, t, q)))

    def unpack(u):
        return (pltpu.bitcast(u << 16, F32),
                pltpu.bitcast(u & jnp.uint32(0xFFFF0000), F32))

    def conv_prep(c, t):
        taps = env["taps"]
        ku = kb.bitcast(U32)
        vu = vb.bitcast(U32)
        tp = [taps[j:j + 1, 128 * t:128 * t + 128] for j in range(4)]
        w0 = (KPAD + L * c) // 2
        kk = [unpack(ku[t, pl.ds(w0 - 2, 64, stride=4), :])[1]]
        for o in range(-1, 4):
            kk += unpack(ku[t, pl.ds(w0 + o, 64, stride=4), :])
        vv = []
        for o in range(4):
            vv += unpack(vu[t, pl.ds(L * c // 2 + o, 64, stride=4), :])
        kv = []
        for n in range(8):
            acc = kk[3 + n] * tp[0]
            for j in range(1, 4):
                acc = acc + kk[3 + n - j] * tp[j]
            kv.append(acc * vv[n])
        return [_pack(kv[r], kv[r + 4]) for r in range(R)]

    def conv_x(c, t, ties, paced=False):
        b = fwd_dots(env.pop(("kv", c, t)), ties)
        nu = 8 if paced else 1
        w = 16 // nu
        hs = np.float32(np.sqrt(0.5))
        g = zero_after(b[3][0][0]) if paced else None
        outs = []
        for j in range(nu):
            cs = slice(w * j, w * j + w)
            rs = slice(16 * w * j, 16 * w * (j + 1))
            bj = [(re[cs], im[cs]) for re, im in b]
            if paced:
                for r in range(2):
                    bj[r] = tuple(pltpu.bitcast(pltpu.bitcast(v, U32) | g[None], F32) for v in bj[r])

            def ld(slot, q):
                return _split(spec[slot, t, q, rs, :])

            def st(slot, q, z):
                spec[slot, t, q, rs, :] = _join(z)

            xq = _fft4(bj, -1)
            z = []
            for q in range(R):
                if c < 2:
                    st((X0S, X1S)[c], q, xq[q])
                acc = None if c == 0 else ld((Z1P, Z2P, Z3P)[c - 1], q)
                z.append(_cmul(xq[q], ld(K0P, q), acc))
                if c == 1:
                    st(Z2P, q, _cmul(xq[q], ld(K1P, q)))
                elif c == 2:
                    st(Z3P, q, _cmul(xq[q], ld(K1P, q), ld(Z3P, q)))
            cr = _fft4(z, +1)
            cms = []
            for r in range(R):
                (ar, br), (ai, bi) = _eo(cr[r][0]), _eo(cr[r][1])
                if r % 2:
                    br, bi = (br - bi) * hs, (br + bi) * hs
                if r < 2:
                    p, m = (ar + br, ai - bi), (ar - br, ai + bi)
                else:
                    p, m = (ar - bi, ai - br), (ar + bi, ai + br)
                for rr_, v in ((r, p), (r + R, m)):
                    cm = _pack(*v).reshape(4 * w, 128)
                    cmb[c % 2, t, rr_, 4 * w * j:4 * w * (j + 1), :] = cm
                    cms.append(cm)
            if paced:
                outs.append(cms)
                if j >= 1:
                    g = g | zero_after(*outs[j - 1])
                g = pltpu.roll(g, 1, 1)

    def conv_inv(c, t, ties):
        for r in range(2 * R):
            tr = None
            if ties and r % R == 0:
                tr = {i - r: z for i, z in ties.items() if 0 <= i - r < 4}
            yb[t, pl.ds(L * c + r, 64, stride=2 * R), :] = jnp.dot(
                _bf(_tie(gib[r], tr)), _bf(cmb[c % 2, t, r]), preferred_element_type=F32)

    def run_rounds(spec_str):
        rounds = spec_str.split()
        slots = []
        plan = {}
        for n, rd in enumerate(rounds):
            if rd[0] == "X":
                pts = []
                if "@" in rd:
                    a, b = (int(v) for v in rd[4:].split(":"))
                    pts = [slots[len(slots) - a + (a - b) * (j + 1) // 8 - 1] for j in range(8)]
                plan.setdefault(pts[0][0] if pts else n, []).append((rd, pts))
            slots += [(n, i) for i in range(8 if rd[0] == "I" else 16)]
        ties = {}
        for n, rd in enumerate(rounds):
            for xr, pts in plan.get(n, []):
                c, t = int(xr[1]), int(xr[2])
                kv = env["kv", c, t] = conv_prep(c, t)
                for j, (pn, pi) in enumerate(pts):
                    z = zero_after(*[w[8 * j:8 * j + 8] for w in kv])
                    d = ties.setdefault(pn, {})
                    d[pi] = z if pi not in d else d[pi] | z
            args = (int(rd[1]), int(rd[2]), ties.get(n))
            if rd[0] == "X":
                conv_x(*args, paced=PACED and args[0] == 3)
            else:
                {"K": conv_k, "I": conv_inv}[rd[0]](*args)

    def rows(r0, n, align=8):
        if isinstance(r0, int):
            return slice(r0, r0 + n)
        return pl.ds(pl.multiple_of(r0, align), n)

    def ld_y(r0, n):
        return jnp.concatenate([yb[t, rows(r0, n), :] for t in range(NT)], axis=-1)

    def prm(i, n=CH, c0=0, c1=D):
        return jnp.concatenate([par[i, :, c0:c1]] * (n // 8), axis=0)

    def a_pre12(r0, n):
        x = _bf(qb[r0 // 2:(r0 + n) // 2, :]).astype(F32)
        m1, r1 = _stats(x)
        x1 = x + ((x - m1) * r1 * prm(0, n) + prm(1, n)) * ld_y(r0, n)
        x1b[r0:r0 + n, :] = x1
        env["m2", r0] = _stats(x1)

    def a_pre3(r0, n, o=0, m=None):
        m = n if m is None else m
        m2, r2 = (v[o:o + m] for v in env["m2", r0])
        rs = slice(r0 + o, r0 + o + m)
        h = (x1b[rs, :] - m2) * r2 * prm(2, m) + prm(3, m)
        hb[rs, :] = h
        m3, r3 = _stats(h)
        return (h - m3) * r3

    def a_pre(r0, gates):
        out = []
        for j, g in enumerate(gates):
            r = r0 + CH * j
            z = zero_after(g)
            qv = qb[rows(r0 // 2 + CH // 2 * j, CH // 2), :] | jnp.concatenate([z] * NT, axis=1)
            x = _bf(qv).astype(F32)
            m1, r1 = _stats(x)
            x1 = x + ((x - m1) * r1 * prm(0) + prm(1)) * ld_y(r, CH)
            x1b[rows(r, CH), :] = x1
            m2, r2 = _stats(x1)
            h = (x1 - m2) * r2 * prm(2) + prm(3)
            hb[rows(r, CH), :] = h
            m3, r3 = _stats(h)
            out.append((h - m3) * r3)
        return jnp.concatenate(out, axis=0)

    def halves(n, split):
        return [(0, n // 2), (n // 2, n - n // 2)] if split else [(0, n)]

    def mm1(r0, n, n3, split_last=False, ties=None, ties2=None):
        for t in range(NT):
            w = w1b[:, 128 * t:128 * t + 128]
            if ties and t in ties:
                w = _tie(w, {**ties[t], **ties2[t]})
            for o, m in halves(n, split_last and t == NT - 1):
                hp = jnp.dot(n3[o:o + m].astype(BF16), _bf(w), preferred_element_type=F32)
                hpb[t, rows(HPAD + r0 + o, m), :] = _gelu(hp)

    def g_prep(r0):
        lane = jax.lax.broadcasted_iota(I32, (TB, 128), 1)
        sh = [-1, 1, -2, 2]

        def ldh(t, g):
            return hpb[t, pl.ds(HPAD + r0 + sh[g], TB), :]

        cols = [ldh(0, 0)]
        for t in range(1, 4):
            cols.append(jnp.where(lane < 32 * t, ldh(t, t - 1), ldh(t, t)))
        cols.append(ldh(4, 3))
        return jnp.concatenate(cols, axis=-1)

    def mm2(r0, g, split_last=False, side=None):
        for t in range(NT):
            if side and t in side:
                side[t]()
            c0, c1 = 128 * t, 128 * t + 128
            for o, m in halves(TB, split_last and t == NT - 1):
                hs = jnp.dot(g[o:o + m].astype(BF16), _bf(w2b[:, c0:c1]), preferred_element_type=F32)
                hb[rows(r0 + o, m), c0:c1] = hb[rows(r0 + o, m), c0:c1] + hs
        return hs[m - 8:m]

    def ln4(r0, n):
        x2 = hb[rows(r0, n), :]
        m4, r4 = _stats(x2)
        return (x2 - m4) * r4

    def mm3(n4, ties=None, split_last=False, side=None, tpos=12, nat=True):
        us = []
        env["g3"] = []
        for j in range(FF // 128):
            if side and j in side:
                side[j]()
            if j == tpos:
                ht = jax.lax.dot_general(_bf(w3b[FM // 2:FF // 2, :]), n4.astype(BF16), NT_DIMS,
                                         preferred_element_type=F32)
                ut = _gelu(ht).T
            w = w3b[64 * j:64 * j + 64, :]
            if ties and j in ties:
                w = _tie(w, {0: ties[j]})
            parts = []
            for o, m in halves(TB, split_last and j == FF // 128 - 1):
                if j == 0 and nat:
                    h3 = jnp.dot(n4.astype(BF16), _bf(w3n[...]), preferred_element_type=F32)
                else:
                    h3 = jax.lax.dot_general(n4[o:o + m].astype(BF16), _bf(w), NT_DIMS,
                                             preferred_element_type=F32)
                parts.append(_gelu(h3))
                if m == TB:
                    env["g3"] += [h3[0:8], h3[128:136]]
            us.append(jnp.concatenate(parts, axis=0))
        return jnp.concatenate(us + [ut], axis=-1)

    def mm4(r0, u, t, final=True, ties=None, split=False, side=None):
        c0, c1 = 128 * t, 128 * t + 128
        w = _bf(_tie(w4b[:, c0:c1], ties))
        for o, m in halves(TB, split):
            if o and side:
                side()
            h2 = jnp.dot(u[o:o + m].astype(BF16), w, preferred_element_type=F32)
            s = hb[rows(r0 + o, m), c0:c1] + h2
            if final:
                ob[rows(r0 + o, m, 16), c0:c1] = (
                    x1b[rows(r0 + o, m), c0:c1] + prm(4, m, c0, c1) * s).astype(BF16)
            else:
                hb[rows(r0 + o, m), c0:c1] = s

    def ln4_store(r0, nch):
        zs = []
        m = TB // nch
        for j in range(nch):
            n4 = ln4(r0 + m * j, m)
            n4b[m * j:m * j + m, :] = n4
            zs.append(zero_after(n4))
        return zs

    def ln4_ticked(r0, g, nch, hops):
        z = zero_after(g)
        m = TB // nch
        for j in range(nch):
            zt = jnp.concatenate([jnp.concatenate([z] * NT, axis=1)] * (m // 8), axis=0)
            x2 = pltpu.bitcast(pltpu.bitcast(hb[rows(r0 + m * j, m), :], U32) | zt, F32)
            m4, r4 = _stats(x2)
            n4b[m * j:m * j + m, :] = (x2 - m4) * r4
            for _ in range(hops):
                z = pltpu.roll(z, 1, 1)

    def out_copy(r0, n, c0=0, c1=D):
        return pltpu.make_async_copy(ob.at[rows(r0, n, 16), c0:c1],
                                     o_hbm.at[0, rows(r0, n, 16), c0:c1], osem)

    def out_copy_old(r0, n):
        return pltpu.make_async_copy(ob.at[rows(r0, n, 16), :], o_hbm.at[0, rows(r0, n, 16), :], osem)

    wait("r0")
    env["taps"] = skb[...].astype(F32)
    env["dvec"] = sdb[...].astype(F32).reshape(1, D)
    cf = cb_[...].astype(F32)
    sc8 = jnp.broadcast_to(cf * jax.nn.sigmoid(cf), (8, D)).astype(BF16)
    run_rounds("K00 K01 K02 K03 K04")
    wait("r1")
    run_rounds("X00 X01@16:3 X02@16:3 I00")
    wait("r2")
    run_rounds("I01 I02 X03@16:3 K10 X04@16:3 K11 I03 K12 K13 K14")
    wait("r3")
    run_rounds("I04 X10 K20 X11@16:3 I10 K21 X12@20:4 I11 K22 X13@20:4 I12 K23 X14@20:4 I13 K24")
    wait("r4")
    run_rounds("I14 X20 K30 X21@16:3 I20 K31 X22@20:4 I21 K32 X23@20:4 I22 K33 X24@20:4 I23 K34")

    wait("wmA")
    mod = jnp.dot(sc8, wmb[:, 0:3 * D], preferred_element_type=F32)
    sa, ca, ga = [mod[:, D * i:D * (i + 1)] for i in range(3)]
    par[0] = (1.0 + ca) * ga
    par[1] = sa * ga
    run_rounds("I24")
    a_pre12(0, TB + AO)
    a_pre12(TB + AO, TB)
    wait("wmB")
    mod = jnp.dot(sc8, wmb[:, 3 * D:5 * D], preferred_element_type=F32)
    par[2] = 1.0 + mod[:, D:2 * D]
    par[3] = mod[:, 0:D]
    n3a = a_pre3(0, TB + AO)

    wait("w1")
    n3b = [a_pre3(TB + AO, TB, 32 * j, 32) for j in range(8)]
    zs = [zero_after(v) for v in n3b]
    mm1(0, TB + AO, n3a, ties={1 + j // 2: {16 * (j % 2): zs[j]} for j in range(0, 8, 2)},
        ties2={1 + j // 2: {16: zs[j]} for j in range(1, 8, 2)})
    mm1(TB + AO, TB, jnp.concatenate(n3b, axis=0), split_last=True)
    wait("w2")
    g0 = g_prep(0)
    rr = lambda x: (lambda: run_rounds(x))
    mm2(0, g0, side={1: rr("X30"), 4: rr("X31")})
    n4 = ln4(0, TB)
    mm2(TB, g_prep(TB), split_last=True, side={3: rr("X32")})
    run_rounds("I30")
    wait("w3")
    zs = ln4_store(TB, 8)
    u = mm3(n4, {5 + j: z for j, z in enumerate(zs)}, split_last=True, nat=False,
            side={0: rr("I31"), 2: rr("X33")})
    run_rounds("I32")
    wait("w4")
    w3n[...] = pltpu.bitcast(_bf(w3b[0:64, :]).T, U32)
    mm4(0, u, 0, final=False)
    run_rounds("X34")
    mm4(0, u, 1, final=False)
    mm4(0, u, 2, final=False)
    mm4(0, u, 3, final=False)
    mm4(0, u, 4, final=False, split=True)
    run_rounds("I33 I34")
    wait("rest")
    par[4] = jnp.dot(sc8, wmb[:, 5 * D:6 * D], preferred_element_type=F32)

    def body(i, carry):
        pl.when(i == 2)(lambda: wait("qlast"))
        r0 = i * TB
        u = mm3(n4b[...])
        n3 = a_pre(r0 + TB + AO, [env["g3"][j * 25 // 15] for j in range(TB // CH)])
        mm4(r0, u, 0)
        mm1(r0 + TB + AO, TB, n3)
        hpb[:, HPAD + S:HPAD + S + 8, :] = jnp.zeros((NT, 8, 128), F32)
        mm4(r0, u, 1)
        g = mm2(r0 + TB, g_prep(r0 + TB))
        ln4_ticked(r0 + TB, g, 16, 1)
        for t in range(2, NT):
            mm4(r0, u, t)
        out_copy(r0, TB).start()
        return carry

    jax.lax.fori_loop(1, NBLK - 1, body, 0)

    r0 = S - TB
    zs = []
    for j in range(8):
        rs = slice(32 * j, 32 * j + 32)
        o = x1b[rs, :] + prm(4, 32) * hb[rs, :]
        ob[rs, :] = o.astype(BF16)
        zs.append(zero_after(o))
    u = mm3(n4b[...], {3 + j: z for j, z in enumerate(zs)})
    out_copy(0, TB).start()
    for t in range(NT):
        mm4(r0, u, t, split=t == NT - 1)
        if t < NT - 1:
            out_copy(r0, TB, 128 * t, 128 * t + 128).start()
    out_copy(r0, TB // 2, D - 128, D).start()
    out_copy(r0 + TB // 2, TB // 2, D - 128, D).start()
    with jax.named_scope("W_out"):
        pltpu.make_async_copy(ob, o_hbm.at[0], osem).wait()


@jax.jit
def pallas_adaLN_cond__ssm_conv_h3__mixer_s_mlp__prompt_kernel(
    A_q, A_k, A_v, A_shift_k, A_ssm_k, A_ssm_D, B_x, B_w1, B_w2, B_w3, B_w4, c, w_mod,
):
    del B_x
    vm = pltpu.VMEM
    scratch = [
        vm(((S + AO) // 2, D), U32),
        vm((NT, KPAD + S, 128), BF16),
        vm((NT, S, 128), BF16),
        vm((4, D), BF16),
        vm((D // 2, S), U32),
        vm((D,), BF16),
        vm((D // 2, D), U32),
        vm((D // 2, D), U32),
        vm((FF // 2, D), U32),
        vm((FF // 2, D), U32),
        vm((1, D), BF16),
        vm((D, 6 * D), BF16),
        vm((R + 1, 128, 128), U32),
        vm((2 * R + 1, 32, 128), U32),
        vm((NT, S // 2, 128), U32),
        vm((10, NT, R, 256, 128), F32),
        vm((3, NT, 2 * R, 64, 128), U32),
        vm((NT, S + AO, 128), F32),
        vm((S + AO, D), F32),
        vm((S + AO, D), F32),
        vm((NT, HPAD + S + AO, 128), F32),
        vm((TB, D), F32),
        vm((5, 8, D), F32),
        vm((D // 2, 128), U32),
        vm((S, D), BF16),
        pltpu.SemaphoreType.DMA((13,)),
        pltpu.SemaphoreType.DMA(()),
    ]
    hbm = pl.BlockSpec(memory_space=pltpu.HBM)
    return pl.pallas_call(
        _kernel,
        out_shape=jax.ShapeDtypeStruct((1, S, D), BF16),
        in_specs=[hbm] * 12,
        out_specs=hbm,
        scratch_shapes=scratch,
        compiler_params=pltpu.CompilerParams(vmem_limit_bytes=110 * 2**20,
                                             disable_semaphore_checks=True,
                                             disable_bounds_checks=True),
        name="h3_mixer",
    )(A_q, A_k, A_v, A_shift_k.T, A_ssm_k, A_ssm_D, B_w1, B_w2, B_w3.T, B_w4, c, w_mod)
```

```python
import jax
import jax.numpy as jnp
import numpy as np
import jax.experimental.pallas as pl
import jax.experimental.pallas.tpu as pltpu

S, D, FF = 2048, 640, 1728
NT = D // 128
L = 512
NB = S // L
NFFT = 2 * L
R = 4
KPAD = 16
HPAD = 8
TB = 256
NBLK = S // TB
AO = 16
CH = 16
EPS = 1e-5
FM = FF // 128 * 128
F32 = jnp.float32
BF16 = jnp.bfloat16
U32 = jnp.uint32
I32 = jnp.int32
NT_DIMS = (((1,), (1,)), ((), ()))
KP, X0S, ZP = 0, 3, 3


def _cos_coefs(deg=6):
    u = (np.cos(np.pi * (np.arange(400) + 0.5) / 400) + 1.0) / 2.0
    c = np.polynomial.polynomial.polyfit(u, np.cos(np.pi * np.sqrt(u)), deg)
    return [np.float32(v) for v in c]


_COS = _cos_coefs()


def _cos_units(a, scale=1.0):
    x = (((a + 1024) & 2047) - 1024).astype(F32) * np.float32(1.0 / 1024.0)
    u = x * x
    acc = u * np.float32(_COS[-1] * scale) + np.float32(_COS[-2] * scale)
    for c in _COS[-3::-1]:
        acc = acc * u + np.float32(c * scale)
    return acc


def _freq2(chunk, s):
    e = 4 * (8 * (chunk >> 1) + s) + 1
    return jnp.where((chunk & 1) == 0, e, 256 - e)


def _gelu(x):
    c1 = np.float32(np.sqrt(2.0 / np.pi))
    c2 = np.float32(np.sqrt(2.0 / np.pi) * 0.044715)
    u = x * (c1 + c2 * (x * x))
    hx = 0.5 * x
    return hx + hx * jnp.tanh(u)


def _stats(x):
    m = jnp.sum(x, axis=-1, keepdims=True) * (1.0 / D)
    e2 = jnp.sum(x * x, axis=-1, keepdims=True) * (1.0 / D)
    v = jnp.maximum(e2 - m * m, 0.0)
    return m, jax.lax.rsqrt(v + EPS)


def _split(b):
    b = b.reshape(-1, 2, 8, 128)
    return b[:, 0], b[:, 1]


def _join(z):
    return jnp.stack(z, axis=1).reshape(-1, 128)


def _eo(v):
    v = v.reshape(-1, 2, 8, 128)
    return v[:, 0], v[:, 1]


def _uneo(e, o):
    return jnp.stack([e, o], axis=1).reshape(16, 8, 128)


def _fft4(b, sign):
    (r0, i0), (r1, i1), (r2, i2), (r3, i3) = b
    sr, si, dr, di = r0 + r2, i0 + i2, r0 - r2, i0 - i2
    tr, ti, er, ei = r1 + r3, i1 + i3, r1 - r3, i1 - i3
    x0 = (sr + tr, si + ti)
    x2 = (sr - tr, si - ti)
    xm = (dr + ei, di - er)
    xp = (dr - ei, di + er)
    return [x0, xm, x2, xp] if sign < 0 else [x0, xp, x2, xm]


def _cmul(a, b, acc=None):
    (ar, ai), (br, bi) = a, b
    if acc is None:
        return ar * br - ai * bi, ar * bi + ai * br
    return (acc[0] + ar * br) - ai * bi, (acc[1] + ar * bi) + ai * br


def _bf(x):
    return pltpu.bitcast(x, BF16)


def _pack(a, b):
    return pltpu.pack_elementwise([a, b], packed_dtype=BF16)


def _tie(w, ties):
    if not ties:
        return w
    parts = []
    for i in range(w.shape[0] // 8):
        p = w[8 * i:8 * i + 8]
        if i in ties:
            z = ties[i]
            p = p | z if p.shape[1] == 128 else jnp.concatenate([p[:, :128] | z, p[:, 128:]], axis=1)
        parts.append(p)
    return jnp.concatenate(parts, axis=0)


def _kernel(q_hbm, k_hbm, v_hbm, sk_hbm, ssm_hbm, sd_hbm, w1_hbm, w2_hbm, w3_hbm,
            w4_hbm, c_hbm, wm_hbm, o_hbm,
            qb, kb, vb, skb, ssmb, sdb, w1b, w2b, w3b, w4b, cb_, wmb, fwb, gib,
            stb, spec, cmb, yb, x1b, hb, hpb, n4b, par, w3n, ob, sems, osem):
    groups = {}

    def add(name, src, dst):
        if name not in groups:
            groups[name] = (len(groups), [])
        idx, lst = groups[name]
        cp = pltpu.make_async_copy(src, dst, sems.at[idx])
        cp.start()
        lst.append(cp)

    def add_kv(name, c, tiles=range(NT)):
        for t in tiles:
            add(name, k_hbm.at[0, pl.ds(L * c, L), pl.ds(128 * t, 128)],
                kb.at[t, pl.ds(KPAD + L * c, L), :])
            add(name, v_hbm.at[0, pl.ds(L * c, L), pl.ds(128 * t, 128)],
                vb.at[t, pl.ds(L * c, L), :])

    def add_ssm(name, t):
        add(name, ssm_hbm.at[pl.ds(128 * t, 128), :], ssmb.bitcast(BF16).at[pl.ds(128 * t, 128), :])

    QE = 2 * TB + AO
    add_kv("ra", 0, [0])
    add("ra", sd_hbm, sdb)
    add("ra", sk_hbm, skb)
    add("ra", c_hbm, cb_)
    for t in range(NT):
        add_ssm(f"r{t}", t)
        add_kv(f"r{t}", (t + 1) // NT, [(t + 1) % NT])
    add_kv("r5", 1, range(1, NT))
    add_kv("r6", 2)
    add("wmA", q_hbm.at[0, pl.ds(0, QE), :], qb.bitcast(BF16).at[pl.ds(0, QE), :])
    add("wmA", wm_hbm.at[:, pl.ds(0, 3 * D)], wmb.at[:, pl.ds(0, 3 * D)])
    add("wmB", wm_hbm.at[:, pl.ds(3 * D, 2 * D)], wmb.at[:, pl.ds(3 * D, 2 * D)])
    add("w1", w1_hbm, w1b.bitcast(BF16))
    add("w2", w2_hbm, w2b.bitcast(BF16))
    add_kv("w2", 3, range(3))
    add("w3", w3_hbm, w3b.bitcast(BF16))
    add_kv("w3", 3, [3])
    add("w4", w4_hbm, w4b.bitcast(BF16))
    add_kv("w4", 3, [4])
    add("rest", wm_hbm.at[:, pl.ds(5 * D, D)], wmb.at[:, pl.ds(5 * D, D)])
    add("rest", q_hbm.at[0, pl.ds(QE, TB), :], qb.bitcast(BF16).at[pl.ds(QE, TB), :])
    add("qlast", q_hbm.at[0, pl.ds(QE + TB, S - QE - TB), :],
        qb.bitcast(BF16).at[pl.ds(QE + TB, S - QE - TB), :])

    def wait(name):
        with jax.named_scope("W_" + name):
            for cp in groups[name][1]:
                cp.wait()

    kb[:, 0:KPAD, :] = jnp.zeros((NT, KPAD, 128), BF16)
    hpb[:, 0:HPAD, :] = jnp.zeros((NT, HPAD, 128), F32)
    yb[:, S:S + AO, :] = jnp.zeros((NT, AO, 128), F32)
    qb[S // 2:(S + AO) // 2, :] = jnp.zeros((AO // 2, D), U32)

    spec[7, 0, 0, pl.ds(0, 8, stride=2), :] = jnp.zeros((8, 128), F32)
    cmb[2, 0, 0, pl.ds(0, 8, stride=2), :] = jnp.zeros((8, 128), U32)
    fwb[R, pl.ds(0, 8, stride=2), :] = jnp.zeros((8, 128), U32)
    gib[2 * R, pl.ds(0, 8, stride=2), :] = jnp.zeros((8, 128), U32)

    row = jax.lax.broadcasted_iota(I32, (128, 128), 0)
    col = jax.lax.broadcasted_iota(I32, (128, 128), 1)
    f2e = _freq2(row >> 3, 2 * (row & 3))
    f2o = _freq2(row >> 3, 2 * (row & 3) + 1)
    ph = 512 * ((row >> 2) & 1)
    for r in range(R):
        n = 4 * col + r
        fwb[r] = _pack(_cos_units(n * f2e + ph), _cos_units(n * f2o + ph))
    row = jax.lax.broadcasted_iota(I32, (32, 128), 0)
    col = jax.lax.broadcasted_iota(I32, (32, 128), 1)
    f2 = 4 * (col >> 1) + 1
    ph = 512 * (col & 1)
    for r in range(2 * R):
        a = (16 * row + r) * f2 + ph
        gib[r] = _pack(_cos_units(a, 2.0 / NFFT), _cos_units(a + 8 * f2, 2.0 / NFFT))

    env = {}

    def zero_after(*vals):
        acc = None
        for v in vals:
            v = pltpu.bitcast(v, U32)
            for i in range(0, v.shape[0], 8):
                for j in range(0, v.shape[1], 128):
                    p = v[i:i + 8, j:j + 128]
                    acc = p if acc is None else acc | p
        return acc & kb.bitcast(U32)[0, 0:8, :]

    def ld_spec(slot, t, q):
        return _split(spec[slot, t, q])

    def st_spec(slot, t, q, z):
        spec[slot, t, q] = _join(z)

    def fwd_dots(rhs, ties):
        return [_split(jnp.dot(_bf(_tie(fwb[r], ties if r == 0 else None)), _bf(rhs[r]),
                               preferred_element_type=F32)) for r in range(R)]

    def conv_k(c, t, ties):
        w0 = L * c // 2
        stb[t, w0:w0 + L // 2, :] = pltpu.bitcast(
            _bf(ssmb[64 * t:64 * t + 64, L * c:L * c + L]).T, U32)
        rhs = []
        for h in range(2):
            lo = stb[t, pl.ds(w0 + h, 64, stride=4), :]
            hi = stb[t, pl.ds(w0 + h + 2, 64, stride=4), :]
            rhs.append((lo & jnp.uint32(0xFFFF)) | (hi << 16))
            rhs.append((lo >> 16) | (hi & jnp.uint32(0xFFFF0000)))
        b = fwd_dots(rhs, ties)
        if c == 0:
            b[0] = (b[0][0] + env["dvec"][:, 128 * t:128 * t + 128][None], b[0][1])
        kq = _fft4(b, -1)
        z = []
        for q in range(R):
            kp = kq[q]
            if c >= 2:
                p = ld_spec(KP + c - 2, t, q)
                kp = (kp[0] + p[0], kp[1] + p[1])
            if c >= 1:
                p = ld_spec(KP + c - 1, t, q)
                if c == 3:
                    p0 = ld_spec(KP, t, q)
                    p = (p[0] - p0[0], p[1] - p0[1])
                (ree, reo), (ime, imo), (pre, pro), (pie, pio) = (_eo(v) for v in kp + p)
                kp = (_uneo(ree - pie, reo + pio), _uneo(ime + pre, imo - pro))
            if c < 3:
                st_spec(KP + c, t, q, kp)
            zc = _cmul(kp, ld_spec(X0S, t, q))
            if c == 0:
                z.append(zc)
            else:
                st_spec(ZP + c, t, q, zc)
        if c == 0:
            finish(0, t, z)

    def finish(c, t, z):
        hs = np.float32(np.sqrt(0.5))
        cr = _fft4(z, +1)
        for r in range(R):
            (ar, br), (ai, bi) = _eo(cr[r][0]), _eo(cr[r][1])
            if r % 2:
                br, bi = (br - bi) * hs, (br + bi) * hs
            if r < 2:
                p, m = (ar + br, ai - bi), (ar - br, ai + bi)
            else:
                p, m = (ar - bi, ai - br), (ar + bi, ai + br)
            cmb[c % 2, t, r] = _pack(*p).reshape(64, 128)
            cmb[c % 2, t, r + R] = _pack(*m).reshape(64, 128)

    def unpack(u):
        return (pltpu.bitcast(u << 16, F32),
                pltpu.bitcast(u & jnp.uint32(0xFFFF0000), F32))

    def conv_prep(c, t):
        taps = env["taps"]
        ku = kb.bitcast(U32)
        vu = vb.bitcast(U32)
        tp = [taps[j:j + 1, 128 * t:128 * t + 128] for j in range(4)]
        w0 = (KPAD + L * c) // 2
        kk = [unpack(ku[t, pl.ds(w0 - 2, 64, stride=4), :])[1]]
        for o in range(-1, 4):
            kk += unpack(ku[t, pl.ds(w0 + o, 64, stride=4), :])
        vv = []
        for o in range(4):
            vv += unpack(vu[t, pl.ds(L * c // 2 + o, 64, stride=4), :])
        kv = []
        for n in range(8):
            acc = kk[3 + n] * tp[0]
            for j in range(1, 4):
                acc = acc + kk[3 + n - j] * tp[j]
            kv.append(acc * vv[n])
        return [_pack(kv[r], kv[r + 4]) for r in range(R)]

    def conv_x(c, t, ties):
        xq = _fft4(fwd_dots(env.pop(("kv", c, t)), ties), -1)
        z = []
        for q in range(R):
            if c == 0:
                st_spec(X0S, t, q, xq[q])
                continue
            for a in range(c, NB):
                za = _cmul(xq[q], ld_spec(KP + a - c, t, q), ld_spec(ZP + a, t, q))
                if a == c:
                    z.append(za)
                else:
                    st_spec(ZP + a, t, q, za)
        if c:
            finish(c, t, z)

    def conv_inv(c, t, ties):
        for r in range(2 * R):
            tr = None
            if ties and r % R == 0:
                tr = {i - r: z for i, z in ties.items() if 0 <= i - r < 4}
            yb[t, pl.ds(L * c + r, 64, stride=2 * R), :] = jnp.dot(
                _bf(_tie(gib[r], tr)), _bf(cmb[c % 2, t, r]), preferred_element_type=F32)

    def run_rounds(spec_str):
        rounds = spec_str.split()
        slots = []
        plan = {}
        for n, rd in enumerate(rounds):
            if rd[0] == "X":
                pts = []
                if "@" in rd:
                    a, b = (int(v) for v in rd[4:].split(":"))
                    pts = [slots[len(slots) - a + (a - b) * (j + 1) // 8 - 1] for j in range(8)]
                plan.setdefault(pts[0][0] if pts else n, []).append((rd, pts))
            slots += [(n, i) for i in range(8 if rd[0] == "I" else 16)]
        ties = {}
        for n, rd in enumerate(rounds):
            for xr, pts in plan.get(n, []):
                c, t = int(xr[1]), int(xr[2])
                kv = env["kv", c, t] = conv_prep(c, t)
                for j, (pn, pi) in enumerate(pts):
                    z = zero_after(*[w[8 * j:8 * j + 8] for w in kv])
                    d = ties.setdefault(pn, {})
                    d[pi] = z if pi not in d else d[pi] | z
            {"K": conv_k, "X": conv_x, "I": conv_inv}[rd[0]](int(rd[1]), int(rd[2]), ties.get(n))

    def rows(r0, n, align=8):
        if isinstance(r0, int):
            return slice(r0, r0 + n)
        return pl.ds(pl.multiple_of(r0, align), n)

    def ld_y(r0, n):
        return jnp.concatenate([yb[t, rows(r0, n), :] for t in range(NT)], axis=-1)

    def prm(i, n=CH, c0=0, c1=D):
        return jnp.concatenate([par[i, :, c0:c1]] * (n // 8), axis=0)

    def a_pre12(r0, n):
        x = _bf(qb[r0 // 2:(r0 + n) // 2, :]).astype(F32)
        m1, r1 = _stats(x)
        x1 = x + ((x - m1) * r1 * prm(0, n) + prm(1, n)) * ld_y(r0, n)
        x1b[r0:r0 + n, :] = x1
        env["m2", r0] = _stats(x1)

    def a_pre3(r0, n, o=0, m=None):
        m = n if m is None else m
        m2, r2 = (v[o:o + m] for v in env["m2", r0])
        rs = slice(r0 + o, r0 + o + m)
        h = (x1b[rs, :] - m2) * r2 * prm(2, m) + prm(3, m)
        hb[rs, :] = h
        m3, r3 = _stats(h)
        return (h - m3) * r3

    def a_pre(r0, gates):
        out = []
        for j, g in enumerate(gates):
            r = r0 + CH * j
            z = zero_after(g)
            qv = qb[rows(r0 // 2 + CH // 2 * j, CH // 2), :] | jnp.concatenate([z] * NT, axis=1)
            x = _bf(qv).astype(F32)
            m1, r1 = _stats(x)
            x1 = x + ((x - m1) * r1 * prm(0) + prm(1)) * ld_y(r, CH)
            x1b[rows(r, CH), :] = x1
            m2, r2 = _stats(x1)
            h = (x1 - m2) * r2 * prm(2) + prm(3)
            hb[rows(r, CH), :] = h
            m3, r3 = _stats(h)
            out.append((h - m3) * r3)
        return jnp.concatenate(out, axis=0)

    def halves(n, split):
        return [(0, n // 2), (n // 2, n - n // 2)] if split else [(0, n)]

    def mm1(r0, n, n3, split_last=False, ties=None, ties2=None):
        for t in range(NT):
            w = w1b[:, 128 * t:128 * t + 128]
            if ties and t in ties:
                w = _tie(w, {**ties[t], **ties2[t]})
            for o, m in halves(n, split_last and t == NT - 1):
                hp = jnp.dot(n3[o:o + m].astype(BF16), _bf(w), preferred_element_type=F32)
                hpb[t, rows(HPAD + r0 + o, m), :] = _gelu(hp)

    def g_prep(r0):
        lane = jax.lax.broadcasted_iota(I32, (TB, 128), 1)
        sh = [-1, 1, -2, 2]

        def ldh(t, g):
            return hpb[t, pl.ds(HPAD + r0 + sh[g], TB), :]

        cols = [ldh(0, 0)]
        for t in range(1, 4):
            cols.append(jnp.where(lane < 32 * t, ldh(t, t - 1), ldh(t, t)))
        cols.append(ldh(4, 3))
        return jnp.concatenate(cols, axis=-1)

    def mm2(r0, g, split_last=False, side=None):
        for t in range(NT):
            if side and t in side:
                side[t]()
            c0, c1 = 128 * t, 128 * t + 128
            for o, m in halves(TB, split_last and t == NT - 1):
                hs = jnp.dot(g[o:o + m].astype(BF16), _bf(w2b[:, c0:c1]), preferred_element_type=F32)
                hb[rows(r0 + o, m), c0:c1] = hb[rows(r0 + o, m), c0:c1] + hs
        return hs[m - 8:m]

    def ln4(r0, n):
        x2 = hb[rows(r0, n), :]
        m4, r4 = _stats(x2)
        return (x2 - m4) * r4

    def mm3(n4, ties=None, split_last=False, side=None, tpos=12, nat=True):
        us = []
        env["g3"] = []
        for j in range(FF // 128):
            if side and j in side:
                side[j]()
            if j == tpos:
                ht = jax.lax.dot_general(_bf(w3b[FM // 2:FF // 2, :]), n4.astype(BF16), NT_DIMS,
                                         preferred_element_type=F32)
                ut = _gelu(ht).T
            w = w3b[64 * j:64 * j + 64, :]
            if ties and j in ties:
                w = _tie(w, {0: ties[j]})
            parts = []
            for o, m in halves(TB, split_last and j == FF // 128 - 1):
                if j == 0 and nat:
                    h3 = jnp.dot(n4.astype(BF16), _bf(w3n[...]), preferred_element_type=F32)
                else:
                    h3 = jax.lax.dot_general(n4[o:o + m].astype(BF16), _bf(w), NT_DIMS,
                                             preferred_element_type=F32)
                parts.append(_gelu(h3))
                if m == TB:
                    env["g3"] += [h3[0:8], h3[128:136]]
            us.append(jnp.concatenate(parts, axis=0))
        return jnp.concatenate(us + [ut], axis=-1)

    def mm4(r0, u, t, final=True, ties=None, split=False, side=None):
        c0, c1 = 128 * t, 128 * t + 128
        w = _bf(_tie(w4b[:, c0:c1], ties))
        for o, m in halves(TB, split):
            if o and side:
                side()
            h2 = jnp.dot(u[o:o + m].astype(BF16), w, preferred_element_type=F32)
            s = hb[rows(r0 + o, m), c0:c1] + h2
            if final:
                ob[rows(r0 + o, m, 16), c0:c1] = (
                    x1b[rows(r0 + o, m), c0:c1] + prm(4, m, c0, c1) * s).astype(BF16)
            else:
                hb[rows(r0 + o, m), c0:c1] = s

    def ln4_store(r0, nch):
        zs = []
        m = TB // nch
        for j in range(nch):
            n4 = ln4(r0 + m * j, m)
            n4b[m * j:m * j + m, :] = n4
            zs.append(zero_after(n4))
        return zs

    def ln4_ticked(r0, g, nch, hops):
        z = zero_after(g)
        m = TB // nch
        for j in range(nch):
            zt = jnp.concatenate([jnp.concatenate([z] * NT, axis=1)] * (m // 8), axis=0)
            x2 = pltpu.bitcast(pltpu.bitcast(hb[rows(r0 + m * j, m), :], U32) | zt, F32)
            m4, r4 = _stats(x2)
            n4b[m * j:m * j + m, :] = (x2 - m4) * r4
            for _ in range(hops):
                z = pltpu.roll(z, 1, 1)

    def out_copy(r0, n, c0=0, c1=D):
        return pltpu.make_async_copy(ob.at[rows(r0, n, 16), c0:c1],
                                     o_hbm.at[0, rows(r0, n, 16), c0:c1], osem)

    def out_copy_old(r0, n):
        return pltpu.make_async_copy(ob.at[rows(r0, n, 16), :], o_hbm.at[0, rows(r0, n, 16), :], osem)

    wait("ra")
    env["taps"] = skb[...].astype(F32)
    env["dvec"] = sdb[...].astype(F32).reshape(1, D)
    cf = cb_[...].astype(F32)
    sc8 = jnp.broadcast_to(cf * jax.nn.sigmoid(cf), (8, D)).astype(BF16)
    run_rounds("X00")
    wait("r0")
    run_rounds("X01 K00 K10 K20 K30")
    for t in range(1, NT):
        wait(f"r{t}")
        run_rounds(f"I0{t - 1} X{(t + 1) // NT}{(t + 1) % NT} K0{t} K1{t} K2{t} K3{t}")
    wait("r5")
    run_rounds("I04 I10 X11 X12@16:3 I11 X13@20:3 I12 X14@20:3")
    wait("r6")
    run_rounds("I13 X20 I14 X21@20:3 I20 X22@20:3 I21 X23@20:3 I22 X24@20:3 I23")

    wait("wmA")
    mod = jnp.dot(sc8, wmb[:, 0:3 * D], preferred_element_type=F32)
    sa, ca, ga = [mod[:, D * i:D * (i + 1)] for i in range(3)]
    par[0] = (1.0 + ca) * ga
    par[1] = sa * ga
    run_rounds("I24")
    a_pre12(0, TB + AO)
    a_pre12(TB + AO, TB)
    wait("wmB")
    mod = jnp.dot(sc8, wmb[:, 3 * D:5 * D], preferred_element_type=F32)
    par[2] = 1.0 + mod[:, D:2 * D]
    par[3] = mod[:, 0:D]
    n3a = a_pre3(0, TB + AO)

    wait("w1")
    n3b = [a_pre3(TB + AO, TB, 32 * j, 32) for j in range(8)]
    zs = [zero_after(v) for v in n3b]
    mm1(0, TB + AO, n3a, ties={1 + j // 2: {16 * (j % 2): zs[j]} for j in range(0, 8, 2)},
        ties2={1 + j // 2: {16: zs[j]} for j in range(1, 8, 2)})
    mm1(TB + AO, TB, jnp.concatenate(n3b, axis=0), split_last=True)
    wait("w2")
    g0 = g_prep(0)
    rr = lambda x: (lambda: run_rounds(x))
    mm2(0, g0, side={1: rr("X30"), 4: rr("X31")})
    n4 = ln4(0, TB)
    mm2(TB, g_prep(TB), split_last=True, side={3: rr("X32")})
    run_rounds("I30")
    wait("w3")
    zs = ln4_store(TB, 8)
    u = mm3(n4, {5 + j: z for j, z in enumerate(zs)}, split_last=True, nat=False,
            side={0: rr("I31"), 2: rr("X33")})
    run_rounds("I32")
    wait("w4")
    w3n[...] = pltpu.bitcast(_bf(w3b[0:64, :]).T, U32)
    mm4(0, u, 0, final=False)
    run_rounds("X34")
    mm4(0, u, 1, final=False)
    mm4(0, u, 2, final=False)
    mm4(0, u, 3, final=False)
    mm4(0, u, 4, final=False, split=True)
    run_rounds("I33 I34")
    wait("rest")
    par[4] = jnp.dot(sc8, wmb[:, 5 * D:6 * D], preferred_element_type=F32)

    def body(i, carry):
        pl.when(i == 2)(lambda: wait("qlast"))
        r0 = i * TB
        u = mm3(n4b[...])
        n3 = a_pre(r0 + TB + AO, [env["g3"][j * 25 // 15] for j in range(TB // CH)])
        mm4(r0, u, 0)
        mm1(r0 + TB + AO, TB, n3)
        hpb[:, HPAD + S:HPAD + S + 8, :] = jnp.zeros((NT, 8, 128), F32)
        mm4(r0, u, 1)
        g = mm2(r0 + TB, g_prep(r0 + TB))
        ln4_ticked(r0 + TB, g, 16, 1)
        for t in range(2, NT):
            mm4(r0, u, t)
        out_copy(r0, TB).start()
        return carry

    jax.lax.fori_loop(1, NBLK - 1, body, 0)

    r0 = S - TB
    zs = []
    for j in range(8):
        rs = slice(32 * j, 32 * j + 32)
        o = x1b[rs, :] + prm(4, 32) * hb[rs, :]
        ob[rs, :] = o.astype(BF16)
        zs.append(zero_after(o))
    u = mm3(n4b[...], {3 + j: z for j, z in enumerate(zs)})
    out_copy(0, TB).start()
    for t in range(NT):
        mm4(r0, u, t, split=t == NT - 1)
        if t < NT - 1:
            out_copy(r0, TB, 128 * t, 128 * t + 128).start()
    out_copy(r0, TB // 2, D - 128, D).start()
    out_copy(r0 + TB // 2, TB // 2, D - 128, D).start()
    with jax.named_scope("W_out"):
        pltpu.make_async_copy(ob, o_hbm.at[0], osem).wait()


@jax.jit
def pallas_adaLN_cond__ssm_conv_h3__mixer_s_mlp__prompt_kernel(
    A_q, A_k, A_v, A_shift_k, A_ssm_k, A_ssm_D, B_x, B_w1, B_w2, B_w3, B_w4, c, w_mod,
):
    del B_x
    vm = pltpu.VMEM
    scratch = [
        vm(((S + AO) // 2, D), U32),
        vm((NT, KPAD + S, 128), BF16),
        vm((NT, S, 128), BF16),
        vm((4, D), BF16),
        vm((D // 2, S), U32),
        vm((D,), BF16),
        vm((D // 2, D), U32),
        vm((D // 2, D), U32),
        vm((FF // 2, D), U32),
        vm((FF // 2, D), U32),
        vm((1, D), BF16),
        vm((D, 6 * D), BF16),
        vm((R + 1, 128, 128), U32),
        vm((2 * R + 1, 32, 128), U32),
        vm((NT, S // 2, 128), U32),
        vm((8, NT, R, 256, 128), F32),
        vm((3, NT, 2 * R, 64, 128), U32),
        vm((NT, S + AO, 128), F32),
        vm((S + AO, D), F32),
        vm((S + AO, D), F32),
        vm((NT, HPAD + S + AO, 128), F32),
        vm((TB, D), F32),
        vm((5, 8, D), F32),
        vm((D // 2, 128), U32),
        vm((S, D), BF16),
        pltpu.SemaphoreType.DMA((16,)),
        pltpu.SemaphoreType.DMA(()),
    ]
    hbm = pl.BlockSpec(memory_space=pltpu.HBM)
    return pl.pallas_call(
        _kernel,
        out_shape=jax.ShapeDtypeStruct((1, S, D), BF16),
        in_specs=[hbm] * 12,
        out_specs=hbm,
        scratch_shapes=scratch,
        compiler_params=pltpu.CompilerParams(vmem_limit_bytes=110 * 2**20,
                                             disable_semaphore_checks=True,
                                             disable_bounds_checks=True),
        name="h3_mixer",
    )(A_q, A_k, A_v, A_shift_k.T, A_ssm_k, A_ssm_D, B_w1, B_w2, B_w3.T, B_w4, c, w_mod)
```

```python
import jax
import jax.numpy as jnp
import numpy as np
import jax.experimental.pallas as pl
import jax.experimental.pallas.tpu as pltpu

S, D, FF = 2048, 640, 1728
NT = D // 128
L = 512
NB = S // L
NFFT = 2 * L
R = 4
KPAD = 16
HPAD = 8
TB = 256
NBLK = S // TB
AO = 16
CH = 16
EPS = 1e-5
NPAD = 1
FM = FF // 128 * 128
F32 = jnp.float32
BF16 = jnp.bfloat16
U32 = jnp.uint32
I32 = jnp.int32
NT_DIMS = (((1,), (1,)), ((), ()))
KP, X0S, ZP = 0, 3, 3


def _cos_coefs(deg=6):
    u = (np.cos(np.pi * (np.arange(400) + 0.5) / 400) + 1.0) / 2.0
    c = np.polynomial.polynomial.polyfit(u, np.cos(np.pi * np.sqrt(u)), deg)
    return [np.float32(v) for v in c]


_COS = _cos_coefs()


def _cos_units(a, scale=1.0):
    x = (((a + 1024) & 2047) - 1024).astype(F32) * np.float32(1.0 / 1024.0)
    u = x * x
    acc = u * np.float32(_COS[-1] * scale) + np.float32(_COS[-2] * scale)
    for c in _COS[-3::-1]:
        acc = acc * u + np.float32(c * scale)
    return acc


def _freq2(chunk, s):
    e = 4 * (8 * (chunk >> 1) + s) + 1
    return jnp.where((chunk & 1) == 0, e, 256 - e)


def _gelu(x):
    c1 = np.float32(np.sqrt(2.0 / np.pi))
    c2 = np.float32(np.sqrt(2.0 / np.pi) * 0.044715)
    u = x * (c1 + c2 * (x * x))
    hx = 0.5 * x
    return hx + hx * jnp.tanh(u)


def _stats(x):
    m = jnp.sum(x, axis=-1, keepdims=True) * (1.0 / D)
    e2 = jnp.sum(x * x, axis=-1, keepdims=True) * (1.0 / D)
    v = jnp.maximum(e2 - m * m, 0.0)
    return m, jax.lax.rsqrt(v + EPS)


def _split(b):
    b = b.reshape(-1, 2, 8, 128)
    return b[:, 0], b[:, 1]


def _join(z):
    return jnp.stack(z, axis=1).reshape(-1, 128)


def _eo(v):
    v = v.reshape(-1, 2, 8, 128)
    return v[:, 0], v[:, 1]


def _uneo(e, o):
    return jnp.stack([e, o], axis=1).reshape(16, 8, 128)


def _fft4(b, sign):
    (r0, i0), (r1, i1), (r2, i2), (r3, i3) = b
    sr, si, dr, di = r0 + r2, i0 + i2, r0 - r2, i0 - i2
    tr, ti, er, ei = r1 + r3, i1 + i3, r1 - r3, i1 - i3
    x0 = (sr + tr, si + ti)
    x2 = (sr - tr, si - ti)
    xm = (dr + ei, di - er)
    xp = (dr - ei, di + er)
    return [x0, xm, x2, xp] if sign < 0 else [x0, xp, x2, xm]


def _cmul(a, b, acc=None):
    (ar, ai), (br, bi) = a, b
    if acc is None:
        return ar * br - ai * bi, ar * bi + ai * br
    return (acc[0] + ar * br) - ai * bi, (acc[1] + ar * bi) + ai * br


def _bf(x):
    return pltpu.bitcast(x, BF16)


def _pack(a, b):
    return pltpu.pack_elementwise([a, b], packed_dtype=BF16)


def _tie(w, ties):
    if not ties:
        return w
    parts = []
    for i in range(w.shape[0] // 8):
        p = w[8 * i:8 * i + 8]
        if i in ties:
            z = ties[i]
            p = p | z if p.shape[1] == 128 else jnp.concatenate([p[:, :128] | z, p[:, 128:]], axis=1)
        parts.append(p)
    return jnp.concatenate(parts, axis=0)


def _kernel(q_hbm, k_hbm, v_hbm, sk_hbm, ssm_hbm, sd_hbm, w1_hbm, w2_hbm, w3_hbm,
            w4_hbm, c_hbm, wm_hbm, o_hbm,
            qb, kb, vb, skb, ssmb, sdb, w1b, w2b, w3b, w4b, cb_, wmb, fwb, gib,
            stb, spec, cmb, yb, x1b, hb, hpb, n4b, par, w3n, ob, sems, osem):
    groups = {}

    def add(name, src, dst):
        if name not in groups:
            groups[name] = (len(groups), [])
        idx, lst = groups[name]
        cp = pltpu.make_async_copy(src, dst, sems.at[idx])
        cp.start()
        lst.append(cp)

    def add_kv(name, c, tiles=range(NT)):
        for t in tiles:
            add(name, k_hbm.at[0, pl.ds(L * c, L), pl.ds(128 * t, 128)],
                kb.at[t, pl.ds(KPAD + L * c, L), :])
            add(name, v_hbm.at[0, pl.ds(L * c, L), pl.ds(128 * t, 128)],
                vb.at[t, pl.ds(L * c, L), :])

    def add_ssm(name, t):
        add(name, ssm_hbm.at[pl.ds(128 * t, 128), :], ssmb.bitcast(BF16).at[pl.ds(128 * t, 128), :])

    QE = 2 * TB + AO
    add_kv("ra", 0, [0])
    add("ra", sd_hbm, sdb)
    add("ra", sk_hbm, skb)
    add("ra", c_hbm, cb_)
    for t in range(NT):
        add_ssm(f"r{t}", t)
        add_kv(f"r{t}", (t + 1) // NT, [(t + 1) % NT])
    add_kv("r5", 1, range(1, NT))
    add_kv("r6", 2)
    add("wmA", q_hbm.at[0, pl.ds(0, QE), :], qb.bitcast(BF16).at[pl.ds(0, QE), :])
    add("wmA", wm_hbm.at[:, pl.ds(0, 3 * D)], wmb.at[:, pl.ds(0, 3 * D)])
    add("wmB", wm_hbm.at[:, pl.ds(3 * D, 2 * D)], wmb.at[:, pl.ds(3 * D, 2 * D)])
    add("w1", w1_hbm, w1b.bitcast(BF16))
    add("w2", w2_hbm, w2b.bitcast(BF16))
    add_kv("w2", 3, range(3))
    add("w3", w3_hbm, w3b.bitcast(BF16))
    add("w4", w4_hbm.at[:, pl.ds(0, D - 128)], w4b.bitcast(BF16).at[:, pl.ds(0, D - 128)])
    add_kv("w4", 3, [3, 4])
    add("rest", w4_hbm.at[:, pl.ds(D - 128, 128)], w4b.bitcast(BF16).at[:, pl.ds(D - 128, 128)])
    add("rest", wm_hbm.at[:, pl.ds(5 * D, D)], wmb.at[:, pl.ds(5 * D, D)])
    add("rest", q_hbm.at[0, pl.ds(QE, TB), :], qb.bitcast(BF16).at[pl.ds(QE, TB), :])
    add("qlast", q_hbm.at[0, pl.ds(QE + TB, S - QE - TB), :],
        qb.bitcast(BF16).at[pl.ds(QE + TB, S - QE - TB), :])

    def wait(name):
        with jax.named_scope("W_" + name):
            for cp in groups[name][1]:
                cp.wait()

    kb[:, 0:KPAD, :] = jnp.zeros((NT, KPAD, 128), BF16)
    hpb[:, 0:HPAD, :] = jnp.zeros((NT, HPAD, 128), F32)
    yb[:, S:S + AO, :] = jnp.zeros((NT, AO, 128), F32)
    qb[S // 2:(S + AO) // 2, :] = jnp.zeros((AO // 2, D), U32)

    spec[7, 0, 0, pl.ds(0, 8, stride=2), :] = jnp.zeros((8, 128), F32)
    cmb[2, 0, 0, pl.ds(0, 8, stride=2), :] = jnp.zeros((8, 128), U32)
    fwb[R, pl.ds(0, 8, stride=2), :] = jnp.zeros((8, 128), U32)
    gib[2 * R, pl.ds(0, 8, stride=2), :] = jnp.zeros((8, 128), U32)

    def make_tables(off):
        row = jax.lax.broadcasted_iota(I32, (128, 128), 0)
        col = jax.lax.broadcasted_iota(I32, (128, 128), 1)
        f2e = _freq2(row >> 3, 2 * (row & 3))
        f2o = _freq2(row >> 3, 2 * (row & 3) + 1)
        ph = 512 * ((row >> 2) & 1) + off
        for r in range(R):
            n = 4 * col + r
            fwb[r] = _pack(_cos_units(n * f2e + ph), _cos_units(n * f2o + ph))
        row = jax.lax.broadcasted_iota(I32, (32, 128), 0)
        col = jax.lax.broadcasted_iota(I32, (32, 128), 1)
        f2 = 4 * (col >> 1) + 1
        ph = 512 * (col & 1) + off
        for r in range(2 * R):
            a = (16 * row + r) * f2 + ph
            gib[r] = _pack(_cos_units(a, 2.0 / NFFT), _cos_units(a + 8 * f2, 2.0 / NFFT))

    make_tables(0)

    env = {}

    def zero_after(*vals):
        acc = None
        for v in vals:
            v = pltpu.bitcast(v, U32)
            for i in range(0, v.shape[0], 8):
                for j in range(0, v.shape[1], 128):
                    p = v[i:i + 8, j:j + 128]
                    acc = p if acc is None else acc | p
        return acc & kb.bitcast(U32)[0, 0:8, :]

    def ld_spec(slot, t, q):
        return _split(spec[slot, t, q])

    def st_spec(slot, t, q, z):
        spec[slot, t, q] = _join(z)

    def fwd_dots(rhs, ties):
        return [_split(jnp.dot(_bf(_tie(fwb[r], ties if r == 0 else None)), _bf(rhs[r]),
                               preferred_element_type=F32)) for r in range(R)]

    def conv_k(c, t, ties):
        w0 = L * c // 2
        stb[t, w0:w0 + L // 2, :] = pltpu.bitcast(
            _bf(ssmb[64 * t:64 * t + 64, L * c:L * c + L]).T, U32)
        rhs = []
        for h in range(2):
            lo = stb[t, pl.ds(w0 + h, 64, stride=4), :]
            hi = stb[t, pl.ds(w0 + h + 2, 64, stride=4), :]
            rhs.append((lo & jnp.uint32(0xFFFF)) | (hi << 16))
            rhs.append((lo >> 16) | (hi & jnp.uint32(0xFFFF0000)))
        b = fwd_dots(rhs, ties)
        if c == 0:
            b[0] = (b[0][0] + env["dvec"][:, 128 * t:128 * t + 128][None], b[0][1])
        kq = _fft4(b, -1)
        z = []
        for q in range(R):
            kp = kq[q]
            if c >= 2:
                p = ld_spec(KP + c - 2, t, q)
                kp = (kp[0] + p[0], kp[1] + p[1])
            if c >= 1:
                p = ld_spec(KP + c - 1, t, q)
                if c == 3:
                    p0 = ld_spec(KP, t, q)
                    p = (p[0] - p0[0], p[1] - p0[1])
                (ree, reo), (ime, imo), (pre, pro), (pie, pio) = (_eo(v) for v in kp + p)
                kp = (_uneo(ree - pie, reo + pio), _uneo(ime + pre, imo - pro))
            if c < 3:
                st_spec(KP + c, t, q, kp)
            zc = _cmul(kp, ld_spec(X0S, t, q))
            if c == 0:
                z.append(zc)
            else:
                st_spec(ZP + c, t, q, zc)
        if c == 0:
            finish(0, t, z)

    def finish(c, t, z):
        hs = np.float32(np.sqrt(0.5))
        cr = _fft4(z, +1)
        for r in range(R):
            (ar, br), (ai, bi) = _eo(cr[r][0]), _eo(cr[r][1])
            if r % 2:
                br, bi = (br - bi) * hs, (br + bi) * hs
            if r < 2:
                p, m = (ar + br, ai - bi), (ar - br, ai + bi)
            else:
                p, m = (ar - bi, ai - br), (ar + bi, ai + br)
            cmb[c % 2, t, r] = _pack(*p).reshape(64, 128)
            cmb[c % 2, t, r + R] = _pack(*m).reshape(64, 128)

    def unpack(u):
        return (pltpu.bitcast(u << 16, F32),
                pltpu.bitcast(u & jnp.uint32(0xFFFF0000), F32))

    def conv_prep(c, t):
        taps = env["taps"]
        ku = kb.bitcast(U32)
        vu = vb.bitcast(U32)
        tp = [taps[j:j + 1, 128 * t:128 * t + 128] for j in range(4)]
        w0 = (KPAD + L * c) // 2
        kk = [unpack(ku[t, pl.ds(w0 - 2, 64, stride=4), :])[1]]
        for o in range(-1, 4):
            kk += unpack(ku[t, pl.ds(w0 + o, 64, stride=4), :])
        vv = []
        for o in range(4):
            vv += unpack(vu[t, pl.ds(L * c // 2 + o, 64, stride=4), :])
        kv = []
        for n in range(8):
            acc = kk[3 + n] * tp[0]
            for j in range(1, 4):
                acc = acc + kk[3 + n - j] * tp[j]
            kv.append(acc * vv[n])
        return [_pack(kv[r], kv[r + 4]) for r in range(R)]

    def conv_x(c, t, ties):
        xq = _fft4(fwd_dots(env.pop(("kv", c, t)), ties), -1)
        z = []
        for q in range(R):
            if c == 0:
                st_spec(X0S, t, q, xq[q])
                continue
            for a in range(c, NB):
                za = _cmul(xq[q], ld_spec(KP + a - c, t, q), ld_spec(ZP + a, t, q))
                if a == c:
                    z.append(za)
                else:
                    st_spec(ZP + a, t, q, za)
        if c:
            finish(c, t, z)

    def conv_inv(c, t, ties):
        for r in range(2 * R):
            tr = None
            if ties and r % R == 0:
                tr = {i - r: z for i, z in ties.items() if 0 <= i - r < 4}
            yb[t, pl.ds(L * c + r, 64, stride=2 * R), :] = jnp.dot(
                _bf(_tie(gib[r], tr)), _bf(cmb[c % 2, t, r]), preferred_element_type=F32)

    def run_rounds(spec_str):
        rounds = spec_str.split()
        slots = []
        plan = {}
        for n, rd in enumerate(rounds):
            if rd[0] == "X":
                pts = []
                if "@" in rd:
                    a, b = (int(v) for v in rd[4:].split(":"))
                    pts = [slots[len(slots) - a + (a - b) * (j + 1) // 8 - 1] for j in range(8)]
                plan.setdefault(pts[0][0] if pts else n, []).append((rd, pts))
            slots += [(n, i) for i in range(8 if rd[0] == "I" else 16)]
        ties = {}
        for n, rd in enumerate(rounds):
            for xr, pts in plan.get(n, []):
                c, t = int(xr[1]), int(xr[2])
                kv = env["kv", c, t] = conv_prep(c, t)
                for j, (pn, pi) in enumerate(pts):
                    z = zero_after(*[w[8 * j:8 * j + 8] for w in kv])
                    d = ties.setdefault(pn, {})
                    d[pi] = z if pi not in d else d[pi] | z
            {"K": conv_k, "X": conv_x, "I": conv_inv}[rd[0]](int(rd[1]), int(rd[2]), ties.get(n))

    def rows(r0, n, align=8):
        if isinstance(r0, int):
            return slice(r0, r0 + n)
        return pl.ds(pl.multiple_of(r0, align), n)

    def ld_y(r0, n):
        return jnp.concatenate([yb[t, rows(r0, n), :] for t in range(NT)], axis=-1)

    def prm(i, n=CH, c0=0, c1=D):
        return jnp.concatenate([par[i, :, c0:c1]] * (n // 8), axis=0)

    def a_pre12(r0, n):
        x = _bf(qb[r0 // 2:(r0 + n) // 2, :]).astype(F32)
        m1, r1 = _stats(x)
        x1 = x + ((x - m1) * r1 * prm(0, n) + prm(1, n)) * ld_y(r0, n)
        x1b[r0:r0 + n, :] = x1
        env["m2", r0] = _stats(x1)

    def a_pre3(r0, n, o=0, m=None):
        m = n if m is None else m
        m2, r2 = (v[o:o + m] for v in env["m2", r0])
        rs = slice(r0 + o, r0 + o + m)
        h = (x1b[rs, :] - m2) * r2 * prm(2, m) + prm(3, m)
        hb[rs, :] = h
        m3, r3 = _stats(h)
        return (h - m3) * r3

    def a_pre(r0, gates):
        out = []
        for j, g in enumerate(gates):
            r = r0 + CH * j
            z = zero_after(g)
            qv = qb[rows(r0 // 2 + CH // 2 * j, CH // 2), :] | jnp.concatenate([z] * NT, axis=1)
            x = _bf(qv).astype(F32)
            m1, r1 = _stats(x)
            x1 = x + ((x - m1) * r1 * prm(0) + prm(1)) * ld_y(r, CH)
            x1b[rows(r, CH), :] = x1
            m2, r2 = _stats(x1)
            h = (x1 - m2) * r2 * prm(2) + prm(3)
            hb[rows(r, CH), :] = h
            m3, r3 = _stats(h)
            out.append((h - m3) * r3)
        return jnp.concatenate(out, axis=0)

    def halves(n, split):
        return [(0, n // 2), (n // 2, n - n // 2)] if split else [(0, n)]

    def mm1(r0, n, n3, split_last=False, ties=None, ties2=None):
        for t in range(NT):
            w = w1b[:, 128 * t:128 * t + 128]
            if ties and t in ties:
                w = _tie(w, {**ties[t], **ties2[t]})
            for o, m in halves(n, split_last and t == NT - 1):
                hp = jnp.dot(n3[o:o + m].astype(BF16), _bf(w), preferred_element_type=F32)
                hpb[t, rows(HPAD + r0 + o, m), :] = _gelu(hp)

    def g_prep(r0):
        lane = jax.lax.broadcasted_iota(I32, (TB, 128), 1)
        sh = [-1, 1, -2, 2]

        def ldh(t, g):
            return hpb[t, pl.ds(HPAD + r0 + sh[g], TB), :]

        cols = [ldh(0, 0)]
        for t in range(1, 4):
            cols.append(jnp.where(lane < 32 * t, ldh(t, t - 1), ldh(t, t)))
        cols.append(ldh(4, 3))
        return jnp.concatenate(cols, axis=-1)

    def mm2(r0, g, split_last=False, side=None):
        for t in range(NT):
            if side and t in side:
                side[t]()
            c0, c1 = 128 * t, 128 * t + 128
            for o, m in halves(TB, split_last and t == NT - 1):
                hs = jnp.dot(g[o:o + m].astype(BF16), _bf(w2b[:, c0:c1]), preferred_element_type=F32)
                hb[rows(r0 + o, m), c0:c1] = hb[rows(r0 + o, m), c0:c1] + hs
        return hs[m - 8:m]

    def ln4(r0, n):
        x2 = hb[rows(r0, n), :]
        m4, r4 = _stats(x2)
        return (x2 - m4) * r4

    def mm3(n4, ties=None, split_last=False, side=None, tpos=12, nat=True):
        us = []
        env["g3"] = []
        for j in range(FF // 128):
            if side and j in side:
                side[j]()
            if j == tpos:
                ht = jax.lax.dot_general(_bf(w3b[FM // 2:FF // 2, :]), n4.astype(BF16), NT_DIMS,
                                         preferred_element_type=F32)
                ut = _gelu(ht).T
            w = w3b[64 * j:64 * j + 64, :]
            if ties and j in ties:
                w = _tie(w, {0: ties[j]})
            parts = []
            for o, m in halves(TB, split_last and j == FF // 128 - 1):
                if j == 0 and nat:
                    h3 = jnp.dot(n4.astype(BF16), _bf(w3n[...]), preferred_element_type=F32)
                else:
                    h3 = jax.lax.dot_general(n4[o:o + m].astype(BF16), _bf(w), NT_DIMS,
                                             preferred_element_type=F32)
                parts.append(_gelu(h3))
                if m == TB:
                    env["g3"] += [h3[0:8], h3[128:136]]
            us.append(jnp.concatenate(parts, axis=0))
        return jnp.concatenate(us + [ut], axis=-1)

    def mm4(r0, u, t, final=True, ties=None, split=False, side=None):
        c0, c1 = 128 * t, 128 * t + 128
        w = _bf(_tie(w4b[:, c0:c1], ties))
        for o, m in halves(TB, split):
            if o and side:
                side()
            h2 = jnp.dot(u[o:o + m].astype(BF16), w, preferred_element_type=F32)
            s = hb[rows(r0 + o, m), c0:c1] + h2
            if final:
                ob[rows(r0 + o, m, 16), c0:c1] = (
                    x1b[rows(r0 + o, m), c0:c1] + prm(4, m, c0, c1) * s).astype(BF16)
            else:
                hb[rows(r0 + o, m), c0:c1] = s

    def ln4_store(r0, nch):
        zs = []
        m = TB // nch
        for j in range(nch):
            n4 = ln4(r0 + m * j, m)
            n4b[m * j:m * j + m, :] = n4
            zs.append(zero_after(n4))
        return zs

    def ln4_ticked(r0, g, nch, hops):
        z = zero_after(g)
        m = TB // nch
        for j in range(nch):
            zt = jnp.concatenate([jnp.concatenate([z] * NT, axis=1)] * (m // 8), axis=0)
            x2 = pltpu.bitcast(pltpu.bitcast(hb[rows(r0 + m * j, m), :], U32) | zt, F32)
            m4, r4 = _stats(x2)
            n4b[m * j:m * j + m, :] = (x2 - m4) * r4
            for _ in range(hops):
                z = pltpu.roll(z, 1, 1)

    def out_copy(r0, n, c0=0, c1=D):
        return pltpu.make_async_copy(ob.at[rows(r0, n, 16), c0:c1],
                                     o_hbm.at[0, rows(r0, n, 16), c0:c1], osem)

    def out_copy_old(r0, n):
        return pltpu.make_async_copy(ob.at[rows(r0, n, 16), :], o_hbm.at[0, rows(r0, n, 16), :], osem)

    wait("ra")
    env["taps"] = skb[...].astype(F32)
    env["dvec"] = sdb[...].astype(F32).reshape(1, D)
    cf = cb_[...].astype(F32)
    sc8 = jnp.broadcast_to(cf * jax.nn.sigmoid(cf), (8, D)).astype(BF16)
    run_rounds("X00")
    wait("r0")
    run_rounds("X01 K00 K10 K20 K30")
    for t in range(1, NT):
        wait(f"r{t}")
        run_rounds(f"I0{t - 1} X{(t + 1) // NT}{(t + 1) % NT} K0{t} K1{t} K2{t} K3{t}")
    wait("r5")
    run_rounds("I04 I10 X11 X12@16:3 I11 X13@20:3 I12 X14@20:3")
    wait("r6")
    run_rounds("I13 X20 I14 X21@20:3 I20 X22@20:3 I21 X23@20:3 I22 X24@20:3 I23")

    flag = kb.bitcast(I32)[0, 0:8, :][0, 0]
    for n in range(NPAD):
        pl.when(flag != 0)(lambda: make_tables(2 * NFFT * (n + 1) * flag))
    wait("wmA")
    mod = jnp.dot(sc8, wmb[:, 0:3 * D], preferred_element_type=F32)
    sa, ca, ga = [mod[:, D * i:D * (i + 1)] for i in range(3)]
    par[0] = (1.0 + ca) * ga
    par[1] = sa * ga
    run_rounds("I24")
    a_pre12(0, TB + AO)
    a_pre12(TB + AO, TB)
    wait("wmB")
    mod = jnp.dot(sc8, wmb[:, 3 * D:5 * D], preferred_element_type=F32)
    par[2] = 1.0 + mod[:, D:2 * D]
    par[3] = mod[:, 0:D]
    n3a = a_pre3(0, TB + AO)

    wait("w1")
    n3b = [a_pre3(TB + AO, TB, 32 * j, 32) for j in range(8)]
    zs = [zero_after(v) for v in n3b]
    mm1(0, TB + AO, n3a, ties={1 + j // 2: {16 * (j % 2): zs[j]} for j in range(0, 8, 2)},
        ties2={1 + j // 2: {16: zs[j]} for j in range(1, 8, 2)})
    mm1(TB + AO, TB, jnp.concatenate(n3b, axis=0), split_last=True)
    wait("w2")
    g0 = g_prep(0)
    rr = lambda x: (lambda: run_rounds(x))
    mm2(0, g0, side={1: rr("X30"), 4: rr("X31")})
    n4 = ln4(0, TB)
    mm2(TB, g_prep(TB), split_last=True, side={3: rr("X32")})
    run_rounds("I30")
    wait("w3")
    zs = ln4_store(TB, 8)
    u = mm3(n4, {5 + j: z for j, z in enumerate(zs)}, split_last=True, nat=False,
            side={0: rr("I31")})
    run_rounds("I32")
    wait("w4")
    w3n[...] = pltpu.bitcast(_bf(w3b[0:64, :]).T, U32)
    mm4(0, u, 0, final=False)
    run_rounds("X33")
    mm4(0, u, 1, final=False)
    run_rounds("X34")
    mm4(0, u, 2, final=False)
    mm4(0, u, 3, final=False, split=True)
    run_rounds("I33")
    wait("rest")

    def gb_tiles(*ts):
        for t in ts:
            par[4, :, 128 * t:128 * t + 128] = jnp.dot(
                sc8, wmb[:, 5 * D + 128 * t:5 * D + 128 * t + 128], preferred_element_type=F32)

    gb_tiles(4, 0, 1)
    mm4(0, u, 4, split=True, side=lambda: gb_tiles(2, 3))
    ob[0:TB, 0:D - 128] = (x1b[0:TB, 0:D - 128]
                           + prm(4, TB, 0, D - 128) * hb[0:TB, 0:D - 128]).astype(BF16)
    run_rounds("I34")
    out_copy(0, TB).start()

    def body(i, carry):
        pl.when(i == 2)(lambda: wait("qlast"))
        r0 = i * TB
        u = mm3(n4b[...])
        n3 = a_pre(r0 + TB + AO, [env["g3"][j * 25 // 15] for j in range(TB // CH)])
        mm4(r0, u, 0)
        mm1(r0 + TB + AO, TB, n3)
        hpb[:, HPAD + S:HPAD + S + 8, :] = jnp.zeros((NT, 8, 128), F32)
        mm4(r0, u, 1)
        g = mm2(r0 + TB, g_prep(r0 + TB))
        ln4_ticked(r0 + TB, g, 16, 1)
        for t in range(2, NT):
            mm4(r0, u, t)
        out_copy(r0, TB).start()
        return carry

    jax.lax.fori_loop(1, NBLK - 1, body, 0)

    r0 = S - TB
    u = mm3(n4b[...])
    for t in range(NT):
        mm4(r0, u, t, split=t == NT - 1)
        if t < NT - 1:
            out_copy(r0, TB, 128 * t, 128 * t + 128).start()
    out_copy(r0, TB // 2, D - 128, D).start()
    out_copy(r0 + TB // 2, TB // 2, D - 128, D).start()
    with jax.named_scope("W_out"):
        pltpu.make_async_copy(ob, o_hbm.at[0], osem).wait()


@jax.jit
def pallas_adaLN_cond__ssm_conv_h3__mixer_s_mlp__prompt_kernel(
    A_q, A_k, A_v, A_shift_k, A_ssm_k, A_ssm_D, B_x, B_w1, B_w2, B_w3, B_w4, c, w_mod,
):
    del B_x
    vm = pltpu.VMEM
    scratch = [
        vm(((S + AO) // 2, D), U32),
        vm((NT, KPAD + S, 128), BF16),
        vm((NT, S, 128), BF16),
        vm((4, D), BF16),
        vm((D // 2, S), U32),
        vm((D,), BF16),
        vm((D // 2, D), U32),
        vm((D // 2, D), U32),
        vm((FF // 2, D), U32),
        vm((FF // 2, D), U32),
        vm((1, D), BF16),
        vm((D, 6 * D), BF16),
        vm((R + 1, 128, 128), U32),
        vm((2 * R + 1, 32, 128), U32),
        vm((NT, S // 2, 128), U32),
        vm((8, NT, R, 256, 128), F32),
        vm((3, NT, 2 * R, 64, 128), U32),
        vm((NT, S + AO, 128), F32),
        vm((S + AO, D), F32),
        vm((S + AO, D), F32),
        vm((NT, HPAD + S + AO, 128), F32),
        vm((TB, D), F32),
        vm((5, 8, D), F32),
        vm((D // 2, 128), U32),
        vm((S, D), BF16),
        pltpu.SemaphoreType.DMA((16,)),
        pltpu.SemaphoreType.DMA(()),
    ]
    hbm = pl.BlockSpec(memory_space=pltpu.HBM)
    return pl.pallas_call(
        _kernel,
        out_shape=jax.ShapeDtypeStruct((1, S, D), BF16),
        in_specs=[hbm] * 12,
        out_specs=hbm,
        scratch_shapes=scratch,
        compiler_params=pltpu.CompilerParams(vmem_limit_bytes=110 * 2**20,
                                             disable_semaphore_checks=True,
                                             disable_bounds_checks=True),
        name="h3_mixer",
    )(A_q, A_k, A_v, A_shift_k.T, A_ssm_k, A_ssm_D, B_w1, B_w2, B_w3.T, B_w4, c, w_mod)
```

```python
import jax
import jax.numpy as jnp
import numpy as np
import jax.experimental.pallas as pl
import jax.experimental.pallas.tpu as pltpu

S, D, FF = 2048, 640, 1728
NT = D // 128
L = 512
NB = S // L
NFFT = 2 * L
R = 4
KPAD = 16
HPAD = 8
TB = 256
NBLK = S // TB
AO = 16
CH = 16
EPS = 1e-5
W1A, W3A, W4A = 256, 1536, 384
NPAD = 1
FM = FF // 128 * 128
F32 = jnp.float32
BF16 = jnp.bfloat16
U32 = jnp.uint32
I32 = jnp.int32
NT_DIMS = (((1,), (1,)), ((), ()))
KP, X0S, ZP = 0, 3, 3


def _cos_coefs(deg=6):
    u = (np.cos(np.pi * (np.arange(400) + 0.5) / 400) + 1.0) / 2.0
    c = np.polynomial.polynomial.polyfit(u, np.cos(np.pi * np.sqrt(u)), deg)
    return [np.float32(v) for v in c]


_COS = _cos_coefs()


def _cos_units(a, scale=1.0):
    x = (((a + 1024) & 2047) - 1024).astype(F32) * np.float32(1.0 / 1024.0)
    u = x * x
    acc = u * np.float32(_COS[-1] * scale) + np.float32(_COS[-2] * scale)
    for c in _COS[-3::-1]:
        acc = acc * u + np.float32(c * scale)
    return acc


def _freq2(chunk, s):
    e = 4 * (8 * (chunk >> 1) + s) + 1
    return jnp.where((chunk & 1) == 0, e, 256 - e)


def _gelu(x):
    c1 = np.float32(np.sqrt(2.0 / np.pi))
    c2 = np.float32(np.sqrt(2.0 / np.pi) * 0.044715)
    u = x * (c1 + c2 * (x * x))
    hx = 0.5 * x
    return hx + hx * jnp.tanh(u)


def _stats(x):
    m = jnp.sum(x, axis=-1, keepdims=True) * (1.0 / D)
    e2 = jnp.sum(x * x, axis=-1, keepdims=True) * (1.0 / D)
    v = jnp.maximum(e2 - m * m, 0.0)
    return m, jax.lax.rsqrt(v + EPS)


def _split(b):
    b = b.reshape(-1, 2, 8, 128)
    return b[:, 0], b[:, 1]


def _join(z):
    return jnp.stack(z, axis=1).reshape(-1, 128)


def _eo(v):
    v = v.reshape(-1, 2, 8, 128)
    return v[:, 0], v[:, 1]


def _uneo(e, o):
    return jnp.stack([e, o], axis=1).reshape(16, 8, 128)


def _fft4(b, sign):
    (r0, i0), (r1, i1), (r2, i2), (r3, i3) = b
    sr, si, dr, di = r0 + r2, i0 + i2, r0 - r2, i0 - i2
    tr, ti, er, ei = r1 + r3, i1 + i3, r1 - r3, i1 - i3
    x0 = (sr + tr, si + ti)
    x2 = (sr - tr, si - ti)
    xm = (dr + ei, di - er)
    xp = (dr - ei, di + er)
    return [x0, xm, x2, xp] if sign < 0 else [x0, xp, x2, xm]


def _cmul(a, b, acc=None):
    (ar, ai), (br, bi) = a, b
    if acc is None:
        return ar * br - ai * bi, ar * bi + ai * br
    return (acc[0] + ar * br) - ai * bi, (acc[1] + ar * bi) + ai * br


def _bf(x):
    return pltpu.bitcast(x, BF16)


def _pack(a, b):
    return pltpu.pack_elementwise([a, b], packed_dtype=BF16)


def _tie(w, ties):
    if not ties:
        return w
    parts = []
    for i in range(w.shape[0] // 8):
        p = w[8 * i:8 * i + 8]
        if i in ties:
            z = ties[i]
            p = p | z if p.shape[1] == 128 else jnp.concatenate([p[:, :128] | z, p[:, 128:]], axis=1)
        parts.append(p)
    return jnp.concatenate(parts, axis=0)


def _kernel(q_hbm, k_hbm, v_hbm, sk_hbm, ssm_hbm, sd_hbm, w1_hbm, w2_hbm, w3_hbm,
            w4_hbm, c_hbm, wm_hbm, o_hbm,
            qb, kb, vb, skb, ssmb, sdb, w1b, w2b, w3b, w4b, cb_, wmb, fwb, gib,
            stb, spec, cmb, yb, x1b, hb, hpb, n4b, par, w3n, ob, sems, osem):
    groups = {}

    def add(name, src, dst):
        if name not in groups:
            groups[name] = (len(groups), [])
        idx, lst = groups[name]
        cp = pltpu.make_async_copy(src, dst, sems.at[idx])
        cp.start()
        lst.append(cp)

    def add_kv(name, c, tiles=range(NT)):
        for t in tiles:
            add(name, k_hbm.at[0, pl.ds(L * c, L), pl.ds(128 * t, 128)],
                kb.at[t, pl.ds(KPAD + L * c, L), :])
            add(name, v_hbm.at[0, pl.ds(L * c, L), pl.ds(128 * t, 128)],
                vb.at[t, pl.ds(L * c, L), :])

    def add_ssm(name, t):
        add(name, ssm_hbm.at[pl.ds(128 * t, 128), :], ssmb.bitcast(BF16).at[pl.ds(128 * t, 128), :])

    QE = 2 * TB + AO
    add_kv("ra", 0, [0])
    add("ra", sd_hbm, sdb)
    add("ra", sk_hbm, skb)
    add("ra", c_hbm, cb_)
    for t in range(NT):
        add_ssm(f"r{t}", t)
        add_kv(f"r{t}", (t + 1) // NT, [(t + 1) % NT])
    add_kv("r5", 1, range(1, NT))
    add_kv("r6", 2)
    add("wmA", q_hbm.at[0, pl.ds(0, QE), :], qb.bitcast(BF16).at[pl.ds(0, QE), :])
    add("wmA", wm_hbm.at[:, pl.ds(0, 3 * D)], wmb.at[:, pl.ds(0, 3 * D)])
    add("wmS", wm_hbm.at[:, pl.ds(3 * D, D + 256)], wmb.at[:, pl.ds(3 * D, D + 256)])
    add("wmB", wm_hbm.at[:, pl.ds(4 * D + 256, D - 256)], wmb.at[:, pl.ds(4 * D + 256, D - 256)])
    add("w1", w1_hbm.at[:, pl.ds(0, W1A)], w1b.bitcast(BF16).at[:, pl.ds(0, W1A)])
    add("w1b", w1_hbm.at[:, pl.ds(W1A, D - W1A)], w1b.bitcast(BF16).at[:, pl.ds(W1A, D - W1A)])
    add_kv("w1b", 3, [0])
    add("w2", w2_hbm, w2b.bitcast(BF16))
    add_kv("w2", 3, [1])
    add("w3", w3_hbm.at[pl.ds(0, W3A), :], w3b.bitcast(BF16).at[pl.ds(0, W3A), :])
    add("w4", w3_hbm.at[pl.ds(W3A, FF - W3A), :], w3b.bitcast(BF16).at[pl.ds(W3A, FF - W3A), :])
    add("w4", w4_hbm.at[:, pl.ds(0, W4A)], w4b.bitcast(BF16).at[:, pl.ds(0, W4A)])
    add_kv("w4", 3, [2, 3])
    add("rest", w4_hbm.at[:, pl.ds(W4A, D - W4A)], w4b.bitcast(BF16).at[:, pl.ds(W4A, D - W4A)])
    add_kv("rest", 3, [4])
    add("rest", wm_hbm.at[:, pl.ds(5 * D, D)], wmb.at[:, pl.ds(5 * D, D)])
    add("qnext", q_hbm.at[0, pl.ds(QE, TB), :], qb.bitcast(BF16).at[pl.ds(QE, TB), :])
    add("qlast", q_hbm.at[0, pl.ds(QE + TB, S - QE - TB), :],
        qb.bitcast(BF16).at[pl.ds(QE + TB, S - QE - TB), :])

    def wait(name):
        with jax.named_scope("W_" + name):
            for cp in groups[name][1]:
                cp.wait()

    kb[:, 0:KPAD, :] = jnp.zeros((NT, KPAD, 128), BF16)
    hpb[:, 0:HPAD, :] = jnp.zeros((NT, HPAD, 128), F32)
    yb[:, S:S + AO, :] = jnp.zeros((NT, AO, 128), F32)
    qb[S // 2:(S + AO) // 2, :] = jnp.zeros((AO // 2, D), U32)

    spec[7, 0, 0, pl.ds(0, 8, stride=2), :] = jnp.zeros((8, 128), F32)
    cmb[2, 0, 0, pl.ds(0, 8, stride=2), :] = jnp.zeros((8, 128), U32)
    fwb[R, pl.ds(0, 8, stride=2), :] = jnp.zeros((8, 128), U32)
    gib[2 * R, pl.ds(0, 8, stride=2), :] = jnp.zeros((8, 128), U32)

    def make_tables(off):
        row = jax.lax.broadcasted_iota(I32, (128, 128), 0)
        col = jax.lax.broadcasted_iota(I32, (128, 128), 1)
        f2e = _freq2(row >> 3, 2 * (row & 3))
        f2o = _freq2(row >> 3, 2 * (row & 3) + 1)
        ph = 512 * ((row >> 2) & 1) + off
        for r in range(R):
            n = 4 * col + r
            fwb[r] = _pack(_cos_units(n * f2e + ph), _cos_units(n * f2o + ph))
        row = jax.lax.broadcasted_iota(I32, (32, 128), 0)
        col = jax.lax.broadcasted_iota(I32, (32, 128), 1)
        f2 = 4 * (col >> 1) + 1
        ph = 512 * (col & 1) + off
        for r in range(2 * R):
            a = (16 * row + r) * f2 + ph
            gib[r] = _pack(_cos_units(a, 2.0 / NFFT), _cos_units(a + 8 * f2, 2.0 / NFFT))

    make_tables(0)

    env = {}

    def zero_after(*vals):
        acc = None
        for v in vals:
            v = pltpu.bitcast(v, U32)
            for i in range(0, v.shape[0], 8):
                for j in range(0, v.shape[1], 128):
                    p = v[i:i + 8, j:j + 128]
                    acc = p if acc is None else acc | p
        return acc & kb.bitcast(U32)[0, 0:8, :]

    def ld_spec(slot, t, q):
        return _split(spec[slot, t, q])

    def st_spec(slot, t, q, z):
        spec[slot, t, q] = _join(z)

    def fwd_dots(rhs, ties):
        return [_split(jnp.dot(_bf(_tie(fwb[r], ties if r == 0 else None)), _bf(rhs[r]),
                               preferred_element_type=F32)) for r in range(R)]

    def conv_k(c, t, ties):
        w0 = L * c // 2
        stb[t, w0:w0 + L // 2, :] = pltpu.bitcast(
            _bf(ssmb[64 * t:64 * t + 64, L * c:L * c + L]).T, U32)
        rhs = []
        for h in range(2):
            lo = stb[t, pl.ds(w0 + h, 64, stride=4), :]
            hi = stb[t, pl.ds(w0 + h + 2, 64, stride=4), :]
            rhs.append((lo & jnp.uint32(0xFFFF)) | (hi << 16))
            rhs.append((lo >> 16) | (hi & jnp.uint32(0xFFFF0000)))
        b = fwd_dots(rhs, ties)
        if c == 0:
            b[0] = (b[0][0] + env["dvec"][:, 128 * t:128 * t + 128][None], b[0][1])
        kq = _fft4(b, -1)
        z = []
        for q in range(R):
            kp = kq[q]
            if c >= 2:
                p = ld_spec(KP + c - 2, t, q)
                kp = (kp[0] + p[0], kp[1] + p[1])
            if c >= 1:
                p = ld_spec(KP + c - 1, t, q)
                if c == 3:
                    p0 = ld_spec(KP, t, q)
                    p = (p[0] - p0[0], p[1] - p0[1])
                (ree, reo), (ime, imo), (pre, pro), (pie, pio) = (_eo(v) for v in kp + p)
                kp = (_uneo(ree - pie, reo + pio), _uneo(ime + pre, imo - pro))
            if c < 3:
                st_spec(KP + c, t, q, kp)
            zc = _cmul(kp, ld_spec(X0S, t, q))
            if c == 0:
                z.append(zc)
            else:
                st_spec(ZP + c, t, q, zc)
        if c == 0:
            finish(0, t, z)

    def finish(c, t, z):
        hs = np.float32(np.sqrt(0.5))
        cr = _fft4(z, +1)
        for r in range(R):
            (ar, br), (ai, bi) = _eo(cr[r][0]), _eo(cr[r][1])
            if r % 2:
                br, bi = (br - bi) * hs, (br + bi) * hs
            if r < 2:
                p, m = (ar + br, ai - bi), (ar - br, ai + bi)
            else:
                p, m = (ar - bi, ai - br), (ar + bi, ai + br)
            cmb[c % 2, t, r] = _pack(*p).reshape(64, 128)
            cmb[c % 2, t, r + R] = _pack(*m).reshape(64, 128)

    def unpack(u):
        return (pltpu.bitcast(u << 16, F32),
                pltpu.bitcast(u & jnp.uint32(0xFFFF0000), F32))

    def conv_prep(c, t):
        taps = env["taps"]
        ku = kb.bitcast(U32)
        vu = vb.bitcast(U32)
        tp = [taps[j:j + 1, 128 * t:128 * t + 128] for j in range(4)]
        w0 = (KPAD + L * c) // 2
        kk = [unpack(ku[t, pl.ds(w0 - 2, 64, stride=4), :])[1]]
        for o in range(-1, 4):
            kk += unpack(ku[t, pl.ds(w0 + o, 64, stride=4), :])
        vv = []
        for o in range(4):
            vv += unpack(vu[t, pl.ds(L * c // 2 + o, 64, stride=4), :])
        kv = []
        for n in range(8):
            acc = kk[3 + n] * tp[0]
            for j in range(1, 4):
                acc = acc + kk[3 + n - j] * tp[j]
            kv.append(acc * vv[n])
        return [_pack(kv[r], kv[r + 4]) for r in range(R)]

    def conv_x(c, t, ties):
        xq = _fft4(fwd_dots(env.pop(("kv", c, t)), ties), -1)
        z = []
        for q in range(R):
            if c == 0:
                st_spec(X0S, t, q, xq[q])
                continue
            for a in range(c, NB):
                za = _cmul(xq[q], ld_spec(KP + a - c, t, q), ld_spec(ZP + a, t, q))
                if a == c:
                    z.append(za)
                else:
                    st_spec(ZP + a, t, q, za)
        if c:
            finish(c, t, z)

    def conv_inv(c, t, ties):
        for r in range(2 * R):
            tr = None
            if ties and r % R == 0:
                tr = {i - r: z for i, z in ties.items() if 0 <= i - r < 4}
            yb[t, pl.ds(L * c + r, 64, stride=2 * R), :] = jnp.dot(
                _bf(_tie(gib[r], tr)), _bf(cmb[c % 2, t, r]), preferred_element_type=F32)

    def run_rounds(spec_str):
        rounds = spec_str.split()
        slots = []
        plan = {}
        for n, rd in enumerate(rounds):
            if rd[0] == "X":
                pts = []
                if "@" in rd:
                    a, b = (int(v) for v in rd[4:].split(":"))
                    pts = [slots[len(slots) - a + (a - b) * (j + 1) // 8 - 1] for j in range(8)]
                plan.setdefault(pts[0][0] if pts else n, []).append((rd, pts))
            slots += [(n, i) for i in range(8 if rd[0] == "I" else 16)]
        ties = {}
        for n, rd in enumerate(rounds):
            for xr, pts in plan.get(n, []):
                c, t = int(xr[1]), int(xr[2])
                kv = env["kv", c, t] = conv_prep(c, t)
                for j, (pn, pi) in enumerate(pts):
                    z = zero_after(*[w[8 * j:8 * j + 8] for w in kv])
                    d = ties.setdefault(pn, {})
                    d[pi] = z if pi not in d else d[pi] | z
            {"K": conv_k, "X": conv_x, "I": conv_inv}[rd[0]](int(rd[1]), int(rd[2]), ties.get(n))

    def rows(r0, n, align=8):
        if isinstance(r0, int):
            return slice(r0, r0 + n)
        return pl.ds(pl.multiple_of(r0, align), n)

    def ld_y(r0, n):
        return jnp.concatenate([yb[t, rows(r0, n), :] for t in range(NT)], axis=-1)

    def prm(i, n=CH, c0=0, c1=D):
        return jnp.concatenate([par[i, :, c0:c1]] * (n // 8), axis=0)

    def a_pre12(r0, n):
        x = _bf(qb[r0 // 2:(r0 + n) // 2, :]).astype(F32)
        m1, r1 = _stats(x)
        x1 = x + ((x - m1) * r1 * prm(0, n) + prm(1, n)) * ld_y(r0, n)
        x1b[r0:r0 + n, :] = x1
        m2, r2 = _stats(x1)
        hb[r0:r0 + n, :] = (x1 - m2) * r2

    def a_pre3(r0, m):
        h = hb[r0:r0 + m, :] * prm(2, m) + prm(3, m)
        hb[r0:r0 + m, :] = h
        m3, r3 = _stats(h)
        return (h - m3) * r3

    def a_pre(r0, gates):
        out = []
        for j, g in enumerate(gates):
            r = r0 + CH * j
            z = zero_after(g)
            qv = qb[rows(r0 // 2 + CH // 2 * j, CH // 2), :] | jnp.concatenate([z] * NT, axis=1)
            x = _bf(qv).astype(F32)
            m1, r1 = _stats(x)
            x1 = x + ((x - m1) * r1 * prm(0) + prm(1)) * ld_y(r, CH)
            x1b[rows(r, CH), :] = x1
            m2, r2 = _stats(x1)
            h = (x1 - m2) * r2 * prm(2) + prm(3)
            hb[rows(r, CH), :] = h
            m3, r3 = _stats(h)
            out.append((h - m3) * r3)
        return jnp.concatenate(out, axis=0)

    def halves(n, split):
        return [(0, n // 2), (n // 2, n - n // 2)] if split else [(0, n)]

    def mm1(r0, n, n3, split_last=False, ties=None, tiles=range(NT)):
        for t in tiles:
            w = _tie(w1b[:, 128 * t:128 * t + 128], ties.get(t) if ties else None)
            for o, m in halves(n, split_last and t == tiles[-1]):
                hp = jnp.dot(n3[o:o + m].astype(BF16), _bf(w), preferred_element_type=F32)
                hpb[t, rows(HPAD + r0 + o, m), :] = _gelu(hp)

    def g_prep(r0):
        lane = jax.lax.broadcasted_iota(I32, (TB, 128), 1)
        sh = [-1, 1, -2, 2]

        def ldh(t, g):
            return hpb[t, pl.ds(HPAD + r0 + sh[g], TB), :]

        cols = [ldh(0, 0)]
        for t in range(1, 4):
            cols.append(jnp.where(lane < 32 * t, ldh(t, t - 1), ldh(t, t)))
        cols.append(ldh(4, 3))
        return jnp.concatenate(cols, axis=-1)

    def mm2(r0, g, split_last=False, side=None):
        for t in range(NT):
            if side and t in side:
                side[t]()
            c0, c1 = 128 * t, 128 * t + 128
            for o, m in halves(TB, split_last and t == NT - 1):
                hs = jnp.dot(g[o:o + m].astype(BF16), _bf(w2b[:, c0:c1]), preferred_element_type=F32)
                hb[rows(r0 + o, m), c0:c1] = hb[rows(r0 + o, m), c0:c1] + hs
        return hs[m - 8:m]

    def ln4(r0, n):
        x2 = hb[rows(r0, n), :]
        m4, r4 = _stats(x2)
        return (x2 - m4) * r4

    def mm3(n4, ties=None, split_at=None, side=None, tpos=12, nat=True):
        us = []
        env["g3"] = []
        for j in range(FF // 128):
            if side and j in side:
                side[j]()
            if j == tpos:
                ht = jax.lax.dot_general(_bf(w3b[FM // 2:FF // 2, :]), n4.astype(BF16), NT_DIMS,
                                         preferred_element_type=F32)
                ut = _gelu(ht).T
            w = w3b[64 * j:64 * j + 64, :]
            if ties and j in ties:
                w = _tie(w, {0: ties[j]})
            parts = []
            for o, m in halves(TB, j == split_at):
                if j == 0 and nat:
                    h3 = jnp.dot(n4.astype(BF16), _bf(w3n[...]), preferred_element_type=F32)
                else:
                    h3 = jax.lax.dot_general(n4[o:o + m].astype(BF16), _bf(w), NT_DIMS,
                                             preferred_element_type=F32)
                parts.append(_gelu(h3))
                if m == TB:
                    env["g3"] += [h3[0:8], h3[128:136]]
            us.append(jnp.concatenate(parts, axis=0))
        return jnp.concatenate(us + [ut], axis=-1)

    def mm4(r0, u, t, final=True, ties=None, split=False, side=None):
        c0, c1 = 128 * t, 128 * t + 128
        w = _bf(_tie(w4b[:, c0:c1], ties))
        for o, m in halves(TB, split):
            if o and side:
                side()
            h2 = jnp.dot(u[o:o + m].astype(BF16), w, preferred_element_type=F32)
            s = hb[rows(r0 + o, m), c0:c1] + h2
            if final:
                ob[rows(r0 + o, m, 16), c0:c1] = (
                    x1b[rows(r0 + o, m), c0:c1] + prm(4, m, c0, c1) * s).astype(BF16)
            else:
                hb[rows(r0 + o, m), c0:c1] = s

    def ln4_store(r0, nch):
        zs = []
        m = TB // nch
        for j in range(nch):
            n4 = ln4(r0 + m * j, m)
            n4b[m * j:m * j + m, :] = n4
            zs.append(zero_after(n4))
        return zs

    def ln4_ticked(r0, g, nch, hops):
        z = zero_after(g)
        m = TB // nch
        for j in range(nch):
            zt = jnp.concatenate([jnp.concatenate([z] * NT, axis=1)] * (m // 8), axis=0)
            x2 = pltpu.bitcast(pltpu.bitcast(hb[rows(r0 + m * j, m), :], U32) | zt, F32)
            m4, r4 = _stats(x2)
            n4b[m * j:m * j + m, :] = (x2 - m4) * r4
            for _ in range(hops):
                z = pltpu.roll(z, 1, 1)

    def out_copy(r0, n, c0=0, c1=D):
        return pltpu.make_async_copy(ob.at[rows(r0, n, 16), c0:c1],
                                     o_hbm.at[0, rows(r0, n, 16), c0:c1], osem)

    def out_copy_old(r0, n):
        return pltpu.make_async_copy(ob.at[rows(r0, n, 16), :], o_hbm.at[0, rows(r0, n, 16), :], osem)

    wait("ra")
    env["taps"] = skb[...].astype(F32)
    env["dvec"] = sdb[...].astype(F32).reshape(1, D)
    cf = cb_[...].astype(F32)
    sc8 = jnp.broadcast_to(cf * jax.nn.sigmoid(cf), (8, D)).astype(BF16)
    run_rounds("X00")
    wait("r0")
    run_rounds("X01 K00 K10 K20 K30")
    for t in range(1, NT):
        wait(f"r{t}")
        run_rounds(f"I0{t - 1} X{(t + 1) // NT}{(t + 1) % NT} K0{t} K1{t} K2{t} K3{t}")
    wait("r5")
    run_rounds("I04 I10 X11 X12@16:3 I11 X13@20:3 I12 X14@20:3")
    wait("r6")
    run_rounds("I13 X20 I14 X21@20:3 I20 X22@20:3 I21 X23@20:3 I22 X24@20:3 I23")

    flag = kb.bitcast(I32)[0, 0:8, :][0, 0]
    for n in range(NPAD):
        pl.when(flag != 0)(lambda: make_tables(2 * NFFT * (n + 1) * flag))
    wait("wmA")
    mod = jnp.dot(sc8, wmb[:, 0:3 * D], preferred_element_type=F32)
    sa, ca, ga = [mod[:, D * i:D * (i + 1)] for i in range(3)]
    par[0] = (1.0 + ca) * ga
    par[1] = sa * ga
    run_rounds("I24")
    a_pre12(0, TB + AO)
    a_pre12(TB + AO, TB)
    wait("wmS")
    mod = jnp.dot(sc8, wmb[:, 3 * D:4 * D + 256], preferred_element_type=F32)
    par[3] = mod[:, 0:D]
    par[2, :, 0:256] = 1.0 + mod[:, D:D + 256]
    wait("wmB")
    par[2, :, 256:D] = 1.0 + jnp.dot(sc8, wmb[:, 4 * D + 256:5 * D], preferred_element_type=F32)
    n3a = a_pre3(0, TB + AO)

    rr = lambda x: (lambda: run_rounds(x))
    ta, tb = range(W1A // 128), range(W1A // 128, NT)
    wait("w1")
    n3b = a_pre3(TB + AO, TB)
    mm1(0, TB + AO, n3a, tiles=ta)
    mm1(TB + AO, TB, n3b, split_last=True, tiles=ta)
    wait("w1b")
    mm1(0, TB + AO, n3a, tiles=tb)
    run_rounds("X30")
    mm1(TB + AO, TB, n3b, split_last=True, tiles=tb)
    wait("w2")
    g0 = g_prep(0)
    mm2(0, g0, side={2: rr("X31")})
    n4 = ln4(0, TB)
    mm2(TB, g_prep(TB), split_last=True)
    run_rounds("I30")
    wait("w3")
    zs = ln4_store(TB, 8)

    def mid():
        run_rounds("I31")
        wait("w4")
        w3n[...] = pltpu.bitcast(_bf(w3b[0:64, :]).T, U32)

    u = mm3(n4, {3 + j: z for j, z in enumerate(zs)}, split_at=W3A // 128 - 1, nat=False,
            side={W3A // 128: mid})
    run_rounds("X32")
    mm4(0, u, 0, final=False)
    run_rounds("X33")
    mm4(0, u, 1, final=False)
    mm4(0, u, 2, final=False, split=True)
    run_rounds("I32")
    wait("rest")

    def gb_tiles(*ts):
        for t in ts:
            par[4, :, 128 * t:128 * t + 128] = jnp.dot(
                sc8, wmb[:, 5 * D + 128 * t:5 * D + 128 * t + 128], preferred_element_type=F32)

    gb_tiles(3, 4)
    mm4(0, u, 3, split=True, side=lambda: (run_rounds("X34"), gb_tiles(0, 1)))
    gb_tiles(2)
    mm4(0, u, 4, split=True)
    ob[0:TB, 0:W4A] = (x1b[0:TB, 0:W4A] + prm(4, TB, 0, W4A) * hb[0:TB, 0:W4A]).astype(BF16)
    run_rounds("I33 I34")
    out_copy(0, TB).start()
    wait("qnext")

    def body(i, carry):
        pl.when(i == 2)(lambda: wait("qlast"))
        r0 = i * TB
        u = mm3(n4b[...])
        n3 = a_pre(r0 + TB + AO, [env["g3"][j * 25 // 15] for j in range(TB // CH)])
        mm4(r0, u, 0)
        mm1(r0 + TB + AO, TB, n3)
        hpb[:, HPAD + S:HPAD + S + 8, :] = jnp.zeros((NT, 8, 128), F32)
        mm4(r0, u, 1)
        g = mm2(r0 + TB, g_prep(r0 + TB))
        ln4_ticked(r0 + TB, g, 16, 1)
        for t in range(2, NT):
            mm4(r0, u, t)
        out_copy(r0, TB).start()
        return carry

    jax.lax.fori_loop(1, NBLK - 1, body, 0)

    r0 = S - TB
    u = mm3(n4b[...])
    for t in range(NT):
        mm4(r0, u, t, split=t == NT - 1)
        if t < NT - 1:
            out_copy(r0, TB, 128 * t, 128 * t + 128).start()
    out_copy(r0, TB // 2, D - 128, D).start()
    out_copy(r0 + TB // 2, TB // 2, D - 128, D).start()
    with jax.named_scope("W_out"):
        pltpu.make_async_copy(ob, o_hbm.at[0], osem).wait()


@jax.jit
def pallas_adaLN_cond__ssm_conv_h3__mixer_s_mlp__prompt_kernel(
    A_q, A_k, A_v, A_shift_k, A_ssm_k, A_ssm_D, B_x, B_w1, B_w2, B_w3, B_w4, c, w_mod,
):
    del B_x
    vm = pltpu.VMEM
    scratch = [
        vm(((S + AO) // 2, D), U32),
        vm((NT, KPAD + S, 128), BF16),
        vm((NT, S, 128), BF16),
        vm((4, D), BF16),
        vm((D // 2, S), U32),
        vm((D,), BF16),
        vm((D // 2, D), U32),
        vm((D // 2, D), U32),
        vm((FF // 2, D), U32),
        vm((FF // 2, D), U32),
        vm((1, D), BF16),
        vm((D, 6 * D), BF16),
        vm((R + 1, 128, 128), U32),
        vm((2 * R + 1, 32, 128), U32),
        vm((NT, S // 2, 128), U32),
        vm((8, NT, R, 256, 128), F32),
        vm((3, NT, 2 * R, 64, 128), U32),
        vm((NT, S + AO, 128), F32),
        vm((S + AO, D), F32),
        vm((S + AO, D), F32),
        vm((NT, HPAD + S + AO, 128), F32),
        vm((TB, D), F32),
        vm((5, 8, D), F32),
        vm((D // 2, 128), U32),
        vm((S, D), BF16),
        pltpu.SemaphoreType.DMA((19,)),
        pltpu.SemaphoreType.DMA(()),
    ]
    hbm = pl.BlockSpec(memory_space=pltpu.HBM)
    return pl.pallas_call(
        _kernel,
        out_shape=jax.ShapeDtypeStruct((1, S, D), BF16),
        in_specs=[hbm] * 12,
        out_specs=hbm,
        scratch_shapes=scratch,
        compiler_params=pltpu.CompilerParams(vmem_limit_bytes=110 * 2**20,
                                             disable_semaphore_checks=True,
                                             disable_bounds_checks=True),
        name="h3_mixer",
    )(A_q, A_k, A_v, A_shift_k.T, A_ssm_k, A_ssm_D, B_w1, B_w2, B_w3.T, B_w4, c, w_mod)
```

```python
import jax
import jax.numpy as jnp
import numpy as np
import jax.experimental.pallas as pl
import jax.experimental.pallas.tpu as pltpu

S, D, FF = 2048, 640, 1728
NT = D // 128
L = 512
NB = S // L
NFFT = 2 * L
R = 4
KPAD = 16
HPAD = 8
TB = 256
NBLK = S // TB
AO = 16
CH = 16
EPS = 1e-5
W1A, W3A, W4A = 256, 1536, 384
NPAD = 1
FM = FF // 128 * 128
F32 = jnp.float32
BF16 = jnp.bfloat16
U32 = jnp.uint32
I32 = jnp.int32
NT_DIMS = (((1,), (1,)), ((), ()))
KP, X0S, ZP = 0, 3, 3


def _cos_coefs(deg=6):
    u = (np.cos(np.pi * (np.arange(400) + 0.5) / 400) + 1.0) / 2.0
    c = np.polynomial.polynomial.polyfit(u, np.cos(np.pi * np.sqrt(u)), deg)
    return [np.float32(v) for v in c]


_COS = _cos_coefs()


def _cos_units(a, scale=1.0):
    x = (((a + 1024) & 2047) - 1024).astype(F32) * np.float32(1.0 / 1024.0)
    u = x * x
    acc = u * np.float32(_COS[-1] * scale) + np.float32(_COS[-2] * scale)
    for c in _COS[-3::-1]:
        acc = acc * u + np.float32(c * scale)
    return acc


def _freq2(chunk, s):
    e = 4 * (8 * (chunk >> 1) + s) + 1
    return jnp.where((chunk & 1) == 0, e, 256 - e)


def _gelu(x):
    c1 = np.float32(np.sqrt(2.0 / np.pi))
    c2 = np.float32(np.sqrt(2.0 / np.pi) * 0.044715)
    u = x * (c1 + c2 * (x * x))
    hx = 0.5 * x
    return hx + hx * jnp.tanh(u)


def _stats(x):
    m = jnp.sum(x, axis=-1, keepdims=True) * (1.0 / D)
    e2 = jnp.sum(x * x, axis=-1, keepdims=True) * (1.0 / D)
    v = jnp.maximum(e2 - m * m, 0.0)
    return m, jax.lax.rsqrt(v + EPS)


def _split(b):
    b = b.reshape(-1, 2, 8, 128)
    return b[:, 0], b[:, 1]


def _join(z):
    return jnp.stack(z, axis=1).reshape(-1, 128)


def _eo(v):
    v = v.reshape(-1, 2, 8, 128)
    return v[:, 0], v[:, 1]


def _uneo(e, o):
    return jnp.stack([e, o], axis=1).reshape(16, 8, 128)


def _fft4(b, sign):
    (r0, i0), (r1, i1), (r2, i2), (r3, i3) = b
    sr, si, dr, di = r0 + r2, i0 + i2, r0 - r2, i0 - i2
    tr, ti, er, ei = r1 + r3, i1 + i3, r1 - r3, i1 - i3
    x0 = (sr + tr, si + ti)
    x2 = (sr - tr, si - ti)
    xm = (dr + ei, di - er)
    xp = (dr - ei, di + er)
    return [x0, xm, x2, xp] if sign < 0 else [x0, xp, x2, xm]


def _cmul(a, b, acc=None):
    (ar, ai), (br, bi) = a, b
    if acc is None:
        return ar * br - ai * bi, ar * bi + ai * br
    return (acc[0] + ar * br) - ai * bi, (acc[1] + ar * bi) + ai * br


def _bf(x):
    return pltpu.bitcast(x, BF16)


def _pack(a, b):
    return pltpu.pack_elementwise([a, b], packed_dtype=BF16)


def _tie(w, ties):
    if not ties:
        return w
    parts = []
    for i in range(w.shape[0] // 8):
        p = w[8 * i:8 * i + 8]
        if i in ties:
            z = ties[i]
            p = p | z if p.shape[1] == 128 else jnp.concatenate([p[:, :128] | z, p[:, 128:]], axis=1)
        parts.append(p)
    return jnp.concatenate(parts, axis=0)


def _kernel(q_hbm, k_hbm, v_hbm, sk_hbm, ssm_hbm, sd_hbm, w1_hbm, w2_hbm, w3_hbm,
            w4_hbm, c_hbm, wm_hbm, o_hbm,
            qb, kb, vb, skb, ssmb, sdb, w1b, w2b, w3b, w4b, cb_, wmb, fwb, gib,
            stb, spec, cmb, yb, x1b, hb, hpb, n4b, par, w3n, ob, sems, osem):
    groups = {}

    def add(name, src, dst):
        if name not in groups:
            groups[name] = (len(groups), [])
        idx, lst = groups[name]
        cp = pltpu.make_async_copy(src, dst, sems.at[idx])
        cp.start()
        lst.append(cp)

    def add_kv(name, c, tiles=range(NT)):
        for t in tiles:
            add(name, k_hbm.at[0, pl.ds(L * c, L), pl.ds(128 * t, 128)],
                kb.at[t, pl.ds(KPAD + L * c, L), :])
            add(name, v_hbm.at[0, pl.ds(L * c, L), pl.ds(128 * t, 128)],
                vb.at[t, pl.ds(L * c, L), :])

    def add_ssm(name, t):
        add(name, ssm_hbm.at[pl.ds(128 * t, 128), :], ssmb.bitcast(BF16).at[pl.ds(128 * t, 128), :])

    QE = 2 * TB + AO
    add_kv("ra", 0, [0])
    add("ra", sd_hbm, sdb)
    add("ra", sk_hbm, skb)
    add("ra", c_hbm, cb_)
    for t in range(NT):
        add_ssm(f"r{t}", t)
        add_kv(f"r{t}", (t + 1) // NT, [(t + 1) % NT])
    add_kv("r5", 1, range(1, NT))
    add_kv("r6", 2)
    add("wmA", q_hbm.at[0, pl.ds(0, QE), :], qb.bitcast(BF16).at[pl.ds(0, QE), :])
    add("wmA", wm_hbm.at[:, pl.ds(0, 3 * D)], wmb.at[:, pl.ds(0, 3 * D)])
    add("wmS", wm_hbm.at[:, pl.ds(3 * D, D + 256)], wmb.at[:, pl.ds(3 * D, D + 256)])
    add("wmB", wm_hbm.at[:, pl.ds(4 * D + 256, D - 256)], wmb.at[:, pl.ds(4 * D + 256, D - 256)])
    add("w1", w1_hbm.at[:, pl.ds(0, W1A)], w1b.bitcast(BF16).at[:, pl.ds(0, W1A)])
    add("w1b", w1_hbm.at[:, pl.ds(W1A, D - W1A)], w1b.bitcast(BF16).at[:, pl.ds(W1A, D - W1A)])
    add_kv("w1b", 3, [0])
    add("w2", w2_hbm, w2b.bitcast(BF16))
    add_kv("w2", 3, [1])
    add("w3", w3_hbm.at[pl.ds(0, W3A), :], w3b.bitcast(BF16).at[pl.ds(0, W3A), :])
    add("w4", w3_hbm.at[pl.ds(W3A, FF - W3A), :], w3b.bitcast(BF16).at[pl.ds(W3A, FF - W3A), :])
    add("w4", w4_hbm.at[:, pl.ds(0, W4A)], w4b.bitcast(BF16).at[:, pl.ds(0, W4A)])
    add_kv("w4", 3, [2, 3])
    add("rest", w4_hbm.at[:, pl.ds(W4A, D - W4A)], w4b.bitcast(BF16).at[:, pl.ds(W4A, D - W4A)])
    add_kv("rest", 3, [4])
    add("rest", wm_hbm.at[:, pl.ds(5 * D, D)], wmb.at[:, pl.ds(5 * D, D)])
    add("qnext", q_hbm.at[0, pl.ds(QE, TB), :], qb.bitcast(BF16).at[pl.ds(QE, TB), :])
    add("qlast", q_hbm.at[0, pl.ds(QE + TB, S - QE - TB), :],
        qb.bitcast(BF16).at[pl.ds(QE + TB, S - QE - TB), :])

    def wait(name):
        with jax.named_scope("W_" + name):
            for cp in groups[name][1]:
                cp.wait()

    kb[:, 0:KPAD, :] = jnp.zeros((NT, KPAD, 128), BF16)
    hpb[:, 0:HPAD, :] = jnp.zeros((NT, HPAD, 128), F32)
    yb[:, S:S + AO, :] = jnp.zeros((NT, AO, 128), F32)
    qb[S // 2:(S + AO) // 2, :] = jnp.zeros((AO // 2, D), U32)

    spec[7, 0, 0, pl.ds(0, 8, stride=2), :] = jnp.zeros((8, 128), F32)
    cmb[2, 0, 0, pl.ds(0, 8, stride=2), :] = jnp.zeros((8, 128), U32)
    fwb[R, pl.ds(0, 8, stride=2), :] = jnp.zeros((8, 128), U32)
    gib[2 * R, pl.ds(0, 8, stride=2), :] = jnp.zeros((8, 128), U32)

    def make_tables(off):
        row = jax.lax.broadcasted_iota(I32, (128, 128), 0)
        col = jax.lax.broadcasted_iota(I32, (128, 128), 1)
        f2e = _freq2(row >> 3, 2 * (row & 3))
        f2o = _freq2(row >> 3, 2 * (row & 3) + 1)
        ph = 512 * ((row >> 2) & 1) + off
        for r in range(R):
            n = 4 * col + r
            fwb[r] = _pack(_cos_units(n * f2e + ph), _cos_units(n * f2o + ph))
        row = jax.lax.broadcasted_iota(I32, (32, 128), 0)
        col = jax.lax.broadcasted_iota(I32, (32, 128), 1)
        f2 = 4 * (col >> 1) + 1
        ph = 512 * (col & 1) + off
        for r in range(2 * R):
            a = (16 * row + r) * f2 + ph
            gib[r] = _pack(_cos_units(a, 2.0 / NFFT), _cos_units(a + 8 * f2, 2.0 / NFFT))

    make_tables(0)

    env = {}

    def zero_after(*vals):
        acc = None
        for v in vals:
            v = pltpu.bitcast(v, U32)
            for i in range(0, v.shape[0], 8):
                for j in range(0, v.shape[1], 128):
                    p = v[i:i + 8, j:j + 128]
                    acc = p if acc is None else acc | p
        return acc & kb.bitcast(U32)[0, 0:8, :]

    def ld_spec(slot, t, q):
        return _split(spec[slot, t, q])

    def st_spec(slot, t, q, z):
        spec[slot, t, q] = _join(z)

    def fwd_dots(rhs, ties):
        return [_split(jnp.dot(_bf(_tie(fwb[r], ties if r == 0 else None)), _bf(rhs[r]),
                               preferred_element_type=F32)) for r in range(R)]

    def conv_k(c, t, ties):
        w0 = L * c // 2
        stb[t, w0:w0 + L // 2, :] = pltpu.bitcast(
            _bf(ssmb[64 * t:64 * t + 64, L * c:L * c + L]).T, U32)
        rhs = []
        for h in range(2):
            lo = stb[t, pl.ds(w0 + h, 64, stride=4), :]
            hi = stb[t, pl.ds(w0 + h + 2, 64, stride=4), :]
            rhs.append((lo & jnp.uint32(0xFFFF)) | (hi << 16))
            rhs.append((lo >> 16) | (hi & jnp.uint32(0xFFFF0000)))
        b = fwd_dots(rhs, ties)
        if c == 0:
            b[0] = (b[0][0] + env["dvec"][:, 128 * t:128 * t + 128][None], b[0][1])
        kq = _fft4(b, -1)
        z = []
        for q in range(R):
            kp = kq[q]
            if c >= 2:
                p = ld_spec(KP + c - 2, t, q)
                kp = (kp[0] + p[0], kp[1] + p[1])
            if c >= 1:
                p = ld_spec(KP + c - 1, t, q)
                if c == 3:
                    p0 = ld_spec(KP, t, q)
                    p = (p[0] - p0[0], p[1] - p0[1])
                (ree, reo), (ime, imo), (pre, pro), (pie, pio) = (_eo(v) for v in kp + p)
                kp = (_uneo(ree - pie, reo + pio), _uneo(ime + pre, imo - pro))
            if c < 3:
                st_spec(KP + c, t, q, kp)
            zc = _cmul(kp, ld_spec(X0S, t, q))
            if c == 0:
                z.append(zc)
            else:
                st_spec(ZP + c, t, q, zc)
        if c == 0:
            finish(0, t, z)

    def finish(c, t, z):
        hs = np.float32(np.sqrt(0.5))
        cr = _fft4(z, +1)
        for r in range(R):
            (ar, br), (ai, bi) = _eo(cr[r][0]), _eo(cr[r][1])
            if r % 2:
                br, bi = (br - bi) * hs, (br + bi) * hs
            if r < 2:
                p, m = (ar + br, ai - bi), (ar - br, ai + bi)
            else:
                p, m = (ar - bi, ai - br), (ar + bi, ai + br)
            cmb[c % 2, t, r] = _pack(*p).reshape(64, 128)
            cmb[c % 2, t, r + R] = _pack(*m).reshape(64, 128)

    def unpack(u):
        return (pltpu.bitcast(u << 16, F32),
                pltpu.bitcast(u & jnp.uint32(0xFFFF0000), F32))

    def conv_prep(c, t):
        taps = env["taps"]
        ku = kb.bitcast(U32)
        vu = vb.bitcast(U32)
        tp = [taps[j:j + 1, 128 * t:128 * t + 128] for j in range(4)]
        w0 = (KPAD + L * c) // 2
        kk = [unpack(ku[t, pl.ds(w0 - 2, 64, stride=4), :])[1]]
        for o in range(-1, 4):
            kk += unpack(ku[t, pl.ds(w0 + o, 64, stride=4), :])
        vv = []
        for o in range(4):
            vv += unpack(vu[t, pl.ds(L * c // 2 + o, 64, stride=4), :])
        kv = []
        for n in range(8):
            acc = kk[3 + n] * tp[0]
            for j in range(1, 4):
                acc = acc + kk[3 + n - j] * tp[j]
            kv.append(acc * vv[n])
        return [_pack(kv[r], kv[r + 4]) for r in range(R)]

    def conv_x(c, t, ties):
        xq = _fft4(fwd_dots(env.pop(("kv", c, t)), ties), -1)
        z = []
        for q in range(R):
            if c == 0:
                st_spec(X0S, t, q, xq[q])
                continue
            for a in range(c, NB):
                za = _cmul(xq[q], ld_spec(KP + a - c, t, q), ld_spec(ZP + a, t, q))
                if a == c:
                    z.append(za)
                else:
                    st_spec(ZP + a, t, q, za)
        if c:
            finish(c, t, z)

    def conv_inv(c, t, ties):
        for r in range(2 * R):
            tr = None
            if ties and r % R == 0:
                tr = {i - r: z for i, z in ties.items() if 0 <= i - r < 4}
            yb[t, pl.ds(L * c + r, 64, stride=2 * R), :] = jnp.dot(
                _bf(_tie(gib[r], tr)), _bf(cmb[c % 2, t, r]), preferred_element_type=F32)

    def run_rounds(spec_str):
        rounds = spec_str.split()
        slots = []
        plan = {}
        for n, rd in enumerate(rounds):
            if rd[0] == "X":
                pts = []
                if "@" in rd:
                    a, b = (int(v) for v in rd[4:].split(":"))
                    pts = [slots[len(slots) - a + (a - b) * (j + 1) // 8 - 1] for j in range(8)]
                plan.setdefault(pts[0][0] if pts else n, []).append((rd, pts))
            slots += [(n, i) for i in range(8 if rd[0] == "I" else 16)]
        ties = {}
        for n, rd in enumerate(rounds):
            for xr, pts in plan.get(n, []):
                c, t = int(xr[1]), int(xr[2])
                kv = env["kv", c, t] = conv_prep(c, t)
                for j, (pn, pi) in enumerate(pts):
                    z = zero_after(*[w[8 * j:8 * j + 8] for w in kv])
                    d = ties.setdefault(pn, {})
                    d[pi] = z if pi not in d else d[pi] | z
            {"K": conv_k, "X": conv_x, "I": conv_inv}[rd[0]](int(rd[1]), int(rd[2]), ties.get(n))

    def rows(r0, n, align=8):
        if isinstance(r0, int):
            return slice(r0, r0 + n)
        return pl.ds(pl.multiple_of(r0, align), n)

    def ld_y(r0, n):
        return jnp.concatenate([yb[t, rows(r0, n), :] for t in range(NT)], axis=-1)

    def prm(i, n=CH, c0=0, c1=D):
        return jnp.concatenate([par[i, :, c0:c1]] * (n // 8), axis=0)

    def a_pre12(r0, n):
        x = _bf(qb[r0 // 2:(r0 + n) // 2, :]).astype(F32)
        m1, r1 = _stats(x)
        x1 = x + ((x - m1) * r1 * prm(0, n) + prm(1, n)) * ld_y(r0, n)
        x1b[r0:r0 + n, :] = x1
        m2, r2 = _stats(x1)
        hb[r0:r0 + n, :] = (x1 - m2) * r2

    def a_pre3(r0, m):
        h = hb[r0:r0 + m, :] * prm(2, m) + prm(3, m)
        hb[r0:r0 + m, :] = h
        m3, r3 = _stats(h)
        return (h - m3) * r3

    def a_pre(r0, gates):
        out = []
        for j, g in enumerate(gates):
            r = r0 + CH * j
            z = zero_after(g)
            qv = qb[rows(r0 // 2 + CH // 2 * j, CH // 2), :] | jnp.concatenate([z] * NT, axis=1)
            x = _bf(qv).astype(F32)
            m1, r1 = _stats(x)
            x1 = x + ((x - m1) * r1 * prm(0) + prm(1)) * ld_y(r, CH)
            x1b[rows(r, CH), :] = x1
            m2, r2 = _stats(x1)
            h = (x1 - m2) * r2 * prm(2) + prm(3)
            hb[rows(r, CH), :] = h
            m3, r3 = _stats(h)
            out.append((h - m3) * r3)
        return jnp.concatenate(out, axis=0)

    def halves(n, split):
        m = n // split if split else n
        return [(o, m) for o in range(0, n, m)]

    def mm1(r0, n, n3, split_last=0, ties=None, tiles=range(NT)):
        for t in tiles:
            w = _tie(w1b[:, 128 * t:128 * t + 128], ties.get(t) if ties else None)
            for o, m in halves(n, split_last if t == tiles[-1] else 0):
                hp = jnp.dot(n3[o:o + m].astype(BF16), _bf(w), preferred_element_type=F32)
                hpb[t, rows(HPAD + r0 + o, m), :] = _gelu(hp)

    def g_prep(r0):
        lane = jax.lax.broadcasted_iota(I32, (TB, 128), 1)
        sh = [-1, 1, -2, 2]

        def ldh(t, g):
            return hpb[t, pl.ds(HPAD + r0 + sh[g], TB), :]

        cols = [ldh(0, 0)]
        for t in range(1, 4):
            cols.append(jnp.where(lane < 32 * t, ldh(t, t - 1), ldh(t, t)))
        cols.append(ldh(4, 3))
        return jnp.concatenate(cols, axis=-1)

    def mm2(r0, g, split_last=0, side=None):
        for t in range(NT):
            if side and t in side:
                side[t]()
            c0, c1 = 128 * t, 128 * t + 128
            for o, m in halves(TB, split_last if t == NT - 1 else 0):
                hs = jnp.dot(g[o:o + m].astype(BF16), _bf(w2b[:, c0:c1]), preferred_element_type=F32)
                hb[rows(r0 + o, m), c0:c1] = hb[rows(r0 + o, m), c0:c1] + hs
        return hs[m - 8:m]

    def ln4(r0, n):
        x2 = hb[rows(r0, n), :]
        m4, r4 = _stats(x2)
        return (x2 - m4) * r4

    def mm3(n4, ties=None, split_at=None, side=None, tpos=12, nat=True):
        us = []
        env["g3"] = []
        for j in range(FF // 128):
            if side and j in side:
                side[j]()
            if j == tpos:
                ht = jax.lax.dot_general(_bf(w3b[FM // 2:FF // 2, :]), n4.astype(BF16), NT_DIMS,
                                         preferred_element_type=F32)
                ut = _gelu(ht).T
            w = w3b[64 * j:64 * j + 64, :]
            if ties and j in ties:
                w = _tie(w, {0: ties[j]})
            parts = []
            for o, m in halves(TB, 2 if j == split_at else 0):
                if j == 0 and nat:
                    h3 = jnp.dot(n4.astype(BF16), _bf(w3n[...]), preferred_element_type=F32)
                else:
                    h3 = jax.lax.dot_general(n4[o:o + m].astype(BF16), _bf(w), NT_DIMS,
                                             preferred_element_type=F32)
                parts.append(_gelu(h3))
                if m == TB:
                    env["g3"] += [h3[0:8], h3[128:136]]
            us.append(jnp.concatenate(parts, axis=0))
        return jnp.concatenate(us + [ut], axis=-1)

    def mm4(r0, u, t, final=True, ties=None, split=0, side=None):
        c0, c1 = 128 * t, 128 * t + 128
        w = _bf(_tie(w4b[:, c0:c1], ties))
        for o, m in halves(TB, split):
            if o and side:
                side()
            h2 = jnp.dot(u[o:o + m].astype(BF16), w, preferred_element_type=F32)
            s = hb[rows(r0 + o, m), c0:c1] + h2
            if final:
                ob[rows(r0 + o, m, 16), c0:c1] = (
                    x1b[rows(r0 + o, m), c0:c1] + prm(4, m, c0, c1) * s).astype(BF16)
            else:
                hb[rows(r0 + o, m), c0:c1] = s

    def ln4_store(r0, nch):
        zs = []
        m = TB // nch
        for j in range(nch):
            n4 = ln4(r0 + m * j, m)
            n4b[m * j:m * j + m, :] = n4
            zs.append(zero_after(n4))
        return zs

    def ln4_ticked(r0, g, nch, hops):
        z = zero_after(g)
        m = TB // nch
        for j in range(nch):
            zt = jnp.concatenate([jnp.concatenate([z] * NT, axis=1)] * (m // 8), axis=0)
            x2 = pltpu.bitcast(pltpu.bitcast(hb[rows(r0 + m * j, m), :], U32) | zt, F32)
            m4, r4 = _stats(x2)
            n4b[m * j:m * j + m, :] = (x2 - m4) * r4
            for _ in range(hops):
                z = pltpu.roll(z, 1, 1)

    def out_copy(r0, n, c0=0, c1=D):
        return pltpu.make_async_copy(ob.at[rows(r0, n, 16), c0:c1],
                                     o_hbm.at[0, rows(r0, n, 16), c0:c1], osem)

    def out_copy_old(r0, n):
        return pltpu.make_async_copy(ob.at[rows(r0, n, 16), :], o_hbm.at[0, rows(r0, n, 16), :], osem)

    wait("ra")
    env["taps"] = skb[...].astype(F32)
    env["dvec"] = sdb[...].astype(F32).reshape(1, D)
    cf = cb_[...].astype(F32)
    sc8 = jnp.broadcast_to(cf * jax.nn.sigmoid(cf), (8, D)).astype(BF16)
    run_rounds("X00")
    wait("r0")
    run_rounds("X01 K00 K10 K20 K30")
    for t in range(1, NT):
        wait(f"r{t}")
        run_rounds(f"I0{t - 1} X{(t + 1) // NT}{(t + 1) % NT} K0{t} K1{t} K2{t} K3{t}")
    wait("r5")
    run_rounds("I04 I10 X11 X12@16:3 I11 X13@20:3 I12 X14@20:3")
    wait("r6")
    run_rounds("I13 X20 I14 X21@20:3 I20 X22@20:3 I21 X23@20:3 I22 X24@20:3 I23")

    flag = kb.bitcast(I32)[0, 0:8, :][0, 0]
    for n in range(NPAD):
        pl.when(flag != 0)(lambda: make_tables(2 * NFFT * (n + 1) * flag))
    wait("wmA")
    mod = jnp.dot(sc8, wmb[:, 0:3 * D], preferred_element_type=F32)
    sa, ca, ga = [mod[:, D * i:D * (i + 1)] for i in range(3)]
    par[0] = (1.0 + ca) * ga
    par[1] = sa * ga
    run_rounds("I24")
    a_pre12(0, TB + AO)
    a_pre12(TB + AO, TB)
    wait("wmS")
    mod = jnp.dot(sc8, wmb[:, 3 * D:4 * D + 256], preferred_element_type=F32)
    par[3] = mod[:, 0:D]
    par[2, :, 0:256] = 1.0 + mod[:, D:D + 256]
    wait("wmB")
    par[2, :, 256:D] = 1.0 + jnp.dot(sc8, wmb[:, 4 * D + 256:5 * D], preferred_element_type=F32)
    n3p = a_pre3(0, 128)

    rr = lambda x: (lambda: run_rounds(x))
    ta, tb = range(W1A // 128), range(W1A // 128, NT)
    wait("w1")
    n3 = jnp.concatenate([n3p, a_pre3(128, QE - 128)], axis=0)
    for a, b in ((0, 128), (128, 256), (256, 400), (400, QE)):
        mm1(a, b - a, n3[a:b], tiles=ta)
    wait("w1b")
    mm1(0, TB + AO, n3[:TB + AO], tiles=tb)
    run_rounds("X30")
    mm1(TB + AO, TB, n3[TB + AO:], split_last=4, tiles=tb)
    wait("w2")
    mm2(0, g_prep(0), side={4: rr("X31")})
    n4 = ln4(0, TB)
    mm2(TB, g_prep(TB), split_last=2)
    wait("w3")
    zs = ln4_store(TB, 8)
    run_rounds("I30")

    def mid():
        wait("w4")
        w3n[...] = pltpu.bitcast(_bf(w3b[0:64, :]).T, U32)
        run_rounds("I31")

    u = mm3(n4, {3 + j: z for j, z in enumerate(zs)}, split_at=W3A // 128 - 1, nat=False,
            side={W3A // 128: mid})
    mm4(0, u, 0, final=False)
    run_rounds("X32")
    mm4(0, u, 1, final=False)
    run_rounds("X33")
    mm4(0, u, 2, final=False, split=4)
    run_rounds("I32")
    wait("rest")

    def gb_tiles(*ts):
        for t in ts:
            par[4, :, 128 * t:128 * t + 128] = jnp.dot(
                sc8, wmb[:, 5 * D + 128 * t:5 * D + 128 * t + 128], preferred_element_type=F32)

    run_rounds("I33")
    gb_tiles(3)
    mm4(0, u, 3, split=2, side=lambda: (gb_tiles(4), run_rounds("X34"), gb_tiles(0)))
    gb_tiles(1)
    mm4(0, u, 4, split=2, side=lambda: gb_tiles(2))
    ob[0:TB, 0:W4A] = (x1b[0:TB, 0:W4A] + prm(4, TB, 0, W4A) * hb[0:TB, 0:W4A]).astype(BF16)
    run_rounds("I34")
    out_copy(0, TB).start()
    wait("qnext")

    def body(i, carry):
        pl.when(i == 2)(lambda: wait("qlast"))
        r0 = i * TB
        u = mm3(n4b[...])
        n3 = a_pre(r0 + TB + AO, [env["g3"][j * 25 // 15] for j in range(TB // CH)])
        mm4(r0, u, 0)
        mm1(r0 + TB + AO, TB, n3)
        hpb[:, HPAD + S:HPAD + S + 8, :] = jnp.zeros((NT, 8, 128), F32)
        mm4(r0, u, 1)
        g = mm2(r0 + TB, g_prep(r0 + TB))
        ln4_ticked(r0 + TB, g, 16, 1)
        for t in range(2, NT):
            mm4(r0, u, t)
        out_copy(r0, TB).start()
        return carry

    jax.lax.fori_loop(1, NBLK - 1, body, 0)

    r0 = S - TB
    u = mm3(n4b[...])
    for t in range(NT):
        mm4(r0, u, t, split=2 if t == NT - 1 else 0)
        if t < NT - 1:
            out_copy(r0, TB, 128 * t, 128 * t + 128).start()
    out_copy(r0, TB // 2, D - 128, D).start()
    out_copy(r0 + TB // 2, TB // 2, D - 128, D).start()
    with jax.named_scope("W_out"):
        pltpu.make_async_copy(ob, o_hbm.at[0], osem).wait()


@jax.jit
def pallas_adaLN_cond__ssm_conv_h3__mixer_s_mlp__prompt_kernel(
    A_q, A_k, A_v, A_shift_k, A_ssm_k, A_ssm_D, B_x, B_w1, B_w2, B_w3, B_w4, c, w_mod,
):
    del B_x
    vm = pltpu.VMEM
    scratch = [
        vm(((S + AO) // 2, D), U32),
        vm((NT, KPAD + S, 128), BF16),
        vm((NT, S, 128), BF16),
        vm((4, D), BF16),
        vm((D // 2, S), U32),
        vm((D,), BF16),
        vm((D // 2, D), U32),
        vm((D // 2, D), U32),
        vm((FF // 2, D), U32),
        vm((FF // 2, D), U32),
        vm((1, D), BF16),
        vm((D, 6 * D), BF16),
        vm((R + 1, 128, 128), U32),
        vm((2 * R + 1, 32, 128), U32),
        vm((NT, S // 2, 128), U32),
        vm((8, NT, R, 256, 128), F32),
        vm((3, NT, 2 * R, 64, 128), U32),
        vm((NT, S + AO, 128), F32),
        vm((S + AO, D), F32),
        vm((S + AO, D), F32),
        vm((NT, HPAD + S + AO, 128), F32),
        vm((TB, D), F32),
        vm((5, 8, D), F32),
        vm((D // 2, 128), U32),
        vm((S, D), BF16),
        pltpu.SemaphoreType.DMA((19,)),
        pltpu.SemaphoreType.DMA(()),
    ]
    hbm = pl.BlockSpec(memory_space=pltpu.HBM)
    return pl.pallas_call(
        _kernel,
        out_shape=jax.ShapeDtypeStruct((1, S, D), BF16),
        in_specs=[hbm] * 12,
        out_specs=hbm,
        scratch_shapes=scratch,
        compiler_params=pltpu.CompilerParams(vmem_limit_bytes=110 * 2**20,
                                             disable_semaphore_checks=True,
                                             disable_bounds_checks=True),
        name="h3_mixer",
    )(A_q, A_k, A_v, A_shift_k.T, A_ssm_k, A_ssm_D, B_w1, B_w2, B_w3.T, B_w4, c, w_mod)
```

```python
import jax
import jax.numpy as jnp
import numpy as np
import jax.experimental.pallas as pl
import jax.experimental.pallas.tpu as pltpu

S, D, FF = 2048, 640, 1728
NT = D // 128
L = 512
NB = S // L
NFFT = 2 * L
R = 4
KPAD = 16
HPAD = 8
TB = 256
NBLK = S // TB
AO = 16
CH = 16
EPS = 1e-5
W1A, W3A, W4A = 256, 1536, 384
NPAD = 1
FM = FF // 128 * 128
F32 = jnp.float32
BF16 = jnp.bfloat16
U32 = jnp.uint32
I32 = jnp.int32
NT_DIMS = (((1,), (1,)), ((), ()))
KP, X0S, ZP = 0, 3, 3


def _cos_coefs(deg=6):
    u = (np.cos(np.pi * (np.arange(400) + 0.5) / 400) + 1.0) / 2.0
    c = np.polynomial.polynomial.polyfit(u, np.cos(np.pi * np.sqrt(u)), deg)
    return [np.float32(v) for v in c]


_COS = _cos_coefs()


def _cos_units(a, scale=1.0):
    x = (((a + 1024) & 2047) - 1024).astype(F32) * np.float32(1.0 / 1024.0)
    u = x * x
    acc = u * np.float32(_COS[-1] * scale) + np.float32(_COS[-2] * scale)
    for c in _COS[-3::-1]:
        acc = acc * u + np.float32(c * scale)
    return acc


def _freq2(chunk, s):
    e = 4 * (8 * (chunk >> 1) + s) + 1
    return jnp.where((chunk & 1) == 0, e, 256 - e)


def _gelu(x):
    c1 = np.float32(np.sqrt(2.0 / np.pi))
    c2 = np.float32(np.sqrt(2.0 / np.pi) * 0.044715)
    u = x * (c1 + c2 * (x * x))
    hx = 0.5 * x
    return hx + hx * jnp.tanh(u)


def _stats(x):
    m = jnp.sum(x, axis=-1, keepdims=True) * (1.0 / D)
    e2 = jnp.sum(x * x, axis=-1, keepdims=True) * (1.0 / D)
    v = jnp.maximum(e2 - m * m, 0.0)
    return m, jax.lax.rsqrt(v + EPS)


def _split(b):
    b = b.reshape(-1, 2, 8, 128)
    return b[:, 0], b[:, 1]


def _join(z):
    return jnp.stack(z, axis=1).reshape(-1, 128)


def _eo(v):
    v = v.reshape(-1, 2, 8, 128)
    return v[:, 0], v[:, 1]


def _uneo(e, o):
    return jnp.stack([e, o], axis=1).reshape(16, 8, 128)


def _fft4(b, sign):
    (r0, i0), (r1, i1), (r2, i2), (r3, i3) = b
    sr, si, dr, di = r0 + r2, i0 + i2, r0 - r2, i0 - i2
    tr, ti, er, ei = r1 + r3, i1 + i3, r1 - r3, i1 - i3
    x0 = (sr + tr, si + ti)
    x2 = (sr - tr, si - ti)
    xm = (dr + ei, di - er)
    xp = (dr - ei, di + er)
    return [x0, xm, x2, xp] if sign < 0 else [x0, xp, x2, xm]


def _cmul(a, b, acc=None):
    (ar, ai), (br, bi) = a, b
    if acc is None:
        return ar * br - ai * bi, ar * bi + ai * br
    return (acc[0] + ar * br) - ai * bi, (acc[1] + ar * bi) + ai * br


def _bf(x):
    return pltpu.bitcast(x, BF16)


def _words(x):
    return pltpu.bitcast(x.astype(BF16), U32)


def _tie(w, ties):
    if not ties:
        return w
    parts = []
    for i in range(w.shape[0] // 8):
        p = w[8 * i:8 * i + 8]
        if i in ties:
            z = ties[i]
            p = p | z if p.shape[1] == 128 else jnp.concatenate([p[:, :128] | z, p[:, 128:]], axis=1)
        parts.append(p)
    return jnp.concatenate(parts, axis=0)


def _kernel(q_hbm, k_hbm, v_hbm, sk_hbm, ssm_hbm, sd_hbm, w1_hbm, w2_hbm, w3_hbm,
            w4_hbm, c_hbm, wm_hbm, o_hbm,
            qb, kb, vb, skb, ssmb, sdb, w1b, w2b, w3b, w4b, cb_, wmb, fwb, gib,
            stb, spec, yb, x1b, hb, hpb, n4b, par, w3n, ob, sems, osem):
    groups = {}

    def add(name, src, dst):
        if name not in groups:
            groups[name] = (len(groups), [])
        idx, lst = groups[name]
        cp = pltpu.make_async_copy(src, dst, sems.at[idx])
        cp.start()
        lst.append(cp)

    def add_kv(name, c, tiles=range(NT)):
        for t in tiles:
            add(name, k_hbm.at[0, pl.ds(L * c, L), pl.ds(128 * t, 128)],
                kb.at[t, pl.ds(KPAD + L * c, L), :])
            add(name, v_hbm.at[0, pl.ds(L * c, L), pl.ds(128 * t, 128)],
                vb.at[t, pl.ds(L * c, L), :])

    def add_ssm(name, t):
        add(name, ssm_hbm.at[pl.ds(128 * t, 128), :], ssmb.bitcast(BF16).at[pl.ds(128 * t, 128), :])

    QE = 2 * TB + AO
    add_kv("ra", 0, [0])
    add("ra", sd_hbm, sdb)
    add("ra", sk_hbm, skb)
    add("ra", c_hbm, cb_)
    for t in range(NT):
        add_ssm(f"r{t}", t)
        add_kv(f"r{t}", (t + 1) // NT, [(t + 1) % NT])
    add_kv("r5", 1, range(1, NT))
    add_kv("r6", 2)
    add("wmA", q_hbm.at[0, pl.ds(0, QE), :], qb.bitcast(BF16).at[pl.ds(0, QE), :])
    add("wmA", wm_hbm.at[:, pl.ds(0, 3 * D)], wmb.at[:, pl.ds(0, 3 * D)])
    add("wmS", wm_hbm.at[:, pl.ds(3 * D, D + 256)], wmb.at[:, pl.ds(3 * D, D + 256)])
    add("wmB", wm_hbm.at[:, pl.ds(4 * D + 256, D - 256)], wmb.at[:, pl.ds(4 * D + 256, D - 256)])
    add("w1", w1_hbm.at[:, pl.ds(0, W1A)], w1b.bitcast(BF16).at[:, pl.ds(0, W1A)])
    add("w1b", w1_hbm.at[:, pl.ds(W1A, D - W1A)], w1b.bitcast(BF16).at[:, pl.ds(W1A, D - W1A)])
    add_kv("w1b", 3, [0])
    add("w2", w2_hbm, w2b.bitcast(BF16))
    add_kv("w2", 3, [1])
    add("w3", w3_hbm.at[pl.ds(0, W3A), :], w3b.bitcast(BF16).at[pl.ds(0, W3A), :])
    add("w4", w3_hbm.at[pl.ds(W3A, FF - W3A), :], w3b.bitcast(BF16).at[pl.ds(W3A, FF - W3A), :])
    add("w4", w4_hbm.at[:, pl.ds(0, W4A)], w4b.bitcast(BF16).at[:, pl.ds(0, W4A)])
    add_kv("w4", 3, [2, 3])
    add("rest", w4_hbm.at[:, pl.ds(W4A, D - W4A)], w4b.bitcast(BF16).at[:, pl.ds(W4A, D - W4A)])
    add_kv("rest", 3, [4])
    add("rest", wm_hbm.at[:, pl.ds(5 * D, D)], wmb.at[:, pl.ds(5 * D, D)])
    add("qnext", q_hbm.at[0, pl.ds(QE, TB), :], qb.bitcast(BF16).at[pl.ds(QE, TB), :])
    add("qlast", q_hbm.at[0, pl.ds(QE + TB, S - QE - TB), :],
        qb.bitcast(BF16).at[pl.ds(QE + TB, S - QE - TB), :])

    def wait(name):
        with jax.named_scope("W_" + name):
            for cp in groups[name][1]:
                cp.wait()

    kb[:, 0:KPAD, :] = jnp.zeros((NT, KPAD, 128), BF16)
    hpb[:, 0:HPAD, :] = jnp.zeros((NT, HPAD, 128), F32)
    yb[:, S:S + AO, :] = jnp.zeros((NT, AO, 128), F32)
    qb[S // 2:(S + AO) // 2, :] = jnp.zeros((AO // 2, D), U32)

    spec[7, 0, 0, pl.ds(0, 8, stride=2), :] = jnp.zeros((8, 128), F32)
    fwb[R, pl.ds(0, 8, stride=2), :] = jnp.zeros((8, 128), U32)
    gib[2 * R, pl.ds(0, 8, stride=2), :] = jnp.zeros((8, 128), U32)

    def make_tables(off):
        row = jax.lax.broadcasted_iota(I32, (256, 128), 0)
        col = jax.lax.broadcasted_iota(I32, (256, 128), 1)
        f2 = _freq2(row >> 4, row & 7)
        ph = 512 * ((row >> 3) & 1) + off
        m = (col & ~15) + 2 * (col & 7) + ((col >> 3) & 1)
        for r in range(R):
            fwb[r] = _words(_cos_units((4 * m + r) * f2 + ph))
        row = jax.lax.broadcasted_iota(I32, (64, 128), 0)
        col = jax.lax.broadcasted_iota(I32, (64, 128), 1)
        f2 = 4 * (8 * (col >> 4) + (col & 7)) + 1
        ph = 512 * ((col >> 3) & 1) + off
        for r in range(2 * R):
            gib[r] = _words(_cos_units((8 * row + r) * f2 + ph, 2.0 / NFFT))

    make_tables(0)

    env = {}

    def zero_after(*vals):
        acc = None
        for v in vals:
            v = pltpu.bitcast(v, U32)
            for i in range(0, v.shape[0], 8):
                for j in range(0, v.shape[1], 128):
                    p = v[i:i + 8, j:j + 128]
                    acc = p if acc is None else acc | p
        return acc & kb.bitcast(U32)[0, 0:8, :]

    def ld_spec(slot, t, q):
        return _split(spec[slot, t, q])

    def st_spec(slot, t, q, z):
        spec[slot, t, q] = _join(z)

    def fwd_dots(rhs, ties):
        return [_split(jnp.dot(_bf(_tie(fwb[r], ties if r == 0 else None)), rhs[r],
                               preferred_element_type=F32)) for r in range(R)]

    def conv_k(c, t, ties):
        w0 = L * c // 2
        stb[t, w0:w0 + L // 2, :] = pltpu.bitcast(
            _bf(ssmb[64 * t:64 * t + 64, L * c:L * c + L]).T, U32)
        rhs = []
        for h in range(2):
            lo = stb[t, pl.ds(w0 + h, 64, stride=4), :]
            hi = stb[t, pl.ds(w0 + h + 2, 64, stride=4), :]
            for e, o in zip(unpack(lo), unpack(hi)):
                rhs.append(_join((e.reshape(8, 8, 128), o.reshape(8, 8, 128))).astype(BF16))
        b = fwd_dots(rhs, ties)
        if c == 0:
            b[0] = (b[0][0] + env["dvec"][:, 128 * t:128 * t + 128][None], b[0][1])
        kq = _fft4(b, -1)
        z = []
        for q in range(R):
            kp = kq[q]
            if c >= 2:
                p = ld_spec(KP + c - 2, t, q)
                kp = (kp[0] + p[0], kp[1] + p[1])
            if c >= 1:
                p = ld_spec(KP + c - 1, t, q)
                if c == 3:
                    p0 = ld_spec(KP, t, q)
                    p = (p[0] - p0[0], p[1] - p0[1])
                (ree, reo), (ime, imo), (pre, pro), (pie, pio) = (_eo(v) for v in kp + p)
                kp = (_uneo(ree - pie, reo + pio), _uneo(ime + pre, imo - pro))
            if c < 3:
                st_spec(KP + c, t, q, kp)
            zc = _cmul(kp, ld_spec(X0S, t, q))
            if c == 0:
                z.append(zc)
            else:
                st_spec(ZP + c, t, q, zc)
        if c == 0:
            finish(0, t, z)

    def finish(c, t, z):
        hs = np.float32(np.sqrt(0.5))
        cr = _fft4(z, +1)
        for r in range(R):
            (ar, br), (ai, bi) = _eo(cr[r][0]), _eo(cr[r][1])
            if r % 2:
                br, bi = (br - bi) * hs, (br + bi) * hs
            if r < 2:
                p, m = (ar + br, ai - bi), (ar - br, ai + bi)
            else:
                p, m = (ar - bi, ai - br), (ar + bi, ai + br)
            env["cm", c, t, r] = _join(p).astype(BF16)
            env["cm", c, t, r + R] = _join(m).astype(BF16)

    def unpack(u):
        return (pltpu.bitcast(u << 16, F32),
                pltpu.bitcast(u & jnp.uint32(0xFFFF0000), F32))

    def conv_prep(c, t):
        taps = env["taps"]
        ku = kb.bitcast(U32)
        vu = vb.bitcast(U32)
        tp = [taps[j:j + 1, 128 * t:128 * t + 128] for j in range(4)]
        w0 = (KPAD + L * c) // 2
        kk = [unpack(ku[t, pl.ds(w0 - 2, 64, stride=4), :])[1]]
        for o in range(-1, 4):
            kk += unpack(ku[t, pl.ds(w0 + o, 64, stride=4), :])
        vv = []
        for o in range(4):
            vv += unpack(vu[t, pl.ds(L * c // 2 + o, 64, stride=4), :])
        kv = []
        for n in range(8):
            acc = kk[3 + n] * tp[0]
            for j in range(1, 4):
                acc = acc + kk[3 + n - j] * tp[j]
            kv.append(acc * vv[n])
        return [_join((kv[r].reshape(8, 8, 128), kv[r + 4].reshape(8, 8, 128))) for r in range(R)]

    def conv_x(c, t, ties):
        xq = _fft4(fwd_dots([v.astype(BF16) for v in env.pop(("kv", c, t))], ties), -1)
        z = []
        for q in range(R):
            if c == 0:
                st_spec(X0S, t, q, xq[q])
                continue
            for a in range(c, NB):
                za = _cmul(xq[q], ld_spec(KP + a - c, t, q), ld_spec(ZP + a, t, q))
                if a == c:
                    z.append(za)
                else:
                    st_spec(ZP + a, t, q, za)
        if c:
            finish(c, t, z)

    def conv_inv(c, t, ties):
        for r in range(2 * R):
            tr = None
            if ties and r % R == 0:
                tr = {i - r: z for i, z in ties.items() if 0 <= i - r < 4}
            yb[t, pl.ds(L * c + r, 64, stride=2 * R), :] = jnp.dot(
                _bf(_tie(gib[r], tr)), env.pop(("cm", c, t, r)), preferred_element_type=F32)

    def run_rounds(spec_str):
        rounds = spec_str.split()
        slots = []
        plan = {}
        for n, rd in enumerate(rounds):
            if rd[0] == "X":
                pts = []
                if "@" in rd:
                    a, b = (int(v) for v in rd[4:].split(":"))
                    pts = [slots[len(slots) - a + (a - b) * (j + 1) // 8 - 1] for j in range(8)]
                plan.setdefault(pts[0][0] if pts else n, []).append((rd, pts))
            slots += [(n, i) for i in range(8 if rd[0] == "I" else 16)]
        ties = {}
        for n, rd in enumerate(rounds):
            for xr, pts in plan.get(n, []):
                c, t = int(xr[1]), int(xr[2])
                kv = env["kv", c, t] = conv_prep(c, t)
                for j, (pn, pi) in enumerate(pts):
                    z = zero_after(*[w[16 * j:16 * j + 16] for w in kv])
                    d = ties.setdefault(pn, {})
                    d[pi] = z if pi not in d else d[pi] | z
            {"K": conv_k, "X": conv_x, "I": conv_inv}[rd[0]](int(rd[1]), int(rd[2]), ties.get(n))

    def rows(r0, n, align=8):
        if isinstance(r0, int):
            return slice(r0, r0 + n)
        return pl.ds(pl.multiple_of(r0, align), n)

    def ld_y(r0, n):
        return jnp.concatenate([yb[t, rows(r0, n), :] for t in range(NT)], axis=-1)

    def prm(i, n=CH, c0=0, c1=D):
        return jnp.concatenate([par[i, :, c0:c1]] * (n // 8), axis=0)

    def a_pre12(r0, n):
        x = _bf(qb[r0 // 2:(r0 + n) // 2, :]).astype(F32)
        m1, r1 = _stats(x)
        x1 = x + ((x - m1) * r1 * prm(0, n) + prm(1, n)) * ld_y(r0, n)
        x1b[r0:r0 + n, :] = x1
        m2, r2 = _stats(x1)
        hb[r0:r0 + n, :] = (x1 - m2) * r2

    def a_pre3(r0, m):
        h = hb[r0:r0 + m, :] * prm(2, m) + prm(3, m)
        hb[r0:r0 + m, :] = h
        m3, r3 = _stats(h)
        return (h - m3) * r3

    def a_pre(r0, gates):
        out = []
        for j, g in enumerate(gates):
            r = r0 + CH * j
            z = zero_after(g)
            qv = qb[rows(r0 // 2 + CH // 2 * j, CH // 2), :] | jnp.concatenate([z] * NT, axis=1)
            x = _bf(qv).astype(F32)
            m1, r1 = _stats(x)
            x1 = x + ((x - m1) * r1 * prm(0) + prm(1)) * ld_y(r, CH)
            x1b[rows(r, CH), :] = x1
            m2, r2 = _stats(x1)
            h = (x1 - m2) * r2 * prm(2) + prm(3)
            hb[rows(r, CH), :] = h
            m3, r3 = _stats(h)
            out.append((h - m3) * r3)
        return jnp.concatenate(out, axis=0)

    def halves(n, split):
        m = n // split if split else n
        return [(o, m) for o in range(0, n, m)]

    def mm1(r0, n, n3, split_last=0, ties=None, tiles=range(NT)):
        for t in tiles:
            w = _tie(w1b[:, 128 * t:128 * t + 128], ties.get(t) if ties else None)
            for o, m in halves(n, split_last if t == tiles[-1] else 0):
                hp = jnp.dot(n3[o:o + m].astype(BF16), _bf(w), preferred_element_type=F32)
                hpb[t, rows(HPAD + r0 + o, m), :] = _gelu(hp)

    def g_prep(r0):
        lane = jax.lax.broadcasted_iota(I32, (TB, 128), 1)
        sh = [-1, 1, -2, 2]

        def ldh(t, g):
            return hpb[t, pl.ds(HPAD + r0 + sh[g], TB), :]

        cols = [ldh(0, 0)]
        for t in range(1, 4):
            cols.append(jnp.where(lane < 32 * t, ldh(t, t - 1), ldh(t, t)))
        cols.append(ldh(4, 3))
        return jnp.concatenate(cols, axis=-1)

    def mm2(r0, g, split_last=0, side=None):
        for t in range(NT):
            if side and t in side:
                side[t]()
            c0, c1 = 128 * t, 128 * t + 128
            for o, m in halves(TB, split_last if t == NT - 1 else 0):
                hs = jnp.dot(g[o:o + m].astype(BF16), _bf(w2b[:, c0:c1]), preferred_element_type=F32)
                hb[rows(r0 + o, m), c0:c1] = hb[rows(r0 + o, m), c0:c1] + hs
        return hs[m - 8:m]

    def ln4(r0, n):
        x2 = hb[rows(r0, n), :]
        m4, r4 = _stats(x2)
        return (x2 - m4) * r4

    def mm3(n4, ties=None, split_at=None, side=None, tpos=12, nat=True):
        us = []
        env["g3"] = []
        for j in range(FF // 128):
            if side and j in side:
                side[j]()
            if j == tpos:
                ht = jax.lax.dot_general(_bf(w3b[FM // 2:FF // 2, :]), n4.astype(BF16), NT_DIMS,
                                         preferred_element_type=F32)
                ut = _gelu(ht).T
            w = w3b[64 * j:64 * j + 64, :]
            if ties and j in ties:
                w = _tie(w, {0: ties[j]})
            parts = []
            for o, m in halves(TB, 2 if j == split_at else 0):
                if j == 0 and nat:
                    h3 = jnp.dot(n4.astype(BF16), _bf(w3n[...]), preferred_element_type=F32)
                else:
                    h3 = jax.lax.dot_general(n4[o:o + m].astype(BF16), _bf(w), NT_DIMS,
                                             preferred_element_type=F32)
                parts.append(_gelu(h3))
                if m == TB:
                    env["g3"] += [h3[0:8], h3[128:136]]
            us.append(jnp.concatenate(parts, axis=0))
        return jnp.concatenate(us + [ut], axis=-1)

    def mm4(r0, u, t, final=True, ties=None, split=0, side=None):
        c0, c1 = 128 * t, 128 * t + 128
        w = _bf(_tie(w4b[:, c0:c1], ties))
        for o, m in halves(TB, split):
            if o and side:
                side()
            h2 = jnp.dot(u[o:o + m].astype(BF16), w, preferred_element_type=F32)
            s = hb[rows(r0 + o, m), c0:c1] + h2
            if final:
                ob[rows(r0 + o, m, 16), c0:c1] = (
                    x1b[rows(r0 + o, m), c0:c1] + prm(4, m, c0, c1) * s).astype(BF16)
            else:
                hb[rows(r0 + o, m), c0:c1] = s

    def ln4_store(r0, nch):
        zs = []
        m = TB // nch
        for j in range(nch):
            n4 = ln4(r0 + m * j, m)
            n4b[m * j:m * j + m, :] = n4
            zs.append(zero_after(n4))
        return zs

    def ln4_ticked(r0, g, nch, hops):
        z = zero_after(g)
        m = TB // nch
        for j in range(nch):
            zt = jnp.concatenate([jnp.concatenate([z] * NT, axis=1)] * (m // 8), axis=0)
            x2 = pltpu.bitcast(pltpu.bitcast(hb[rows(r0 + m * j, m), :], U32) | zt, F32)
            m4, r4 = _stats(x2)
            n4b[m * j:m * j + m, :] = (x2 - m4) * r4
            for _ in range(hops):
                z = pltpu.roll(z, 1, 1)

    def out_copy(r0, n, c0=0, c1=D):
        return pltpu.make_async_copy(ob.at[rows(r0, n, 16), c0:c1],
                                     o_hbm.at[0, rows(r0, n, 16), c0:c1], osem)

    def out_copy_old(r0, n):
        return pltpu.make_async_copy(ob.at[rows(r0, n, 16), :], o_hbm.at[0, rows(r0, n, 16), :], osem)

    wait("ra")
    env["taps"] = skb[...].astype(F32)
    env["dvec"] = sdb[...].astype(F32).reshape(1, D)
    cf = cb_[...].astype(F32)
    sc8 = jnp.broadcast_to(cf * jax.nn.sigmoid(cf), (8, D)).astype(BF16)
    run_rounds("X00")
    wait("r0")
    run_rounds("X01 K00 K10 K20 K30")
    for t in range(1, NT):
        wait(f"r{t}")
        run_rounds(f"I0{t - 1} X{(t + 1) // NT}{(t + 1) % NT} K0{t} K1{t} K2{t} K3{t}")
    wait("r5")
    run_rounds("I04 I10 X11 X12@16:3 I11 X13@20:3 I12 X14@20:3")
    wait("r6")
    run_rounds("I13 X20 I14 X21@20:3 I20 X22@20:3 I21 X23@20:3 I22 X24@20:3 I23")

    flag = kb.bitcast(I32)[0, 0:8, :][0, 0]
    for n in range(NPAD):
        pl.when(flag != 0)(lambda: make_tables(2 * NFFT * (n + 1) * flag))
    wait("wmA")
    mod = jnp.dot(sc8, wmb[:, 0:3 * D], preferred_element_type=F32)
    sa, ca, ga = [mod[:, D * i:D * (i + 1)] for i in range(3)]
    par[0] = (1.0 + ca) * ga
    par[1] = sa * ga
    run_rounds("I24")
    a_pre12(0, TB + AO)
    a_pre12(TB + AO, TB)
    wait("wmS")
    mod = jnp.dot(sc8, wmb[:, 3 * D:4 * D + 256], preferred_element_type=F32)
    par[3] = mod[:, 0:D]
    par[2, :, 0:256] = 1.0 + mod[:, D:D + 256]
    wait("wmB")
    par[2, :, 256:D] = 1.0 + jnp.dot(sc8, wmb[:, 4 * D + 256:5 * D], preferred_element_type=F32)
    n3p = a_pre3(0, 128)

    rr = lambda x: (lambda: run_rounds(x))
    ta, tb = range(W1A // 128), range(W1A // 128, NT)
    wait("w1")
    n3 = jnp.concatenate([n3p, a_pre3(128, QE - 128)], axis=0)
    for a, b in ((0, 128), (128, 256), (256, 400), (400, QE)):
        mm1(a, b - a, n3[a:b], tiles=ta)
    wait("w1b")
    mm1(0, TB + AO, n3[:TB + AO], tiles=tb)
    run_rounds("X30")
    mm1(TB + AO, TB, n3[TB + AO:], split_last=4, tiles=tb)
    wait("w2")
    mm2(0, g_prep(0), side={4: rr("X31")})
    n4 = ln4(0, TB)
    mm2(TB, g_prep(TB), split_last=2)
    wait("w3")
    zs = ln4_store(TB, 8)
    run_rounds("I30")

    def mid():
        wait("w4")
        w3n[...] = pltpu.bitcast(_bf(w3b[0:64, :]).T, U32)
        run_rounds("I31")

    u = mm3(n4, {3 + j: z for j, z in enumerate(zs)}, split_at=W3A // 128 - 1, nat=False,
            side={W3A // 128: mid})
    mm4(0, u, 0, final=False)
    run_rounds("X32")
    mm4(0, u, 1, final=False)
    run_rounds("X33")
    mm4(0, u, 2, final=False, split=4)
    run_rounds("I32")
    wait("rest")

    def gb_tiles(*ts):
        for t in ts:
            par[4, :, 128 * t:128 * t + 128] = jnp.dot(
                sc8, wmb[:, 5 * D + 128 * t:5 * D + 128 * t + 128], preferred_element_type=F32)

    run_rounds("I33")
    gb_tiles(3)
    mm4(0, u, 3, split=2, side=lambda: (gb_tiles(4), run_rounds("X34"), gb_tiles(0)))
    gb_tiles(1)
    mm4(0, u, 4, split=2, side=lambda: gb_tiles(2))
    ob[0:TB, 0:W4A] = (x1b[0:TB, 0:W4A] + prm(4, TB, 0, W4A) * hb[0:TB, 0:W4A]).astype(BF16)
    run_rounds("I34")
    out_copy(0, TB).start()
    wait("qnext")

    def body(i, carry):
        pl.when(i == 2)(lambda: wait("qlast"))
        r0 = i * TB
        u = mm3(n4b[...])
        n3 = a_pre(r0 + TB + AO, [env["g3"][j * 25 // 15] for j in range(TB // CH)])
        mm4(r0, u, 0)
        mm1(r0 + TB + AO, TB, n3)
        hpb[:, HPAD + S:HPAD + S + 8, :] = jnp.zeros((NT, 8, 128), F32)
        mm4(r0, u, 1)
        g = mm2(r0 + TB, g_prep(r0 + TB))
        ln4_ticked(r0 + TB, g, 16, 1)
        for t in range(2, NT):
            mm4(r0, u, t)
        out_copy(r0, TB).start()
        return carry

    jax.lax.fori_loop(1, NBLK - 1, body, 0)

    r0 = S - TB
    u = mm3(n4b[...])
    for t in range(NT):
        mm4(r0, u, t, split=2 if t == NT - 1 else 0)
        if t < NT - 1:
            out_copy(r0, TB, 128 * t, 128 * t + 128).start()
    out_copy(r0, TB // 2, D - 128, D).start()
    out_copy(r0 + TB // 2, TB // 2, D - 128, D).start()
    with jax.named_scope("W_out"):
        pltpu.make_async_copy(ob, o_hbm.at[0], osem).wait()


@jax.jit
def pallas_adaLN_cond__ssm_conv_h3__mixer_s_mlp__prompt_kernel(
    A_q, A_k, A_v, A_shift_k, A_ssm_k, A_ssm_D, B_x, B_w1, B_w2, B_w3, B_w4, c, w_mod,
):
    del B_x
    vm = pltpu.VMEM
    scratch = [
        vm(((S + AO) // 2, D), U32),
        vm((NT, KPAD + S, 128), BF16),
        vm((NT, S, 128), BF16),
        vm((4, D), BF16),
        vm((D // 2, S), U32),
        vm((D,), BF16),
        vm((D // 2, D), U32),
        vm((D // 2, D), U32),
        vm((FF // 2, D), U32),
        vm((FF // 2, D), U32),
        vm((1, D), BF16),
        vm((D, 6 * D), BF16),
        vm((R + 1, 128, 128), U32),
        vm((2 * R + 1, 32, 128), U32),
        vm((NT, S // 2, 128), U32),
        vm((8, NT, R, 256, 128), F32),
        vm((NT, S + AO, 128), F32),
        vm((S + AO, D), F32),
        vm((S + AO, D), F32),
        vm((NT, HPAD + S + AO, 128), F32),
        vm((TB, D), F32),
        vm((5, 8, D), F32),
        vm((D // 2, 128), U32),
        vm((S, D), BF16),
        pltpu.SemaphoreType.DMA((19,)),
        pltpu.SemaphoreType.DMA(()),
    ]
    hbm = pl.BlockSpec(memory_space=pltpu.HBM)
    return pl.pallas_call(
        _kernel,
        out_shape=jax.ShapeDtypeStruct((1, S, D), BF16),
        in_specs=[hbm] * 12,
        out_specs=hbm,
        scratch_shapes=scratch,
        compiler_params=pltpu.CompilerParams(vmem_limit_bytes=110 * 2**20,
                                             disable_semaphore_checks=True,
                                             disable_bounds_checks=True),
        name="h3_mixer",
    )(A_q, A_k, A_v, A_shift_k.T, A_ssm_k, A_ssm_D, B_w1, B_w2, B_w3.T, B_w4, c, w_mod)
```

```python
import jax
import jax.numpy as jnp
import numpy as np
import jax.experimental.pallas as pl
import jax.experimental.pallas.tpu as pltpu

S, D, FF = 2048, 640, 1728
NT = D // 128
L = 512
NB = S // L
NFFT = 2 * L
R = 4
KPAD = 16
HPAD = 8
TB = 256
NBLK = S // TB
AO = 16
CH = 16
EPS = 1e-5
W1A, W3A, W4A = 256, 1536, 384
NPAD = 1
FM = FF // 128 * 128
F32 = jnp.float32
BF16 = jnp.bfloat16
U32 = jnp.uint32
I32 = jnp.int32
NT_DIMS = (((1,), (1,)), ((), ()))
KP, X0S, ZP = 0, 3, 3


def _cos_coefs(deg=6):
    u = (np.cos(np.pi * (np.arange(400) + 0.5) / 400) + 1.0) / 2.0
    c = np.polynomial.polynomial.polyfit(u, np.cos(np.pi * np.sqrt(u)), deg)
    return [np.float32(v) for v in c]


_COS = _cos_coefs()


def _cos_units(a, scale=1.0):
    x = (((a + 1024) & 2047) - 1024).astype(F32) * np.float32(1.0 / 1024.0)
    u = x * x
    acc = u * np.float32(_COS[-1] * scale) + np.float32(_COS[-2] * scale)
    for c in _COS[-3::-1]:
        acc = acc * u + np.float32(c * scale)
    return acc


def _freq2(chunk, s):
    e = 4 * (8 * (chunk >> 1) + s) + 1
    return jnp.where((chunk & 1) == 0, e, 256 - e)


def _gelu(x):
    c1 = np.float32(np.sqrt(2.0 / np.pi))
    c2 = np.float32(np.sqrt(2.0 / np.pi) * 0.044715)
    u = x * (c1 + c2 * (x * x))
    hx = 0.5 * x
    return hx + hx * jnp.tanh(u)


def _stats(x):
    m = jnp.sum(x, axis=-1, keepdims=True) * (1.0 / D)
    e2 = jnp.sum(x * x, axis=-1, keepdims=True) * (1.0 / D)
    v = jnp.maximum(e2 - m * m, 0.0)
    return m, jax.lax.rsqrt(v + EPS)


def _split(b):
    b = b.reshape(-1, 2, 8, 128)
    return b[:, 0], b[:, 1]


def _join(z):
    return jnp.stack(z, axis=1).reshape(-1, 128)


def _eo(v):
    v = v.reshape(-1, 2, 8, 128)
    return v[:, 0], v[:, 1]


def _uneo(e, o):
    return jnp.stack([e, o], axis=1).reshape(16, 8, 128)


def _fft4(b, sign):
    (r0, i0), (r1, i1), (r2, i2), (r3, i3) = b
    sr, si, dr, di = r0 + r2, i0 + i2, r0 - r2, i0 - i2
    tr, ti, er, ei = r1 + r3, i1 + i3, r1 - r3, i1 - i3
    x0 = (sr + tr, si + ti)
    x2 = (sr - tr, si - ti)
    xm = (dr + ei, di - er)
    xp = (dr - ei, di + er)
    return [x0, xm, x2, xp] if sign < 0 else [x0, xp, x2, xm]


def _cmul(a, b, acc=None):
    (ar, ai), (br, bi) = a, b
    if acc is None:
        return ar * br - ai * bi, ar * bi + ai * br
    return (acc[0] + ar * br) - ai * bi, (acc[1] + ar * bi) + ai * br


def _bf(x):
    return pltpu.bitcast(x, BF16)


def _words(x):
    return pltpu.bitcast(x.astype(BF16), U32)


def _tie(w, ties):
    if not ties:
        return w
    parts = []
    for i in range(w.shape[0] // 8):
        p = w[8 * i:8 * i + 8]
        if i in ties:
            z = ties[i]
            p = p | z if p.shape[1] == 128 else jnp.concatenate([p[:, :128] | z, p[:, 128:]], axis=1)
        parts.append(p)
    return jnp.concatenate(parts, axis=0)


def _kernel(q_hbm, k_hbm, v_hbm, sk_hbm, ssm_hbm, sd_hbm, w1_hbm, w2_hbm, w3_hbm,
            w4_hbm, c_hbm, wm_hbm, o_hbm,
            qb, kb, vb, skb, ssmb, sdb, w1b, w2b, w3b, w4b, cb_, wmb, fwb, gib,
            stb, spec, yb, x1b, hb, eb, hpb, n4b, par, w3n, ob, sems, osem):
    groups = {}

    def add(name, src, dst):
        if name not in groups:
            groups[name] = (len(groups), [])
        idx, lst = groups[name]
        cp = pltpu.make_async_copy(src, dst, sems.at[idx])
        cp.start()
        lst.append(cp)

    def add_kv(name, c, tiles=range(NT)):
        for t in tiles:
            add(name, k_hbm.at[0, pl.ds(L * c, L), pl.ds(128 * t, 128)],
                kb.at[t, pl.ds(KPAD + L * c, L), :])
            add(name, v_hbm.at[0, pl.ds(L * c, L), pl.ds(128 * t, 128)],
                vb.at[t, pl.ds(L * c, L), :])

    def add_ssm(name, t):
        add(name, ssm_hbm.at[pl.ds(128 * t, 128), :], ssmb.bitcast(BF16).at[pl.ds(128 * t, 128), :])

    QE = 2 * TB + AO
    add_kv("ra", 0, [0])
    add("ra", sd_hbm, sdb)
    add("ra", sk_hbm, skb)
    add("ra", c_hbm, cb_)
    for t in range(NT):
        add_ssm(f"r{t}", t)
        add_kv(f"r{t}", (t + 1) // NT, [(t + 1) % NT])
    add_kv("r5", 1, range(1, NT))
    add_kv("r6", 2)
    add("wmA", q_hbm.at[0, pl.ds(0, QE), :], qb.bitcast(BF16).at[pl.ds(0, QE), :])
    add("wmA", wm_hbm.at[:, pl.ds(0, 3 * D)], wmb.at[:, pl.ds(0, 3 * D)])
    add("wmS", wm_hbm.at[:, pl.ds(3 * D, D + 256)], wmb.at[:, pl.ds(3 * D, D + 256)])
    add("wmB", wm_hbm.at[:, pl.ds(4 * D + 256, D - 256)], wmb.at[:, pl.ds(4 * D + 256, D - 256)])
    add("w1", w1_hbm.at[:, pl.ds(0, W1A)], w1b.bitcast(BF16).at[:, pl.ds(0, W1A)])
    add("w1b", w1_hbm.at[:, pl.ds(W1A, D - W1A)], w1b.bitcast(BF16).at[:, pl.ds(W1A, D - W1A)])
    add_kv("w1b", 3, [0])
    add("w2", w2_hbm, w2b.bitcast(BF16))
    add_kv("w2", 3, [1])
    add("w3", w3_hbm.at[pl.ds(0, W3A), :], w3b.bitcast(BF16).at[pl.ds(0, W3A), :])
    add("w4", w3_hbm.at[pl.ds(W3A, FF - W3A), :], w3b.bitcast(BF16).at[pl.ds(W3A, FF - W3A), :])
    add("w4", w4_hbm.at[:, pl.ds(0, W4A)], w4b.bitcast(BF16).at[:, pl.ds(0, W4A)])
    add_kv("w4", 3, [2, 3])
    add("rest", w4_hbm.at[:, pl.ds(W4A, D - W4A)], w4b.bitcast(BF16).at[:, pl.ds(W4A, D - W4A)])
    add_kv("rest", 3, [4])
    add("rest", wm_hbm.at[:, pl.ds(5 * D, D)], wmb.at[:, pl.ds(5 * D, D)])
    add("qnext", q_hbm.at[0, pl.ds(QE, TB), :], qb.bitcast(BF16).at[pl.ds(QE, TB), :])
    add("qlast", q_hbm.at[0, pl.ds(QE + TB, S - QE - TB), :],
        qb.bitcast(BF16).at[pl.ds(QE + TB, S - QE - TB), :])

    def wait(name):
        with jax.named_scope("W_" + name):
            for cp in groups[name][1]:
                cp.wait()

    kb[:, 0:KPAD, :] = jnp.zeros((NT, KPAD, 128), BF16)
    hpb[:, 0:HPAD, :] = jnp.zeros((NT, HPAD, 128), F32)
    yb[:, S:S + AO, :] = jnp.zeros((NT, AO, 128), F32)
    qb[S // 2:(S + AO) // 2, :] = jnp.zeros((AO // 2, D), U32)

    spec[7, 0, 0, pl.ds(0, 8, stride=2), :] = jnp.zeros((8, 128), F32)
    fwb[R, pl.ds(0, 8, stride=2), :] = jnp.zeros((8, 128), U32)
    gib[2 * R, pl.ds(0, 8, stride=2), :] = jnp.zeros((8, 128), U32)

    def make_tables(off):
        row = jax.lax.broadcasted_iota(I32, (256, 128), 0)
        col = jax.lax.broadcasted_iota(I32, (256, 128), 1)
        f2 = _freq2(row >> 4, row & 7)
        ph = 512 * ((row >> 3) & 1) + off
        m = (col & ~15) + 2 * (col & 7) + ((col >> 3) & 1)
        for r in range(R):
            fwb[r] = _words(_cos_units((4 * m + r) * f2 + ph))
        row = jax.lax.broadcasted_iota(I32, (64, 128), 0)
        col = jax.lax.broadcasted_iota(I32, (64, 128), 1)
        f2 = 4 * (8 * (col >> 4) + (col & 7)) + 1
        ph = 512 * ((col >> 3) & 1) + off
        for r in range(2 * R):
            gib[r] = _words(_cos_units((8 * row + r) * f2 + ph, 2.0 / NFFT))

    make_tables(0)

    env = {}

    def zero_after(*vals):
        acc = None
        for v in vals:
            v = pltpu.bitcast(v, U32)
            for i in range(0, v.shape[0], 8):
                for j in range(0, v.shape[1], 128):
                    p = v[i:i + 8, j:j + 128]
                    acc = p if acc is None else acc | p
        return acc & kb.bitcast(U32)[0, 0:8, :]

    def ld_spec(slot, t, q):
        return _split(spec[slot, t, q])

    def st_spec(slot, t, q, z):
        spec[slot, t, q] = _join(z)

    def fwd_dots(rhs, ties):
        return [_split(jnp.dot(_bf(_tie(fwb[r], ties if r == 0 else None)), rhs[r],
                               preferred_element_type=F32)) for r in range(R)]

    def conv_k(c, t, ties):
        w0 = L * c // 2
        stb[t, w0:w0 + L // 2, :] = pltpu.bitcast(
            _bf(ssmb[64 * t:64 * t + 64, L * c:L * c + L]).T, U32)
        rhs = []
        for h in range(2):
            lo = stb[t, pl.ds(w0 + h, 64, stride=4), :]
            hi = stb[t, pl.ds(w0 + h + 2, 64, stride=4), :]
            for e, o in zip(unpack(lo), unpack(hi)):
                rhs.append(_join((e.reshape(8, 8, 128), o.reshape(8, 8, 128))).astype(BF16))
        b = fwd_dots(rhs, ties)
        if c == 0:
            b[0] = (b[0][0] + env["dvec"][:, 128 * t:128 * t + 128][None], b[0][1])
        kq = _fft4(b, -1)
        z = []
        for q in range(R):
            kp = kq[q]
            if c >= 2:
                p = ld_spec(KP + c - 2, t, q)
                kp = (kp[0] + p[0], kp[1] + p[1])
            if c >= 1:
                p = ld_spec(KP + c - 1, t, q)
                if c == 3:
                    p0 = ld_spec(KP, t, q)
                    p = (p[0] - p0[0], p[1] - p0[1])
                (ree, reo), (ime, imo), (pre, pro), (pie, pio) = (_eo(v) for v in kp + p)
                kp = (_uneo(ree - pie, reo + pio), _uneo(ime + pre, imo - pro))
            if c < 3:
                st_spec(KP + c, t, q, kp)
            zc = _cmul(kp, ld_spec(X0S, t, q))
            if c == 0:
                z.append(zc)
            else:
                st_spec(ZP + c, t, q, zc)
        if c == 0:
            finish(0, t, z)

    def finish(c, t, z):
        hs = np.float32(np.sqrt(0.5))
        cr = _fft4(z, +1)
        for r in range(R):
            (ar, br), (ai, bi) = _eo(cr[r][0]), _eo(cr[r][1])
            if r % 2:
                br, bi = (br - bi) * hs, (br + bi) * hs
            if r < 2:
                p, m = (ar + br, ai - bi), (ar - br, ai + bi)
            else:
                p, m = (ar - bi, ai - br), (ar + bi, ai + br)
            env["cm", c, t, r] = _join(p).astype(BF16)
            env["cm", c, t, r + R] = _join(m).astype(BF16)

    def unpack(u):
        return (pltpu.bitcast(u << 16, F32),
                pltpu.bitcast(u & jnp.uint32(0xFFFF0000), F32))

    def conv_prep(c, t):
        taps = env["taps"]
        ku = kb.bitcast(U32)
        vu = vb.bitcast(U32)
        tp = [taps[j:j + 1, 128 * t:128 * t + 128] for j in range(4)]
        w0 = (KPAD + L * c) // 2
        kk = [unpack(ku[t, pl.ds(w0 - 2, 64, stride=4), :])[1]]
        for o in range(-1, 4):
            kk += unpack(ku[t, pl.ds(w0 + o, 64, stride=4), :])
        vv = []
        for o in range(4):
            vv += unpack(vu[t, pl.ds(L * c // 2 + o, 64, stride=4), :])
        kv = []
        for n in range(8):
            acc = kk[3 + n] * tp[0]
            for j in range(1, 4):
                acc = acc + kk[3 + n - j] * tp[j]
            kv.append(acc * vv[n])
        return [_join((kv[r].reshape(8, 8, 128), kv[r + 4].reshape(8, 8, 128))) for r in range(R)]

    def conv_x(c, t, ties):
        xq = _fft4(fwd_dots([v.astype(BF16) for v in env.pop(("kv", c, t))], ties), -1)
        z = []
        for q in range(R):
            if c == 0:
                st_spec(X0S, t, q, xq[q])
                continue
            for a in range(c, NB):
                za = _cmul(xq[q], ld_spec(KP + a - c, t, q), ld_spec(ZP + a, t, q))
                if a == c:
                    z.append(za)
                else:
                    st_spec(ZP + a, t, q, za)
        if c:
            finish(c, t, z)

    def conv_inv(c, t, ties):
        for r in range(2 * R):
            tr = None
            if ties and r % R == 0:
                tr = {i - r: z for i, z in ties.items() if 0 <= i - r < 4}
            yb[t, pl.ds(L * c + r, 64, stride=2 * R), :] = jnp.dot(
                _bf(_tie(gib[r], tr)), env.pop(("cm", c, t, r)), preferred_element_type=F32)

    def run_rounds(spec_str):
        rounds = spec_str.split()
        slots = []
        plan = {}
        for n, rd in enumerate(rounds):
            if rd[0] == "X":
                pts = []
                if "@" in rd:
                    a, b = (int(v) for v in rd[4:].split(":"))
                    pts = [slots[len(slots) - a + (a - b) * (j + 1) // 8 - 1] for j in range(8)]
                plan.setdefault(pts[0][0] if pts else n, []).append((rd, pts))
            slots += [(n, i) for i in range(8 if rd[0] == "I" else 16)]
        ties = {}
        for n, rd in enumerate(rounds):
            for xr, pts in plan.get(n, []):
                c, t = int(xr[1]), int(xr[2])
                kv = env["kv", c, t] = conv_prep(c, t)
                for j, (pn, pi) in enumerate(pts):
                    z = zero_after(*[w[16 * j:16 * j + 16] for w in kv])
                    d = ties.setdefault(pn, {})
                    d[pi] = z if pi not in d else d[pi] | z
            {"K": conv_k, "X": conv_x, "I": conv_inv}[rd[0]](int(rd[1]), int(rd[2]), ties.get(n))

    def rows(r0, n, align=8):
        if isinstance(r0, int):
            return slice(r0, r0 + n)
        return pl.ds(pl.multiple_of(r0, align), n)

    def ld_y(r0, n):
        return jnp.concatenate([yb[t, rows(r0, n), :] for t in range(NT)], axis=-1)

    def prm(i, n=CH, c0=0, c1=D):
        return jnp.concatenate([par[i, :, c0:c1]] * (n // 8), axis=0)

    def a_pre12(r0, n):
        x = _bf(qb[r0 // 2:(r0 + n) // 2, :]).astype(F32)
        m1, r1 = _stats(x)
        x1 = x + ((x - m1) * r1 * prm(0, n) + prm(1, n)) * ld_y(r0, n)
        x1b[r0:r0 + n, :] = x1
        m2, r2 = _stats(x1)
        hb[r0:r0 + n, :] = (x1 - m2) * r2

    def a_pre3(r0, m):
        h = hb[r0:r0 + m, :] * prm(2, m) + prm(3, m)
        hb[r0:r0 + m, :] = h
        m3, r3 = _stats(h)
        return (h - m3) * r3

    def halves(n, split):
        m = n // split if split else n
        return [(o, m) for o in range(0, n, m)]

    def mm1(r0, n, n3, split_last=0, ties=None, tiles=range(NT)):
        for t in tiles:
            w = _tie(w1b[:, 128 * t:128 * t + 128], ties.get(t) if ties else None)
            for o, m in halves(n, split_last if t == tiles[-1] else 0):
                hp = jnp.dot(n3[o:o + m].astype(BF16), _bf(w), preferred_element_type=F32)
                hpb[t, rows(HPAD + r0 + o, m), :] = _gelu(hp)

    def g_prep(r0):
        lane = jax.lax.broadcasted_iota(I32, (TB, 128), 1)
        sh = [-1, 1, -2, 2]

        def ldh(t, g):
            return hpb[t, pl.ds(HPAD + r0 + sh[g], TB), :]

        cols = [ldh(0, 0)]
        for t in range(1, 4):
            cols.append(jnp.where(lane < 32 * t, ldh(t, t - 1), ldh(t, t)))
        cols.append(ldh(4, 3))
        return jnp.concatenate(cols, axis=-1)

    def mm2(r0, g, split_last=0, side=None):
        for t in range(NT):
            if side and t in side:
                side[t]()
            c0, c1 = 128 * t, 128 * t + 128
            for o, m in halves(TB, split_last if t == NT - 1 else 0):
                hs = jnp.dot(g[o:o + m].astype(BF16), _bf(w2b[:, c0:c1]), preferred_element_type=F32)
                hb[rows(r0 + o, m), c0:c1] = hb[rows(r0 + o, m), c0:c1] + hs
        return hs[m - 8:m]

    def ln4(r0, n):
        x2 = hb[rows(r0, n), :]
        m4, r4 = _stats(x2)
        return (x2 - m4) * r4

    def mm3(n4, ties=None, split_at=None, side=None, tpos=12, nat=True):
        us = []
        env["g3"] = []
        for j in range(FF // 128):
            if side and j in side:
                side[j]()
            if j == tpos:
                ht = jax.lax.dot_general(_bf(w3b[FM // 2:FF // 2, :]), n4.astype(BF16), NT_DIMS,
                                         preferred_element_type=F32)
                ut = _gelu(ht).T
            w = w3b[64 * j:64 * j + 64, :]
            if ties and j in ties:
                w = _tie(w, {0: ties[j]})
            parts = []
            for o, m in halves(TB, 2 if j == split_at else 0):
                if j == 0 and nat:
                    h3 = jnp.dot(n4.astype(BF16), _bf(w3n[...]), preferred_element_type=F32)
                else:
                    h3 = jax.lax.dot_general(n4[o:o + m].astype(BF16), _bf(w), NT_DIMS,
                                             preferred_element_type=F32)
                parts.append(_gelu(h3))
                if m == TB:
                    env["g3"] += [h3[0:8], h3[128:136]]
            us.append(jnp.concatenate(parts, axis=0))
        return jnp.concatenate(us + [ut], axis=-1)

    def mm4(r0, u, t, final=True, ties=None, split=0, side=None):
        c0, c1 = 128 * t, 128 * t + 128
        w = _bf(_tie(w4b[:, c0:c1], ties))
        for o, m in halves(TB, split):
            if o and side:
                side()
            h2 = jnp.dot(u[o:o + m].astype(BF16), w, preferred_element_type=F32)
            s = hb[rows(r0 + o, m), c0:c1] + h2
            if final:
                ob[rows(r0 + o, m, 16), c0:c1] = (
                    x1b[rows(r0 + o, m), c0:c1] + prm(4, m, c0, c1) * s).astype(BF16)
            else:
                hb[rows(r0 + o, m), c0:c1] = s

    def ln4_store(r0, nch):
        zs = []
        m = TB // nch
        for j in range(nch):
            n4 = ln4(r0 + m * j, m)
            n4b[m * j:m * j + m, :] = n4
            zs.append(zero_after(n4))
        return zs

    def out_copy(r0, n, c0=0, c1=D):
        return pltpu.make_async_copy(ob.at[rows(r0, n, 16), c0:c1],
                                     o_hbm.at[0, rows(r0, n, 16), c0:c1], osem)

    wait("ra")
    env["taps"] = skb[...].astype(F32)
    env["dvec"] = sdb[...].astype(F32).reshape(1, D)
    cf = cb_[...].astype(F32)
    sc8 = jnp.broadcast_to(cf * jax.nn.sigmoid(cf), (8, D)).astype(BF16)
    run_rounds("X00")
    wait("r0")
    run_rounds("X01 K00 K10 K20 K30")
    for t in range(1, NT):
        wait(f"r{t}")
        run_rounds(f"I0{t - 1} X{(t + 1) // NT}{(t + 1) % NT} K0{t} K1{t} K2{t} K3{t}")
    wait("r5")
    run_rounds("I04 I10 X11 X12@16:3 I11 X13@20:3 I12 X14@20:3")
    wait("r6")
    run_rounds("I13 X20 I14 X21@20:3 I20 X22@20:3 I21 X23@20:3 I22 X24@20:3 I23")

    flag = kb.bitcast(I32)[0, 0:8, :][0, 0]
    for n in range(NPAD):
        pl.when(flag != 0)(lambda: make_tables(2 * NFFT * (n + 1) * flag))
    wait("wmA")
    mod = jnp.dot(sc8, wmb[:, 0:3 * D], preferred_element_type=F32)
    sa, ca, ga = [mod[:, D * i:D * (i + 1)] for i in range(3)]
    par[0] = (1.0 + ca) * ga
    par[1] = sa * ga
    run_rounds("I24")
    a_pre12(0, TB + AO)
    a_pre12(TB + AO, TB)
    wait("wmS")
    mod = jnp.dot(sc8, wmb[:, 3 * D:4 * D + 256], preferred_element_type=F32)
    par[3] = mod[:, 0:D]
    par[2, :, 0:256] = 1.0 + mod[:, D:D + 256]
    wait("wmB")
    par[2, :, 256:D] = 1.0 + jnp.dot(sc8, wmb[:, 4 * D + 256:5 * D], preferred_element_type=F32)
    n3p = a_pre3(0, 128)

    rr = lambda x: (lambda: run_rounds(x))
    ta, tb = range(W1A // 128), range(W1A // 128, NT)
    wait("w1")
    n3 = jnp.concatenate([n3p, a_pre3(128, QE - 128)], axis=0)
    for a, b in ((0, 128), (128, 256), (256, 400), (400, QE)):
        mm1(a, b - a, n3[a:b], tiles=ta)
    wait("w1b")
    mm1(0, TB + AO, n3[:TB + AO], tiles=tb)
    run_rounds("X30")
    mm1(TB + AO, TB, n3[TB + AO:], split_last=4, tiles=tb)
    wait("w2")
    mm2(0, g_prep(0), side={4: rr("X31")})
    n4 = ln4(0, TB)
    mm2(TB, g_prep(TB), split_last=2)
    wait("w3")
    zs = ln4_store(TB, 8)
    run_rounds("I30")

    def mid():
        wait("w4")
        w3n[...] = pltpu.bitcast(_bf(w3b[0:64, :]).T, U32)
        run_rounds("I31")

    u = mm3(n4, {3 + j: z for j, z in enumerate(zs)}, split_at=W3A // 128 - 1, nat=False,
            side={W3A // 128: mid})
    mm4(0, u, 0, final=False)
    run_rounds("X32")
    mm4(0, u, 1, final=False)
    run_rounds("X33")
    mm4(0, u, 2, final=False, split=4)
    run_rounds("I32")
    wait("rest")

    def gb_tiles(*ts):
        for t in ts:
            par[4, :, 128 * t:128 * t + 128] = jnp.dot(
                sc8, wmb[:, 5 * D + 128 * t:5 * D + 128 * t + 128], preferred_element_type=F32)

    run_rounds("I33")
    gb_tiles(3)
    mm4(0, u, 3, split=2, side=lambda: (gb_tiles(4), run_rounds("X34"), gb_tiles(0)))
    gb_tiles(1)
    mm4(0, u, 4, split=2, side=lambda: gb_tiles(2))
    ob[0:TB, 0:W4A] = (x1b[0:TB, 0:W4A] + prm(4, TB, 0, W4A) * hb[0:TB, 0:W4A]).astype(BF16)
    eb[TB:2 * TB, :] = x1b[TB:2 * TB, :] + prm(4, TB) * hb[TB:2 * TB, :]
    run_rounds("I34")
    out_copy(0, TB).start()
    wait("qnext")

    def gated(v, z):
        zt = jnp.concatenate([jnp.concatenate([z] * NT, axis=1)] * (v.shape[0] // 8), axis=0)
        return pltpu.bitcast(v, U32) | zt

    def mm4e(ev, ov, u, t, split=0):
        c0, c1 = 128 * t, 128 * t + 128
        for o, m in halves(TB, split):
            h2 = jnp.dot(u[o:o + m].astype(BF16), _bf(w4b[:, c0:c1]), preferred_element_type=F32)
            ov[o:o + m, c0:c1] = (ev[o:o + m, c0:c1] + prm(4, m, c0, c1) * h2).astype(BF16)

    def body(i, carry):
        pl.when(i == 2)(lambda: wait("qlast"))
        r0 = pl.multiple_of(i * TB, TB)
        ev = eb.at[pl.ds(r0, 2 * TB), :]
        ov = ob.at[pl.ds(r0, TB), :]
        u = mm3(n4b[...])
        hpb[:, TB:TB + HPAD + AO, :] = hpb[:, 2 * TB:2 * TB + HPAD + AO, :]
        x1s, hs, n3 = [x1b[2 * TB:QE, :]], [hb[2 * TB:QE, :]], []
        for j in range(TB // CH):
            r = r0 + TB + AO + CH * j
            z = zero_after(env["g3"][j * 25 // 15])
            x = _bf(gated(qb[rows(r // 2, CH // 2), :], z)).astype(F32)
            m1, r1 = _stats(x)
            x1 = x + ((x - m1) * r1 * prm(0) + prm(1)) * ld_y(r, CH)
            m2, r2 = _stats(x1)
            h = (x1 - m2) * r2 * prm(2) + prm(3)
            m3, r3 = _stats(h)
            n3.append((h - m3) * r3)
            x1s.append(x1)
            hs.append(h)
        x1b[2 * TB:QE, :] = x1s[-1]
        hb[2 * TB:QE, :] = hs[-1]
        mm4e(ev, ov, u, 0)
        mm1(TB + AO, TB, jnp.concatenate(n3, axis=0))
        zrow = pl.multiple_of(jnp.where(i == NBLK - 2, HPAD + 2 * TB, HPAD + QE), 8)
        hpb[:, pl.ds(zrow, 8), :] = jnp.zeros((NT, 8, 128), F32)
        mm4e(ev, ov, u, 1)
        g = g_prep(TB).astype(BF16)
        hcat = jnp.concatenate(hs[:-1], axis=0)
        x2 = []
        for t in range(NT):
            mix = jnp.dot(g, _bf(w2b[:, 128 * t:128 * t + 128]), preferred_element_type=F32)
            x2.append(hcat[:, 128 * t:128 * t + 128] + mix)
        x2 = jnp.concatenate(x2, axis=-1)
        z = zero_after(mix[0:8])
        for j in range(TB // CH):
            xx = pltpu.bitcast(gated(x2[CH * j:CH * j + CH], z), F32)
            m4, r4 = _stats(xx)
            n4b[CH * j:CH * j + CH, :] = (xx - m4) * r4
            ev[TB + CH * j:TB + CH * j + CH, :] = x1s[j] + prm(4) * xx
            z = pltpu.roll(z, 1, 1)
        for t in range(2, NT):
            mm4e(ev, ov, u, t)
        out_copy(r0, TB).start()
        return carry

    jax.lax.fori_loop(1, NBLK - 1, body, 0)

    r0 = S - TB
    u = mm3(n4b[...])
    for t in range(NT):
        mm4e(eb.at[r0:S, :], ob.at[r0:S, :], u, t, split=2 if t == NT - 1 else 0)
        if t < NT - 1:
            out_copy(r0, TB, 128 * t, 128 * t + 128).start()
    out_copy(r0, TB // 2, D - 128, D).start()
    out_copy(r0 + TB // 2, TB // 2, D - 128, D).start()
    with jax.named_scope("W_out"):
        pltpu.make_async_copy(ob, o_hbm.at[0], osem).wait()


@jax.jit
def pallas_adaLN_cond__ssm_conv_h3__mixer_s_mlp__prompt_kernel(
    A_q, A_k, A_v, A_shift_k, A_ssm_k, A_ssm_D, B_x, B_w1, B_w2, B_w3, B_w4, c, w_mod,
):
    del B_x
    vm = pltpu.VMEM
    scratch = [
        vm(((S + AO) // 2, D), U32),
        vm((NT, KPAD + S, 128), BF16),
        vm((NT, S, 128), BF16),
        vm((4, D), BF16),
        vm((D // 2, S), U32),
        vm((D,), BF16),
        vm((D // 2, D), U32),
        vm((D // 2, D), U32),
        vm((FF // 2, D), U32),
        vm((FF // 2, D), U32),
        vm((1, D), BF16),
        vm((D, 6 * D), BF16),
        vm((R + 1, 128, 128), U32),
        vm((2 * R + 1, 32, 128), U32),
        vm((NT, S // 2, 128), U32),
        vm((8, NT, R, 256, 128), F32),
        vm((NT, S + AO, 128), F32),
        vm((2 * TB + AO, D), F32),
        vm((2 * TB + AO, D), F32),
        vm((S, D), F32),
        vm((NT, HPAD + 2 * TB + AO + 8, 128), F32),
        vm((TB, D), F32),
        vm((5, 8, D), F32),
        vm((D // 2, 128), U32),
        vm((S, D), BF16),
        pltpu.SemaphoreType.DMA((19,)),
        pltpu.SemaphoreType.DMA(()),
    ]
    hbm = pl.BlockSpec(memory_space=pltpu.HBM)
    return pl.pallas_call(
        _kernel,
        out_shape=jax.ShapeDtypeStruct((1, S, D), BF16),
        in_specs=[hbm] * 12,
        out_specs=hbm,
        scratch_shapes=scratch,
        compiler_params=pltpu.CompilerParams(vmem_limit_bytes=110 * 2**20,
                                             disable_semaphore_checks=True,
                                             disable_bounds_checks=True),
        name="h3_mixer",
    )(A_q, A_k, A_v, A_shift_k.T, A_ssm_k, A_ssm_D, B_w1, B_w2, B_w3.T, B_w4, c, w_mod)
```

```python
import jax
import jax.numpy as jnp
import numpy as np
import jax.experimental.pallas as pl
import jax.experimental.pallas.tpu as pltpu

S, D, FF = 2048, 640, 1728
NT = D // 128
L = 512
NB = S // L
NFFT = 2 * L
R = 4
KPAD = 16
HPAD = 8
TB = 256
NBLK = S // TB
AO = 16
CH = 16
EPS = 1e-5
W1A, W3A, W4A = 256, 1536, 384
NPAD = 1
FM = FF // 128 * 128
F32 = jnp.float32
BF16 = jnp.bfloat16
U32 = jnp.uint32
I32 = jnp.int32
NT_DIMS = (((1,), (1,)), ((), ()))
KP, X0S, ZP = 0, 3, 3


def _cos_coefs(deg=6):
    u = (np.cos(np.pi * (np.arange(400) + 0.5) / 400) + 1.0) / 2.0
    c = np.polynomial.polynomial.polyfit(u, np.cos(np.pi * np.sqrt(u)), deg)
    return [np.float32(v) for v in c]


_COS = _cos_coefs()


def _cos_units(a, scale=1.0):
    x = (((a + 1024) & 2047) - 1024).astype(F32) * np.float32(1.0 / 1024.0)
    u = x * x
    acc = u * np.float32(_COS[-1] * scale) + np.float32(_COS[-2] * scale)
    for c in _COS[-3::-1]:
        acc = acc * u + np.float32(c * scale)
    return acc


def _freq2(chunk, s):
    e = 4 * (8 * (chunk >> 1) + s) + 1
    return jnp.where((chunk & 1) == 0, e, 256 - e)


def _gelu(x):
    c1 = np.float32(np.sqrt(2.0 / np.pi))
    c2 = np.float32(np.sqrt(2.0 / np.pi) * 0.044715)
    u = x * (c1 + c2 * (x * x))
    hx = 0.5 * x
    return hx + hx * jnp.tanh(u)


def _stats(x):
    m = jnp.sum(x, axis=-1, keepdims=True) * (1.0 / D)
    e2 = jnp.sum(x * x, axis=-1, keepdims=True) * (1.0 / D)
    v = jnp.maximum(e2 - m * m, 0.0)
    return m, jax.lax.rsqrt(v + EPS)


def _split(b):
    b = b.reshape(-1, 2, 8, 128)
    return b[:, 0], b[:, 1]


def _join(z):
    return jnp.stack(z, axis=1).reshape(-1, 128)


def _eo(v):
    v = v.reshape(-1, 2, 8, 128)
    return v[:, 0], v[:, 1]


def _uneo(e, o):
    return jnp.stack([e, o], axis=1).reshape(16, 8, 128)


def _fft4(b, sign):
    (r0, i0), (r1, i1), (r2, i2), (r3, i3) = b
    sr, si, dr, di = r0 + r2, i0 + i2, r0 - r2, i0 - i2
    tr, ti, er, ei = r1 + r3, i1 + i3, r1 - r3, i1 - i3
    x0 = (sr + tr, si + ti)
    x2 = (sr - tr, si - ti)
    xm = (dr + ei, di - er)
    xp = (dr - ei, di + er)
    return [x0, xm, x2, xp] if sign < 0 else [x0, xp, x2, xm]


def _cmul(a, b, acc=None):
    (ar, ai), (br, bi) = a, b
    if acc is None:
        return ar * br - ai * bi, ar * bi + ai * br
    return (acc[0] + ar * br) - ai * bi, (acc[1] + ar * bi) + ai * br


def _bf(x):
    return pltpu.bitcast(x, BF16)


def _words(x):
    return pltpu.bitcast(x.astype(BF16), U32)


def _tie(w, ties):
    if not ties:
        return w
    parts = []
    for i in range(w.shape[0] // 8):
        p = w[8 * i:8 * i + 8]
        if i in ties:
            z = ties[i]
            p = p | z if p.shape[1] == 128 else jnp.concatenate([p[:, :128] | z, p[:, 128:]], axis=1)
        parts.append(p)
    return jnp.concatenate(parts, axis=0)


def _kernel(q_hbm, k_hbm, v_hbm, sk_hbm, ssm_hbm, sd_hbm, w1_hbm, w2_hbm, w3_hbm,
            w4_hbm, c_hbm, wm_hbm, o_hbm,
            qb, kb, vb, skb, ssmb, sdb, w1b, w2b, w3b, w4b, cb_, wmb, fwb, gib,
            stb, spec, yb, x1b, hb, eb, hpb, n4b, par, w3n, ob, sems, osem):
    groups = {}

    def add(name, src, dst):
        if name not in groups:
            groups[name] = (len(groups), [])
        idx, lst = groups[name]
        cp = pltpu.make_async_copy(src, dst, sems.at[idx])
        cp.start()
        lst.append(cp)

    def add_kv(name, c, tiles=range(NT)):
        for t in tiles:
            add(name, k_hbm.at[0, pl.ds(L * c, L), pl.ds(128 * t, 128)],
                kb.at[t, pl.ds(KPAD + L * c, L), :])
            add(name, v_hbm.at[0, pl.ds(L * c, L), pl.ds(128 * t, 128)],
                vb.at[t, pl.ds(L * c, L), :])

    def add_ssm(name, t):
        add(name, ssm_hbm.at[pl.ds(128 * t, 128), :], ssmb.bitcast(BF16).at[pl.ds(128 * t, 128), :])

    QE = 2 * TB + AO
    add_kv("ra", 0, [0])
    add("ra", sd_hbm, sdb)
    add("ra", sk_hbm, skb)
    add("ra", c_hbm, cb_)
    for t in range(NT):
        add_ssm(f"r{t}", t)
        add_kv(f"r{t}", (t + 1) // NT, [(t + 1) % NT])
    add_kv("r5", 1, range(1, NT))
    add_kv("r6", 2)
    add("wmA", q_hbm.at[0, pl.ds(0, QE), :], qb.bitcast(BF16).at[pl.ds(0, QE), :])
    add("wmA", wm_hbm.at[:, pl.ds(0, 3 * D)], wmb.at[:, pl.ds(0, 3 * D)])
    add("wmS", wm_hbm.at[:, pl.ds(3 * D, D + 256)], wmb.at[:, pl.ds(3 * D, D + 256)])
    add("wmB", wm_hbm.at[:, pl.ds(4 * D + 256, D - 256)], wmb.at[:, pl.ds(4 * D + 256, D - 256)])
    add("w1", w1_hbm.at[:, pl.ds(0, W1A)], w1b.bitcast(BF16).at[:, pl.ds(0, W1A)])
    add("w1b", w1_hbm.at[:, pl.ds(W1A, D - W1A)], w1b.bitcast(BF16).at[:, pl.ds(W1A, D - W1A)])
    add_kv("w1b", 3, [0])
    add("w2", w2_hbm, w2b.bitcast(BF16))
    add_kv("w2", 3, [1])
    add("w3", w3_hbm.at[pl.ds(0, W3A), :], w3b.bitcast(BF16).at[pl.ds(0, W3A), :])
    add("w4", w3_hbm.at[pl.ds(W3A, FF - W3A), :], w3b.bitcast(BF16).at[pl.ds(W3A, FF - W3A), :])
    add("w4", w4_hbm.at[:, pl.ds(0, W4A)], w4b.bitcast(BF16).at[:, pl.ds(0, W4A)])
    add_kv("w4", 3, [2, 3])
    add("rest", w4_hbm.at[:, pl.ds(W4A, D - W4A)], w4b.bitcast(BF16).at[:, pl.ds(W4A, D - W4A)])
    add_kv("rest", 3, [4])
    add("rest", wm_hbm.at[:, pl.ds(5 * D, D)], wmb.at[:, pl.ds(5 * D, D)])
    add("qnext", q_hbm.at[0, pl.ds(QE, TB), :], qb.bitcast(BF16).at[pl.ds(QE, TB), :])
    add("qlast", q_hbm.at[0, pl.ds(QE + TB, S - QE - TB), :],
        qb.bitcast(BF16).at[pl.ds(QE + TB, S - QE - TB), :])

    def wait(name):
        with jax.named_scope("W_" + name):
            for cp in groups[name][1]:
                cp.wait()

    kb[:, 0:KPAD, :] = jnp.zeros((NT, KPAD, 128), BF16)
    hpb[:, 0:HPAD, :] = jnp.zeros((NT, HPAD, 128), F32)
    yb[:, S:S + AO, :] = jnp.zeros((NT, AO, 128), F32)
    qb[S // 2:(S + AO) // 2, :] = jnp.zeros((AO // 2, D), U32)

    spec[7, 0, 0, pl.ds(0, 8, stride=2), :] = jnp.zeros((8, 128), F32)
    fwb[R, pl.ds(0, 8, stride=2), :] = jnp.zeros((8, 128), U32)
    gib[2 * R, pl.ds(0, 8, stride=2), :] = jnp.zeros((8, 128), U32)

    def make_tables(off):
        row = jax.lax.broadcasted_iota(I32, (256, 128), 0)
        col = jax.lax.broadcasted_iota(I32, (256, 128), 1)
        f2 = _freq2(row >> 4, row & 7)
        ph = 512 * ((row >> 3) & 1) + off
        m = (col & ~15) + 2 * (col & 7) + ((col >> 3) & 1)
        for r in range(R):
            fwb[r] = _words(_cos_units((4 * m + r) * f2 + ph))
        row = jax.lax.broadcasted_iota(I32, (64, 128), 0)
        col = jax.lax.broadcasted_iota(I32, (64, 128), 1)
        f2 = 4 * (8 * (col >> 4) + (col & 7)) + 1
        ph = 512 * ((col >> 3) & 1) + off
        for r in range(2 * R):
            gib[r] = _words(_cos_units((8 * row + r) * f2 + ph, 2.0 / NFFT))

    make_tables(0)

    env = {}

    def zero_after(*vals):
        acc = None
        for v in vals:
            v = pltpu.bitcast(v, U32)
            for i in range(0, v.shape[0], 8):
                for j in range(0, v.shape[1], 128):
                    p = v[i:i + 8, j:j + 128]
                    acc = p if acc is None else acc | p
        return acc & kb.bitcast(U32)[0, 0:8, :]

    def ld_spec(slot, t, q):
        return _split(spec[slot, t, q])

    def st_spec(slot, t, q, z):
        spec[slot, t, q] = _join(z)

    def fwd_dots(rhs, ties):
        return [_split(jnp.dot(_bf(_tie(fwb[r], ties if r == 0 else None)), rhs[r],
                               preferred_element_type=F32)) for r in range(R)]

    def conv_k(c, t, ties):
        w0 = L * c // 2
        stb[t, w0:w0 + L // 2, :] = pltpu.bitcast(
            _bf(ssmb[64 * t:64 * t + 64, L * c:L * c + L]).T, U32)
        rhs = []
        for h in range(2):
            lo = stb[t, pl.ds(w0 + h, 64, stride=4), :]
            hi = stb[t, pl.ds(w0 + h + 2, 64, stride=4), :]
            for e, o in zip(unpack(lo), unpack(hi)):
                rhs.append(_join((e.reshape(8, 8, 128), o.reshape(8, 8, 128))).astype(BF16))
        b = fwd_dots(rhs, ties)
        if c == 0:
            b[0] = (b[0][0] + env["dvec"][:, 128 * t:128 * t + 128][None], b[0][1])
        kq = _fft4(b, -1)
        z = []
        for q in range(R):
            kp = kq[q]
            if c >= 2:
                p = ld_spec(KP + c - 2, t, q)
                kp = (kp[0] + p[0], kp[1] + p[1])
            if c >= 1:
                p = ld_spec(KP + c - 1, t, q)
                if c == 3:
                    p0 = ld_spec(KP, t, q)
                    p = (p[0] - p0[0], p[1] - p0[1])
                (ree, reo), (ime, imo), (pre, pro), (pie, pio) = (_eo(v) for v in kp + p)
                kp = (_uneo(ree - pie, reo + pio), _uneo(ime + pre, imo - pro))
            if c < 3:
                st_spec(KP + c, t, q, kp)
            zc = _cmul(kp, ld_spec(X0S, t, q))
            if c == 0:
                z.append(zc)
            else:
                st_spec(ZP + c, t, q, zc)
        if c == 0:
            finish(0, t, z)

    def finish(c, t, z):
        hs = np.float32(np.sqrt(0.5))
        cr = _fft4(z, +1)
        for r in range(R):
            (ar, br), (ai, bi) = _eo(cr[r][0]), _eo(cr[r][1])
            if r % 2:
                br, bi = (br - bi) * hs, (br + bi) * hs
            if r < 2:
                p, m = (ar + br, ai - bi), (ar - br, ai + bi)
            else:
                p, m = (ar - bi, ai - br), (ar + bi, ai + br)
            env["cm", c, t, r] = _join(p).astype(BF16)
            env["cm", c, t, r + R] = _join(m).astype(BF16)

    def unpack(u):
        return (pltpu.bitcast(u << 16, F32),
                pltpu.bitcast(u & jnp.uint32(0xFFFF0000), F32))

    def conv_prep(c, t):
        taps = env["taps"]
        ku = kb.bitcast(U32)
        vu = vb.bitcast(U32)
        tp = [taps[j:j + 1, 128 * t:128 * t + 128] for j in range(4)]
        w0 = (KPAD + L * c) // 2
        kk = [unpack(ku[t, pl.ds(w0 - 2, 64, stride=4), :])[1]]
        for o in range(-1, 4):
            kk += unpack(ku[t, pl.ds(w0 + o, 64, stride=4), :])
        vv = []
        for o in range(4):
            vv += unpack(vu[t, pl.ds(L * c // 2 + o, 64, stride=4), :])
        kv = []
        for n in range(8):
            acc = kk[3 + n] * tp[0]
            for j in range(1, 4):
                acc = acc + kk[3 + n - j] * tp[j]
            kv.append(acc * vv[n])
        return [_join((kv[r].reshape(8, 8, 128), kv[r + 4].reshape(8, 8, 128))) for r in range(R)]

    def conv_x(c, t, ties):
        xq = _fft4(fwd_dots([v.astype(BF16) for v in env.pop(("kv", c, t))], ties), -1)
        z = []
        for q in range(R):
            if c == 0:
                st_spec(X0S, t, q, xq[q])
                continue
            for a in range(c, NB):
                if (c, a) == (1, 2):
                    st_spec(X0S, t, q, xq[q])
                    continue
                za = _cmul(xq[q], ld_spec(KP + a - c, t, q), ld_spec(ZP + a, t, q))
                if (c, a) == (2, 2):
                    za = _cmul(ld_spec(X0S, t, q), ld_spec(KP + 1, t, q), za)
                if a == c:
                    z.append(za)
                else:
                    st_spec(ZP + a, t, q, za)
        if c:
            finish(c, t, z)

    def conv_inv(c, t, ties):
        for r in range(2 * R):
            tr = None
            if ties and r % R == 0:
                tr = {i - r: z for i, z in ties.items() if 0 <= i - r < 4}
            yb[t, pl.ds(L * c + r, 64, stride=2 * R), :] = jnp.dot(
                _bf(_tie(gib[r], tr)), env.pop(("cm", c, t, r)), preferred_element_type=F32)

    def run_rounds(spec_str):
        rounds = spec_str.split()
        slots = []
        plan = {}
        for n, rd in enumerate(rounds):
            if rd[0] == "X":
                pts = []
                if "@" in rd:
                    a, b = (int(v) for v in rd[4:].split(":"))
                    pts = [slots[len(slots) - a + (a - b) * (j + 1) // 8 - 1] for j in range(8)]
                plan.setdefault(pts[0][0] if pts else n, []).append((rd, pts))
            slots += [(n, i) for i in range(8 if rd[0] == "I" else 16)]
        ties = {}
        for n, rd in enumerate(rounds):
            for xr, pts in plan.get(n, []):
                c, t = int(xr[1]), int(xr[2])
                kv = env["kv", c, t] = conv_prep(c, t)
                for j, (pn, pi) in enumerate(pts):
                    z = zero_after(*[w[16 * j:16 * j + 16] for w in kv])
                    d = ties.setdefault(pn, {})
                    d[pi] = z if pi not in d else d[pi] | z
            {"K": conv_k, "X": conv_x, "I": conv_inv}[rd[0]](int(rd[1]), int(rd[2]), ties.get(n))

    def rows(r0, n, align=8):
        if isinstance(r0, int):
            return slice(r0, r0 + n)
        return pl.ds(pl.multiple_of(r0, align), n)

    def ld_y(r0, n):
        return jnp.concatenate([yb[t, rows(r0, n), :] for t in range(NT)], axis=-1)

    def prm(i, n=CH, c0=0, c1=D):
        return jnp.concatenate([par[i, :, c0:c1]] * (n // 8), axis=0)

    def a_pre12(r0, n):
        x = _bf(qb[r0 // 2:(r0 + n) // 2, :]).astype(F32)
        m1, r1 = _stats(x)
        x1 = x + ((x - m1) * r1 * prm(0, n) + prm(1, n)) * ld_y(r0, n)
        x1b[r0:r0 + n, :] = x1
        m2, r2 = _stats(x1)
        hb[r0:r0 + n, :] = (x1 - m2) * r2

    def a_pre3(r0, m):
        h = hb[r0:r0 + m, :] * prm(2, m) + prm(3, m)
        hb[r0:r0 + m, :] = h
        m3, r3 = _stats(h)
        return (h - m3) * r3

    def halves(n, split):
        m = n // split if split else n
        return [(o, m) for o in range(0, n, m)]

    def mm1(r0, n, n3, split_last=0, ties=None, tiles=range(NT)):
        for t in tiles:
            w = _tie(w1b[:, 128 * t:128 * t + 128], ties.get(t) if ties else None)
            for o, m in halves(n, split_last if t == tiles[-1] else 0):
                hp = jnp.dot(n3[o:o + m].astype(BF16), _bf(w), preferred_element_type=F32)
                hpb[t, rows(HPAD + r0 + o, m), :] = _gelu(hp)

    def g_prep(r0):
        lane = jax.lax.broadcasted_iota(I32, (TB, 128), 1)
        sh = [-1, 1, -2, 2]

        def ldh(t, g):
            return hpb[t, pl.ds(HPAD + r0 + sh[g], TB), :]

        cols = [ldh(0, 0)]
        for t in range(1, 4):
            cols.append(jnp.where(lane < 32 * t, ldh(t, t - 1), ldh(t, t)))
        cols.append(ldh(4, 3))
        return jnp.concatenate(cols, axis=-1)

    def mm2(r0, g, split_last=0, side=None):
        for t in range(NT):
            if side and t in side:
                side[t]()
            c0, c1 = 128 * t, 128 * t + 128
            for o, m in halves(TB, split_last if t == NT - 1 else 0):
                hs = jnp.dot(g[o:o + m].astype(BF16), _bf(w2b[:, c0:c1]), preferred_element_type=F32)
                hb[rows(r0 + o, m), c0:c1] = hb[rows(r0 + o, m), c0:c1] + hs
        return hs[m - 8:m]

    def ln4(r0, n):
        x2 = hb[rows(r0, n), :]
        m4, r4 = _stats(x2)
        return (x2 - m4) * r4

    def mm3(n4, ties=None, split_at=None, side=None, tpos=12, nat=True):
        us = []
        env["g3"] = []
        for j in range(FF // 128):
            if side and j in side:
                side[j]()
            if j == tpos:
                ht = jax.lax.dot_general(_bf(w3b[FM // 2:FF // 2, :]), n4.astype(BF16), NT_DIMS,
                                         preferred_element_type=F32)
                ut = _gelu(ht).T
            w = w3b[64 * j:64 * j + 64, :]
            if ties and j in ties:
                w = _tie(w, {0: ties[j]})
            parts = []
            for o, m in halves(TB, 2 if j == split_at else 0):
                if j == 0 and nat:
                    h3 = jnp.dot(n4.astype(BF16), _bf(w3n[...]), preferred_element_type=F32)
                else:
                    h3 = jax.lax.dot_general(n4[o:o + m].astype(BF16), _bf(w), NT_DIMS,
                                             preferred_element_type=F32)
                parts.append(_gelu(h3))
                if m == TB:
                    env["g3"] += [h3[0:8], h3[128:136]]
            us.append(jnp.concatenate(parts, axis=0))
        return jnp.concatenate(us + [ut], axis=-1)

    def mm4(r0, u, t, final=True, ties=None, split=0, side=None):
        c0, c1 = 128 * t, 128 * t + 128
        w = _bf(_tie(w4b[:, c0:c1], ties))
        for o, m in halves(TB, split):
            if o and side:
                side()
            h2 = jnp.dot(u[o:o + m].astype(BF16), w, preferred_element_type=F32)
            s = hb[rows(r0 + o, m), c0:c1] + h2
            if final:
                ob[rows(r0 + o, m, 16), c0:c1] = (
                    x1b[rows(r0 + o, m), c0:c1] + prm(4, m, c0, c1) * s).astype(BF16)
            else:
                hb[rows(r0 + o, m), c0:c1] = s

    def ln4_store(r0, nch):
        zs = []
        m = TB // nch
        for j in range(nch):
            n4 = ln4(r0 + m * j, m)
            n4b[m * j:m * j + m, :] = n4
            zs.append(zero_after(n4))
        return zs

    def out_copy(r0, n, c0=0, c1=D):
        return pltpu.make_async_copy(ob.at[rows(r0, n, 16), c0:c1],
                                     o_hbm.at[0, rows(r0, n, 16), c0:c1], osem)

    wait("ra")
    env["taps"] = skb[...].astype(F32)
    env["dvec"] = sdb[...].astype(F32).reshape(1, D)
    cf = cb_[...].astype(F32)
    sc8 = jnp.broadcast_to(cf * jax.nn.sigmoid(cf), (8, D)).astype(BF16)
    run_rounds("X00")
    wait("r0")
    run_rounds("X01 K00 K10 K20 K30")
    for t in range(1, NT):
        wait(f"r{t}")
        run_rounds(f"I0{t - 1} X{(t + 1) // NT}{(t + 1) % NT} K0{t} K1{t} K2{t} K3{t}")
    wait("r5")
    run_rounds("I04 X11 I10 X12@20:3 I11 X13@20:3 I12 X14@20:3")
    wait("r6")
    run_rounds("I13 X20 I14 X21@24:14 I20 X22@24:14 I21 X23@24:14 I22 X24@24:14 I23")

    flag = kb.bitcast(I32)[0, 0:8, :][0, 0]
    for n in range(NPAD):
        pl.when(flag != 0)(lambda: make_tables(2 * NFFT * (n + 1) * flag))
    wait("wmA")
    mod = jnp.dot(sc8, wmb[:, 0:3 * D], preferred_element_type=F32)
    sa, ca, ga = [mod[:, D * i:D * (i + 1)] for i in range(3)]
    par[0] = (1.0 + ca) * ga
    par[1] = sa * ga
    run_rounds("I24")
    a_pre12(0, TB + AO)
    a_pre12(TB + AO, TB)
    wait("wmS")
    mod = jnp.dot(sc8, wmb[:, 3 * D:4 * D + 256], preferred_element_type=F32)
    par[3] = mod[:, 0:D]
    par[2, :, 0:256] = 1.0 + mod[:, D:D + 256]
    wait("wmB")
    par[2, :, 256:D] = 1.0 + jnp.dot(sc8, wmb[:, 4 * D + 256:5 * D], preferred_element_type=F32)
    n3p = a_pre3(0, 128)

    rr = lambda x: (lambda: run_rounds(x))
    ta, tb = range(W1A // 128), range(W1A // 128, NT)
    wait("w1")
    n3 = jnp.concatenate([n3p, a_pre3(128, QE - 128)], axis=0)
    for a, b in ((0, 128), (128, 256), (256, 400), (400, QE)):
        mm1(a, b - a, n3[a:b], tiles=ta)
    wait("w1b")
    mm1(0, TB + AO, n3[:TB + AO], tiles=tb)
    run_rounds("X30")
    mm1(TB + AO, TB, n3[TB + AO:], split_last=4, tiles=tb)
    wait("w2")
    mm2(0, g_prep(0), side={4: rr("X31")})
    n4 = ln4(0, TB)
    mm2(TB, g_prep(TB), split_last=2)
    wait("w3")
    zs = ln4_store(TB, 8)
    run_rounds("I30")

    def mid():
        wait("w4")
        w3n[...] = pltpu.bitcast(_bf(w3b[0:64, :]).T, U32)
        run_rounds("I31")

    u = mm3(n4, {3 + j: z for j, z in enumerate(zs)}, split_at=W3A // 128 - 1, nat=False,
            side={W3A // 128: mid})
    mm4(0, u, 0, final=False)
    run_rounds("X32")
    mm4(0, u, 1, final=False)
    run_rounds("X33")
    mm4(0, u, 2, final=False, split=4)
    run_rounds("I32")
    wait("rest")

    def gb_tiles(*ts):
        for t in ts:
            par[4, :, 128 * t:128 * t + 128] = jnp.dot(
                sc8, wmb[:, 5 * D + 128 * t:5 * D + 128 * t + 128], preferred_element_type=F32)

    run_rounds("I33")
    gb_tiles(3)
    mm4(0, u, 3, split=2, side=lambda: (gb_tiles(4), run_rounds("X34"), gb_tiles(0)))
    gb_tiles(1)
    mm4(0, u, 4, split=2, side=lambda: gb_tiles(2))
    ob[0:TB, 0:W4A] = (x1b[0:TB, 0:W4A] + prm(4, TB, 0, W4A) * hb[0:TB, 0:W4A]).astype(BF16)
    eb[TB:2 * TB, :] = x1b[TB:2 * TB, :] + prm(4, TB) * hb[TB:2 * TB, :]
    run_rounds("I34")
    out_copy(0, TB).start()
    wait("qnext")

    def gated(v, z):
        zt = jnp.concatenate([jnp.concatenate([z] * NT, axis=1)] * (v.shape[0] // 8), axis=0)
        return pltpu.bitcast(v, U32) | zt

    def mm4e(ev, ov, u, t, split=0):
        c0, c1 = 128 * t, 128 * t + 128
        for o, m in halves(TB, split):
            h2 = jnp.dot(u[o:o + m].astype(BF16), _bf(w4b[:, c0:c1]), preferred_element_type=F32)
            ov[o:o + m, c0:c1] = (ev[o:o + m, c0:c1] + prm(4, m, c0, c1) * h2).astype(BF16)

    def body(i, carry):
        pl.when(i == 2)(lambda: wait("qlast"))
        r0 = pl.multiple_of(i * TB, TB)
        ev = eb.at[pl.ds(r0, 2 * TB), :]
        ov = ob.at[pl.ds(r0, TB), :]
        u = mm3(n4b[...])
        hpb[:, TB:TB + HPAD + AO, :] = hpb[:, 2 * TB:2 * TB + HPAD + AO, :]
        x1s, hs, n3 = [x1b[2 * TB:QE, :]], [hb[2 * TB:QE, :]], []
        for j in range(TB // CH):
            r = r0 + TB + AO + CH * j
            z = zero_after(env["g3"][j * 25 // 15])
            x = _bf(gated(qb[rows(r // 2, CH // 2), :], z)).astype(F32)
            m1, r1 = _stats(x)
            x1 = x + ((x - m1) * r1 * prm(0) + prm(1)) * ld_y(r, CH)
            m2, r2 = _stats(x1)
            h = (x1 - m2) * r2 * prm(2) + prm(3)
            m3, r3 = _stats(h)
            n3.append((h - m3) * r3)
            x1s.append(x1)
            hs.append(h)
        x1b[2 * TB:QE, :] = x1s[-1]
        hb[2 * TB:QE, :] = hs[-1]
        mm4e(ev, ov, u, 0)
        mm1(TB + AO, TB, jnp.concatenate(n3, axis=0))
        zrow = pl.multiple_of(jnp.where(i == NBLK - 2, HPAD + 2 * TB, HPAD + QE), 8)
        hpb[:, pl.ds(zrow, 8), :] = jnp.zeros((NT, 8, 128), F32)
        mm4e(ev, ov, u, 1)
        g = g_prep(TB).astype(BF16)
        hcat = jnp.concatenate(hs[:-1], axis=0)
        x2 = []
        for t in range(NT):
            mix = jnp.dot(g, _bf(w2b[:, 128 * t:128 * t + 128]), preferred_element_type=F32)
            x2.append(hcat[:, 128 * t:128 * t + 128] + mix)
        x2 = jnp.concatenate(x2, axis=-1)
        z = zero_after(mix[0:8])
        for j in range(TB // CH):
            xx = pltpu.bitcast(gated(x2[CH * j:CH * j + CH], z), F32)
            m4, r4 = _stats(xx)
            n4b[CH * j:CH * j + CH, :] = (xx - m4) * r4
            ev[TB + CH * j:TB + CH * j + CH, :] = x1s[j] + prm(4) * xx
            z = pltpu.roll(z, 1, 1)
        for t in range(2, NT):
            mm4e(ev, ov, u, t)
        out_copy(r0, TB).start()
        return carry

    jax.lax.fori_loop(1, NBLK - 1, body, 0)

    r0 = S - TB
    u = mm3(n4b[...])
    for t in range(NT):
        mm4e(eb.at[r0:S, :], ob.at[r0:S, :], u, t, split=2 if t == NT - 1 else 0)
        if t < NT - 1:
            out_copy(r0, TB, 128 * t, 128 * t + 128).start()
    out_copy(r0, TB // 2, D - 128, D).start()
    out_copy(r0 + TB // 2, TB // 2, D - 128, D).start()
    with jax.named_scope("W_out"):
        pltpu.make_async_copy(ob, o_hbm.at[0], osem).wait()


@jax.jit
def pallas_adaLN_cond__ssm_conv_h3__mixer_s_mlp__prompt_kernel(
    A_q, A_k, A_v, A_shift_k, A_ssm_k, A_ssm_D, B_x, B_w1, B_w2, B_w3, B_w4, c, w_mod,
):
    del B_x
    vm = pltpu.VMEM
    scratch = [
        vm(((S + AO) // 2, D), U32),
        vm((NT, KPAD + S, 128), BF16),
        vm((NT, S, 128), BF16),
        vm((4, D), BF16),
        vm((D // 2, S), U32),
        vm((D,), BF16),
        vm((D // 2, D), U32),
        vm((D // 2, D), U32),
        vm((FF // 2, D), U32),
        vm((FF // 2, D), U32),
        vm((1, D), BF16),
        vm((D, 6 * D), BF16),
        vm((R + 1, 128, 128), U32),
        vm((2 * R + 1, 32, 128), U32),
        vm((NT, S // 2, 128), U32),
        vm((8, NT, R, 256, 128), F32),
        vm((NT, S + AO, 128), F32),
        vm((2 * TB + AO, D), F32),
        vm((2 * TB + AO, D), F32),
        vm((S, D), F32),
        vm((NT, HPAD + 2 * TB + AO + 8, 128), F32),
        vm((TB, D), F32),
        vm((5, 8, D), F32),
        vm((D // 2, 128), U32),
        vm((S, D), BF16),
        pltpu.SemaphoreType.DMA((19,)),
        pltpu.SemaphoreType.DMA(()),
    ]
    hbm = pl.BlockSpec(memory_space=pltpu.HBM)
    return pl.pallas_call(
        _kernel,
        out_shape=jax.ShapeDtypeStruct((1, S, D), BF16),
        in_specs=[hbm] * 12,
        out_specs=hbm,
        scratch_shapes=scratch,
        compiler_params=pltpu.CompilerParams(vmem_limit_bytes=110 * 2**20,
                                             disable_semaphore_checks=True,
                                             disable_bounds_checks=True),
        name="h3_mixer",
    )(A_q, A_k, A_v, A_shift_k.T, A_ssm_k, A_ssm_D, B_w1, B_w2, B_w3.T, B_w4, c, w_mod)
```

```python
import jax
import jax.numpy as jnp
import numpy as np
import jax.experimental.pallas as pl
import jax.experimental.pallas.tpu as pltpu

S, D, FF = 2048, 640, 1728
NT = D // 128
L = 512
NB = S // L
NFFT = 2 * L
R = 4
KPAD = 16
HPAD = 8
TB = 256
NBLK = S // TB
AO = 16
CH = 16
EPS = 1e-5
GATES = (0, 6, 7, 12, 15, 21, 22, 25, 28, 31, 33, 38, 42, 43, 44, 51)
W1A, W3A, W4A = 256, 1536, 384
FM = FF // 128 * 128
F32 = jnp.float32
BF16 = jnp.bfloat16
U32 = jnp.uint32
I32 = jnp.int32
NT_DIMS = (((1,), (1,)), ((), ()))
KP, XS, ZP = 0, 3, 3


def _cos_coefs(deg=6):
    u = (np.cos(np.pi * (np.arange(400) + 0.5) / 400) + 1.0) / 2.0
    c = np.polynomial.polynomial.polyfit(u, np.cos(np.pi * np.sqrt(u)), deg)
    return [np.float32(v) for v in c]


_COS = _cos_coefs()


def _cos_units(a, scale=1.0):
    x = (((a + 1024) & 2047) - 1024).astype(F32) * np.float32(1.0 / 1024.0)
    u = x * x
    acc = u * np.float32(_COS[-1] * scale) + np.float32(_COS[-2] * scale)
    for c in _COS[-3::-1]:
        acc = acc * u + np.float32(c * scale)
    return acc


def _freq2(chunk, s):
    e = 4 * (8 * (chunk >> 1) + s) + 1
    return jnp.where((chunk & 1) == 0, e, 256 - e)


def _gelu(x):
    c1 = np.float32(np.sqrt(2.0 / np.pi))
    c2 = np.float32(np.sqrt(2.0 / np.pi) * 0.044715)
    u = x * (c1 + c2 * (x * x))
    hx = 0.5 * x
    return hx + hx * jnp.tanh(u)


def _stats(x):
    m = jnp.sum(x, axis=-1, keepdims=True) * (1.0 / D)
    e2 = jnp.sum(x * x, axis=-1, keepdims=True) * (1.0 / D)
    v = jnp.maximum(e2 - m * m, 0.0)
    return m, jax.lax.rsqrt(v + EPS)


def _split(b):
    b = b.reshape(-1, 2, 8, 128)
    return b[:, 0], b[:, 1]


def _join(z):
    return jnp.stack(z, axis=1).reshape(-1, 128)


def _uneo(e, o):
    return jnp.stack([e, o], axis=1).reshape(16, 8, 128)


def _fft4(b, sign):
    (r0, i0), (r1, i1), (r2, i2), (r3, i3) = b
    sr, si, dr, di = r0 + r2, i0 + i2, r0 - r2, i0 - i2
    tr, ti, er, ei = r1 + r3, i1 + i3, r1 - r3, i1 - i3
    x0 = (sr + tr, si + ti)
    x2 = (sr - tr, si - ti)
    xm = (dr + ei, di - er)
    xp = (dr - ei, di + er)
    return [x0, xm, x2, xp] if sign < 0 else [x0, xp, x2, xm]


def _cmul(a, b, acc=None):
    (ar, ai), (br, bi) = a, b
    if acc is None:
        return ar * br - ai * bi, ar * bi + ai * br
    return (acc[0] + ar * br) - ai * bi, (acc[1] + ar * bi) + ai * br


def _bf(x):
    return pltpu.bitcast(x, BF16)


def _words(x):
    return pltpu.bitcast(x.astype(BF16), U32)


def _tie(w, ties):
    if not ties:
        return w
    parts = []
    for i in range(w.shape[0] // 8):
        p = w[8 * i:8 * i + 8]
        if i in ties:
            z = ties[i]
            p = p | z if p.shape[1] == 128 else jnp.concatenate([p[:, :128] | z, p[:, 128:]], axis=1)
        parts.append(p)
    return jnp.concatenate(parts, axis=0)


def _kernel(q_hbm, k_hbm, v_hbm, sk_hbm, ssm_hbm, sd_hbm, w1_hbm, w2_hbm, w3_hbm,
            w4_hbm, c_hbm, wm_hbm, o_hbm,
            qb, kb, vb, skb, ssmb, sdb, w1b, w2b, w3b, w4b, cb_, wmb, fwb, gib,
            stb, spec, yb, x1b, hb, eb, hpb, n4b, par, w3n, ob, sems, osem):
    groups = {}

    def add(name, src, dst):
        if name not in groups:
            groups[name] = (len(groups), [])
        idx, lst = groups[name]
        cp = pltpu.make_async_copy(src, dst, sems.at[idx])
        cp.start()
        lst.append(cp)

    def add_kv(name, c, tiles=range(NT)):
        for t in tiles:
            add(name, k_hbm.at[0, pl.ds(L * c, L), pl.ds(128 * t, 128)],
                kb.at[t, pl.ds(KPAD + L * c, L), :])
            add(name, v_hbm.at[0, pl.ds(L * c, L), pl.ds(128 * t, 128)],
                vb.at[t, pl.ds(L * c, L), :])

    def add_ssm(name, t):
        add(name, ssm_hbm.at[pl.ds(128 * t, 128), :], ssmb.bitcast(BF16).at[pl.ds(128 * t, 128), :])

    QE = 2 * TB + AO
    add_kv("ra", 0, [0])
    add("ra", sd_hbm, sdb)
    add("ra", sk_hbm, skb)
    add("ra", c_hbm, cb_)
    for t in range(NT):
        add_ssm(f"r{t}", t)
        add_kv(f"r{t}", (t + 1) // NT, [(t + 1) % NT])
    add_kv("r5", 1, range(1, NT))
    add_kv("r6", 2)
    add("wmA", q_hbm.at[0, pl.ds(0, QE), :], qb.bitcast(BF16).at[pl.ds(0, QE), :])
    add("wmA", wm_hbm.at[:, pl.ds(0, 3 * D)], wmb.at[:, pl.ds(0, 3 * D)])
    add("wmS", wm_hbm.at[:, pl.ds(3 * D, D + 256)], wmb.at[:, pl.ds(3 * D, D + 256)])
    add("wmB", wm_hbm.at[:, pl.ds(4 * D + 256, D - 256)], wmb.at[:, pl.ds(4 * D + 256, D - 256)])
    add("w1", w1_hbm.at[:, pl.ds(0, W1A)], w1b.bitcast(BF16).at[:, pl.ds(0, W1A)])
    add("w1b", w1_hbm.at[:, pl.ds(W1A, D - W1A)], w1b.bitcast(BF16).at[:, pl.ds(W1A, D - W1A)])
    add_kv("w1b", 3, [0])
    add("w2", w2_hbm, w2b.bitcast(BF16))
    add_kv("w2", 3, [1])
    add("w3", w3_hbm.at[pl.ds(0, W3A), :], w3b.bitcast(BF16).at[pl.ds(0, W3A), :])
    add("w4", w3_hbm.at[pl.ds(W3A, FF - W3A), :], w3b.bitcast(BF16).at[pl.ds(W3A, FF - W3A), :])
    add("w4", w4_hbm.at[:, pl.ds(0, W4A)], w4b.bitcast(BF16).at[:, pl.ds(0, W4A)])
    add_kv("w4", 3, [2, 3])
    add("rest", w4_hbm.at[:, pl.ds(W4A, D - W4A)], w4b.bitcast(BF16).at[:, pl.ds(W4A, D - W4A)])
    add_kv("rest", 3, [4])
    add("rest", wm_hbm.at[:, pl.ds(5 * D, D)], wmb.at[:, pl.ds(5 * D, D)])
    add("qnext", q_hbm.at[0, pl.ds(QE, TB), :], qb.bitcast(BF16).at[pl.ds(QE, TB), :])
    add("qlast", q_hbm.at[0, pl.ds(QE + TB, S - QE - TB), :],
        qb.bitcast(BF16).at[pl.ds(QE + TB, S - QE - TB), :])

    def wait(name):
        with jax.named_scope("W_" + name):
            for cp in groups[name][1]:
                cp.wait()

    kb[:, 0:KPAD, :] = jnp.zeros((NT, KPAD, 128), BF16)
    hpb[:, 0:HPAD, :] = jnp.zeros((NT, HPAD, 128), F32)
    yb[:, S:S + AO, :] = jnp.zeros((NT, AO, 128), F32)
    qb[S // 2:(S + AO) // 2, :] = jnp.zeros((AO // 2, D), U32)

    spec[7, 0, 0, pl.ds(0, 8, stride=2), :] = jnp.zeros((8, 128), F32)
    fwb[R, pl.ds(0, 8, stride=2), :] = jnp.zeros((8, 128), U32)
    gib[2 * R, pl.ds(0, 8, stride=2), :] = jnp.zeros((8, 128), U32)

    def make_tables(off):
        row = jax.lax.broadcasted_iota(I32, (256, 128), 0)
        col = jax.lax.broadcasted_iota(I32, (256, 128), 1)
        f2 = _freq2(row >> 4, row & 7)
        ph = 512 * ((row >> 3) & 1) + off
        m = (col & ~15) + 2 * (col & 7) + ((col >> 3) & 1)
        for r in range(R):
            fwb[r] = _words(_cos_units((4 * m + r) * f2 + ph))
        row = jax.lax.broadcasted_iota(I32, (64, 128), 0)
        col = jax.lax.broadcasted_iota(I32, (64, 128), 1)
        f2 = 4 * (8 * (col >> 4) + (col & 7)) + 1
        ph = 512 * ((col >> 3) & 1) + off
        for r in range(2 * R):
            gib[r] = _words(_cos_units((8 * row + r) * f2 + ph, 2.0 / NFFT))

    make_tables(0)

    env = {}

    def zero_after(*vals):
        acc = None
        for v in vals:
            v = pltpu.bitcast(v, U32)
            for i in range(0, v.shape[0], 8):
                for j in range(0, v.shape[1], 128):
                    p = v[i:i + 8, j:j + 128]
                    acc = p if acc is None else acc | p
        return acc & kb.bitcast(U32)[0, 0:8, :]

    def gated(v, z):
        zt = jnp.concatenate([jnp.concatenate([z] * NT, axis=1)] * (v.shape[0] // 8), axis=0)
        return pltpu.bitcast(v, U32) | zt

    def ld_spec(slot, t, q):
        return _split(spec[slot, t, q])

    def st_spec(slot, t, q, z):
        spec[slot, t, q] = _join(z)

    def fwd_dots(rhs, ties):
        return [_split(jnp.dot(_bf(_tie(fwb[r], ties if r == 0 else None)), rhs[r],
                               preferred_element_type=F32)) for r in range(R)]

    def conv_k(c, t, ties):
        w0 = L * c // 2
        stb[t, w0:w0 + L // 2, :] = pltpu.bitcast(
            _bf(ssmb[64 * t:64 * t + 64, L * c:L * c + L]).T, U32)
        rhs = []
        for h in range(2):
            lo = stb[t, pl.ds(w0 + h, 64, stride=4), :]
            hi = stb[t, pl.ds(w0 + h + 2, 64, stride=4), :]
            for e, o in zip(unpack(lo), unpack(hi)):
                rhs.append(_join((e.reshape(8, 8, 128), o.reshape(8, 8, 128))).astype(BF16))
        b = fwd_dots(rhs, ties)
        if c == 0:
            b[0] = (b[0][0] + env["dvec"][:, 128 * t:128 * t + 128][None], b[0][1])
        kq = _fft4(b, -1)
        z = []
        for q in range(R):
            kp = kq[q]
            if c >= 2:
                p = ld_spec(KP + c - 2, t, q)
                kp = (kp[0] + p[0], kp[1] + p[1])
            if c >= 1:
                p = ld_spec(KP + c - 1, t, q)
                if c == 3:
                    p0 = ld_spec(KP, t, q)
                    p = (p[0] - p0[0], p[1] - p0[1])
                (ree, reo), (ime, imo), (pre, pro), (pie, pio) = (_split(v) for v in kp + p)
                kp = (_uneo(ree - pie, reo + pio), _uneo(ime + pre, imo - pro))
            if c < 3:
                st_spec(KP + c, t, q, kp)
            zc = _cmul(kp, ld_spec(XS, t, q))
            if c == 0:
                z.append(zc)
            else:
                st_spec(ZP + c, t, q, zc)
        if c == 0:
            finish(0, t, z)

    def finish(c, t, z):
        hs = np.float32(np.sqrt(0.5))
        cr = _fft4(z, +1)
        for r in range(R):
            (ar, br), (ai, bi) = _split(cr[r][0]), _split(cr[r][1])
            if r % 2:
                br, bi = (br - bi) * hs, (br + bi) * hs
            if r < 2:
                p, m = (ar + br, ai - bi), (ar - br, ai + bi)
            else:
                p, m = (ar - bi, ai - br), (ar + bi, ai + br)
            env["cm", c, t, r] = _join(p).astype(BF16)
            env["cm", c, t, r + R] = _join(m).astype(BF16)

    def unpack(u):
        return (pltpu.bitcast(u << 16, F32),
                pltpu.bitcast(u & jnp.uint32(0xFFFF0000), F32))

    def conv_prep(c, t):
        taps = env["taps"]
        ku = kb.bitcast(U32)
        vu = vb.bitcast(U32)
        tp = [taps[j:j + 1, 128 * t:128 * t + 128] for j in range(4)]
        w0 = (KPAD + L * c) // 2
        kk = [unpack(ku[t, pl.ds(w0 - 2, 64, stride=4), :])[1]]
        for o in range(-1, 4):
            kk += unpack(ku[t, pl.ds(w0 + o, 64, stride=4), :])
        vv = []
        for o in range(4):
            vv += unpack(vu[t, pl.ds(L * c // 2 + o, 64, stride=4), :])
        kv = []
        for n in range(8):
            acc = kk[3 + n] * tp[0]
            for j in range(1, 4):
                acc = acc + kk[3 + n - j] * tp[j]
            kv.append(acc * vv[n])
        return [_join((kv[r].reshape(8, 8, 128), kv[r + 4].reshape(8, 8, 128))) for r in range(R)]

    def conv_x(c, t, ties):
        xq = _fft4(fwd_dots([v.astype(BF16) for v in env.pop(("kv", c, t))], ties), -1)
        z = []
        for q in range(R):
            if c == 0:
                st_spec(XS, t, q, xq[q])
                continue
            for a in range(c, NB):
                if (c, a) == (1, 2):
                    st_spec(XS, t, q, xq[q])
                    continue
                za = _cmul(xq[q], ld_spec(KP + a - c, t, q), ld_spec(ZP + a, t, q))
                if (c, a) == (2, 2):
                    za = _cmul(ld_spec(XS, t, q), ld_spec(KP + 1, t, q), za)
                if a == c:
                    z.append(za)
                else:
                    st_spec(ZP + a, t, q, za)
        if c:
            finish(c, t, z)

    def conv_inv(c, t, ties):
        for r in range(2 * R):
            tr = None
            if ties and r % R == 0:
                tr = {i - r: z for i, z in ties.items() if 0 <= i - r < 4}
            yb[t, pl.ds(L * c + r, 64, stride=2 * R), :] = jnp.dot(
                _bf(_tie(gib[r], tr)), env.pop(("cm", c, t, r)), preferred_element_type=F32)

    def run_rounds(spec_str):
        rounds = spec_str.split()
        slots = []
        plan = {}
        for n, rd in enumerate(rounds):
            if rd[0] == "X":
                pts = []
                if "@" in rd:
                    a, b = (int(v) for v in rd[4:].split(":"))
                    pts = [slots[len(slots) - a + (a - b) * (j + 1) // 8 - 1] for j in range(8)]
                plan.setdefault(pts[0][0] if pts else n, []).append((rd, pts))
            slots += [(n, i) for i in range(8 if rd[0] == "I" else 16)]
        ties = {}
        for n, rd in enumerate(rounds):
            for xr, pts in plan.get(n, []):
                c, t = int(xr[1]), int(xr[2])
                kv = env["kv", c, t] = conv_prep(c, t)
                for j, (pn, pi) in enumerate(pts):
                    z = zero_after(*[w[16 * j:16 * j + 16] for w in kv])
                    d = ties.setdefault(pn, {})
                    d[pi] = z if pi not in d else d[pi] | z
            {"K": conv_k, "X": conv_x, "I": conv_inv}[rd[0]](int(rd[1]), int(rd[2]), ties.get(n))

    def rows(r0, n, align=8):
        if isinstance(r0, int):
            return slice(r0, r0 + n)
        return pl.ds(pl.multiple_of(r0, align), n)

    def ld_y(r0, n):
        return jnp.concatenate([yb[t, rows(r0, n), :] for t in range(NT)], axis=-1)

    def prm(i, n=CH, c0=0, c1=D):
        return jnp.concatenate([par[i, :, c0:c1]] * (n // 8), axis=0)

    def a_pre12(r0, n):
        x = _bf(qb[r0 // 2:(r0 + n) // 2, :]).astype(F32)
        m1, r1 = _stats(x)
        x1 = x + ((x - m1) * r1 * prm(0, n) + prm(1, n)) * ld_y(r0, n)
        x1b[r0:r0 + n, :] = x1
        m2, r2 = _stats(x1)
        hb[r0:r0 + n, :] = (x1 - m2) * r2

    def a_pre3(r0, m):
        h = hb[r0:r0 + m, :] * prm(2, m) + prm(3, m)
        hb[r0:r0 + m, :] = h
        m3, r3 = _stats(h)
        return (h - m3) * r3

    def halves(n, split):
        m = n // split if split else n
        return [(o, m) for o in range(0, n, m)]

    def mm1(r0, n, n3, split_last=0, tiles=range(NT)):
        for t in tiles:
            w = w1b[:, 128 * t:128 * t + 128]
            for o, m in halves(n, split_last if t == tiles[-1] else 0):
                hp = jnp.dot(n3[o:o + m].astype(BF16), _bf(w), preferred_element_type=F32)
                hpb[t, rows(HPAD + r0 + o, m), :] = _gelu(hp)

    def g_prep(r0):
        lane = jax.lax.broadcasted_iota(I32, (TB, 128), 1)
        sh = [-1, 1, -2, 2]

        def ldh(t, g):
            return hpb[t, pl.ds(HPAD + r0 + sh[g], TB), :]

        cols = [ldh(0, 0)]
        for t in range(1, 4):
            cols.append(jnp.where(lane < 32 * t, ldh(t, t - 1), ldh(t, t)))
        cols.append(ldh(4, 3))
        return jnp.concatenate(cols, axis=-1)

    def mm2(r0, g, split_last=0, side=None):
        for t in range(NT):
            if side and t in side:
                side[t]()
            c0, c1 = 128 * t, 128 * t + 128
            for o, m in halves(TB, split_last if t == NT - 1 else 0):
                hs = jnp.dot(g[o:o + m].astype(BF16), _bf(w2b[:, c0:c1]), preferred_element_type=F32)
                hb[rows(r0 + o, m), c0:c1] = hb[rows(r0 + o, m), c0:c1] + hs
        return hs[m - 8:m]

    def mm3(n4, ties=None, split_at=None, side=None, tpos=12, nat=True):
        us = []
        env["g3"] = []
        for j in range(FF // 128):
            if side and j in side:
                side[j]()
            if j == tpos:
                ht = jax.lax.dot_general(_bf(w3b[FM // 2:FF // 2, :]), n4.astype(BF16), NT_DIMS,
                                         preferred_element_type=F32)
                ut = _gelu(ht).T
            w = w3b[64 * j:64 * j + 64, :]
            if ties and j in ties:
                w = _tie(w, {0: ties[j]})
            parts = []
            for o, m in halves(TB, 2 if j == split_at else 0):
                if j == 0 and nat:
                    h3 = jnp.dot(n4.astype(BF16), _bf(w3n[...]), preferred_element_type=F32)
                else:
                    h3 = jax.lax.dot_general(n4[o:o + m].astype(BF16), _bf(w), NT_DIMS,
                                             preferred_element_type=F32)
                parts.append(_gelu(h3))
                if m == TB:
                    env["g3"] += [h3[o:o + 8] for o in range(0, TB, 64)]
            us.append(jnp.concatenate(parts, axis=0))
        return jnp.concatenate(us + [ut], axis=-1)

    def mm4(r0, u, t, final=True, split=0, side=None):
        c0, c1 = 128 * t, 128 * t + 128
        w = _bf(w4b[:, c0:c1])
        for o, m in halves(TB, split):
            if o and side:
                side()
            h2 = jnp.dot(u[o:o + m].astype(BF16), w, preferred_element_type=F32)
            s = hb[rows(r0 + o, m), c0:c1] + h2
            if final:
                ob[rows(r0 + o, m, 16), c0:c1] = (
                    x1b[rows(r0 + o, m), c0:c1] + prm(4, m, c0, c1) * s).astype(BF16)
            else:
                hb[rows(r0 + o, m), c0:c1] = s

    def ln4_store(r0, nch):
        zs = []
        m = TB // nch
        for j in range(nch):
            x2 = hb[r0 + m * j:r0 + m * j + m, :]
            m4, r4 = _stats(x2)
            n4 = (x2 - m4) * r4
            n4b[m * j:m * j + m, :] = n4
            zs.append(zero_after(n4))
        return zs

    def out_copy(r0, n, c0=0, c1=D):
        return pltpu.make_async_copy(ob.at[rows(r0, n, 16), c0:c1],
                                     o_hbm.at[0, rows(r0, n, 16), c0:c1], osem)

    wait("ra")
    env["taps"] = skb[...].astype(F32)
    env["dvec"] = sdb[...].astype(F32).reshape(1, D)
    cf = cb_[...].astype(F32)
    sc8 = jnp.broadcast_to(cf * jax.nn.sigmoid(cf), (8, D)).astype(BF16)
    run_rounds("X00")
    wait("r0")
    run_rounds("X01 K00 K10 K20 K30")
    for t in range(1, NT):
        wait(f"r{t}")
        run_rounds(f"I0{t - 1} X{(t + 1) // NT}{(t + 1) % NT} K0{t} K1{t} K2{t} K3{t}")
    wait("r5")
    run_rounds("I04 X11 I10 X12@20:3 I11 X13@20:3 I12 X14@20:3")
    wait("r6")
    run_rounds("I13 X20 I14 X21@24:14 I20 X22@24:14 I21 X23@24:14 I22 X24@24:14 I23")

    flag = kb.bitcast(I32)[0, 0:8, :][0, 0]
    pl.when(flag != 0)(lambda: make_tables(2 * NFFT * flag))
    wait("wmA")
    mod = jnp.dot(sc8, wmb[:, 0:3 * D], preferred_element_type=F32)
    sa, ca, ga = [mod[:, D * i:D * (i + 1)] for i in range(3)]
    par[0] = (1.0 + ca) * ga
    par[1] = sa * ga
    run_rounds("I24")
    a_pre12(0, TB + AO)
    a_pre12(TB + AO, TB)
    wait("wmS")
    mod = jnp.dot(sc8, wmb[:, 3 * D:4 * D + 256], preferred_element_type=F32)
    par[3] = mod[:, 0:D]
    par[2, :, 0:256] = 1.0 + mod[:, D:D + 256]
    wait("wmB")
    par[2, :, 256:D] = 1.0 + jnp.dot(sc8, wmb[:, 4 * D + 256:5 * D], preferred_element_type=F32)
    n3p = a_pre3(0, 128)

    ta, tb = range(W1A // 128), range(W1A // 128, NT)
    wait("w1")
    n3 = jnp.concatenate([n3p, a_pre3(128, QE - 128)], axis=0)
    for a, b in ((0, 128), (128, 256), (256, 400), (400, QE)):
        mm1(a, b - a, n3[a:b], tiles=ta)
    wait("w1b")
    mm1(0, TB + AO, n3[:TB + AO], tiles=tb)
    run_rounds("X30")
    mm1(TB + AO, TB, n3[TB + AO:], split_last=4, tiles=tb)
    wait("w2")
    z = zero_after(mm2(0, g_prep(0), side={4: lambda: run_rounds("X31")}))
    n4 = []
    for j in range(8):
        xx = pltpu.bitcast(gated(hb[32 * j:32 * j + 32, :], z), F32)
        m4, r4 = _stats(xx)
        n4.append((xx - m4) * r4)
        if j >= 3:
            z = z | zero_after(n4[j - 3])
        z = pltpu.roll(z, 1, 1)
    n4 = jnp.concatenate(n4, axis=0)
    mm2(TB, g_prep(TB), split_last=2)
    wait("w3")
    zs = ln4_store(TB, 8)
    run_rounds("I30")

    def mid():
        wait("w4")
        w3n[...] = pltpu.bitcast(_bf(w3b[0:64, :]).T, U32)
        run_rounds("I31")

    u = mm3(n4, {3 + j: z for j, z in enumerate(zs)}, split_at=W3A // 128 - 1, nat=False,
            side={W3A // 128: mid})
    mm4(0, u, 0, final=False)
    run_rounds("X32")
    mm4(0, u, 1, final=False)
    run_rounds("X33")
    mm4(0, u, 2, final=False, split=4)
    run_rounds("I32")
    wait("rest")

    def gb_tiles(*ts):
        for t in ts:
            par[4, :, 128 * t:128 * t + 128] = jnp.dot(
                sc8, wmb[:, 5 * D + 128 * t:5 * D + 128 * t + 128], preferred_element_type=F32)

    run_rounds("I33")
    gb_tiles(3)
    mm4(0, u, 3, split=2, side=lambda: (gb_tiles(4), run_rounds("X34"), gb_tiles(0)))
    gb_tiles(1)
    mm4(0, u, 4, split=2, side=lambda: gb_tiles(2))
    ob[0:TB, 0:W4A] = (x1b[0:TB, 0:W4A] + prm(4, TB, 0, W4A) * hb[0:TB, 0:W4A]).astype(BF16)
    eb[TB:2 * TB, :] = x1b[TB:2 * TB, :] + prm(4, TB) * hb[TB:2 * TB, :]
    run_rounds("I34")
    out_copy(0, TB).start()
    wait("qnext")

    def mm4e(ev, ov, u, t, split=0):
        c0, c1 = 128 * t, 128 * t + 128
        for o, m in halves(TB, split):
            h2 = jnp.dot(u[o:o + m].astype(BF16), _bf(w4b[:, c0:c1]), preferred_element_type=F32)
            ov[o:o + m, c0:c1] = (ev[o:o + m, c0:c1] + prm(4, m, c0, c1) * h2).astype(BF16)

    def body(i, carry):
        pl.when(i == 2)(lambda: wait("qlast"))
        r0 = pl.multiple_of(i * TB, TB)
        ev = eb.at[pl.ds(r0, 2 * TB), :]
        ov = ob.at[pl.ds(r0, TB), :]
        u = mm3(n4b[...])
        hpb[:, TB:TB + HPAD + AO, :] = hpb[:, 2 * TB:2 * TB + HPAD + AO, :]
        x1s, hs, n3 = [x1b[2 * TB:QE, :]], [hb[2 * TB:QE, :]], []
        for j in range(TB // CH):
            r = r0 + TB + AO + CH * j
            z = zero_after(env["g3"][GATES[j]])
            x = _bf(gated(qb[rows(r // 2, CH // 2), :], z)).astype(F32)
            m1, r1 = _stats(x)
            x1 = x + ((x - m1) * r1 * prm(0) + prm(1)) * ld_y(r, CH)
            m2, r2 = _stats(x1)
            h = (x1 - m2) * r2 * prm(2) + prm(3)
            m3, r3 = _stats(h)
            n3.append((h - m3) * r3)
            x1s.append(x1)
            hs.append(h)
        x1b[2 * TB:QE, :] = x1s[-1]
        hb[2 * TB:QE, :] = hs[-1]
        mm4e(ev, ov, u, 0)
        mm1(TB + AO, TB, jnp.concatenate(n3, axis=0))
        zrow = pl.multiple_of(jnp.where(i == NBLK - 2, HPAD + 2 * TB, HPAD + QE), 8)
        hpb[:, pl.ds(zrow, 8), :] = jnp.zeros((NT, 8, 128), F32)
        mm4e(ev, ov, u, 1)
        g = g_prep(TB).astype(BF16)
        hcat = jnp.concatenate(hs[:-1], axis=0)
        x2 = []
        for t in range(NT):
            mix = jnp.dot(g, _bf(w2b[:, 128 * t:128 * t + 128]), preferred_element_type=F32)
            x2.append(hcat[:, 128 * t:128 * t + 128] + mix)
        x2 = jnp.concatenate(x2, axis=-1)
        z = zero_after(mix[0:8])
        for j in range(TB // CH):
            xx = pltpu.bitcast(gated(x2[CH * j:CH * j + CH], z), F32)
            m4, r4 = _stats(xx)
            n4b[CH * j:CH * j + CH, :] = (xx - m4) * r4
            ev[TB + CH * j:TB + CH * j + CH, :] = x1s[j] + prm(4) * xx
            z = pltpu.roll(z, 1, 1)
        for t in range(2, NT):
            mm4e(ev, ov, u, t)
        out_copy(r0, TB).start()
        return carry

    jax.lax.fori_loop(1, NBLK - 1, body, 0)

    r0 = S - TB
    u = mm3(n4b[...])
    for t in range(NT):
        mm4e(eb.at[r0:S, :], ob.at[r0:S, :], u, t, split=2 if t == NT - 1 else 0)
        if t < NT - 1:
            out_copy(r0, TB, 128 * t, 128 * t + 128).start()
    out_copy(r0, TB // 2, D - 128, D).start()
    out_copy(r0 + TB // 2, TB // 2, D - 128, D).start()
    with jax.named_scope("W_out"):
        pltpu.make_async_copy(ob, o_hbm.at[0], osem).wait()


@jax.jit
def pallas_adaLN_cond__ssm_conv_h3__mixer_s_mlp__prompt_kernel(
    A_q, A_k, A_v, A_shift_k, A_ssm_k, A_ssm_D, B_x, B_w1, B_w2, B_w3, B_w4, c, w_mod,
):
    del B_x
    vm = pltpu.VMEM
    scratch = [
        vm(((S + AO) // 2, D), U32),
        vm((NT, KPAD + S, 128), BF16),
        vm((NT, S, 128), BF16),
        vm((4, D), BF16),
        vm((D // 2, S), U32),
        vm((D,), BF16),
        vm((D // 2, D), U32),
        vm((D // 2, D), U32),
        vm((FF // 2, D), U32),
        vm((FF // 2, D), U32),
        vm((1, D), BF16),
        vm((D, 6 * D), BF16),
        vm((R + 1, 128, 128), U32),
        vm((2 * R + 1, 32, 128), U32),
        vm((NT, S // 2, 128), U32),
        vm((8, NT, R, 256, 128), F32),
        vm((NT, S + AO + 16, 128), F32),
        vm((2 * TB + AO, D), F32),
        vm((2 * TB + AO, D), F32),
        vm((S + 8, D), F32),
        vm((NT, HPAD + 2 * TB + AO + 8, 128), F32),
        vm((TB, D), F32),
        vm((5, 8, D), F32),
        vm((D // 2, 128), U32),
        vm((S, D), BF16),
        pltpu.SemaphoreType.DMA((19,)),
        pltpu.SemaphoreType.DMA(()),
    ]
    hbm = pl.BlockSpec(memory_space=pltpu.HBM)
    return pl.pallas_call(
        _kernel,
        out_shape=jax.ShapeDtypeStruct((1, S, D), BF16),
        in_specs=[hbm] * 12,
        out_specs=hbm,
        scratch_shapes=scratch,
        compiler_params=pltpu.CompilerParams(vmem_limit_bytes=110 * 2**20,
                                             disable_semaphore_checks=True,
                                             disable_bounds_checks=True),
        name="h3_mixer",
    )(A_q, A_k, A_v, A_shift_k.T, A_ssm_k, A_ssm_D, B_w1, B_w2, B_w3.T, B_w4, c, w_mod)
```

```python
import jax
import jax.numpy as jnp
import numpy as np
import jax.experimental.pallas as pl
import jax.experimental.pallas.tpu as pltpu

S, D, FF = 2048, 640, 1728
NT = D // 128
L = 512
NB = S // L
NFFT = 2 * L
R = 4
KPAD = 16
HPAD = 8
TB = 256
NBLK = S // TB
AO = 16
CH = 16
EPS = 1e-5
GATES = (0, 6, 7, 12, 15, 21, 22, 25, 28, 31, 33, 38, 42, 43, 44, 51)
W1A, W3A, W4A = 256, 1536, 384
FM = FF // 128 * 128
F32 = jnp.float32
BF16 = jnp.bfloat16
U32 = jnp.uint32
I32 = jnp.int32
NT_DIMS = (((1,), (1,)), ((), ()))
KP, XS, ZP = 0, 3, 3


def _cos_coefs(deg=6):
    u = (np.cos(np.pi * (np.arange(400) + 0.5) / 400) + 1.0) / 2.0
    c = np.polynomial.polynomial.polyfit(u, np.cos(np.pi * np.sqrt(u)), deg)
    return [np.float32(v) for v in c]


_COS = _cos_coefs()


def _cos_units(a, scale=1.0):
    x = (((a + 1024) & 2047) - 1024).astype(F32) * np.float32(1.0 / 1024.0)
    u = x * x
    acc = u * np.float32(_COS[-1] * scale) + np.float32(_COS[-2] * scale)
    for c in _COS[-3::-1]:
        acc = acc * u + np.float32(c * scale)
    return acc


def _freq2(chunk, s):
    e = 4 * (8 * (chunk >> 1) + s) + 1
    return jnp.where((chunk & 1) == 0, e, 256 - e)


def _gelu(x):
    c1 = np.float32(np.sqrt(2.0 / np.pi))
    c2 = np.float32(np.sqrt(2.0 / np.pi) * 0.044715)
    u = x * (c1 + c2 * (x * x))
    hx = 0.5 * x
    return hx + hx * jnp.tanh(u)


def _stats(x):
    m = jnp.sum(x, axis=-1, keepdims=True) * (1.0 / D)
    e2 = jnp.sum(x * x, axis=-1, keepdims=True) * (1.0 / D)
    v = jnp.maximum(e2 - m * m, 0.0)
    return m, jax.lax.rsqrt(v + EPS)


def _split(b):
    b = b.reshape(-1, 2, 8, 128)
    return b[:, 0], b[:, 1]


def _join(z):
    return jnp.stack(z, axis=1).reshape(-1, 128)


def _uneo(e, o):
    return jnp.stack([e, o], axis=1).reshape(16, 8, 128)


def _fft4(b, sign):
    (r0, i0), (r1, i1), (r2, i2), (r3, i3) = b
    sr, si, dr, di = r0 + r2, i0 + i2, r0 - r2, i0 - i2
    tr, ti, er, ei = r1 + r3, i1 + i3, r1 - r3, i1 - i3
    x0 = (sr + tr, si + ti)
    x2 = (sr - tr, si - ti)
    xm = (dr + ei, di - er)
    xp = (dr - ei, di + er)
    return [x0, xm, x2, xp] if sign < 0 else [x0, xp, x2, xm]


def _cmul(a, b, acc=None):
    (ar, ai), (br, bi) = a, b
    if acc is None:
        return ar * br - ai * bi, ar * bi + ai * br
    return (acc[0] + ar * br) - ai * bi, (acc[1] + ar * bi) + ai * br


def _bf(x):
    return pltpu.bitcast(x, BF16)


def _words(x):
    return pltpu.bitcast(x.astype(BF16), U32)


def _tie(w, ties):
    if not ties:
        return w
    parts = []
    for i in range(w.shape[0] // 8):
        p = w[8 * i:8 * i + 8]
        if i in ties:
            z = ties[i]
            p = p | z if p.shape[1] == 128 else jnp.concatenate([p[:, :128] | z, p[:, 128:]], axis=1)
        parts.append(p)
    return jnp.concatenate(parts, axis=0)


def _kernel(q_hbm, k_hbm, v_hbm, sk_hbm, ssm_hbm, sd_hbm, w1_hbm, w2_hbm, w3_hbm,
            w4_hbm, c_hbm, wm_hbm, o_hbm,
            qb, kb, vb, skb, ssmb, sdb, w1b, w2b, w3b, w4b, cb_, wmb, fwb, gib,
            stb, spec, yb, x1b, hb, eb, hpb, n4b, par, w3n, ob, sems, osem):
    groups = {}

    def add(name, src, dst):
        if name not in groups:
            groups[name] = (len(groups), [])
        idx, lst = groups[name]
        cp = pltpu.make_async_copy(src, dst, sems.at[idx])
        cp.start()
        lst.append(cp)

    def add_kv(name, c, tiles=range(NT)):
        for t in tiles:
            add(name, k_hbm.at[0, pl.ds(L * c, L), pl.ds(128 * t, 128)],
                kb.at[t, pl.ds(KPAD + L * c, L), :])
            add(name, v_hbm.at[0, pl.ds(L * c, L), pl.ds(128 * t, 128)],
                vb.at[t, pl.ds(L * c, L), :])

    def add_ssm(name, t):
        add(name, ssm_hbm.at[pl.ds(128 * t, 128), :], ssmb.bitcast(BF16).at[pl.ds(128 * t, 128), :])

    QE = 2 * TB + AO
    add_kv("ra", 0, [0])
    add("ra", sd_hbm, sdb)
    add("ra", sk_hbm, skb)
    add("ra", c_hbm, cb_)
    for t in range(NT):
        add_ssm(f"r{t}", t)
        add_kv(f"r{t}", (t + 1) // NT, [(t + 1) % NT])
    add_kv("r5", 1, range(1, NT))
    add_kv("r6", 2)
    add("wmA", q_hbm.at[0, pl.ds(0, QE), :], qb.bitcast(BF16).at[pl.ds(0, QE), :])
    add("wmA", wm_hbm.at[:, pl.ds(0, 3 * D)], wmb.at[:, pl.ds(0, 3 * D)])
    add("wmS", wm_hbm.at[:, pl.ds(3 * D, D + 256)], wmb.at[:, pl.ds(3 * D, D + 256)])
    add("wmB", wm_hbm.at[:, pl.ds(4 * D + 256, D - 256)], wmb.at[:, pl.ds(4 * D + 256, D - 256)])
    add("w1", w1_hbm.at[:, pl.ds(0, W1A)], w1b.bitcast(BF16).at[:, pl.ds(0, W1A)])
    add("w1b", w1_hbm.at[:, pl.ds(W1A, D - W1A)], w1b.bitcast(BF16).at[:, pl.ds(W1A, D - W1A)])
    add_kv("w1b", 3, [0])
    add("w2", w2_hbm, w2b.bitcast(BF16))
    add_kv("w2", 3, [1])
    add("w3", w3_hbm.at[pl.ds(0, W3A), :], w3b.bitcast(BF16).at[pl.ds(0, W3A), :])
    add("w4", w3_hbm.at[pl.ds(W3A, FF - W3A), :], w3b.bitcast(BF16).at[pl.ds(W3A, FF - W3A), :])
    add("w4", w4_hbm.at[:, pl.ds(0, W4A)], w4b.bitcast(BF16).at[:, pl.ds(0, W4A)])
    add_kv("w4", 3, [2, 3])
    add("rest", w4_hbm.at[:, pl.ds(W4A, D - W4A)], w4b.bitcast(BF16).at[:, pl.ds(W4A, D - W4A)])
    add_kv("rest", 3, [4])
    add("rest", wm_hbm.at[:, pl.ds(5 * D, D)], wmb.at[:, pl.ds(5 * D, D)])
    add("qnext", q_hbm.at[0, pl.ds(QE, TB), :], qb.bitcast(BF16).at[pl.ds(QE, TB), :])
    add("qlast", q_hbm.at[0, pl.ds(QE + TB, S - QE - TB), :],
        qb.bitcast(BF16).at[pl.ds(QE + TB, S - QE - TB), :])

    def wait(name):
        with jax.named_scope("W_" + name):
            for cp in groups[name][1]:
                cp.wait()

    kb[:, 0:KPAD, :] = jnp.zeros((NT, KPAD, 128), BF16)
    hpb[:, 0:HPAD, :] = jnp.zeros((NT, HPAD, 128), F32)
    yb[:, S:S + AO, :] = jnp.zeros((NT, AO, 128), F32)
    qb[S // 2:(S + AO) // 2, :] = jnp.zeros((AO // 2, D), U32)

    spec[7, 0, 0, pl.ds(0, 8, stride=2), :] = jnp.zeros((8, 128), F32)
    fwb[R, pl.ds(0, 8, stride=2), :] = jnp.zeros((8, 128), U32)
    gib[2 * R, pl.ds(0, 8, stride=2), :] = jnp.zeros((8, 128), U32)

    def make_tables(off):
        row = jax.lax.broadcasted_iota(I32, (256, 128), 0)
        col = jax.lax.broadcasted_iota(I32, (256, 128), 1)
        f2 = _freq2(row >> 4, row & 7)
        ph = 512 * ((row >> 3) & 1) + off
        m = (col & ~15) + 2 * (col & 7) + ((col >> 3) & 1)
        for r in range(R):
            fwb[r] = _words(_cos_units((4 * m + r) * f2 + ph))
        row = jax.lax.broadcasted_iota(I32, (64, 128), 0)
        col = jax.lax.broadcasted_iota(I32, (64, 128), 1)
        f2 = 4 * (8 * (col >> 4) + (col & 7)) + 1
        ph = 512 * ((col >> 3) & 1) + off
        for r in range(2 * R):
            gib[r] = _words(_cos_units((8 * row + r) * f2 + ph, 2.0 / NFFT))

    make_tables(0)

    env = {}

    def zero_after(*vals):
        acc = None
        for v in vals:
            v = pltpu.bitcast(v, U32)
            for i in range(0, v.shape[0], 8):
                for j in range(0, v.shape[1], 128):
                    p = v[i:i + 8, j:j + 128]
                    acc = p if acc is None else acc | p
        return acc & kb.bitcast(U32)[0, 0:8, :]

    def gated(v, z):
        zt = jnp.concatenate([jnp.concatenate([z] * NT, axis=1)] * (v.shape[0] // 8), axis=0)
        return pltpu.bitcast(v, U32) | zt

    def ld_spec(slot, t, q):
        return _split(spec[slot, t, q])

    def st_spec(slot, t, q, z):
        spec[slot, t, q] = _join(z)

    def fwd_dots(rhs, ties):
        return [_split(jnp.dot(_bf(_tie(fwb[r], ties if r == 0 else None)), rhs[r],
                               preferred_element_type=F32)) for r in range(R)]

    def conv_k(c, t, ties):
        w0 = L * c // 2
        stb[t, w0:w0 + L // 2, :] = pltpu.bitcast(
            _bf(ssmb[64 * t:64 * t + 64, L * c:L * c + L]).T, U32)
        rhs = []
        for h in range(2):
            lo = stb[t, pl.ds(w0 + h, 64, stride=4), :]
            hi = stb[t, pl.ds(w0 + h + 2, 64, stride=4), :]
            for e, o in zip(unpack(lo), unpack(hi)):
                rhs.append(_join((e.reshape(8, 8, 128), o.reshape(8, 8, 128))).astype(BF16))
        b = fwd_dots(rhs, ties)
        if c == 0:
            b[0] = (b[0][0] + env["dvec"][:, 128 * t:128 * t + 128][None], b[0][1])
        kq = _fft4(b, -1)
        z = []
        for q in range(R):
            kp = kq[q]
            if c >= 2:
                p = ld_spec(KP + c - 2, t, q)
                kp = (kp[0] + p[0], kp[1] + p[1])
            if c >= 1:
                p = ld_spec(KP + c - 1, t, q)
                if c == 3:
                    p0 = ld_spec(KP, t, q)
                    p = (p[0] - p0[0], p[1] - p0[1])
                (ree, reo), (ime, imo), (pre, pro), (pie, pio) = (_split(v) for v in kp + p)
                kp = (_uneo(ree - pie, reo + pio), _uneo(ime + pre, imo - pro))
            if c < 3:
                st_spec(KP + c, t, q, kp)
            zc = _cmul(kp, ld_spec(XS, t, q))
            if c == 0:
                z.append(zc)
            else:
                st_spec(ZP + c, t, q, zc)
        if c == 0:
            finish(0, t, z)

    def finish(c, t, z):
        hs = np.float32(np.sqrt(0.5))
        cr = _fft4(z, +1)
        for r in range(R):
            (ar, br), (ai, bi) = _split(cr[r][0]), _split(cr[r][1])
            if r % 2:
                br, bi = (br - bi) * hs, (br + bi) * hs
            if r < 2:
                p, m = (ar + br, ai - bi), (ar - br, ai + bi)
            else:
                p, m = (ar - bi, ai - br), (ar + bi, ai + br)
            env["cm", c, t, r] = _join(p).astype(BF16)
            env["cm", c, t, r + R] = _join(m).astype(BF16)

    def unpack(u):
        return (pltpu.bitcast(u << 16, F32),
                pltpu.bitcast(u & jnp.uint32(0xFFFF0000), F32))

    def conv_prep(c, t):
        taps = env["taps"]
        ku = kb.bitcast(U32)
        vu = vb.bitcast(U32)
        tp = [taps[j:j + 1, 128 * t:128 * t + 128] for j in range(4)]
        w0 = (KPAD + L * c) // 2
        kk = [unpack(ku[t, pl.ds(w0 - 2, 64, stride=4), :])[1]]
        for o in range(-1, 4):
            kk += unpack(ku[t, pl.ds(w0 + o, 64, stride=4), :])
        vv = []
        for o in range(4):
            vv += unpack(vu[t, pl.ds(L * c // 2 + o, 64, stride=4), :])
        kv = []
        for n in range(8):
            acc = kk[3 + n] * tp[0]
            for j in range(1, 4):
                acc = acc + kk[3 + n - j] * tp[j]
            kv.append(acc * vv[n])
        return [_join((kv[r].reshape(8, 8, 128), kv[r + 4].reshape(8, 8, 128))) for r in range(R)]

    def conv_x(c, t, ties):
        xq = _fft4(fwd_dots([v.astype(BF16) for v in env.pop(("kv", c, t))], ties), -1)
        z = []
        for q in range(R):
            if c == 0:
                st_spec(XS, t, q, xq[q])
                continue
            for a in range(c, NB):
                if (c, a) == (1, 2):
                    st_spec(XS, t, q, xq[q])
                    continue
                za = _cmul(xq[q], ld_spec(KP + a - c, t, q), ld_spec(ZP + a, t, q))
                if (c, a) == (2, 2):
                    za = _cmul(ld_spec(XS, t, q), ld_spec(KP + 1, t, q), za)
                if a == c:
                    z.append(za)
                else:
                    st_spec(ZP + a, t, q, za)
        if c:
            finish(c, t, z)

    def conv_inv(c, t, ties):
        for r in range(2 * R):
            tr = None
            if ties and r % R == 0:
                tr = {i - r: z for i, z in ties.items() if 0 <= i - r < 4}
            yb[t, pl.ds(L * c + r, 64, stride=2 * R), :] = jnp.dot(
                _bf(_tie(gib[r], tr)), env.pop(("cm", c, t, r)), preferred_element_type=F32)

    def run_rounds(spec_str):
        rounds = spec_str.split()
        slots = []
        plan = {}
        for n, rd in enumerate(rounds):
            if rd[0] == "X":
                pts = []
                if "@" in rd:
                    a, b = (int(v) for v in rd[4:].split(":"))
                    pts = [slots[len(slots) - a + (a - b) * (j + 1) // 8 - 1] for j in range(8)]
                plan.setdefault(pts[0][0] if pts else n, []).append((rd, pts))
            slots += [(n, i) for i in range(8 if rd[0] == "I" else 16)]
        ties = {}
        for n, rd in enumerate(rounds):
            for xr, pts in plan.get(n, []):
                c, t = int(xr[1]), int(xr[2])
                kv = env["kv", c, t] = conv_prep(c, t)
                for j, (pn, pi) in enumerate(pts):
                    z = zero_after(*[w[16 * j:16 * j + 16] for w in kv])
                    d = ties.setdefault(pn, {})
                    d[pi] = z if pi not in d else d[pi] | z
            {"K": conv_k, "X": conv_x, "I": conv_inv}[rd[0]](int(rd[1]), int(rd[2]), ties.get(n))

    def rows(r0, n, align=8):
        if isinstance(r0, int):
            return slice(r0, r0 + n)
        return pl.ds(pl.multiple_of(r0, align), n)

    def ld_y(r0, n):
        return jnp.concatenate([yb[t, rows(r0, n), :] for t in range(NT)], axis=-1)

    def prm(i, n=CH, c0=0, c1=D):
        return jnp.concatenate([par[i, :, c0:c1]] * (n // 8), axis=0)

    def a_pre12(r0, n):
        x = _bf(qb[r0 // 2:(r0 + n) // 2, :]).astype(F32)
        m1, r1 = _stats(x)
        x1 = x + ((x - m1) * r1 * prm(0, n) + prm(1, n)) * ld_y(r0, n)
        x1b[r0:r0 + n, :] = x1
        m2, r2 = _stats(x1)
        hb[r0:r0 + n, :] = (x1 - m2) * r2

    def a_pre3(r0, m):
        h = hb[r0:r0 + m, :] * prm(2, m) + prm(3, m)
        hb[r0:r0 + m, :] = h
        m3, r3 = _stats(h)
        return (h - m3) * r3

    def halves(n, split):
        m = n // split if split else n
        return [(o, m) for o in range(0, n, m)]

    def mm1(r0, n, n3, split_last=0, tiles=range(NT)):
        for t in tiles:
            w = w1b[:, 128 * t:128 * t + 128]
            for o, m in halves(n, split_last if t == tiles[-1] else 0):
                hp = jnp.dot(n3[o:o + m].astype(BF16), _bf(w), preferred_element_type=F32)
                hpb[t, rows(HPAD + r0 + o, m), :] = _gelu(hp)

    def g_prep(r0):
        lane = jax.lax.broadcasted_iota(I32, (TB, 128), 1)
        sh = [-1, 1, -2, 2]

        def ldh(t, g):
            return hpb[t, pl.ds(HPAD + r0 + sh[g], TB), :]

        cols = [ldh(0, 0)]
        for t in range(1, 4):
            cols.append(jnp.where(lane < 32 * t, ldh(t, t - 1), ldh(t, t)))
        cols.append(ldh(4, 3))
        return jnp.concatenate(cols, axis=-1)

    def mm2(r0, g, split_last=0, side=None):
        for t in range(NT):
            if side and t in side:
                side[t]()
            c0, c1 = 128 * t, 128 * t + 128
            for o, m in halves(TB, split_last if t == NT - 1 else 0):
                hs = jnp.dot(g[o:o + m].astype(BF16), _bf(w2b[:, c0:c1]), preferred_element_type=F32)
                hb[rows(r0 + o, m), c0:c1] = hb[rows(r0 + o, m), c0:c1] + hs
        return hs[m - 8:m]

    def mm3(n4, ties=None, split_at=None, side=None, tpos=12, nat=True):
        us = []
        env["g3"] = []
        for j in range(FF // 128):
            if side and j in side:
                side[j]()
            if j == tpos:
                ht = jax.lax.dot_general(_bf(w3b[FM // 2:FF // 2, :]), n4.astype(BF16), NT_DIMS,
                                         preferred_element_type=F32)
                ut = _gelu(ht).T
            w = w3b[64 * j:64 * j + 64, :]
            if ties and j in ties:
                w = _tie(w, {0: ties[j]})
            parts = []
            for o, m in halves(TB, 2 if j == split_at else 0):
                if j == 0 and nat:
                    h3 = jnp.dot(n4.astype(BF16), _bf(w3n[...]), preferred_element_type=F32)
                else:
                    h3 = jax.lax.dot_general(n4[o:o + m].astype(BF16), _bf(w), NT_DIMS,
                                             preferred_element_type=F32)
                parts.append(_gelu(h3))
                if m == TB:
                    env["g3"] += [h3[o:o + 8] for o in range(0, TB, 64)]
            us.append(jnp.concatenate(parts, axis=0))
        return jnp.concatenate(us + [ut], axis=-1)

    def mm4(r0, u, t, final=True, split=0, side=None):
        c0, c1 = 128 * t, 128 * t + 128
        w = _bf(w4b[:, c0:c1])
        for o, m in halves(TB, split):
            if o and side:
                side()
            h2 = jnp.dot(u[o:o + m].astype(BF16), w, preferred_element_type=F32)
            s = hb[rows(r0 + o, m), c0:c1] + h2
            if final:
                ob[rows(r0 + o, m, 16), c0:c1] = (
                    x1b[rows(r0 + o, m), c0:c1] + prm(4, m, c0, c1) * s).astype(BF16)
            else:
                hb[rows(r0 + o, m), c0:c1] = s

    def ln4_store(r0, nch):
        zs = []
        m = TB // nch
        for j in range(nch):
            x2 = hb[r0 + m * j:r0 + m * j + m, :]
            m4, r4 = _stats(x2)
            n4 = (x2 - m4) * r4
            n4b[m * j:m * j + m, :] = n4
            zs.append(zero_after(n4))
        return zs

    def out_copy(r0, n, c0=0, c1=D):
        return pltpu.make_async_copy(ob.at[rows(r0, n, 16), c0:c1],
                                     o_hbm.at[0, rows(r0, n, 16), c0:c1], osem)

    wait("ra")
    env["taps"] = skb[...].astype(F32)
    env["dvec"] = sdb[...].astype(F32).reshape(1, D)
    cf = cb_[...].astype(F32)
    sc8 = jnp.broadcast_to(cf * jax.nn.sigmoid(cf), (8, D)).astype(BF16)
    run_rounds("X00")
    wait("r0")
    run_rounds("X01 K00 K10 K20 K30")
    for t in range(1, NT):
        wait(f"r{t}")
        run_rounds(f"I0{t - 1} X{(t + 1) // NT}{(t + 1) % NT} K0{t} K1{t} K2{t} K3{t}")
    wait("r5")
    run_rounds("I04 X11 I10 X12@20:3 I11 X13@20:3 I12 X14@20:3")
    wait("r6")
    run_rounds("I13 X20 I14 X21@24:14 I20 X22@24:14 I21 X23@24:14 I22 X24@24:14 I23")

    flag = kb.bitcast(I32)[0, 0:8, :][0, 0]
    pl.when(flag != 0)(lambda: make_tables(2 * NFFT * flag))
    wait("wmA")
    mod = jnp.dot(sc8, wmb[:, 0:3 * D], preferred_element_type=F32)
    sa, ca, ga = [mod[:, D * i:D * (i + 1)] for i in range(3)]
    par[0] = (1.0 + ca) * ga
    par[1] = sa * ga
    run_rounds("I24")
    a_pre12(0, TB + AO)
    a_pre12(TB + AO, TB)
    wait("wmS")
    mod = jnp.dot(sc8, wmb[:, 3 * D:4 * D + 256], preferred_element_type=F32)
    par[3] = mod[:, 0:D]
    par[2, :, 0:256] = 1.0 + mod[:, D:D + 256]
    wait("wmB")
    par[2, :, 256:D] = 1.0 + jnp.dot(sc8, wmb[:, 4 * D + 256:5 * D], preferred_element_type=F32)
    n3p = a_pre3(0, 128)

    ta, tb = range(W1A // 128), range(W1A // 128, NT)
    wait("w1")
    n3 = jnp.concatenate([n3p, a_pre3(128, QE - 128)], axis=0)
    for a, b in ((0, 128), (128, 256), (256, 400), (400, QE)):
        mm1(a, b - a, n3[a:b], tiles=ta)
    wait("w1b")
    mm1(0, TB + AO, n3[:TB + AO], tiles=tb)
    run_rounds("X30")
    mm1(TB + AO, TB, n3[TB + AO:], split_last=4, tiles=tb)
    wait("w2")
    z = zero_after(mm2(0, g_prep(0), side={4: lambda: run_rounds("X31")}))
    n4 = []
    for j in range(8):
        xx = pltpu.bitcast(gated(hb[32 * j:32 * j + 32, :], z), F32)
        m4, r4 = _stats(xx)
        n4.append((xx - m4) * r4)
        if j >= 3:
            z = z | zero_after(n4[j - 3])
        z = pltpu.roll(z, 1, 1)
    n4 = jnp.concatenate(n4, axis=0)
    mm2(TB, g_prep(TB), split_last=2)
    wait("w3")
    zs = ln4_store(TB, 8)
    w3n[...] = pltpu.bitcast(_bf(w3b[0:64, :]).T, U32)
    run_rounds("I30")

    def mid():
        wait("w4")
        run_rounds("I31")

    u = mm3(n4, {3 + j: z for j, z in enumerate(zs)}, split_at=W3A // 128 - 1, nat=False,
            side={W3A // 128: mid})
    mm4(0, u, 0, final=False)
    run_rounds("X32")
    run_rounds("X33")
    mm4(0, u, 1, final=False)
    mm4(0, u, 2, final=False)
    run_rounds("I32")
    wait("rest")

    def gb_tiles(*ts):
        for t in ts:
            par[4, :, 128 * t:128 * t + 128] = jnp.dot(
                sc8, wmb[:, 5 * D + 128 * t:5 * D + 128 * t + 128], preferred_element_type=F32)

    def finalize(t):
        c0, c1 = 128 * t, 128 * t + 128
        if c0 < W4A:
            ob[0:TB, c0:c1] = (x1b[0:TB, c0:c1] + prm(4, TB, c0, c1) * hb[0:TB, c0:c1]).astype(BF16)
        eb[TB:2 * TB, c0:c1] = x1b[TB:2 * TB, c0:c1] + prm(4, TB, c0, c1) * hb[TB:2 * TB, c0:c1]

    run_rounds("I33")
    gb_tiles(3, 4, 0)
    mm4(0, u, 3, split=2, side=lambda: run_rounds("X34"))
    gb_tiles(1)
    mm4(0, u, 4, split=2, side=lambda: gb_tiles(2))
    for t in range(NT - 1):
        finalize(t)
    run_rounds("I34")
    finalize(NT - 1)
    out_copy(0, TB).start()
    wait("qnext")

    def mm4e(ev, ov, u, t, split=0):
        c0, c1 = 128 * t, 128 * t + 128
        for o, m in halves(TB, split):
            h2 = jnp.dot(u[o:o + m].astype(BF16), _bf(w4b[:, c0:c1]), preferred_element_type=F32)
            ov[o:o + m, c0:c1] = (ev[o:o + m, c0:c1] + prm(4, m, c0, c1) * h2).astype(BF16)

    def body(i, carry):
        pl.when(i == 2)(lambda: wait("qlast"))
        r0 = pl.multiple_of(i * TB, TB)
        ev = eb.at[pl.ds(r0, 2 * TB), :]
        ov = ob.at[pl.ds(r0, TB), :]
        u = mm3(n4b[...])
        hpb[:, TB:TB + HPAD + AO, :] = hpb[:, 2 * TB:2 * TB + HPAD + AO, :]
        x1s, hs, n3 = [x1b[2 * TB:QE, :]], [hb[2 * TB:QE, :]], []
        for j in range(TB // CH):
            r = r0 + TB + AO + CH * j
            z = zero_after(env["g3"][GATES[j]])
            x = _bf(gated(qb[rows(r // 2, CH // 2), :], z)).astype(F32)
            m1, r1 = _stats(x)
            x1 = x + ((x - m1) * r1 * prm(0) + prm(1)) * ld_y(r, CH)
            m2, r2 = _stats(x1)
            h = (x1 - m2) * r2 * prm(2) + prm(3)
            m3, r3 = _stats(h)
            n3.append((h - m3) * r3)
            x1s.append(x1)
            hs.append(h)
        x1b[2 * TB:QE, :] = x1s[-1]
        hb[2 * TB:QE, :] = hs[-1]
        mm4e(ev, ov, u, 0)
        mm1(TB + AO, TB, jnp.concatenate(n3, axis=0))
        zrow = pl.multiple_of(jnp.where(i == NBLK - 2, HPAD + 2 * TB, HPAD + QE), 8)
        hpb[:, pl.ds(zrow, 8), :] = jnp.zeros((NT, 8, 128), F32)
        mm4e(ev, ov, u, 1)
        g = g_prep(TB).astype(BF16)
        hcat = jnp.concatenate(hs[:-1], axis=0)
        x2 = []
        for t in range(NT):
            mix = jnp.dot(g, _bf(w2b[:, 128 * t:128 * t + 128]), preferred_element_type=F32)
            x2.append(hcat[:, 128 * t:128 * t + 128] + mix)
        x2 = jnp.concatenate(x2, axis=-1)
        z = zero_after(mix[0:8])
        for j in range(TB // CH):
            xx = pltpu.bitcast(gated(x2[CH * j:CH * j + CH], z), F32)
            m4, r4 = _stats(xx)
            n4b[CH * j:CH * j + CH, :] = (xx - m4) * r4
            ev[TB + CH * j:TB + CH * j + CH, :] = x1s[j] + prm(4) * xx
            z = pltpu.roll(z, 1, 1)
        for t in range(2, NT):
            mm4e(ev, ov, u, t)
        out_copy(r0, TB).start()
        return carry

    jax.lax.fori_loop(1, NBLK - 1, body, 0)

    r0 = S - TB
    u = mm3(n4b[...])
    for t in range(NT):
        mm4e(eb.at[r0:S, :], ob.at[r0:S, :], u, t, split=2 if t == NT - 1 else 0)
        if t < NT - 1:
            out_copy(r0, TB, 128 * t, 128 * t + 128).start()
    out_copy(r0, TB // 2, D - 128, D).start()
    out_copy(r0 + TB // 2, TB // 2, D - 128, D).start()
    with jax.named_scope("W_out"):
        pltpu.make_async_copy(ob, o_hbm.at[0], osem).wait()


@jax.jit
def pallas_adaLN_cond__ssm_conv_h3__mixer_s_mlp__prompt_kernel(
    A_q, A_k, A_v, A_shift_k, A_ssm_k, A_ssm_D, B_x, B_w1, B_w2, B_w3, B_w4, c, w_mod,
):
    del B_x
    vm = pltpu.VMEM
    scratch = [
        vm(((S + AO) // 2, D), U32),
        vm((NT, KPAD + S, 128), BF16),
        vm((NT, S, 128), BF16),
        vm((4, D), BF16),
        vm((D // 2, S), U32),
        vm((D,), BF16),
        vm((D // 2, D), U32),
        vm((D // 2, D), U32),
        vm((FF // 2, D), U32),
        vm((FF // 2, D), U32),
        vm((1, D), BF16),
        vm((D, 6 * D), BF16),
        vm((R + 1, 128, 128), U32),
        vm((2 * R + 1, 32, 128), U32),
        vm((NT, S // 2, 128), U32),
        vm((8, NT, R, 256, 128), F32),
        vm((NT, S + AO + 16, 128), F32),
        vm((2 * TB + AO, D), F32),
        vm((2 * TB + AO, D), F32),
        vm((S + 8, D), F32),
        vm((NT, HPAD + 2 * TB + AO + 8, 128), F32),
        vm((TB, D), F32),
        vm((5, 8, D), F32),
        vm((D // 2, 128), U32),
        vm((S, D), BF16),
        pltpu.SemaphoreType.DMA((19,)),
        pltpu.SemaphoreType.DMA(()),
    ]
    hbm = pl.BlockSpec(memory_space=pltpu.HBM)
    return pl.pallas_call(
        _kernel,
        out_shape=jax.ShapeDtypeStruct((1, S, D), BF16),
        in_specs=[hbm] * 12,
        out_specs=hbm,
        scratch_shapes=scratch,
        compiler_params=pltpu.CompilerParams(vmem_limit_bytes=110 * 2**20,
                                             disable_semaphore_checks=True,
                                             disable_bounds_checks=True),
        name="h3_mixer",
    )(A_q, A_k, A_v, A_shift_k.T, A_ssm_k, A_ssm_D, B_w1, B_w2, B_w3.T, B_w4, c, w_mod)
```

```python
import jax
import jax.numpy as jnp
import numpy as np
import jax.experimental.pallas as pl
import jax.experimental.pallas.tpu as pltpu

S, D, FF = 2048, 640, 1728
NT = D // 128
L = 512
NB = S // L
NFFT = 2 * L
R = 4
KPAD = 16
HPAD = 8
TB = 256
NBLK = S // TB
AO = 16
CH = 16
EPS = 1e-5
GATES = (0, 6, 7, 12, 15, 21, 22, 25, 28, 31, 33, 38, 42, 43, 44, 51)
W1A, W3A, W4A = 256, 1536, 384
FM = FF // 128 * 128
F32 = jnp.float32
BF16 = jnp.bfloat16
U32 = jnp.uint32
I32 = jnp.int32
NT_DIMS = (((1,), (1,)), ((), ()))
KP, XS, ZP = 0, 3, 3


def _cos_coefs(deg=6):
    u = (np.cos(np.pi * (np.arange(400) + 0.5) / 400) + 1.0) / 2.0
    c = np.polynomial.polynomial.polyfit(u, np.cos(np.pi * np.sqrt(u)), deg)
    return [np.float32(v) for v in c]


_COS = _cos_coefs()


def _cos_units(a, scale=1.0):
    x = (((a + 1024) & 2047) - 1024).astype(F32) * np.float32(1.0 / 1024.0)
    u = x * x
    acc = u * np.float32(_COS[-1] * scale) + np.float32(_COS[-2] * scale)
    for c in _COS[-3::-1]:
        acc = acc * u + np.float32(c * scale)
    return acc


def _freq2(chunk, s):
    e = 4 * (8 * (chunk >> 1) + s) + 1
    return jnp.where((chunk & 1) == 0, e, 256 - e)


def _gelu(x):
    c1 = np.float32(np.sqrt(2.0 / np.pi))
    c2 = np.float32(np.sqrt(2.0 / np.pi) * 0.044715)
    u = x * (c1 + c2 * (x * x))
    hx = 0.5 * x
    return hx + hx * jnp.tanh(u)


def _stats(x):
    m = jnp.sum(x, axis=-1, keepdims=True) * (1.0 / D)
    e2 = jnp.sum(x * x, axis=-1, keepdims=True) * (1.0 / D)
    v = jnp.maximum(e2 - m * m, 0.0)
    return m, jax.lax.rsqrt(v + EPS)


def _split(b):
    b = b.reshape(-1, 2, 8, 128)
    return b[:, 0], b[:, 1]


def _join(z):
    return jnp.stack(z, axis=1).reshape(-1, 128)


def _uneo(e, o):
    return jnp.stack([e, o], axis=1).reshape(16, 8, 128)


def _fft4(b, sign):
    (r0, i0), (r1, i1), (r2, i2), (r3, i3) = b
    sr, si, dr, di = r0 + r2, i0 + i2, r0 - r2, i0 - i2
    tr, ti, er, ei = r1 + r3, i1 + i3, r1 - r3, i1 - i3
    x0 = (sr + tr, si + ti)
    x2 = (sr - tr, si - ti)
    xm = (dr + ei, di - er)
    xp = (dr - ei, di + er)
    return [x0, xm, x2, xp] if sign < 0 else [x0, xp, x2, xm]


def _cmul(a, b, acc=None):
    (ar, ai), (br, bi) = a, b
    if acc is None:
        return ar * br - ai * bi, ar * bi + ai * br
    return (acc[0] + ar * br) - ai * bi, (acc[1] + ar * bi) + ai * br


def _bf(x):
    return pltpu.bitcast(x, BF16)


def _words(x):
    return pltpu.bitcast(x.astype(BF16), U32)


def _tie(w, ties):
    if not ties:
        return w
    parts = []
    for i in range(w.shape[0] // 8):
        p = w[8 * i:8 * i + 8]
        if i in ties:
            z = ties[i]
            p = p | z if p.shape[1] == 128 else jnp.concatenate([p[:, :128] | z, p[:, 128:]], axis=1)
        parts.append(p)
    return jnp.concatenate(parts, axis=0)


def _kernel(q_hbm, k_hbm, v_hbm, sk_hbm, ssm_hbm, sd_hbm, w1_hbm, w2_hbm, w3_hbm,
            w4_hbm, c_hbm, wm_hbm, o_hbm,
            qb, kb, vb, skb, ssmb, sdb, w1b, w2b, w3b, w4b, cb_, wmb, fwb, gib,
            stb, spec, yb, x1b, hb, eb, hpb, n4b, par, w3n, ob, sems, osem):
    groups = {}

    def add(name, src, dst):
        if name not in groups:
            groups[name] = (len(groups), [])
        idx, lst = groups[name]
        cp = pltpu.make_async_copy(src, dst, sems.at[idx])
        cp.start()
        lst.append(cp)

    def add_kv(name, c, tiles=range(NT)):
        for t in tiles:
            add(name, k_hbm.at[0, pl.ds(L * c, L), pl.ds(128 * t, 128)],
                kb.at[t, pl.ds(KPAD + L * c, L), :])
            add(name, v_hbm.at[0, pl.ds(L * c, L), pl.ds(128 * t, 128)],
                vb.at[t, pl.ds(L * c, L), :])

    def add_ssm(name, t):
        add(name, ssm_hbm.at[pl.ds(128 * t, 128), :], ssmb.bitcast(BF16).at[pl.ds(128 * t, 128), :])

    QE = 2 * TB + AO
    add_kv("ra", 0, [0])
    add("ra", sd_hbm, sdb)
    add("ra", sk_hbm, skb)
    add("ra", c_hbm, cb_)
    for t in range(NT):
        add_ssm(f"r{t}", t)
        add_kv(f"r{t}", (t + 1) // NT, [(t + 1) % NT])
    add_kv("r5", 1, range(1, NT))
    add_kv("r6", 2)
    add("wmA", q_hbm.at[0, pl.ds(0, QE), :], qb.bitcast(BF16).at[pl.ds(0, QE), :])
    add("wmA", wm_hbm.at[:, pl.ds(0, 3 * D)], wmb.at[:, pl.ds(0, 3 * D)])
    add("wmS", wm_hbm.at[:, pl.ds(3 * D, D + 256)], wmb.at[:, pl.ds(3 * D, D + 256)])
    add("wmB", wm_hbm.at[:, pl.ds(4 * D + 256, D - 256)], wmb.at[:, pl.ds(4 * D + 256, D - 256)])
    add("w1", w1_hbm.at[:, pl.ds(0, W1A)], w1b.bitcast(BF16).at[:, pl.ds(0, W1A)])
    add("w1b", w1_hbm.at[:, pl.ds(W1A, D - W1A)], w1b.bitcast(BF16).at[:, pl.ds(W1A, D - W1A)])
    add_kv("w1b", 3, [0])
    add("w2", w2_hbm, w2b.bitcast(BF16))
    add_kv("w2", 3, [1])
    add("w3", w3_hbm.at[pl.ds(0, W3A), :], w3b.bitcast(BF16).at[pl.ds(0, W3A), :])
    add("w4", w3_hbm.at[pl.ds(W3A, FF - W3A), :], w3b.bitcast(BF16).at[pl.ds(W3A, FF - W3A), :])
    add("w4", w4_hbm.at[:, pl.ds(0, W4A)], w4b.bitcast(BF16).at[:, pl.ds(0, W4A)])
    add_kv("w4", 3, [2, 3])
    add("rest", w4_hbm.at[:, pl.ds(W4A, D - W4A)], w4b.bitcast(BF16).at[:, pl.ds(W4A, D - W4A)])
    add_kv("rest", 3, [4])
    add("rest", wm_hbm.at[:, pl.ds(5 * D, D)], wmb.at[:, pl.ds(5 * D, D)])
    add("qnext", q_hbm.at[0, pl.ds(QE, TB), :], qb.bitcast(BF16).at[pl.ds(QE, TB), :])
    add("qlast", q_hbm.at[0, pl.ds(QE + TB, S - QE - TB), :],
        qb.bitcast(BF16).at[pl.ds(QE + TB, S - QE - TB), :])

    def wait(name):
        with jax.named_scope("W_" + name):
            for cp in groups[name][1]:
                cp.wait()

    kb[:, 0:KPAD, :] = jnp.zeros((NT, KPAD, 128), BF16)
    hpb[:, 0:HPAD, :] = jnp.zeros((NT, HPAD, 128), F32)
    qb[S // 2:(S + AO) // 2, :] = jnp.zeros((AO // 2, D), U32)

    spec[7, 0, 0, pl.ds(0, 8, stride=2), :] = jnp.zeros((8, 128), F32)
    fwb[R, pl.ds(0, 8, stride=2), :] = jnp.zeros((8, 128), U32)
    gib[2 * R, pl.ds(0, 8, stride=2), :] = jnp.zeros((8, 128), U32)

    row = jax.lax.broadcasted_iota(I32, (256, 128), 0)
    col = jax.lax.broadcasted_iota(I32, (256, 128), 1)
    f2 = _freq2(row >> 4, row & 7)
    ph = 512 * ((row >> 3) & 1)
    m = (col & ~15) + 2 * (col & 7) + ((col >> 3) & 1)
    for r in range(R):
        fwb[r] = _words(_cos_units((4 * m + r) * f2 + ph))
    row = jax.lax.broadcasted_iota(I32, (64, 128), 0)
    col = jax.lax.broadcasted_iota(I32, (64, 128), 1)
    f2 = 4 * (8 * (col >> 4) + (col & 7)) + 1
    ph = 512 * ((col >> 3) & 1)
    for r in range(2 * R):
        gib[r] = _words(_cos_units((8 * row + r) * f2 + ph, 2.0 / NFFT))

    env = {}

    def zero_after(*vals):
        acc = None
        for v in vals:
            v = pltpu.bitcast(v, U32)
            for i in range(0, v.shape[0], 8):
                for j in range(0, v.shape[1], 128):
                    p = v[i:i + 8, j:j + 128]
                    acc = p if acc is None else acc | p
        return acc & kb.bitcast(U32)[0, 0:8, :]

    def gated(v, z):
        zt = jnp.concatenate([jnp.concatenate([z] * NT, axis=1)] * (v.shape[0] // 8), axis=0)
        return pltpu.bitcast(v, U32) | zt

    def ld_spec(slot, t, q):
        return _split(spec[slot, t, q])

    def st_spec(slot, t, q, z):
        spec[slot, t, q] = _join(z)

    def fwd_dots(rhs, ties):
        return [_split(jnp.dot(_bf(_tie(fwb[r], ties if r == 0 else None)), rhs[r],
                               preferred_element_type=F32)) for r in range(R)]

    def conv_k(c, t, ties):
        w0 = L * c // 2
        stb[t, w0:w0 + L // 2, :] = pltpu.bitcast(
            _bf(ssmb[64 * t:64 * t + 64, L * c:L * c + L]).T, U32)
        rhs = []
        for h in range(2):
            lo = stb[t, pl.ds(w0 + h, 64, stride=4), :]
            hi = stb[t, pl.ds(w0 + h + 2, 64, stride=4), :]
            for e, o in zip(unpack(lo), unpack(hi)):
                rhs.append(_join((e.reshape(8, 8, 128), o.reshape(8, 8, 128))).astype(BF16))
        b = fwd_dots(rhs, ties)
        if c == 0:
            b[0] = (b[0][0] + env["dvec"][:, 128 * t:128 * t + 128][None], b[0][1])
        kq = _fft4(b, -1)
        z = []
        for q in range(R):
            kp = kq[q]
            if c >= 2:
                p = ld_spec(KP + c - 2, t, q)
                kp = (kp[0] + p[0], kp[1] + p[1])
            if c >= 1:
                p = ld_spec(KP + c - 1, t, q)
                if c == 3:
                    p0 = ld_spec(KP, t, q)
                    p = (p[0] - p0[0], p[1] - p0[1])
                (ree, reo), (ime, imo), (pre, pro), (pie, pio) = (_split(v) for v in kp + p)
                kp = (_uneo(ree - pie, reo + pio), _uneo(ime + pre, imo - pro))
            if c < 3:
                st_spec(KP + c, t, q, kp)
            zc = _cmul(kp, ld_spec(XS, t, q))
            if c == 0:
                z.append(zc)
            else:
                st_spec(ZP + c, t, q, zc)
        if c == 0:
            finish(0, t, z)

    def finish(c, t, z):
        hs = np.float32(np.sqrt(0.5))
        cr = _fft4(z, +1)
        for r in range(R):
            (ar, br), (ai, bi) = _split(cr[r][0]), _split(cr[r][1])
            if r % 2:
                br, bi = (br - bi) * hs, (br + bi) * hs
            if r < 2:
                p, m = (ar + br, ai - bi), (ar - br, ai + bi)
            else:
                p, m = (ar - bi, ai - br), (ar + bi, ai + br)
            env["cm", c, t, r] = _join(p).astype(BF16)
            env["cm", c, t, r + R] = _join(m).astype(BF16)

    def unpack(u):
        return (pltpu.bitcast(u << 16, F32),
                pltpu.bitcast(u & jnp.uint32(0xFFFF0000), F32))

    def conv_prep(c, t):
        taps = env["taps"]
        ku = kb.bitcast(U32)
        vu = vb.bitcast(U32)
        tp = [taps[j:j + 1, 128 * t:128 * t + 128] for j in range(4)]
        w0 = (KPAD + L * c) // 2
        kk = [unpack(ku[t, pl.ds(w0 - 2, 64, stride=4), :])[1]]
        for o in range(-1, 4):
            kk += unpack(ku[t, pl.ds(w0 + o, 64, stride=4), :])
        vv = []
        for o in range(4):
            vv += unpack(vu[t, pl.ds(L * c // 2 + o, 64, stride=4), :])
        kv = []
        for n in range(8):
            acc = kk[3 + n] * tp[0]
            for j in range(1, 4):
                acc = acc + kk[3 + n - j] * tp[j]
            kv.append(acc * vv[n])
        return [_join((kv[r].reshape(8, 8, 128), kv[r + 4].reshape(8, 8, 128))) for r in range(R)]

    def conv_x(c, t, ties):
        xq = _fft4(fwd_dots([v.astype(BF16) for v in env.pop(("kv", c, t))], ties), -1)
        z = []
        for q in range(R):
            if c == 0:
                st_spec(XS, t, q, xq[q])
                continue
            for a in range(c, NB):
                if (c, a) == (1, 2):
                    st_spec(XS, t, q, xq[q])
                    continue
                za = _cmul(xq[q], ld_spec(KP + a - c, t, q), ld_spec(ZP + a, t, q))
                if (c, a) == (2, 2):
                    za = _cmul(ld_spec(XS, t, q), ld_spec(KP + 1, t, q), za)
                if a == c:
                    z.append(za)
                else:
                    st_spec(ZP + a, t, q, za)
        if c:
            finish(c, t, z)

    def conv_inv(c, t, ties):
        for r in range(2 * R):
            tr = None
            if ties and r % R == 0:
                tr = {i - r: z for i, z in ties.items() if 0 <= i - r < 4}
            yb[t, pl.ds(L * c + r, 64, stride=2 * R), :] = jnp.dot(
                _bf(_tie(gib[r], tr)), env.pop(("cm", c, t, r)), preferred_element_type=F32)

    def run_rounds(spec_str):
        rounds = spec_str.split()
        slots = []
        plan = {}
        for n, rd in enumerate(rounds):
            if rd[0] == "X":
                pts = []
                if "@" in rd:
                    a, b = (int(v) for v in rd[4:].split(":"))
                    pts = [slots[len(slots) - a + (a - b) * (j + 1) // 8 - 1] for j in range(8)]
                plan.setdefault(pts[0][0] if pts else n, []).append((rd, pts))
            slots += [(n, i) for i in range(8 if rd[0] == "I" else 16)]
        ties = {}
        for n, rd in enumerate(rounds):
            for xr, pts in plan.get(n, []):
                c, t = int(xr[1]), int(xr[2])
                kv = env["kv", c, t] = conv_prep(c, t)
                for j, (pn, pi) in enumerate(pts):
                    z = zero_after(*[w[16 * j:16 * j + 16] for w in kv])
                    d = ties.setdefault(pn, {})
                    d[pi] = z if pi not in d else d[pi] | z
            {"K": conv_k, "X": conv_x, "I": conv_inv}[rd[0]](int(rd[1]), int(rd[2]), ties.get(n))

    def rows(r0, n, align=8):
        if isinstance(r0, int):
            return slice(r0, r0 + n)
        return pl.ds(pl.multiple_of(r0, align), n)

    def ld_y(r0, n):
        return jnp.concatenate([yb[t, rows(r0, n), :] for t in range(NT)], axis=-1)

    def prm(i, n=CH, c0=0, c1=D):
        return jnp.concatenate([par[i, :, c0:c1]] * (n // 8), axis=0)

    def a_pre12(r0, n):
        x = _bf(qb[r0 // 2:(r0 + n) // 2, :]).astype(F32)
        m1, r1 = _stats(x)
        x1 = x + ((x - m1) * r1 * prm(0, n) + prm(1, n)) * ld_y(r0, n)
        x1b[r0:r0 + n, :] = x1
        m2, r2 = _stats(x1)
        hb[r0:r0 + n, :] = (x1 - m2) * r2

    def a_pre3(r0, m):
        h = hb[r0:r0 + m, :] * prm(2, m) + prm(3, m)
        hb[r0:r0 + m, :] = h
        m3, r3 = _stats(h)
        return (h - m3) * r3

    def halves(n, split):
        m = n // split if split else n
        return [(o, m) for o in range(0, n, m)]

    def mm1(r0, n, n3, split_last=0, tiles=range(NT)):
        for t in tiles:
            w = w1b[:, 128 * t:128 * t + 128]
            for o, m in halves(n, split_last if t == tiles[-1] else 0):
                hp = jnp.dot(n3[o:o + m].astype(BF16), _bf(w), preferred_element_type=F32)
                hpb[t, rows(HPAD + r0 + o, m), :] = _gelu(hp)

    def g_prep(r0):
        lane = jax.lax.broadcasted_iota(I32, (TB, 128), 1)
        sh = [-1, 1, -2, 2]

        def ldh(t, g):
            return hpb[t, pl.ds(HPAD + r0 + sh[g], TB), :]

        cols = [ldh(0, 0)]
        for t in range(1, 4):
            cols.append(jnp.where(lane < 32 * t, ldh(t, t - 1), ldh(t, t)))
        cols.append(ldh(4, 3))
        return jnp.concatenate(cols, axis=-1)

    def mm2(r0, g, split_last=0, side=None):
        for t in range(NT):
            if side and t in side:
                side[t]()
            c0, c1 = 128 * t, 128 * t + 128
            for o, m in halves(TB, split_last if t == NT - 1 else 0):
                hs = jnp.dot(g[o:o + m].astype(BF16), _bf(w2b[:, c0:c1]), preferred_element_type=F32)
                hb[rows(r0 + o, m), c0:c1] = hb[rows(r0 + o, m), c0:c1] + hs
        return hs[m - 8:m]

    def mm3(n4, ties=None, split_at=None, side=None, tpos=12, nat=True):
        us = []
        env["g3"] = []
        for j in range(FF // 128):
            if side and j in side:
                side[j]()
            if j == tpos:
                ht = jax.lax.dot_general(_bf(w3b[FM // 2:FF // 2, :]), n4.astype(BF16), NT_DIMS,
                                         preferred_element_type=F32)
                ut = _gelu(ht).T
            w = w3b[64 * j:64 * j + 64, :]
            if ties and j in ties:
                w = _tie(w, {0: ties[j]})
            parts = []
            for o, m in halves(TB, 2 if j == split_at else 0):
                if j == 0 and nat:
                    h3 = jnp.dot(n4.astype(BF16), _bf(w3n[...]), preferred_element_type=F32)
                else:
                    h3 = jax.lax.dot_general(n4[o:o + m].astype(BF16), _bf(w), NT_DIMS,
                                             preferred_element_type=F32)
                parts.append(_gelu(h3))
                if m == TB:
                    env["g3"] += [h3[o:o + 8] for o in range(0, TB, 64)]
            us.append(jnp.concatenate(parts, axis=0))
        return jnp.concatenate(us + [ut], axis=-1)

    def mm4(r0, u, t, final=True, split=0, side=None):
        c0, c1 = 128 * t, 128 * t + 128
        w = _bf(w4b[:, c0:c1])
        for o, m in halves(TB, split):
            if o and side:
                side()
            h2 = jnp.dot(u[o:o + m].astype(BF16), w, preferred_element_type=F32)
            s = hb[rows(r0 + o, m), c0:c1] + h2
            if final:
                ob[rows(r0 + o, m, 16), c0:c1] = (
                    x1b[rows(r0 + o, m), c0:c1] + prm(4, m, c0, c1) * s).astype(BF16)
            else:
                hb[rows(r0 + o, m), c0:c1] = s

    def ln4_store(r0, nch):
        zs = []
        m = TB // nch
        for j in range(nch):
            x2 = hb[r0 + m * j:r0 + m * j + m, :]
            m4, r4 = _stats(x2)
            n4 = (x2 - m4) * r4
            n4b[m * j:m * j + m, :] = n4
            zs.append(zero_after(n4))
        return zs

    def out_copy(r0, n, c0=0, c1=D):
        return pltpu.make_async_copy(ob.at[rows(r0, n, 16), c0:c1],
                                     o_hbm.at[0, rows(r0, n, 16), c0:c1], osem)

    wait("ra")
    env["taps"] = skb[...].astype(F32)
    env["dvec"] = sdb[...].astype(F32).reshape(1, D)
    cf = cb_[...].astype(F32)
    sc8 = jnp.broadcast_to(cf * jax.nn.sigmoid(cf), (8, D)).astype(BF16)
    run_rounds("X00")
    wait("r0")
    run_rounds("X01 K00 K10 K20 K30")
    for t in range(1, NT):
        wait(f"r{t}")
        run_rounds(f"I0{t - 1} X{(t + 1) // NT}{(t + 1) % NT} K0{t} K1{t} K2{t} K3{t}")
    wait("r5")
    run_rounds("I04 X11 I10 X12@20:3 I11 X13@20:3 I12 X14@20:3")
    wait("r6")
    run_rounds("I13 X20 I14 X21@24:14 I20 X22@24:14 I21 X23@24:14 I22 X24@24:14 I23")

    def zero_tail(t, carry):
        yb[t, S:S + AO, :] = jnp.zeros((AO, 128), F32)
        return carry

    jax.lax.fori_loop(0, NT, zero_tail, 0)
    wait("wmA")
    mod = jnp.dot(sc8, wmb[:, 0:3 * D], preferred_element_type=F32)
    sa, ca, ga = [mod[:, D * i:D * (i + 1)] for i in range(3)]
    par[0] = (1.0 + ca) * ga
    par[1] = sa * ga
    run_rounds("I24")
    a_pre12(0, TB + AO)
    a_pre12(TB + AO, TB)
    wait("wmS")
    mod = jnp.dot(sc8, wmb[:, 3 * D:4 * D + 256], preferred_element_type=F32)
    par[3] = mod[:, 0:D]
    par[2, :, 0:256] = 1.0 + mod[:, D:D + 256]
    wait("wmB")
    par[2, :, 256:D] = 1.0 + jnp.dot(sc8, wmb[:, 4 * D + 256:5 * D], preferred_element_type=F32)
    n3p = a_pre3(0, 128)

    ta, tb = range(W1A // 128), range(W1A // 128, NT)
    wait("w1")
    n3 = jnp.concatenate([n3p, a_pre3(128, QE - 128)], axis=0)
    for a, b in ((0, 128), (128, 256), (256, 400), (400, QE)):
        mm1(a, b - a, n3[a:b], tiles=ta)
    wait("w1b")
    mm1(0, TB + AO, n3[:TB + AO], tiles=tb)
    run_rounds("X30")
    mm1(TB + AO, TB, n3[TB + AO:], split_last=4, tiles=tb)
    wait("w2")
    z = zero_after(mm2(0, g_prep(0), side={4: lambda: run_rounds("X31")}))
    n4 = []
    for j in range(8):
        xx = pltpu.bitcast(gated(hb[32 * j:32 * j + 32, :], z), F32)
        m4, r4 = _stats(xx)
        n4.append((xx - m4) * r4)
        if j >= 3:
            z = z | zero_after(n4[j - 3])
        z = pltpu.roll(z, 1, 1)
    n4 = jnp.concatenate(n4, axis=0)
    mm2(TB, g_prep(TB), split_last=2)
    wait("w3")
    zs = ln4_store(TB, 8)
    w3n[...] = pltpu.bitcast(_bf(w3b[0:64, :]).T, U32)
    run_rounds("I30")

    def mid():
        wait("w4")
        run_rounds("I31")

    u = mm3(n4, {3 + j: z for j, z in enumerate(zs)}, split_at=W3A // 128 - 1, nat=False,
            side={W3A // 128: mid})
    mm4(0, u, 0, final=False)
    run_rounds("X32")
    run_rounds("X33")
    mm4(0, u, 1, final=False)
    mm4(0, u, 2, final=False)
    run_rounds("I32")
    wait("rest")

    def gb_tiles(*ts):
        for t in ts:
            par[4, :, 128 * t:128 * t + 128] = jnp.dot(
                sc8, wmb[:, 5 * D + 128 * t:5 * D + 128 * t + 128], preferred_element_type=F32)

    def finalize(t):
        c0, c1 = 128 * t, 128 * t + 128
        if c0 < W4A:
            ob[0:TB, c0:c1] = (x1b[0:TB, c0:c1] + prm(4, TB, c0, c1) * hb[0:TB, c0:c1]).astype(BF16)
        eb[TB:2 * TB, c0:c1] = x1b[TB:2 * TB, c0:c1] + prm(4, TB, c0, c1) * hb[TB:2 * TB, c0:c1]

    run_rounds("I33")
    gb_tiles(3, 4, 0)
    mm4(0, u, 3, split=2, side=lambda: run_rounds("X34"))
    gb_tiles(1)
    mm4(0, u, 4, split=2, side=lambda: gb_tiles(2))
    for t in range(NT - 1):
        finalize(t)
    run_rounds("I34")
    finalize(NT - 1)
    out_copy(0, TB).start()
    wait("qnext")

    def mm4e(ev, ov, u, t, split=0):
        c0, c1 = 128 * t, 128 * t + 128
        for o, m in halves(TB, split):
            h2 = jnp.dot(u[o:o + m].astype(BF16), _bf(w4b[:, c0:c1]), preferred_element_type=F32)
            ov[o:o + m, c0:c1] = (ev[o:o + m, c0:c1] + prm(4, m, c0, c1) * h2).astype(BF16)

    def body(i, carry):
        pl.when(i == 2)(lambda: wait("qlast"))
        r0 = pl.multiple_of(i * TB, TB)
        ev = eb.at[pl.ds(r0, 2 * TB), :]
        ov = ob.at[pl.ds(r0, TB), :]
        u = mm3(n4b[...])
        hpb[:, TB:TB + HPAD + AO, :] = hpb[:, 2 * TB:2 * TB + HPAD + AO, :]
        x1s, hs, n3 = [x1b[2 * TB:QE, :]], [hb[2 * TB:QE, :]], []
        for j in range(TB // CH):
            r = r0 + TB + AO + CH * j
            z = zero_after(env["g3"][GATES[j]])
            x = _bf(gated(qb[rows(r // 2, CH // 2), :], z)).astype(F32)
            m1, r1 = _stats(x)
            x1 = x + ((x - m1) * r1 * prm(0) + prm(1)) * ld_y(r, CH)
            m2, r2 = _stats(x1)
            h = (x1 - m2) * r2 * prm(2) + prm(3)
            m3, r3 = _stats(h)
            n3.append((h - m3) * r3)
            x1s.append(x1)
            hs.append(h)
        x1b[2 * TB:QE, :] = x1s[-1]
        hb[2 * TB:QE, :] = hs[-1]
        mm4e(ev, ov, u, 0)
        mm1(TB + AO, TB, jnp.concatenate(n3, axis=0))
        zrow = pl.multiple_of(jnp.where(i == NBLK - 2, HPAD + 2 * TB, HPAD + QE), 8)
        hpb[:, pl.ds(zrow, 8), :] = jnp.zeros((NT, 8, 128), F32)
        mm4e(ev, ov, u, 1)
        g = g_prep(TB).astype(BF16)
        hcat = jnp.concatenate(hs[:-1], axis=0)
        x2 = []
        for t in range(NT):
            mix = jnp.dot(g, _bf(w2b[:, 128 * t:128 * t + 128]), preferred_element_type=F32)
            x2.append(hcat[:, 128 * t:128 * t + 128] + mix)
        x2 = jnp.concatenate(x2, axis=-1)
        z = zero_after(mix[0:8])
        for j in range(TB // CH):
            xx = pltpu.bitcast(gated(x2[CH * j:CH * j + CH], z), F32)
            m4, r4 = _stats(xx)
            n4b[CH * j:CH * j + CH, :] = (xx - m4) * r4
            ev[TB + CH * j:TB + CH * j + CH, :] = x1s[j] + prm(4) * xx
            z = pltpu.roll(z, 1, 1)
        for t in range(2, NT):
            mm4e(ev, ov, u, t)
        out_copy(r0, TB).start()
        return carry

    jax.lax.fori_loop(1, NBLK - 1, body, 0)

    r0 = S - TB
    u = mm3(n4b[...])
    for t in range(NT):
        mm4e(eb.at[r0:S, :], ob.at[r0:S, :], u, t, split=2 if t == NT - 1 else 0)
        if t < NT - 1:
            out_copy(r0, TB, 128 * t, 128 * t + 128).start()
    out_copy(r0, TB // 2, D - 128, D).start()
    out_copy(r0 + TB // 2, TB // 2, D - 128, D).start()
    with jax.named_scope("W_out"):
        pltpu.make_async_copy(ob, o_hbm.at[0], osem).wait()


@jax.jit
def pallas_adaLN_cond__ssm_conv_h3__mixer_s_mlp__prompt_kernel(
    A_q, A_k, A_v, A_shift_k, A_ssm_k, A_ssm_D, B_x, B_w1, B_w2, B_w3, B_w4, c, w_mod,
):
    del B_x
    vm = pltpu.VMEM
    scratch = [
        vm(((S + AO) // 2, D), U32),
        vm((NT, KPAD + S, 128), BF16),
        vm((NT, S, 128), BF16),
        vm((4, D), BF16),
        vm((D // 2, S), U32),
        vm((D,), BF16),
        vm((D // 2, D), U32),
        vm((D // 2, D), U32),
        vm((FF // 2, D), U32),
        vm((FF // 2, D), U32),
        vm((1, D), BF16),
        vm((D, 6 * D), BF16),
        vm((R + 1, 128, 128), U32),
        vm((2 * R + 1, 32, 128), U32),
        vm((NT, S // 2, 128), U32),
        vm((8, NT, R, 256, 128), F32),
        vm((NT, S + AO + 16, 128), F32),
        vm((2 * TB + AO, D), F32),
        vm((2 * TB + AO, D), F32),
        vm((S + 8, D), F32),
        vm((NT, HPAD + 2 * TB + AO + 8, 128), F32),
        vm((TB, D), F32),
        vm((5, 8, D), F32),
        vm((D // 2, 128), U32),
        vm((S, D), BF16),
        pltpu.SemaphoreType.DMA((19,)),
        pltpu.SemaphoreType.DMA(()),
    ]
    hbm = pl.BlockSpec(memory_space=pltpu.HBM)
    return pl.pallas_call(
        _kernel,
        out_shape=jax.ShapeDtypeStruct((1, S, D), BF16),
        in_specs=[hbm] * 12,
        out_specs=hbm,
        scratch_shapes=scratch,
        compiler_params=pltpu.CompilerParams(vmem_limit_bytes=110 * 2**20,
                                             disable_semaphore_checks=True,
                                             disable_bounds_checks=True),
        name="h3_mixer",
    )(A_q, A_k, A_v, A_shift_k.T, A_ssm_k, A_ssm_D, B_w1, B_w2, B_w3.T, B_w4, c, w_mod)
```

```python
import jax
import jax.numpy as jnp
import numpy as np
import jax.experimental.pallas as pl
import jax.experimental.pallas.tpu as pltpu

S, D, FF = 2048, 640, 1728
NT = D // 128
L = 512
NB = S // L
NFFT = 2 * L
R = 4
KPAD = 16
HPAD = 8
TB = 256
NBLK = S // TB
AO = 16
CH = 16
EPS = 1e-5
GATES = (0, 6, 7, 12, 15, 21, 22, 25, 28, 31, 33, 38, 42, 43, 44, 51)
W1A, W3A, W4A = 256, 1536, 384
FM = FF // 128 * 128
F32 = jnp.float32
BF16 = jnp.bfloat16
U32 = jnp.uint32
I32 = jnp.int32
NT_DIMS = (((1,), (1,)), ((), ()))
KP, XS, ZP = 0, 3, 3


def _cos_coefs(deg=6):
    u = (np.cos(np.pi * (np.arange(400) + 0.5) / 400) + 1.0) / 2.0
    c = np.polynomial.polynomial.polyfit(u, np.cos(np.pi * np.sqrt(u)), deg)
    return [np.float32(v) for v in c]


_COS = _cos_coefs()


def _cos_units(a, scale=1.0):
    x = (((a + 1024) & 2047) - 1024).astype(F32) * np.float32(1.0 / 1024.0)
    u = x * x
    acc = u * np.float32(_COS[-1] * scale) + np.float32(_COS[-2] * scale)
    for c in _COS[-3::-1]:
        acc = acc * u + np.float32(c * scale)
    return acc


def _freq2(chunk, s):
    e = 4 * (8 * (chunk >> 1) + s) + 1
    return jnp.where((chunk & 1) == 0, e, 256 - e)


def _gelu(x):
    c1 = np.float32(np.sqrt(2.0 / np.pi))
    c2 = np.float32(np.sqrt(2.0 / np.pi) * 0.044715)
    u = x * (c1 + c2 * (x * x))
    hx = 0.5 * x
    return hx + hx * jnp.tanh(u)


def _stats(x):
    m = jnp.sum(x, axis=-1, keepdims=True) * (1.0 / D)
    e2 = jnp.sum(x * x, axis=-1, keepdims=True) * (1.0 / D)
    v = jnp.maximum(e2 - m * m, 0.0)
    return m, jax.lax.rsqrt(v + EPS)


def _split(b):
    b = b.reshape(-1, 2, 8, 128)
    return b[:, 0], b[:, 1]


def _join(z):
    return jnp.stack(z, axis=1).reshape(-1, 128)


def _uneo(e, o):
    return jnp.stack([e, o], axis=1).reshape(16, 8, 128)


def _fft4(b, sign):
    (r0, i0), (r1, i1), (r2, i2), (r3, i3) = b
    sr, si, dr, di = r0 + r2, i0 + i2, r0 - r2, i0 - i2
    tr, ti, er, ei = r1 + r3, i1 + i3, r1 - r3, i1 - i3
    x0 = (sr + tr, si + ti)
    x2 = (sr - tr, si - ti)
    xm = (dr + ei, di - er)
    xp = (dr - ei, di + er)
    return [x0, xm, x2, xp] if sign < 0 else [x0, xp, x2, xm]


def _cmul(a, b, acc=None):
    (ar, ai), (br, bi) = a, b
    if acc is None:
        return ar * br - ai * bi, ar * bi + ai * br
    return (acc[0] + ar * br) - ai * bi, (acc[1] + ar * bi) + ai * br


def _bf(x):
    return pltpu.bitcast(x, BF16)


def _words(x):
    return pltpu.bitcast(x.astype(BF16), U32)


def _tie(w, ties):
    if not ties:
        return w
    parts = []
    for i in range(w.shape[0] // 8):
        p = w[8 * i:8 * i + 8]
        if i in ties:
            z = ties[i]
            p = p | z if p.shape[1] == 128 else jnp.concatenate([p[:, :128] | z, p[:, 128:]], axis=1)
        parts.append(p)
    return jnp.concatenate(parts, axis=0)


def _kernel(q_hbm, k_hbm, v_hbm, sk_hbm, ssm_hbm, sd_hbm, w1_hbm, w2_hbm, w3_hbm,
            w4_hbm, c_hbm, wm_hbm, o_hbm,
            qb, kb, vb, skb, ssmb, sdb, w1b, w2b, w3b, w4b, cb_, wmb, fwb, gib,
            stb, spec, yb, x1b, hb, eb, hpb, n4b, par, w3n, ob, sems, osem):
    groups = {}

    def add(name, src, dst):
        if name not in groups:
            groups[name] = (len(groups), [])
        idx, lst = groups[name]
        cp = pltpu.make_async_copy(src, dst, sems.at[idx])
        cp.start()
        lst.append(cp)

    def add_kv(name, c, tiles=range(NT)):
        for t in tiles:
            add(name, k_hbm.at[0, pl.ds(L * c, L), pl.ds(128 * t, 128)],
                kb.at[t, pl.ds(KPAD + L * c, L), :])
            add(name, v_hbm.at[0, pl.ds(L * c, L), pl.ds(128 * t, 128)],
                vb.at[t, pl.ds(L * c, L), :])

    def add_ssm(name, t):
        add(name, ssm_hbm.at[pl.ds(128 * t, 128), :], ssmb.bitcast(BF16).at[pl.ds(128 * t, 128), :])

    QE = 2 * TB + AO
    add_kv("ra", 0, [0])
    add("ra", sd_hbm, sdb)
    add("ra", sk_hbm, skb)
    add("ra", c_hbm, cb_)
    for t in range(NT):
        add_ssm(f"r{t}", t)
        add_kv(f"r{t}", (t + 1) // NT, [(t + 1) % NT])
    add_kv("r5", 1, range(1, NT))
    add_kv("r6", 2)
    add("wmA", q_hbm.at[0, pl.ds(0, QE), :], qb.bitcast(BF16).at[pl.ds(0, QE), :])
    add("wmA", wm_hbm.at[:, pl.ds(0, 3 * D)], wmb.at[:, pl.ds(0, 3 * D)])
    add("wmS", wm_hbm.at[:, pl.ds(3 * D, D + 256)], wmb.at[:, pl.ds(3 * D, D + 256)])
    add("wmB", wm_hbm.at[:, pl.ds(4 * D + 256, D - 256)], wmb.at[:, pl.ds(4 * D + 256, D - 256)])
    add("w1", w1_hbm.at[:, pl.ds(0, W1A)], w1b.bitcast(BF16).at[:, pl.ds(0, W1A)])
    add("w1b", w1_hbm.at[:, pl.ds(W1A, D - W1A)], w1b.bitcast(BF16).at[:, pl.ds(W1A, D - W1A)])
    add_kv("w1b", 3, [0])
    add("w2", w2_hbm, w2b.bitcast(BF16))
    add_kv("w2", 3, [1])
    add("w3", w3_hbm.at[pl.ds(0, W3A), :], w3b.bitcast(BF16).at[pl.ds(0, W3A), :])
    add("w4", w3_hbm.at[pl.ds(W3A, FF - W3A), :], w3b.bitcast(BF16).at[pl.ds(W3A, FF - W3A), :])
    add("w4", w4_hbm.at[:, pl.ds(0, W4A)], w4b.bitcast(BF16).at[:, pl.ds(0, W4A)])
    add_kv("w4", 3, [2, 3])
    add("rest", w4_hbm.at[:, pl.ds(W4A, D - W4A)], w4b.bitcast(BF16).at[:, pl.ds(W4A, D - W4A)])
    add_kv("rest", 3, [4])
    add("rest", wm_hbm.at[:, pl.ds(5 * D, D)], wmb.at[:, pl.ds(5 * D, D)])
    add("qnext", q_hbm.at[0, pl.ds(QE, TB), :], qb.bitcast(BF16).at[pl.ds(QE, TB), :])
    add("qlast", q_hbm.at[0, pl.ds(QE + TB, S - QE - TB), :],
        qb.bitcast(BF16).at[pl.ds(QE + TB, S - QE - TB), :])

    def wait(name):
        with jax.named_scope("W_" + name):
            for cp in groups[name][1]:
                cp.wait()

    kb[:, 0:KPAD, :] = jnp.zeros((NT, KPAD, 128), BF16)
    hpb[:, 0:HPAD, :] = jnp.zeros((NT, HPAD, 128), F32)
    qb[S // 2:(S + AO) // 2, :] = jnp.zeros((AO // 2, D), U32)

    spec[7, 0, 0, pl.ds(0, 8, stride=2), :] = jnp.zeros((8, 128), F32)
    fwb[R, pl.ds(0, 8, stride=2), :] = jnp.zeros((8, 128), U32)
    gib[2 * R, pl.ds(0, 8, stride=2), :] = jnp.zeros((8, 128), U32)

    row = jax.lax.broadcasted_iota(I32, (256, 128), 0)
    col = jax.lax.broadcasted_iota(I32, (256, 128), 1)
    f2 = _freq2(row >> 4, row & 7)
    ph = 512 * ((row >> 3) & 1)
    m = (col & ~15) + 2 * (col & 7) + ((col >> 3) & 1)
    for r in range(R):
        fwb[r] = _words(_cos_units((4 * m + r) * f2 + ph))
    row = jax.lax.broadcasted_iota(I32, (64, 128), 0)
    col = jax.lax.broadcasted_iota(I32, (64, 128), 1)
    f2 = 4 * (8 * (col >> 4) + (col & 7)) + 1
    ph = 512 * ((col >> 3) & 1)
    for r in range(2 * R):
        gib[r] = _words(_cos_units((8 * row + r) * f2 + ph, 2.0 / NFFT))

    env = {}

    def zero_after(*vals):
        acc = None
        for v in vals:
            v = pltpu.bitcast(v, U32)
            for i in range(0, v.shape[0], 8):
                for j in range(0, v.shape[1], 128):
                    p = v[i:i + 8, j:j + 128]
                    acc = p if acc is None else acc | p
        return acc & kb.bitcast(U32)[0, 0:8, :]

    def gated(v, z):
        zt = jnp.concatenate([jnp.concatenate([z] * NT, axis=1)] * (v.shape[0] // 8), axis=0)
        return pltpu.bitcast(v, U32) | zt

    def ld_spec(slot, t, q):
        return _split(spec[slot, t, q])

    def st_spec(slot, t, q, z):
        spec[slot, t, q] = _join(z)

    def fwd_dots(rhs, ties):
        return [_split(jnp.dot(_bf(_tie(fwb[r], ties if r == 0 else None)), rhs[r],
                               preferred_element_type=F32)) for r in range(R)]

    def conv_k(c, t, ties):
        w0 = L * c // 2
        stb[t, w0:w0 + L // 2, :] = pltpu.bitcast(
            _bf(ssmb[64 * t:64 * t + 64, L * c:L * c + L]).T, U32)
        rhs = []
        for h in range(2):
            lo = stb[t, pl.ds(w0 + h, 64, stride=4), :]
            hi = stb[t, pl.ds(w0 + h + 2, 64, stride=4), :]
            for e, o in zip(unpack(lo), unpack(hi)):
                rhs.append(_join((e.reshape(8, 8, 128), o.reshape(8, 8, 128))).astype(BF16))
        b = fwd_dots(rhs, ties)
        if c == 0:
            b[0] = (b[0][0] + env["dvec"][:, 128 * t:128 * t + 128][None], b[0][1])
        kq = _fft4(b, -1)
        z = []
        for q in range(R):
            kp = kq[q]
            if c >= 2:
                p = ld_spec(KP + c - 2, t, q)
                kp = (kp[0] + p[0], kp[1] + p[1])
            if c >= 1:
                p = ld_spec(KP + c - 1, t, q)
                if c == 3:
                    p0 = ld_spec(KP, t, q)
                    p = (p[0] - p0[0], p[1] - p0[1])
                (ree, reo), (ime, imo), (pre, pro), (pie, pio) = (_split(v) for v in kp + p)
                kp = (_uneo(ree - pie, reo + pio), _uneo(ime + pre, imo - pro))
            if c < 3:
                st_spec(KP + c, t, q, kp)
            zc = _cmul(kp, ld_spec(XS, t, q))
            if c == 0:
                z.append(zc)
            else:
                st_spec(ZP + c, t, q, zc)
        if c == 0:
            finish(0, t, z)

    def finish(c, t, z):
        hs = np.float32(np.sqrt(0.5))
        cr = _fft4(z, +1)
        for r in range(R):
            (ar, br), (ai, bi) = _split(cr[r][0]), _split(cr[r][1])
            if r % 2:
                br, bi = (br - bi) * hs, (br + bi) * hs
            if r < 2:
                p, m = (ar + br, ai - bi), (ar - br, ai + bi)
            else:
                p, m = (ar - bi, ai - br), (ar + bi, ai + br)
            env["cm", c, t, r] = _join(p).astype(BF16)
            env["cm", c, t, r + R] = _join(m).astype(BF16)

    def unpack(u):
        return (pltpu.bitcast(u << 16, F32),
                pltpu.bitcast(u & jnp.uint32(0xFFFF0000), F32))

    def conv_prep(c, t):
        taps = env["taps"]
        ku = kb.bitcast(U32)
        vu = vb.bitcast(U32)
        tp = [taps[j:j + 1, 128 * t:128 * t + 128] for j in range(4)]
        w0 = (KPAD + L * c) // 2
        kk = [unpack(ku[t, pl.ds(w0 - 2, 64, stride=4), :])[1]]
        for o in range(-1, 4):
            kk += unpack(ku[t, pl.ds(w0 + o, 64, stride=4), :])
        vv = []
        for o in range(4):
            vv += unpack(vu[t, pl.ds(L * c // 2 + o, 64, stride=4), :])
        kv = []
        for n in range(8):
            acc = kk[3 + n] * tp[0]
            for j in range(1, 4):
                acc = acc + kk[3 + n - j] * tp[j]
            kv.append(acc * vv[n])
        return [_join((kv[r].reshape(8, 8, 128), kv[r + 4].reshape(8, 8, 128))) for r in range(R)]

    def conv_x(c, t, ties):
        xq = _fft4(fwd_dots([v.astype(BF16) for v in env.pop(("kv", c, t))], ties), -1)
        z = []
        for q in range(R):
            if c == 0:
                st_spec(XS, t, q, xq[q])
                continue
            for a in range(c, NB):
                if (c, a) == (1, 2):
                    st_spec(XS, t, q, xq[q])
                    continue
                za = _cmul(xq[q], ld_spec(KP + a - c, t, q), ld_spec(ZP + a, t, q))
                if (c, a) == (2, 2):
                    za = _cmul(ld_spec(XS, t, q), ld_spec(KP + 1, t, q), za)
                if a == c:
                    z.append(za)
                else:
                    st_spec(ZP + a, t, q, za)
        if c:
            finish(c, t, z)

    def conv_inv(c, t, ties):
        for r in range(2 * R):
            tr = None
            if ties and r % R == 0:
                tr = {i - r: z for i, z in ties.items() if 0 <= i - r < 4}
            yb[t, pl.ds(L * c + r, 64, stride=2 * R), :] = jnp.dot(
                _bf(_tie(gib[r], tr)), env.pop(("cm", c, t, r)), preferred_element_type=F32)

    def run_rounds(spec_str):
        rounds = spec_str.split()
        slots = []
        plan = {}
        for n, rd in enumerate(rounds):
            if rd[0] == "X":
                pts = []
                if "@" in rd:
                    a, b = (int(v) for v in rd[4:].split(":"))
                    pts = [slots[len(slots) - a + (a - b) * (j + 1) // 8 - 1] for j in range(8)]
                plan.setdefault(pts[0][0] if pts else n, []).append((rd, pts))
            slots += [(n, i) for i in range(8 if rd[0] == "I" else 16)]
        ties = {}
        for n, rd in enumerate(rounds):
            for xr, pts in plan.get(n, []):
                c, t = int(xr[1]), int(xr[2])
                kv = env["kv", c, t] = conv_prep(c, t)
                for j, (pn, pi) in enumerate(pts):
                    z = zero_after(*[w[16 * j:16 * j + 16] for w in kv])
                    d = ties.setdefault(pn, {})
                    d[pi] = z if pi not in d else d[pi] | z
            {"K": conv_k, "X": conv_x, "I": conv_inv}[rd[0]](int(rd[1]), int(rd[2]), ties.get(n))

    def rows(r0, n, align=8):
        if isinstance(r0, int):
            return slice(r0, r0 + n)
        return pl.ds(pl.multiple_of(r0, align), n)

    def ld_y(r0, n):
        return jnp.concatenate([yb[t, rows(r0, n), :] for t in range(NT)], axis=-1)

    def prm(i, n=CH, c0=0, c1=D):
        return jnp.concatenate([par[i, :, c0:c1]] * (n // 8), axis=0)

    def a_pre12(r0, n):
        x = _bf(qb[r0 // 2:(r0 + n) // 2, :]).astype(F32)
        m1, r1 = _stats(x)
        x1 = x + ((x - m1) * r1 * prm(0, n) + prm(1, n)) * ld_y(r0, n)
        x1b[r0:r0 + n, :] = x1
        m2, r2 = _stats(x1)
        hb[r0:r0 + n, :] = (x1 - m2) * r2

    def a_pre3(r0, m):
        h = hb[r0:r0 + m, :] * prm(2, m) + prm(3, m)
        hb[r0:r0 + m, :] = h
        m3, r3 = _stats(h)
        return (h - m3) * r3

    def halves(n, split):
        m = n // split if split else n
        return [(o, m) for o in range(0, n, m)]

    def mm1(r0, n, n3, split_last=0, tiles=range(NT)):
        for t in tiles:
            w = w1b[:, 128 * t:128 * t + 128]
            for o, m in halves(n, split_last if t == tiles[-1] else 0):
                hp = jnp.dot(n3[o:o + m].astype(BF16), _bf(w), preferred_element_type=F32)
                hpb[t, rows(HPAD + r0 + o, m), :] = _gelu(hp)

    def g_prep(r0):
        lane = jax.lax.broadcasted_iota(I32, (TB, 128), 1)
        sh = [-1, 1, -2, 2]

        def ldh(t, g):
            return hpb[t, pl.ds(HPAD + r0 + sh[g], TB), :]

        cols = [ldh(0, 0)]
        for t in range(1, 4):
            cols.append(jnp.where(lane < 32 * t, ldh(t, t - 1), ldh(t, t)))
        cols.append(ldh(4, 3))
        return jnp.concatenate(cols, axis=-1)

    def mm2(r0, g, split_last=0, side=None):
        for t in range(NT):
            if side and t in side:
                side[t]()
            c0, c1 = 128 * t, 128 * t + 128
            for o, m in halves(TB, split_last if t == NT - 1 else 0):
                hs = jnp.dot(g[o:o + m].astype(BF16), _bf(w2b[:, c0:c1]), preferred_element_type=F32)
                hb[rows(r0 + o, m), c0:c1] = hb[rows(r0 + o, m), c0:c1] + hs
        return hs[m - 8:m]

    def mm3(n4, ties=None, split_at=None, side=None, tpos=12, nat=True):
        us = []
        env["g3"] = []
        for j in range(FF // 128):
            if side and j in side:
                side[j]()
            if j == tpos:
                ht = jax.lax.dot_general(_bf(w3b[FM // 2:FF // 2, :]), n4.astype(BF16), NT_DIMS,
                                         preferred_element_type=F32)
                ut = _gelu(ht).T
            w = w3b[64 * j:64 * j + 64, :]
            if ties and j in ties:
                w = _tie(w, {0: ties[j]})
            parts = []
            for o, m in halves(TB, 2 if j == split_at else 0):
                if j == 0 and nat:
                    h3 = jnp.dot(n4.astype(BF16), _bf(w3n[...]), preferred_element_type=F32)
                else:
                    h3 = jax.lax.dot_general(n4[o:o + m].astype(BF16), _bf(w), NT_DIMS,
                                             preferred_element_type=F32)
                parts.append(_gelu(h3))
                if m == TB:
                    env["g3"] += [h3[o:o + 8] for o in range(0, TB, 64)]
            us.append(jnp.concatenate(parts, axis=0))
        return jnp.concatenate(us + [ut], axis=-1)

    def mm4(r0, u, t, final=True, split=0, side=None):
        c0, c1 = 128 * t, 128 * t + 128
        w = _bf(w4b[:, c0:c1])
        for o, m in halves(TB, split):
            if o and side:
                side()
            h2 = jnp.dot(u[o:o + m].astype(BF16), w, preferred_element_type=F32)
            s = hb[rows(r0 + o, m), c0:c1] + h2
            if final:
                ob[rows(r0 + o, m, 16), c0:c1] = (
                    x1b[rows(r0 + o, m), c0:c1] + prm(4, m, c0, c1) * s).astype(BF16)
            else:
                hb[rows(r0 + o, m), c0:c1] = s

    def ln4_store(r0, nch):
        zs = []
        m = TB // nch
        for j in range(nch):
            x2 = hb[r0 + m * j:r0 + m * j + m, :]
            m4, r4 = _stats(x2)
            n4 = (x2 - m4) * r4
            n4b[m * j:m * j + m, :] = n4
            zs.append(zero_after(n4))
        return zs

    def out_copy(r0, n, c0=0, c1=D):
        return pltpu.make_async_copy(ob.at[rows(r0, n, 16), c0:c1],
                                     o_hbm.at[0, rows(r0, n, 16), c0:c1], osem)

    wait("ra")
    env["taps"] = skb[...].astype(F32)
    env["dvec"] = sdb[...].astype(F32).reshape(1, D)
    cf = cb_[...].astype(F32)
    sc8 = jnp.broadcast_to(cf * jax.nn.sigmoid(cf), (8, D)).astype(BF16)
    run_rounds("X00")
    wait("r0")
    run_rounds("X01 K00 K10 K20 K30")
    for t in range(1, NT):
        wait(f"r{t}")
        run_rounds(f"I0{t - 1} X{(t + 1) // NT}{(t + 1) % NT} K0{t} K1{t} K2{t} K3{t}")
    wait("r5")
    run_rounds("I04 X11 I10 X12@20:3 I11 X13@20:3 I12 X14@20:3")
    wait("r6")
    run_rounds("I13 X20 I14 X21@24:14 I20 X22@24:14 I21 X23@24:14 I22 X24@24:14 I23")

    def zero_tail(t, carry):
        yb[t, S:S + AO, :] = jnp.zeros((AO, 128), F32)
        return carry

    jax.lax.fori_loop(0, NT, zero_tail, 0)
    wait("wmA")
    mod = jnp.dot(sc8, wmb[:, 0:3 * D], preferred_element_type=F32)
    sa, ca, ga = [mod[:, D * i:D * (i + 1)] for i in range(3)]
    par[0] = (1.0 + ca) * ga
    par[1] = sa * ga
    run_rounds("I24")
    a_pre12(0, TB + AO)
    a_pre12(TB + AO, TB)
    wait("wmS")
    mod = jnp.dot(sc8, wmb[:, 3 * D:4 * D + 256], preferred_element_type=F32)
    par[3] = mod[:, 0:D]
    par[2, :, 0:256] = 1.0 + mod[:, D:D + 256]
    wait("wmB")
    par[2, :, 256:D] = 1.0 + jnp.dot(sc8, wmb[:, 4 * D + 256:5 * D], preferred_element_type=F32)
    n3p = a_pre3(0, 128)

    ta, tb = range(W1A // 128), range(W1A // 128, NT)
    wait("w1")
    n3 = jnp.concatenate([n3p, a_pre3(128, QE - 128)], axis=0)
    for a, b in ((0, 128), (128, 256), (256, 400), (400, QE)):
        mm1(a, b - a, n3[a:b], tiles=ta)
    wait("w1b")
    mm1(0, TB + AO, n3[:TB + AO], tiles=tb)
    run_rounds("X30")
    mm1(TB + AO, TB, n3[TB + AO:], split_last=4, tiles=tb)
    wait("w2")
    z = zero_after(mm2(0, g_prep(0), side={4: lambda: run_rounds("X31")}))
    n4 = []
    for j in range(8):
        xx = pltpu.bitcast(gated(hb[32 * j:32 * j + 32, :], z), F32)
        m4, r4 = _stats(xx)
        n4.append((xx - m4) * r4)
        if j >= 3:
            z = z | zero_after(n4[j - 3])
        z = pltpu.roll(z, 1, 1)
    n4 = jnp.concatenate(n4, axis=0)
    mm2(TB, g_prep(TB), split_last=2)
    wait("w3")
    zs = ln4_store(TB, 8)
    w3n[...] = pltpu.bitcast(_bf(w3b[0:64, :]).T, U32)
    run_rounds("I30")

    def mid():
        wait("w4")
        run_rounds("I31")

    u = mm3(n4, {3 + j: z for j, z in enumerate(zs)}, split_at=W3A // 128 - 1, nat=False,
            side={W3A // 128: mid})
    mm4(0, u, 0, final=False)
    run_rounds("X32")
    run_rounds("X33")
    mm4(0, u, 1, final=False)
    mm4(0, u, 2, final=False)
    run_rounds("I32")
    wait("rest")

    def gb_tiles(*ts):
        for t in ts:
            par[4, :, 128 * t:128 * t + 128] = jnp.dot(
                sc8, wmb[:, 5 * D + 128 * t:5 * D + 128 * t + 128], preferred_element_type=F32)

    def finalize(t):
        c0, c1 = 128 * t, 128 * t + 128
        if c0 < W4A:
            ob[0:TB, c0:c1] = (x1b[0:TB, c0:c1] + prm(4, TB, c0, c1) * hb[0:TB, c0:c1]).astype(BF16)
        eb[TB:2 * TB, c0:c1] = x1b[TB:2 * TB, c0:c1] + prm(4, TB, c0, c1) * hb[TB:2 * TB, c0:c1]

    run_rounds("I33")
    gb_tiles(3, 4, 0)
    mm4(0, u, 3, split=2, side=lambda: run_rounds("X34"))
    gb_tiles(1)
    mm4(0, u, 4, split=2, side=lambda: gb_tiles(2))
    for t in range(NT - 1):
        finalize(t)
    run_rounds("I34")
    finalize(NT - 1)
    out_copy(0, TB).start()
    wait("qnext")

    def mm4e(ev, ov, u, t, o=0, m=TB):
        c0, c1 = 128 * t, 128 * t + 128
        h2 = jnp.dot(u[o:o + m].astype(BF16), _bf(w4b[:, c0:c1]), preferred_element_type=F32)
        ov[o:o + m, c0:c1] = (ev[o:o + m, c0:c1] + prm(4, m, c0, c1) * h2).astype(BF16)

    def body(i, carry):
        pl.when(i == 2)(lambda: wait("qlast"))
        r0 = pl.multiple_of(i * TB, TB)
        ev = eb.at[pl.ds(r0, 2 * TB), :]
        ov = ob.at[pl.ds(r0, TB), :]
        u = mm3(n4b[...])
        hpb[:, TB:TB + HPAD + AO, :] = hpb[:, 2 * TB:2 * TB + HPAD + AO, :]
        x1s, hs, n3 = [x1b[2 * TB:QE, :]], [hb[2 * TB:QE, :]], []
        for j in range(TB // CH):
            r = r0 + TB + AO + CH * j
            z = zero_after(env["g3"][GATES[j]])
            x = _bf(gated(qb[rows(r // 2, CH // 2), :], z)).astype(F32)
            m1, r1 = _stats(x)
            x1 = x + ((x - m1) * r1 * prm(0) + prm(1)) * ld_y(r, CH)
            m2, r2 = _stats(x1)
            h = (x1 - m2) * r2 * prm(2) + prm(3)
            m3, r3 = _stats(h)
            n3.append((h - m3) * r3)
            x1s.append(x1)
            hs.append(h)
        x1b[2 * TB:QE, :] = x1s[-1]
        hb[2 * TB:QE, :] = hs[-1]
        mm4e(ev, ov, u, 0)
        mm1(TB + AO, TB, jnp.concatenate(n3, axis=0))
        zrow = pl.multiple_of(jnp.where(i == NBLK - 2, HPAD + 2 * TB, HPAD + QE), 8)
        hpb[:, pl.ds(zrow, 8), :] = jnp.zeros((NT, 8, 128), F32)
        mm4e(ev, ov, u, 1)
        g = g_prep(TB).astype(BF16)
        hcat = jnp.concatenate(hs[:-1], axis=0)
        x2 = []
        for t in range(NT):
            mix = jnp.dot(g, _bf(w2b[:, 128 * t:128 * t + 128]), preferred_element_type=F32)
            x2.append(hcat[:, 128 * t:128 * t + 128] + mix)
        x2 = jnp.concatenate(x2, axis=-1)
        z = zero_after(mix[0:8])
        for j in range(TB // CH):
            xx = pltpu.bitcast(gated(x2[CH * j:CH * j + CH], z), F32)
            m4, r4 = _stats(xx)
            n4b[CH * j:CH * j + CH, :] = (xx - m4) * r4
            ev[TB + CH * j:TB + CH * j + CH, :] = x1s[j] + prm(4) * xx
            z = pltpu.roll(z, 1, 1)
        for t in range(2, NT):
            mm4e(ev, ov, u, t)
        out_copy(r0, TB).start()
        return carry

    jax.lax.fori_loop(1, NBLK - 1, body, 0)

    r0 = S - TB
    u = mm3(n4b[...])
    for t in range(NT - 1):
        mm4e(eb.at[r0:S, :], ob.at[r0:S, :], u, t)
        out_copy(r0, TB, 128 * t, 128 * t + 128).start()
    c0 = D - 128
    for o, m, cuts in ((0, 128, (0, 128)), (128, 128, (0, 64, 112, 128))):
        h2 = jnp.dot(u[o:o + m].astype(BF16), _bf(w4b[:, c0:D]), preferred_element_type=F32)
        for a, b in zip(cuts, cuts[1:]):
            rs = slice(r0 + o + a, r0 + o + b)
            ob[rs, c0:D] = (eb[rs, c0:D] + prm(4, b - a, c0, D) * h2[a:b]).astype(BF16)
            out_copy(r0 + o + a, b - a, c0, D).start()
    with jax.named_scope("W_out"):
        pltpu.make_async_copy(ob, o_hbm.at[0], osem).wait()


@jax.jit
def pallas_adaLN_cond__ssm_conv_h3__mixer_s_mlp__prompt_kernel(
    A_q, A_k, A_v, A_shift_k, A_ssm_k, A_ssm_D, B_x, B_w1, B_w2, B_w3, B_w4, c, w_mod,
):
    del B_x
    vm = pltpu.VMEM
    scratch = [
        vm(((S + AO) // 2, D), U32),
        vm((NT, KPAD + S, 128), BF16),
        vm((NT, S, 128), BF16),
        vm((4, D), BF16),
        vm((D // 2, S), U32),
        vm((D,), BF16),
        vm((D // 2, D), U32),
        vm((D // 2, D), U32),
        vm((FF // 2, D), U32),
        vm((FF // 2, D), U32),
        vm((1, D), BF16),
        vm((D, 6 * D), BF16),
        vm((R + 1, 128, 128), U32),
        vm((2 * R + 1, 32, 128), U32),
        vm((NT, S // 2, 128), U32),
        vm((8, NT, R, 256, 128), F32),
        vm((NT, S + AO + 16, 128), F32),
        vm((2 * TB + AO, D), F32),
        vm((2 * TB + AO, D), F32),
        vm((S + 8, D), F32),
        vm((NT, HPAD + 2 * TB + AO + 8, 128), F32),
        vm((TB, D), F32),
        vm((5, 8, D), F32),
        vm((D // 2, 128), U32),
        vm((S, D), BF16),
        pltpu.SemaphoreType.DMA((19,)),
        pltpu.SemaphoreType.DMA(()),
    ]
    hbm = pl.BlockSpec(memory_space=pltpu.HBM)
    return pl.pallas_call(
        _kernel,
        out_shape=jax.ShapeDtypeStruct((1, S, D), BF16),
        in_specs=[hbm] * 12,
        out_specs=hbm,
        scratch_shapes=scratch,
        compiler_params=pltpu.CompilerParams(vmem_limit_bytes=110 * 2**20,
                                             disable_semaphore_checks=True,
                                             disable_bounds_checks=True),
        name="h3_mixer",
    )(A_q, A_k, A_v, A_shift_k.T, A_ssm_k, A_ssm_D, B_w1, B_w2, B_w3.T, B_w4, c, w_mod)
```
